```python
import jax
import jax.numpy as jnp

def _softmax(x, axis=-1):
    return jax.nn.softmax(x, axis=axis)

def _gelu(x):
    return jax.nn.gelu(x, approximate=True)

def _silu(x):
    return jax.nn.silu(x)

def _sigmoid(x):
    return jax.nn.sigmoid(x)

def _layernorm(x, axis=-1, eps=1e-05):
    m = jnp.mean(x, axis=axis, keepdims=True)
    v = jnp.var(x, axis=axis, keepdims=True)
    return (x - m) / jnp.sqrt(v + eps)

def _scatter_add(tgt, idx, src, axis=0):
    return tgt.at[idx].add(src)

def _segment_sum(src, seg, n):
    return jax.ops.segment_sum(src, seg, n)

class _Rng:

    def __init__(self, key):
        self._k = key

    def _next(self):
        self._k, sub = jax.random.split(self._k)
        return sub

    def normal(self, shape):
        return jax.random.normal(self._next(), shape, dtype=jnp.bfloat16)

    def randint(self, lo, hi, shape):
        return jax.random.randint(self._next(), shape, lo, hi, dtype=jnp.int32)

    def uniform(self, shape, lo=0.0, hi=1.0):
        return jax.random.uniform(self._next(), shape, jnp.bfloat16, lo, hi)

    def permutation(self, n):
        return jax.random.permutation(self._next(), n)
kernel_name = 'adaLN_cond__sliding_block_cached__moe_arch_mod__prompt'

def setup_inputs():
    _rng = _Rng(jax.random.key(int.from_bytes(__import__("os").urandom(4), "little")))
    _w = lambda a: (lambda t: t.astype(jnp.bfloat16) if jnp.issubdtype(t.dtype, jnp.floating) else t)(jnp.asarray(a))

    def _A_setup():
        B, Sq, D = (1, 2048, 1024)
        Hq, Hkv, Sk, Dh = (32, 4, 2048, 128)
        assert Hq % Hkv == 0, (Hq, Hkv)
        return {'x': _w((lambda *s: _rng.normal(s) * 0.05)(B, Sq, D)), 'k_cache': _w((lambda *s: _rng.normal(s) * 0.05)(B, Hkv, Sk, Dh)), 'v_cache': _w((lambda *s: _rng.normal(s) * 0.05)(B, Hkv, Sk, Dh)), 'wq': _w((lambda *s: _rng.normal(s) * 0.05)(D, Hq * Dh) * D ** (-0.5)), 'wo': _w((lambda *s: _rng.normal(s) * 0.05)(Hq * Dh, D) * (Hq * Dh) ** (-0.5))}
    _A_in = _A_setup()

    def _B_setup():
        B, S, D, F, C = (1, 2048, 1024, 3584, 1)
        return {'x': _w((lambda *s: _rng.normal(s) * 0.05)(B, S, D)), 'w_r': _w((lambda *s: _rng.normal(s) * 0.05)(D)), 'w_gate': _w((lambda *s: _rng.normal(s) * 0.05)(D, F)), 'w_up': _w((lambda *s: _rng.normal(s) * 0.05)(D, F)), 'w_down': _w((lambda *s: _rng.normal(s) * 0.05)(F, D))}
    _B_in = _B_setup()
    return {'A_x': _A_in['x'], 'A_k_cache': _A_in['k_cache'], 'A_v_cache': _A_in['v_cache'], 'A_wq': _A_in['wq'], 'A_wo': _A_in['wo'], 'B_x': _B_in['x'], 'B_w_r': _B_in['w_r'], 'B_w_gate': _B_in['w_gate'], 'B_w_up': _B_in['w_up'], 'B_w_down': _B_in['w_down'], 'c': _w((lambda *s: _rng.normal(s) * 0.05)(1, 1024)), 'w_mod': _w((lambda *s: _rng.normal(s) * 0.05)(1024, 6 * 1024) * 1024 ** (-0.5))}

def reference(A_x, A_k_cache, A_v_cache, A_wq, A_wo, B_x, B_w_r, B_w_gate, B_w_up, B_w_down, c, w_mod):

    def _A_ref(x, k_cache, v_cache, wq, wo):
        B, Sq, D = x.shape
        Hq, Dh = (32, 128)
        Hkv, Sk = (k_cache.shape[1], k_cache.shape[2])
        W = min(4096, max(256, Sk // 4))
        rep = Hq // Hkv
        q = (lambda x, *d: x.transpose(*d))((x @ wq).reshape(B, Sq, Hq, Dh), 0, 2, 1, 3)
        k = jnp.repeat(k_cache[:, :, Sk - W:, :], rep, axis=1)
        v = jnp.repeat(v_cache[:, :, Sk - W:, :], rep, axis=1)
        scores = jnp.einsum('bhqd,bhkd->bhqk', q, k) * Dh ** (-0.5)
        p = _softmax(scores, axis=-1)
        o = jnp.einsum('bhqk,bhkd->bhqd', p, v)
        return (lambda x, *d: x.transpose(*d))(o, 0, 2, 1, 3).reshape(B, Sq, Hq * Dh) @ wo

    def _B_ref(x, w_r, w_gate, w_up, w_down):
        B, S, D = x.shape
        C = 1
        r = x @ w_r
        idx = jnp.argsort(-r, axis=-1)[:, :C]
        idx_e = jnp.repeat(idx.reshape(B, C, 1), D, axis=2)
        x_sel = jnp.take_along_axis(x, idx_e, axis=1)
        g = _silu(x_sel @ w_gate)
        u = x_sel @ w_up
        y = g * u @ w_down
        r_sel = _sigmoid(jnp.take_along_axis(r, idx, axis=1))
        y = y * r_sel.reshape(B, C, 1)
        b_off = (jnp.arange(B) * S).reshape(B, 1)
        flat_idx = (idx + b_off).reshape(B * C)
        zero = (x * 0.0).reshape(B * S, D)
        upd = _scatter_add(zero, flat_idx, y.reshape(B * C, D), axis=0)
        return x + upd.reshape(B, S, D)
    x = A_x
    mod = (_silu(c) @ w_mod).reshape(c.shape[0], 6, 1, -1)
    sa, ca, ga, sb, cb, gb = (mod[:, 0].copy(), mod[:, 1].copy(), mod[:, 2].copy(), mod[:, 3].copy(), mod[:, 4].copy(), mod[:, 5].copy())
    h = _layernorm(x, axis=-1) * (1 + ca) + sa
    x = x + ga * _A_ref(h, A_k_cache, A_v_cache, A_wq, A_wo)
    h = _layernorm(x, axis=-1) * (1 + cb) + sb
    x = x + gb * _B_ref(h, B_w_r, B_w_gate, B_w_up, B_w_down)
    return x
```

```python
import contextlib
import math
import os

import jax
import jax.numpy as jnp
from jax import lax
from jax.experimental import pallas as pl
from jax.experimental.pallas import tpu as pltpu

S = 2048
D = 1024
HQ = 32
HKV = 4
REP = HQ // HKV
DH = 128
GW = REP * DH
W = 512
F = 3584
EPS = 1e-5
TQ = int(os.environ.get('KP_TQ', 256))
NT = S // TQ
NIT = NT * HKV
CH = TQ // HKV
ORDER = os.environ.get('KP_ORDER', 'h1')
NEWTON = int(os.environ.get('KP_NEWTON', 1))
PACK = int(os.environ.get('KP_PACK', 1))
SCOPES = int(os.environ.get('KP_SCOPES', 0))
NPIECE = int(os.environ.get('KP_NPIECE', 4))
NOCOPY = int(os.environ.get('KP_NOCOPY', 0))
NOLN = int(os.environ.get('KP_NOLN', 0))
LATEFFN = int(os.environ.get('KP_LATEFFN', 0))
QSCALE = (DH ** -0.5) * math.log2(math.e)

f32 = jnp.float32
bf16 = jnp.bfloat16
u32 = jnp.uint32


def _scope(name):
    return jax.named_scope(name) if SCOPES else contextlib.nullcontext()


def _ln(x):
    m = jnp.mean(x, axis=-1, keepdims=True)
    xc = x - m
    v = jnp.mean(xc * xc, axis=-1, keepdims=True)
    return xc * lax.rsqrt(v + EPS)


def _recip(l):
    r = pl.reciprocal(l, approx=True)
    if NEWTON:
        r = r * (2.0 - l * r)
    return r


def _pk(x):
    return pltpu.bitcast(x, u32) if PACK else x


def _unpk(x):
    return pltpu.bitcast(x, bf16) if PACK else x


PD = 2 if PACK else 1
PT = u32 if PACK else bf16


def _kernel(x_hbm, k_hbm, v_hbm, wq_hbm, wo_hbm, wr_hbm, wg_hbm, wu_hbm, wd_hbm, c_hbm, wmod_hbm,
            out_hbm,
            xo_v, wmod_v, wq_v, wo_v, wg_v, wu_v, wd_v, k_v, v_v, kt_p, v_p, c_v, wr_v, mod_v,
            q_v, h_v, acc_v, best_v, bidx_v, sems, wqsem, wosem, osem):
    sk = k_hbm.shape[2]

    def cp(src, dst, i):
        return pltpu.make_async_copy(src, dst, sems.at[i])

    c_v = c_v.at[0]
    wr_v = wr_v.at[0]
    best_v = best_v.at[0]
    bidx_v = bidx_v.at[0]
    c_cp = cp(c_hbm, c_v, 0)
    wr_cp = cp(wr_hbm, wr_v, 1)
    wm0_cp = cp(wmod_hbm.at[:, pl.ds(0, 2 * D)], wmod_v.at[:, pl.ds(0, 2 * D)], 2)
    x0_cp = cp(x_hbm.at[0, pl.ds(0, TQ), :], xo_v.at[pl.ds(0, TQ), :], 3)
    x1_cp = cp(x_hbm.at[0, pl.ds(TQ, TQ), :], xo_v.at[pl.ds(TQ, TQ), :], 4)
    x2_cp = cp(x_hbm.at[0, pl.ds(2 * TQ, S - 2 * TQ), :], xo_v.at[pl.ds(2 * TQ, S - 2 * TQ), :], 7)
    k_cp = cp(k_hbm.at[0, :, pl.ds(sk - W, W), :], k_v, 5)
    v_cp = cp(v_hbm.at[0, :, pl.ds(sk - W, W), :], v_v, 6)
    wm1_cp = cp(wmod_hbm.at[:, pl.ds(2 * D, 4 * D)], wmod_v.at[:, pl.ds(2 * D, 4 * D)], 8)
    wg_cp = cp(wg_hbm, wg_v, 9)
    wu_cp = cp(wu_hbm, wu_v, 10)
    wd_cp = cp(wd_hbm, wd_v, 11)

    def wq_cp(g):
        return pltpu.make_async_copy(wq_hbm.at[:, pl.ds(g * GW, GW)], wq_v.at[g], wqsem.at[g])

    def wo_cp(g):
        return pltpu.make_async_copy(wo_hbm.at[pl.ds(g * GW, GW), :], wo_v.at[g], wosem.at[g])

    def out_copy(r0, n):
        return pltpu.make_async_copy(xo_v.at[pl.ds(S + r0, n), :], out_hbm.at[0, pl.ds(r0, n), :], osem.at[0])

    for c_ in (c_cp, wr_cp, wm0_cp, x0_cp, wq_cp(0), k_cp, v_cp):
        c_.start()

    def ln1_rows(r0, n, slot, d0):
        x = xo_v[pl.ds(r0, n), :].astype(f32)
        sa = mod_v[0:1, 0 * D:1 * D]
        ca = mod_v[0:1, 1 * D:2 * D]
        d0p = d0 // PD if isinstance(d0, int) else pl.multiple_of(d0 // PD, 16 // PD)
        h_v[slot, pl.ds(d0p, n // PD), :] = _pk((_ln(x) * (1.0 + ca) + sa).astype(bf16))

    def ln2_rows(r0, n, attn):
        ga = mod_v[0:1, 2 * D:3 * D]
        sb = mod_v[0:1, 3 * D:4 * D]
        cb = mod_v[0:1, 4 * D:5 * D]
        gb = mod_v[0:1, 5 * D:6 * D]
        x = xo_v[pl.ds(r0, n), :].astype(f32)
        x2b = (x + ga * attn).astype(bf16)
        xo_v[pl.ds(r0, n), :] = x2b
        x2 = x2b.astype(f32)
        h2 = (_ln(x2) * (1.0 + cb) + sb).astype(bf16).astype(f32)
        ro = S + r0 if isinstance(r0, int) else pl.multiple_of(S + r0, 16)
        xo_v[pl.ds(ro, n), :] = (x2 + gb * h2).astype(bf16)
        r = jnp.sum(h2 * wr_v[...].astype(f32), axis=-1, keepdims=True)
        r = r.astype(bf16).astype(f32)
        best = best_v[...]
        bidx = bidx_v[...]
        rows = lax.broadcasted_iota(jnp.int32, (8, 1), 0)
        for j in range(n // 8):
            rj = r[8 * j:8 * (j + 1), :]
            upd = rj > best
            best = jnp.where(upd, rj, best)
            bidx = jnp.where(upd, rows + (r0 + 8 * j), bidx)
        best_v[...] = best
        bidx_v[...] = bidx

    with _scope('P0_wait_c_wm0'):
        c_cp.wait()
        cf = c_v[...].astype(f32)
        sc = (cf * jax.nn.sigmoid(cf)).astype(bf16)
        sc8 = jnp.broadcast_to(sc, (8, D))
        best_v[...] = jnp.full(best_v.shape, -jnp.inf, f32)
        bidx_v[...] = jnp.zeros(bidx_v.shape, jnp.int32)
        wm0_cp.wait()
    with _scope('P1_mod_ln1_kt'):
        mod_v[:, 0:2 * D] = jnp.dot(sc8, wmod_v[:, 0:2 * D], preferred_element_type=f32).astype(bf16).astype(f32)
        x0_cp.wait()
        ln1_rows(0, TQ, 0, 0)
        k_cp.wait()
        for g in range(HKV):
            kt_p[g] = _pk(k_v[g].T)
        v_cp.wait()
        for g in range(HKV):
            v_p[g] = _pk(v_v[g])
    with _scope('P2_wq_qproj'):
        wq_cp(0).wait()
        for c_ in (x1_cp, wq_cp(1), wo_cp(0)):
            c_.start()
        q = jnp.dot(_unpk(h_v[0]), wq_v[0], preferred_element_type=f32)
        q_v[0] = _pk((q * QSCALE).astype(bf16))
    with _scope('P3_waitx1'):
        x1_cp.wait()
        ln1_rows(TQ, CH, 1, 0)

    def body(it, with_ln2, with_next):
        t = it // HKV
        g = it % HKV
        qslot = it % 2
        aslot = t % 2
        nit = it + 1
        hslot = (nit // HKV) % 2
        ng = nit % HKV
        PR = CH // NPIECE
        tl1 = nit // HKV + 1
        tl1c = jnp.minimum(tl1, NT - 1)

        def ln_piece(j):
            if NOLN:
                return
            if with_ln2:
                r0 = pl.multiple_of((t - 1) * TQ + g * CH + j * PR, PR)
                a0 = pl.multiple_of(g * CH + j * PR, PR)
                ln2_rows(r0, PR, acc_v[(t - 1) % 2, pl.ds(a0, PR), :])
            if with_next:
                d0 = pl.multiple_of(ng * CH + j * PR, PR)
                ln1_rows(pl.multiple_of(tl1c * TQ + d0, PR), PR, tl1 % 2, d0)

        def qk(hh):
            qh = _unpk(q_v[qslot, :, hh * DH:(hh + 1) * DH])
            s = jnp.dot(qh, _unpk(kt_p[g]), preferred_element_type=f32)
            m = jnp.max(s, axis=-1, keepdims=True)
            p = jnp.exp2(s - m)
            l = jnp.sum(p, axis=-1, keepdims=True)
            return p.astype(bf16), l

        def pv(pl_):
            p, l = pl_
            o = jnp.dot(p, _unpk(v_p[g]), preferred_element_type=f32)
            return o * _recip(l)

        def qp(h0, n):
            if not with_next:
                return
            q = jnp.dot(_unpk(h_v[hslot]), wq_v[ng, :, h0 * DH:(h0 + n) * DH], preferred_element_type=f32)
            q_v[1 - qslot, :, h0 * DH:(h0 + n) * DH] = _pk((q * QSCALE).astype(bf16))

        def op(os_, h0):
            n = len(os_)
            o = os_[0] if n == 1 else jnp.concatenate(os_, axis=1)
            y = jnp.dot(o.astype(bf16), wo_v[g, h0 * DH:(h0 + n) * DH, :], preferred_element_type=f32)
            if h0 == 0:
                acc_v[aslot] = jnp.where(g == 0, 0.0, acc_v[aslot]) + y
            else:
                acc_v[aslot] += y

        os_ = []
        if ORDER == 'h1':
            step = REP // NPIECE
            for hh in range(REP):
                sp = qk(hh)
                if hh % step == step - 1:
                    ln_piece(hh // step)
                if hh > 0:
                    op([os_[hh - 1]], hh - 1)
                os_.append(pv(sp))
                qp(hh, 1)
            op([os_[REP - 1]], REP - 1)
        elif ORDER == 'h2':
            assert NPIECE == 4
            for hp in range(REP // 2):
                a = qk(2 * hp)
                b = qk(2 * hp + 1)
                os_.append(pv(a))
                os_.append(pv(b))
                ln_piece(hp)
                qp(2 * hp, 2)
                op(os_[2 * hp:2 * hp + 2], 2 * hp)
        elif ORDER == 'h2b':
            assert NPIECE == 4
            for hp in range(REP // 2):
                a = qk(2 * hp)
                b = qk(2 * hp + 1)
                os_.append(pv(a))
                os_.append(pv(b))
                qp(2 * hp, 1)
                ln_piece(hp)
                qp(2 * hp + 1, 1)
                op(os_[2 * hp:2 * hp + 2], 2 * hp)
        elif ORDER == 'h4':
            assert NPIECE == 4
            for hp in range(2):
                a = qk(4 * hp)
                for j in range(4):
                    b = qk(4 * hp + j + 1) if j < 3 else None
                    os_.append(pv(a))
                    a = b
                qp(4 * hp, 2)
                ln_piece(2 * hp)
                qp(4 * hp + 2, 1)
                ln_piece(2 * hp + 1)
                qp(4 * hp + 3, 1)
                op(os_[4 * hp:4 * hp + 4], 4 * hp)
        if with_ln2 and not NOCOPY:
            out_copy(pl.multiple_of((t - 1) * TQ + g * CH, CH), CH).start()

    def first_body(it, carry):
        wo_cp(it).wait()

        @pl.when(it < HKV - 1)
        def _():
            wq_cp(it + 1).wait()
            wo_cp(it + 1).start()

        @pl.when(it < HKV - 2)
        def _():
            wq_cp(it + 2).start()

        @pl.when(it == 1)
        def _():
            x2_cp.start()

        @pl.when(it == 2)
        def _():
            wm1_cp.start()

        @pl.when(it == 3)
        def _():
            x2_cp.wait()

        body(it, False, True)
        return carry

    with _scope('L1_first'):
        lax.fori_loop(0, HKV, first_body, 0)

    with _scope('M_mid'):
        wm1_cp.wait()
        if not LATEFFN:
            for c_ in (wg_cp, wu_cp, wd_cp):
                c_.start()
        mod_v[:, 2 * D:6 * D] = jnp.dot(sc8, wmod_v[:, 2 * D:6 * D], preferred_element_type=f32).astype(bf16).astype(f32)
        wr_cp.wait()

    def main_body(it, carry):
        body(it, True, True)
        return carry

    with _scope('L2_main'):
        lax.fori_loop(HKV, NIT - 1, main_body, 0)

    with _scope('E1_last'):
        body(NIT - 1, True, False)
        r0 = (NT - 1) * TQ
        ln2_rows(r0, TQ, acc_v[(NT - 1) % 2])
        if NOCOPY:
            out_copy(0, S).start()
        else:
            out_copy(r0, TQ).start()
        if LATEFFN:
            for c_ in (wg_cp, wu_cp, wd_cp):
                c_.start()

    with _scope('E2_ffn'):
        best = best_v[...]
        bidx = bidx_v[...]
        rmax = jnp.max(best, axis=0, keepdims=True)
        idx_v = jnp.min(jnp.where(best == rmax, bidx, S), axis=0, keepdims=True)
        idx = jnp.minimum(idx_v[0, 0], S - 1)
        g0 = pl.multiple_of((idx // 16) * 16, 16)
        sb = mod_v[0:1, 3 * D:4 * D]
        cb = mod_v[0:1, 4 * D:5 * D]
        gb = mod_v[0:1, 5 * D:6 * D]
        x2 = xo_v[pl.ds(g0, 16), :].astype(f32)
        h2b = (_ln(x2) * (1.0 + cb) + sb).astype(bf16)
        wg_cp.wait()
        wu_cp.wait()
        gt = jnp.dot(h2b, wg_v[...], preferred_element_type=f32)
        up = jnp.dot(h2b, wu_v[...], preferred_element_type=f32)
        a = (gt * jax.nn.sigmoid(gt) * up).astype(bf16)
        wd_cp.wait()
        y = jnp.dot(a, wd_v[...], preferred_element_type=f32)
        y = y * jax.nn.sigmoid(rmax)
        rows16 = lax.broadcasted_iota(jnp.int32, (16, 1), 0) + g0
        y = jnp.where(rows16 == idx, y, 0.0)
        out_copy(0, S).wait()
        xo_v[pl.ds(pl.multiple_of(S + g0, 16), 16), :] = (x2 + gb * (h2b.astype(f32) + y)).astype(bf16)
        fix = out_copy(g0, 16)
        fix.start()
        fix.wait()


@jax.jit
def pallas_adaLN_cond__sliding_block_cached__moe_arch_mod__prompt_kernel(
    A_x, A_k_cache, A_v_cache, A_wq, A_wo, B_x, B_w_r, B_w_gate, B_w_up, B_w_down, c, w_mod,
):
    del B_x
    any_spec = pl.BlockSpec(memory_space=pl.ANY)
    return pl.pallas_call(
        _kernel,
        out_shape=jax.ShapeDtypeStruct(A_x.shape, A_x.dtype),
        in_specs=[any_spec] * 11,
        out_specs=any_spec,
        scratch_shapes=[
            pltpu.VMEM((2 * S, D), bf16),
            pltpu.VMEM((D, 6 * D), bf16),
            pltpu.VMEM((HKV, D, GW), bf16),
            pltpu.VMEM((HKV, GW, D), bf16),
            pltpu.VMEM((D, F), bf16),
            pltpu.VMEM((D, F), bf16),
            pltpu.VMEM((F, D), bf16),
            pltpu.VMEM((HKV, W, DH), bf16),
            pltpu.VMEM((HKV, W, DH), bf16),
            pltpu.VMEM((HKV, DH // PD, W), PT),
            pltpu.VMEM((HKV, W // PD, DH), PT),
            pltpu.VMEM((8, 1, D), bf16),
            pltpu.VMEM((8, 1, D), bf16),
            pltpu.VMEM((8, 6 * D), f32),
            pltpu.VMEM((2, TQ // PD, GW), PT),
            pltpu.VMEM((2, TQ // PD, D), PT),
            pltpu.VMEM((2, TQ, D), f32),
            pltpu.VMEM((8, 8, 1), f32),
            pltpu.VMEM((8, 8, 1), jnp.int32),
            pltpu.SemaphoreType.DMA((12,)),
            pltpu.SemaphoreType.DMA((HKV,)),
            pltpu.SemaphoreType.DMA((HKV,)),
            pltpu.SemaphoreType.DMA((1,)),
        ],
        compiler_params=pltpu.CompilerParams(vmem_limit_bytes=110 * 1024 * 1024),
    )(A_x, A_k_cache, A_v_cache, A_wq, A_wo, B_w_r.reshape(1, D), B_w_gate, B_w_up, B_w_down, c, w_mod)
```

```python
import contextlib
import math
import os

import jax
import jax.numpy as jnp
from jax import lax
from jax.experimental import pallas as pl
from jax.experimental.pallas import tpu as pltpu

S = 2048
D = 1024
HQ = 32
HKV = 4
REP = HQ // HKV
DH = 128
GW = REP * DH
W = 512
F = 3584
EPS = 1e-5
TQ = 256
NT = S // TQ
NIT = NT * HKV
NQS = NT
PADC = 128
TP = 512
SEQ_A = os.environ.get('KP_SEQA', 'KOV')
SEQ_B = os.environ.get('KP_SEQB', 'KQVOM')
SEQ_C = os.environ.get('KP_SEQC', 'KQVLO')
SEQ_D = os.environ.get('KP_SEQD', 'KOVL')
PINLO = os.environ.get('KP_PINLO', 'Q')
UNA = int(os.environ.get('KP_UNA', 1))
UNB = int(os.environ.get('KP_UNB', 1))
UNC = int(os.environ.get('KP_UNC', 1))
P0PIN = int(os.environ.get('KP_P0PIN', 1))
LAG0 = int(os.environ.get('KP_LAG0', 2))
SCOPES = int(os.environ.get('KP_SCOPES', 0))
QSCALE = (DH ** -0.5) * math.log2(math.e)
PR = TQ // REP

f32 = jnp.float32
bf16 = jnp.bfloat16

(SEM_C, SEM_WR, SEM_X0, SEM_WM1, SEM_K, SEM_V, SEM_WG, SEM_WU, SEM_WD, SEM_OUT) = range(10)
SEM_X = 10
SEM_WQ = SEM_X + NT
SEM_WO = SEM_WQ + HKV
SEM_WQ0 = SEM_WO + HKV
SEM_WMS = SEM_WQ0 + 4
SEM_WMC = SEM_WMS + 4
NSEM = SEM_WMC + 4


def _scope(name):
    return jax.named_scope(name) if SCOPES else contextlib.nullcontext()


def _ln(x):
    m = jnp.mean(x, axis=-1, keepdims=True)
    xc = x - m
    v = jnp.mean(xc * xc, axis=-1, keepdims=True)
    return xc * lax.rsqrt(v + EPS)


def _recip(l):
    r = pl.reciprocal(l, approx=True)
    return r * (2.0 - l * r)


def _mo(x, m):
    return x if isinstance(x, int) else pl.multiple_of(x, m)


def _gate(x, flag, tok):
    n = x.shape[0]
    xs = jnp.where(flag, jnp.concatenate([tok] * (n // 8), axis=0), x[:, 0:128])
    return jnp.concatenate([xs, x[:, 128:]], axis=1)


def _gate1(x, flag, tok):
    r = tok.shape[0]
    x0 = jnp.where(flag, tok, x[0:r, 0:128])
    if x.shape[1] > 128:
        x0 = jnp.concatenate([x0, x[0:r, 128:]], axis=1)
    return jnp.concatenate([x0, x[r:]], axis=0)


def _token(y):
    t = y[:, 0:128]
    for j in range(1, y.shape[1] // 128):
        t = jnp.maximum(t, y[:, j * 128:(j + 1) * 128])
    u = t[0:8]
    for j in range(1, y.shape[0] // 8):
        u = jnp.maximum(u, t[8 * j:8 * (j + 1)])
    return u


def _kernel(x_hbm, k_hbm, v_hbm, wq_hbm, wo_hbm, wr_hbm, wg_hbm, wu_hbm, wd_hbm, c_hbm, wmod_hbm,
            out_hbm,
            x_v, out_v, h_v, q_v, acc_v, wmod_v, wq_v, wo_v, wg_v, wu_v, wd_v, k_v, v_v, kt_v,
            c_v8, wr_v8, sc_v, mod_v, best_v8, bidx_v8, cand_v, flag_s, sems):
    sk = k_hbm.shape[2]
    c_v = c_v8.at[0]
    wr_v = wr_v8.at[0]
    best_v = best_v8.at[0]
    bidx_v = bidx_v8.at[0]

    def cp(src, dst, i):
        return pltpu.make_async_copy(src, dst, sems.at[i])

    c_cp = cp(c_hbm, c_v, SEM_C)
    wr_cp = cp(wr_hbm, wr_v, SEM_WR)
    x0_cp = cp(x_hbm.at[0, pl.ds(0, TP), :], x_v.at[pl.ds(0, TP), :], SEM_X0)
    wm1_cp = cp(wmod_hbm.at[:, pl.ds(2 * D, 4 * D)], wmod_v.at[:, pl.ds(2 * D, 4 * D)], SEM_WM1)
    k_cp = cp(k_hbm.at[0, :, pl.ds(sk - W, W), :], k_v, SEM_K)
    v_cp = cp(v_hbm.at[0, :, pl.ds(sk - W, W), :], v_v, SEM_V)
    wg_cp = cp(wg_hbm, wg_v, SEM_WG)
    wu_cp = cp(wu_hbm, wu_v, SEM_WU)
    wd_cp = cp(wd_hbm, wd_v.at[:, pl.ds(0, D)], SEM_WD)

    def x_cp(t):
        r0 = _mo(t * TQ, TQ)
        return cp(x_hbm.at[0, pl.ds(r0, TQ), :], x_v.at[pl.ds(r0, TQ), :], SEM_X + t)

    def wm_cp(part, j):
        c0 = _mo(part * D + j * 256, 256)
        return cp(wmod_hbm.at[:, pl.ds(c0, 256)], wmod_v.at[:, pl.ds(c0, 256)], (SEM_WMS, SEM_WMC)[part] + j)

    def wq0_cp(j):
        return cp(wq_hbm.at[:, pl.ds(j * 256, 256)], wq_v.at[0, :, pl.ds(j * 256, 256)], SEM_WQ0 + j)

    def wq_cp(g):
        return cp(wq_hbm.at[:, pl.ds(_mo(g * GW, GW), GW)], wq_v.at[g], SEM_WQ + g)

    def wo_cp(g):
        return cp(wo_hbm.at[pl.ds(_mo(g * GW, GW), GW), :], wo_v.at[g], SEM_WO + g)

    def out_copy(r0, n):
        return cp(out_v.at[pl.ds(r0, n), :], out_hbm.at[0, pl.ds(r0, n), :], SEM_OUT)

    for c_ in ([c_cp, wr_cp, x0_cp] + [wm_cp(p_, j) for j in range(4) for p_ in range(2)]
               + [wq0_cp(j) for j in range(4)] + [x_cp(2), x_cp(3), k_cp]
               + [x_cp(t) for t in range(4, NT)]
               + [v_cp, wo_cp(0), wq_cp(1), wm1_cp,
                  wo_cp(1), wq_cp(2), wo_cp(2), wq_cp(3), wo_cp(3), wg_cp, wu_cp, wd_cp]):
        c_.start()

    def ln1_rows(r0, n, lo=None):
        x = x_v[pl.ds(r0, n), :].astype(f32)
        if lo is not None:
            x = _gate(x, *lo)
        sa = mod_v[0:1, 0 * D:1 * D]
        ca = mod_v[0:1, 1 * D:2 * D]
        y = _ln(x) * (1.0 + ca) + sa
        h_v[pl.ds(r0, n), :] = y.astype(bf16)
        return y

    def ln2_rows(r0, n, valid=None, lo=None):
        sb = mod_v[0:1, 3 * D:4 * D]
        cb = mod_v[0:1, 4 * D:5 * D]
        gb = mod_v[0:1, 5 * D:6 * D]
        x2 = x_v[pl.ds(r0, n), :].astype(f32)
        if lo is not None:
            x2 = _gate(x2, *lo)
        h2 = (_ln(x2) * (1.0 + cb) + sb).astype(bf16).astype(f32)
        y = x2 + gb * h2
        out_v[pl.ds(r0, n), :] = y.astype(bf16)
        r = jnp.sum(h2 * wr_v[...].astype(f32), axis=-1, keepdims=True)
        r = r.astype(bf16).astype(f32)
        if valid is not None:
            r = jnp.where(valid, r, -jnp.inf)
        r = jnp.broadcast_to(r, (n, 128))
        best = best_v[...]
        bidx = bidx_v[...]
        cand = cand_v[...]
        rows = lax.broadcasted_iota(jnp.int32, (8, 128), 0)
        for j in range(n // 8):
            rj = r[8 * j:8 * (j + 1), :]
            upd = rj > best
            best = jnp.where(upd, rj, best)
            bidx = jnp.where(upd, rows + (r0 + 8 * j), bidx)
            cand = jnp.where(jnp.concatenate([upd] * (D // 128), axis=1), h2[8 * j:8 * (j + 1), :], cand)
        best_v[...] = best
        bidx_v[...] = bidx
        cand_v[...] = cand
        return y, cand

    def mod_cols(c0, n):
        m = jnp.dot(sc_v[...], wmod_v[:, pl.ds(c0, n)], preferred_element_type=f32)
        mod_v[:, pl.ds(c0, n)] = m[0:8].astype(bf16).astype(f32)

    def qproj(hr0, qr0, n, g, c0, nc, hi=None, h=None):
        if h is None:
            h = h_v[pl.ds(hr0, n), :]
        if hi is not None:
            flag, tok = hi
            h = _gate1(h, flag, jnp.concatenate([tok, tok], axis=0).astype(bf16))
        q = jnp.dot(h, wq_v[g, :, c0:c0 + nc], preferred_element_type=f32)
        q_v[pl.ds(qr0, n), c0:c0 + nc] = (q * QSCALE).astype(bf16)
        return q

    with _scope('P0_wait_c_wm0'):
        flag_s[0] = 0
        c_cp.wait()
        cf = c_v[...].astype(f32)
        sc = (cf * jax.nn.sigmoid(cf)).astype(bf16)
        sc_v[...] = jnp.broadcast_to(sc, (16, D))
        best_v[...] = jnp.full(best_v.shape, -jnp.inf, f32)
        bidx_v[...] = jnp.zeros(bidx_v.shape, jnp.int32)
        cand_v[...] = jnp.zeros(cand_v.shape, f32)
        x0_cp.wait()
        for i in range(TP // 128):
            acc_v[i * 128:(i + 1) * 128, :] = _ln(x_v[i * 128:(i + 1) * 128, :].astype(f32))

    def mod_chunk(j, carry):
        wm_cp(0, j).wait()
        wm_cp(1, j).wait()
        c0 = pl.multiple_of(j * 256, 256)
        scv = sc_v[...]
        sa = jnp.dot(scv, wmod_v[:, pl.ds(c0, 256)], preferred_element_type=f32)[0:8].astype(bf16).astype(f32)
        ca = jnp.dot(scv, wmod_v[:, pl.ds(D + c0, 256)], preferred_element_type=f32)[0:8].astype(bf16).astype(f32)
        mod_v[:, pl.ds(c0, 256)] = sa
        mod_v[:, pl.ds(D + c0, 256)] = ca
        h_v[0:TP, pl.ds(c0, 256)] = (acc_v[0:TP, pl.ds(c0, 256)] * (1.0 + ca[0:1]) + sa[0:1]).astype(bf16)
        return carry

    with _scope('P1_mod'):
        lax.fori_loop(0, 4, mod_chunk, 0)

    def q0_cols(r0, n, j0, j1, ln_r0):
        flag = flag_s[0] > 0
        h = h_v[pl.ds(r0, n), :]
        toks = {}
        npc = (j1 - j0) - LAG0
        base, extra = divmod(TQ // 16, npc)
        sizes = [(base + (1 if i < extra else 0)) * 16 for i in range(npc)]
        off = 0
        for i, j in enumerate(range(j0, j1)):
            hi = (flag, toks[i - LAG0]) if (i - LAG0) in toks else None
            q = qproj(r0, r0, n, 0, j * DH, DH, hi, h)
            if i < npc:
                lo = (flag, q[0:8]) if P0PIN else None
                toks[i] = _token(ln1_rows(_mo(ln_r0 + off, 16), sizes[i], lo))
                off += sizes[i]

    with _scope('P2_q0'):
        wq0_cp(0).wait()
        qproj(0, 0, TP, 0, 0, 256)
        wq0_cp(1).wait()
        qproj(0, 0, TP, 0, 256, 256)
        wq0_cp(2).wait()
        wq0_cp(3).wait()
        x_cp(2).wait()
        q0_cols(0, TP, 4, 8, 2 * TQ)
        k_cp.wait()

    def q0_tile(t, carry):
        tn = jnp.minimum(t + 1, NT - 1)

        @pl.when(t + 1 < NT)
        def _():
            x_cp(t + 1).wait()

        q0_cols(pl.multiple_of(t * TQ, TQ), TQ, 0, REP, tn * TQ)
        gk = jnp.minimum(t - 2, HKV - 1)
        kt_v[gk] = k_v[gk].T
        return carry

    with _scope('P3_q0'):
        lax.fori_loop(2, NT, q0_tile, 0)
        v_cp.wait()
        wo_cp(0).wait()

    def body(its, seq, phase):
        flag = flag_s[0] > 0
        st = dict(lo=None, hi=None, pend=None, next=None)

        def flush_op():
            if st['pend'] is not None:
                st['pend']()
                st['pend'] = None

        for it in its:
            g = it // NT
            t = it % NT
            a0 = _mo(t * TQ, TQ)
            q0 = _mo((it % NQS) * TQ, TQ)
            nit = it + 1

            def ln_piece(j, t=t, n=PR):
                lo = (flag, st['lo']) if st['lo'] is not None else None
                if isinstance(t, int):
                    y, b = ln2_rows((t - 1) * TQ + j * n, n, None, lo)
                else:
                    tl = jnp.maximum(t - 1, 0)
                    y, b = ln2_rows(_mo(tl * TQ + j * n, n), n, t > 0, lo)
                st['hi'] = jnp.maximum(_token(y), _token(b))

            def qk(hh, g=g, q0=q0):
                qh = q_v[pl.ds(q0, TQ), hh * DH:(hh + 1) * DH]
                s = jnp.dot(qh, kt_v[g], preferred_element_type=f32)
                if st['hi'] is not None:
                    s = _gate1(s, flag, st['hi'])
                    st['hi'] = None
                m = jnp.max(s, axis=-1, keepdims=True)
                p = jnp.exp2(s - m)
                l = jnp.sum(p, axis=-1, keepdims=True)
                return p.astype(bf16), l

            def pv(pl_, g=g):
                p, l = pl_
                o = jnp.dot(p, v_v[g], preferred_element_type=f32)
                if PINLO == 'V' or 'Q' not in seq:
                    st['lo'] = o[0:8]
                return o * _recip(l)

            def op(o, hh, g=g, a0=a0):
                y = jnp.dot(o.astype(bf16), wo_v[g, hh * DH:(hh + 1) * DH, :], preferred_element_type=f32)
                if hh == 0 and phase == 'A':
                    acc_v[pl.ds(a0, TQ), :] = y
                elif hh == 0 and phase == 'B':
                    acc_v[pl.ds(a0, TQ), :] = jnp.where(g == 0, 0.0, acc_v[pl.ds(a0, TQ), :]) + y
                elif hh == REP - 1 and phase == 'C':
                    ga = mod_v[0:1, 2 * D:3 * D]
                    x = x_v[pl.ds(a0, TQ), :].astype(f32)
                    x_v[pl.ds(a0, TQ), :] = (x + ga * (acc_v[pl.ds(a0, TQ), :] + y)).astype(bf16)
                else:
                    acc_v[pl.ds(a0, TQ), :] += y

            sp = None
            for hh in range(REP):
                for tok in seq:
                    if tok == 'K':
                        sp = qk(hh)
                    elif tok == 'V':
                        o = pv(sp)
                        new_pend = (lambda o=o, hh=hh, op=op: op(o, hh))
                        if 'O' in seq[seq.index('V'):]:
                            st['next'] = new_pend
                        else:
                            st['pend'] = new_pend
                    elif tok == 'O':
                        flush_op()
                        if st['next'] is not None:
                            st['pend'] = st['next']
                            st['next'] = None
                    elif tok == 'L':
                        ln_piece(hh)
                    elif tok == 'Q':
                        q = qproj(_mo((nit % NT) * TQ, TQ), _mo((nit % NQS) * TQ, TQ), TQ, nit // NT, hh * DH, DH)
                        if PINLO == 'Q':
                            st['lo'] = q[0:8]
                    elif tok == 'M':
                        if hh in (2, 5):
                            mod_cols(pl.multiple_of(2 * D + jnp.maximum(it - NT, 0) * 256 + (hh // 4) * 128, 128), 128)
            if phase == 'C':
                flush_op()
        flush_op()
        if phase == 'C':
            for it in its:
                t = it % NT
                if isinstance(t, int):
                    out_copy((t - 1) * TQ, TQ).start()
                else:
                    @pl.when(t > 0)
                    def _():
                        out_copy(_mo((t - 1) * TQ, TQ), TQ).start()

    def body_a(i, carry):
        body([i], SEQ_A, 'A')
        return carry

    with _scope('LA'):
        lax.fori_loop(0, NT - 1, body_a, 0)

    wq_cp(1).wait()
    wm1_cp.wait()
    wo_cp(1).wait()
    wq_cp(2).wait()
    wo_cp(2).wait()
    wq_cp(3).wait()

    def body_b(i, carry):
        body([i], SEQ_B, 'B')
        return carry

    with _scope('LB'):
        lax.fori_loop(NT - 1, 3 * NT, body_b, 0)

    wr_cp.wait()
    wo_cp(3).wait()

    def body_c(i, carry):
        body([i], SEQ_C, 'C')
        return carry

    with _scope('LC'):
        lax.fori_loop(3 * NT, NIT - 1, body_c, 0)

    with _scope('E1_last'):
        wg_cp.wait()
        wu_cp.wait()
        wd_cp.wait()
        body([NIT - 1], SEQ_D, 'C')
        r0 = (NT - 1) * TQ
        ln2_rows(r0, TQ)
        out_copy(r0, TQ).start()

    with _scope('E2_ffn'):
        best = best_v[...]
        bidx = bidx_v[...]
        cand = cand_v[...]
        rmax = jnp.max(best, axis=0, keepdims=True)
        idx_v = jnp.min(jnp.where(best == rmax, bidx, S), axis=0, keepdims=True)
        idx_v = jnp.minimum(idx_v, S - 1)
        idx = idx_v[0, 0]
        g0 = pl.multiple_of((idx // 8) * 8, 8)
        gb = mod_v[0:1, 5 * D:6 * D]
        h2b = cand.astype(bf16)
        gt = jnp.dot(h2b, wg_v[...], preferred_element_type=f32)
        up = jnp.dot(h2b, wu_v[...], preferred_element_type=f32)
        a = (gt * jax.nn.sigmoid(gt) * up).astype(bf16)
        y = jnp.dot(a, wd_v[:, 0:D], preferred_element_type=f32)
        y = y * jax.nn.sigmoid(rmax[:, 0:1])
        x2 = x_v[pl.ds(g0, 8), :].astype(f32)
        rows8 = lax.broadcasted_iota(jnp.int32, (8, 1), 0) + g0
        out_copy(0, S).wait()
        new = (x2 + gb * (cand + y)).astype(bf16)
        out_v[pl.ds(g0, 8), :] = jnp.where(rows8 == idx, new, out_v[pl.ds(g0, 8), :])
        fix = out_copy(g0, 8)
        fix.start()
        fix.wait()


@jax.jit
def pallas_adaLN_cond__sliding_block_cached__moe_arch_mod__prompt_kernel(
    A_x, A_k_cache, A_v_cache, A_wq, A_wo, B_x, B_w_r, B_w_gate, B_w_up, B_w_down, c, w_mod,
):
    del B_x
    any_spec = pl.BlockSpec(memory_space=pl.ANY)
    return pl.pallas_call(
        _kernel,
        out_shape=jax.ShapeDtypeStruct(A_x.shape, A_x.dtype),
        in_specs=[any_spec] * 11,
        out_specs=any_spec,
        scratch_shapes=[
            pltpu.VMEM((S, D), bf16),
            pltpu.VMEM((S, D), bf16),
            pltpu.VMEM((S, D), bf16),
            pltpu.VMEM((NQS * TQ, GW), bf16),
            pltpu.VMEM((S, D), f32),
            pltpu.VMEM((D, 6 * D + PADC), bf16),
            pltpu.VMEM((HKV, D, GW), bf16),
            pltpu.VMEM((HKV, GW, D), bf16),
            pltpu.VMEM((D, F), bf16),
            pltpu.VMEM((D, F), bf16),
            pltpu.VMEM((F, D + PADC), bf16),
            pltpu.VMEM((HKV, W, DH), bf16),
            pltpu.VMEM((HKV, W, DH), bf16),
            pltpu.VMEM((HKV, DH, W), bf16),
            pltpu.VMEM((8, 1, D), bf16),
            pltpu.VMEM((8, 1, D), bf16),
            pltpu.VMEM((16, D), bf16),
            pltpu.VMEM((8, 6 * D), f32),
            pltpu.VMEM((8, 8, 128), f32),
            pltpu.VMEM((8, 8, 128), jnp.int32),
            pltpu.VMEM((8, D), f32),
            pltpu.SMEM((1,), jnp.int32),
            pltpu.SemaphoreType.DMA((NSEM,)),
        ],
        compiler_params=pltpu.CompilerParams(vmem_limit_bytes=110 * 1024 * 1024),
    )(A_x, A_k_cache, A_v_cache, A_wq, A_wo, B_w_r.reshape(1, D), B_w_gate, B_w_up, B_w_down, c, w_mod)
```

```python
import contextlib
import math
import os

import jax
import jax.numpy as jnp
from jax import lax
from jax.experimental import pallas as pl
from jax.experimental.pallas import tpu as pltpu

S = 2048
D = 1024
HQ = 32
HKV = 4
REP = HQ // HKV
DH = 128
GW = REP * DH
W = 512
F = 3584
EPS = 1e-5
TQ = 256
NT = S // TQ
NIT = NT * HKV
NQS = NT
PADC = 128
TP = 512
SEQ_A = os.environ.get('KP_SEQA', 'KOV')
SEQ_B = os.environ.get('KP_SEQB', 'KQVOM')
SEQ_C = os.environ.get('KP_SEQC', 'KQVOL')
SEQ_D = os.environ.get('KP_SEQD', 'KoVOL')
PINLO = os.environ.get('KP_PINLO', 'Q')
UNA = int(os.environ.get('KP_UNA', 1))
UNB = int(os.environ.get('KP_UNB', 2))
UNC = int(os.environ.get('KP_UNC', 2))
P0PIN = int(os.environ.get('KP_P0PIN', 0))
LAG0 = int(os.environ.get('KP_LAG0', 2))
LPC = os.environ.get('KP_LPC', 'Q0,O128').split(',')
LPD = os.environ.get('KP_LPD', 'V0,V128,O0,O128').split(',')
LPE = os.environ.get('KP_LPE', 'O192,O256,O320,O384').split(',')
NKC = int(os.environ.get('KP_NKC', 4))
KC = D // NKC
UNP = int(os.environ.get('KP_UNP', 1))
OS = int(os.environ.get('KP_OS', 32))
SCOPES = int(os.environ.get('KP_SCOPES', 0))
QSCALE = (DH ** -0.5) * math.log2(math.e)
PR = TQ // REP

f32 = jnp.float32
bf16 = jnp.bfloat16

(SEM_C, SEM_WR, SEM_X0, SEM_WM1, SEM_K, SEM_V, SEM_WG, SEM_WU, SEM_WD, SEM_OUT, SEM_K0, SEM_WM2) = range(12)
SEM_X = 12
SEM_WQ = SEM_X + NT
SEM_WO = SEM_WQ + HKV
SEM_WQ0 = SEM_WO + HKV
SEM_WMS = SEM_WQ0 + NKC
SEM_WMC = SEM_WMS + NKC
NSEM = SEM_WMC + NKC


def _scope(name):
    return jax.named_scope(name) if SCOPES else contextlib.nullcontext()


def _ln(x):
    m = jnp.mean(x, axis=-1, keepdims=True)
    xc = x - m
    v = jnp.mean(xc * xc, axis=-1, keepdims=True)
    return xc * lax.rsqrt(v + EPS)


def _recip(l):
    r = pl.reciprocal(l, approx=True)
    return r * (2.0 - l * r)


def _mo(x, m):
    return x if isinstance(x, int) else pl.multiple_of(x, m)


def _gate(x, flag, tok):
    n = x.shape[0]
    xs = jnp.where(flag, jnp.concatenate([tok] * (n // 8), axis=0), x[:, 0:128])
    return jnp.concatenate([xs, x[:, 128:]], axis=1)


def _gate1(x, flag, tok):
    r = tok.shape[0]
    x0 = jnp.where(flag, tok, x[0:r, 0:128])
    if x.shape[1] > 128:
        x0 = jnp.concatenate([x0, x[0:r, 128:]], axis=1)
    return jnp.concatenate([x0, x[r:]], axis=0)


def _rows(v8, n):
    return v8 if n == 8 else jnp.concatenate([v8] * (n // 8), axis=0)


def _token(y):
    t = y[:, 0:128]
    for j in range(1, y.shape[1] // 128):
        t = jnp.maximum(t, y[:, j * 128:(j + 1) * 128])
    u = t[0:8]
    for j in range(1, y.shape[0] // 8):
        u = jnp.maximum(u, t[8 * j:8 * (j + 1)])
    return u


def _kernel(x_hbm, k_hbm, v_hbm, wq_hbm, wo_hbm, wr_hbm, wg_hbm, wu_hbm, wd_hbm, c_hbm, wmod_hbm,
            out_hbm,
            x_v, out_v, h_v, q_v, acc_v, wmod_v, wq_v, wo_v, wg_v, wu_v, wd_v, k_v, v_v, kt_v,
            c_v8, wr_v8, sc_v, mod_v, best_v, bidx_v, aux_v, flag_s, sems):
    sk = k_hbm.shape[2]
    c_v = c_v8.at[0]
    wr_v = wr_v8.at[0]

    def cp(src, dst, i):
        return pltpu.make_async_copy(src, dst, sems.at[i])

    c_cp = cp(c_hbm, c_v, SEM_C)
    wr_cp = cp(wr_hbm, wr_v, SEM_WR)
    x0_cp = cp(x_hbm.at[0, pl.ds(0, TP), :], x_v.at[pl.ds(0, TP), :], SEM_X0)
    wm1_cp = cp(wmod_hbm.at[:, pl.ds(2 * D, D)], wmod_v.at[:, pl.ds(2 * D, D)], SEM_WM1)
    wm2_cp = cp(wmod_hbm.at[:, pl.ds(3 * D, 3 * D)], wmod_v.at[:, pl.ds(3 * D, 3 * D)], SEM_WM2)
    k0_cp = cp(k_hbm.at[0, 0, pl.ds(sk - W, W), :], k_v.at[0], SEM_K0)
    k_cp = cp(k_hbm.at[0, pl.ds(1, HKV - 1), pl.ds(sk - W, W), :], k_v.at[pl.ds(1, HKV - 1)], SEM_K)
    v_cp = cp(v_hbm.at[0, :, pl.ds(sk - W, W), :], v_v, SEM_V)
    wg_cp = cp(wg_hbm, wg_v, SEM_WG)
    wu_cp = cp(wu_hbm, wu_v, SEM_WU)
    wd_cp = cp(wd_hbm, wd_v.at[:, pl.ds(0, D)], SEM_WD)

    def x_cp(t):
        r0 = _mo(t * TQ, TQ)
        return cp(x_hbm.at[0, pl.ds(r0, TQ), :], x_v.at[pl.ds(r0, TQ), :], SEM_X + t)

    def wm_cp(part, j):
        c0 = _mo(part * D + j * KC, KC)
        return cp(wmod_hbm.at[:, pl.ds(c0, KC)], wmod_v.at[:, pl.ds(c0, KC)], (SEM_WMS, SEM_WMC)[part] + j)

    def wq0_cp(j):
        r0 = _mo(j * KC, KC)
        return cp(wq_hbm.at[pl.ds(r0, KC), pl.ds(0, GW)], wq_v.at[0, pl.ds(r0, KC), :], SEM_WQ0 + j)

    def wq_cp(g):
        return cp(wq_hbm.at[:, pl.ds(_mo(g * GW, GW), GW)], wq_v.at[g], SEM_WQ + g)

    def wo_cp(g):
        return cp(wo_hbm.at[pl.ds(_mo(g * GW, GW), GW), :], wo_v.at[g], SEM_WO + g)

    def out_copy(r0, n):
        return cp(out_v.at[pl.ds(r0, n), :], out_hbm.at[0, pl.ds(r0, n), :], SEM_OUT)

    for c_ in ([c_cp, x0_cp] + [c_ for j in range(NKC) for c_ in (wm_cp(0, j), wm_cp(1, j), wq0_cp(j))]
               + [x_cp(2), k0_cp, x_cp(3), k_cp, wr_cp]
               + [x_cp(t) for t in range(4, NT)]
               + [v_cp, wo_cp(0), wq_cp(1), wm1_cp, wm2_cp,
                  wo_cp(1), wq_cp(2), wo_cp(2), wq_cp(3), wo_cp(3), wg_cp, wu_cp, wd_cp]):
        c_.start()

    def ln1_rows(r0, n, lo=None):
        x = x_v[pl.ds(r0, n), :].astype(f32)
        if lo is not None:
            x = _gate(x, *lo)
        y = _ln(x) * _rows(mod_v[:, D:2 * D], n) + _rows(mod_v[:, 0:D], n)
        h_v[pl.ds(r0, n), :] = y.astype(bf16)
        return y

    def ln2_rows(r0, n, valid=None, lo=None):
        av = _rows(aux_v[0], n)
        bv = _rows(aux_v[1], n)
        rv = _rows(aux_v[2], n)
        r_c = _rows(aux_v[3, :, 0:128], n)
        x2 = x_v[pl.ds(r0, n), :].astype(f32)
        if lo is not None:
            x2 = _gate(x2, *lo)
        m = jnp.mean(x2, axis=-1, keepdims=True)
        xc = x2 - m
        var = jnp.mean(xc * xc, axis=-1, keepdims=True)
        rs = lax.rsqrt(var + EPS)
        y = (x2 + bv) + (xc * rs) * av
        out_v[pl.ds(r0, n), :] = y.astype(bf16)
        r = jnp.sum(xc * rv, axis=-1, keepdims=True) * rs
        r = (jnp.broadcast_to(r, (n, 128)) + r_c).astype(bf16).astype(f32)
        if valid is not None:
            r = jnp.where(valid, r, -jnp.inf)
        mb = jnp.broadcast_to(m, (n, 128))
        rsb = jnp.broadcast_to(rs, (n, 128))
        best = best_v[0]
        bm = best_v[1]
        brs = best_v[2]
        bidx = bidx_v[0]
        rows = lax.broadcasted_iota(jnp.int32, (8, 128), 0)
        for j in range(n // 8):
            sl = slice(8 * j, 8 * (j + 1))
            upd = r[sl] > best
            best = jnp.where(upd, r[sl], best)
            bm = jnp.where(upd, mb[sl], bm)
            brs = jnp.where(upd, rsb[sl], brs)
            bidx = jnp.where(upd, rows + (r0 + 8 * j), bidx)
        best_v[0] = best
        best_v[1] = bm
        best_v[2] = brs
        bidx_v[0] = bidx
        return y, best

    def mod_cols(c0, n):
        m = jnp.dot(sc_v[...], wmod_v[:, pl.ds(c0, n)], preferred_element_type=f32)
        mod_v[:, pl.ds(c0, n)] = m[0:8].astype(bf16).astype(f32)

    def qproj(hr0, qr0, n, g, c0, nc, hi=None, h=None):
        if h is None:
            h = h_v[pl.ds(hr0, n), :]
        if hi is not None:
            flag, tok = hi
            h = _gate1(h, flag, jnp.concatenate([tok, tok], axis=0).astype(bf16))
        q = jnp.dot(h, wq_v[g, :, c0:c0 + nc], preferred_element_type=f32)
        q_v[pl.ds(qr0, n), c0:c0 + nc] = (q * QSCALE).astype(bf16)
        return q

    with _scope('P0_wait_c_wm0'):
        flag_s[0] = 0
        c_cp.wait()
        cf = c_v[...].astype(f32)
        sc = (cf * jax.nn.sigmoid(cf)).astype(bf16)
        sc_v[...] = jnp.broadcast_to(sc, (16, D))
        best_v[0] = jnp.full((8, 128), -jnp.inf, f32)
        best_v[1] = jnp.zeros((8, 128), f32)
        best_v[2] = jnp.zeros((8, 128), f32)
        bidx_v[0] = jnp.zeros((8, 128), jnp.int32)
        x0_cp.wait()

        def norm_rows(i, carry):
            r0 = pl.multiple_of(i * 128, 128)
            acc_v[pl.ds(r0, 128), :] = _ln(x_v[pl.ds(r0, 128), :].astype(f32))
            return carry

        lax.fori_loop(0, TP // 128, norm_rows, 0)

    def k_chunk(j, carry):
        wm_cp(0, j).wait()
        wm_cp(1, j).wait()
        c0 = pl.multiple_of(j * KC, KC)
        scv = sc_v[...]
        sa = jnp.dot(scv, wmod_v[:, pl.ds(c0, KC)], preferred_element_type=f32)[0:8].astype(bf16).astype(f32)
        ca = jnp.dot(scv, wmod_v[:, pl.ds(D + c0, KC)], preferred_element_type=f32)[0:8].astype(bf16).astype(f32)
        mod_v[:, pl.ds(c0, KC)] = sa
        mod_v[:, pl.ds(D + c0, KC)] = 1.0 + ca
        h_v[0:TP, pl.ds(c0, KC)] = (acc_v[0:TP, pl.ds(c0, KC)] * _rows(1.0 + ca, TP) + _rows(sa, TP)).astype(bf16)
        wq0_cp(j).wait()
        part = jnp.dot(h_v[0:TP, pl.ds(c0, KC)], wq_v[0, pl.ds(c0, KC), :], preferred_element_type=f32)
        tot = jnp.where(j == 0, 0.0, acc_v[TP:2 * TP, :]) + part
        acc_v[TP:2 * TP, :] = tot
        q_v[0:TP, :] = (tot * QSCALE).astype(bf16)
        return carry

    with _scope('P1_kchunks'):
        lax.fori_loop(0, NKC, k_chunk, 0)

    def q0_cols(r0, n, j0, j1, ln_r0):
        flag = flag_s[0] > 0
        h = h_v[pl.ds(r0, n), :]
        toks = {}
        npc = (j1 - j0) - LAG0
        base, extra = divmod(TQ // 16, npc)
        sizes = [(base + (1 if i < extra else 0)) * 16 for i in range(npc)]
        off = 0
        for i, j in enumerate(range(j0, j1)):
            hi = (flag, toks[i - LAG0]) if (i - LAG0) in toks else None
            q = qproj(r0, r0, n, 0, j * DH, DH, hi, h)
            if i < npc:
                lo = (flag, q[0:8]) if P0PIN else None
                toks[i] = _token(ln1_rows(_mo(ln_r0 + off, 16), sizes[i], lo))
                off += sizes[i]

    with _scope('P2_ln'):
        x_cp(2).wait()
        ln1_rows(2 * TQ, TQ)
        k0_cp.wait()

    def q0_tile(i, carry):
        for u in range(UNP):
            t = 2 + i * UNP + u

            @pl.when(t + 1 < NT)
            def _():
                x_cp(t + 1).wait()

        @pl.when(i == 1)
        def _():
            k_cp.wait()

        for u in range(UNP):
            t = 2 + i * UNP + u
            q0_cols(pl.multiple_of(t * TQ, TQ), TQ, 0, REP, jnp.minimum(t + 1, NT - 1) * TQ)
            gk = jnp.clip(t - 2 - (UNP - 1), 0, HKV - 1)
            kt_v[gk] = k_v[gk].T
        return carry

    with _scope('P3_q0'):
        lax.fori_loop(0, (NT - 2) // UNP, q0_tile, 0)
        v_cp.wait()
        wm1_cp.wait()

    def body(its, seq, phase, pins=None):
        flag = flag_s[0] > 0
        st = dict(lo=None, hi=None, pend=None, next=None)

        def flush_op(rb=TQ):
            if st['pend'] is not None:
                st['pend'](st.get('done', 0), rb)
                st['done'] = rb % TQ
                if rb == TQ:
                    st['pend'] = None

        for u_, it in enumerate(its):
            g = it // NT
            t = it % NT
            a0 = _mo(t * TQ, TQ)
            q0 = a0

            def ln_step(j, pins, t=t):
                n = PR // len(pins)
                hi = st['hi']
                for i, pin in enumerate(pins):
                    src_ = st.get(pin[0])
                    if src_ is None:
                        src_, r_ = st['V'], 0
                    else:
                        r_ = int(pin[1:])
                    c_ = 512 if r_ >= TQ else 0
                    r_ = r_ % TQ
                    lo = (flag, src_[r_:r_ + 8, c_:c_ + 128])
                    off = j * PR + i * n
                    if isinstance(t, int):
                        y, b = ln2_rows((t - 1) * TQ + off, n, None, lo)
                    else:
                        tl = jnp.maximum(t - 1, 0)
                        y, b = ln2_rows(_mo(tl * TQ + off, n), n, t > 0, lo)
                    tk = jnp.maximum(_token(y), b)
                    hi = tk if hi is None else jnp.maximum(hi, tk)
                st['hi'] = hi

            def qk(hh, g=g, q0=q0):
                qh = q_v[pl.ds(q0, TQ), hh * DH:(hh + 1) * DH]
                s = jnp.dot(qh, kt_v[g], preferred_element_type=f32)
                if st['hi'] is not None:
                    s = _gate1(s, flag, st['hi'])
                    st['hi'] = None
                m = jnp.max(s, axis=-1, keepdims=True)
                p = jnp.exp2(s - m)
                st['K'] = s
                st['P'] = p
                l = jnp.sum(p, axis=-1, keepdims=True)
                return p.astype(bf16), l

            def pv(pl_, g=g):
                p, l = pl_
                o = jnp.dot(p, v_v[g], preferred_element_type=f32)
                st['V'] = o
                return o * _recip(l)

            def op(o, hh, ra, rb, g=g, a0=a0):
                n = rb - ra
                r0 = _mo(a0 + ra, 16)
                y = jnp.dot(o[ra:rb].astype(bf16), wo_v[g, hh * DH:(hh + 1) * DH, :], preferred_element_type=f32)
                st['O'] = y
                if hh == 0 and phase == 'B':
                    acc_v[pl.ds(r0, n), :] = jnp.where(g == 0, 0.0, acc_v[pl.ds(r0, n), :]) + y
                elif hh == REP - 1 and phase == 'C':
                    ga = _rows(mod_v[:, 2 * D:3 * D], n)
                    x = x_v[pl.ds(r0, n), :].astype(f32)
                    x_v[pl.ds(r0, n), :] = (x + ga * (acc_v[pl.ds(r0, n), :] + y)).astype(bf16)
                else:
                    acc_v[pl.ds(r0, n), :] += y

            sp = None
            for hh in range(REP):
                for tok in seq:
                    if tok == 'K':
                        sp = qk(hh)
                    elif tok == 'V':
                        o = pv(sp)
                        new_pend = (lambda ra, rb, o=o, hh=hh, op=op: op(o, hh, ra, rb))
                        if 'O' in seq[seq.index('V'):]:
                            st['next'] = new_pend
                        else:
                            st['pend'] = new_pend
                    elif tok == 'O':
                        flush_op()
                        if st['next'] is not None:
                            st['pend'] = st['next']
                            st['next'] = None
                    elif tok == 'o':
                        flush_op(OS)
                    elif tok == 'L':
                        if hh > 0:
                            ln_step(hh - 1, pins)
                        if hh == REP - 1:
                            ln_step(hh, LPE)
                    elif tok == 'Q':
                        q = qproj(a0, a0, TQ, g + 1, hh * DH, DH)
                        st['Q'] = q
                    elif tok == 'M':
                        pos = u_ * REP + hh
                        nm = -(-32 * UNB // (3 * NT))
                        spots = [(2 * k_ + 1) * REP * UNB // (2 * nm) for k_ in range(nm)]
                        if pos in spots:
                            j = jnp.minimum((its[0] // UNB) * nm + spots.index(pos), 31)
                            mod_cols(pl.multiple_of(2 * D + j * 128, 128), 128)
            if phase == 'C':
                flush_op()
        flush_op()
        if phase == 'C':
            for it in its:
                t = it % NT
                if isinstance(t, int):
                    out_copy((t - 1) * TQ, TQ).start()
                else:
                    @pl.when(t > 0)
                    def _():
                        out_copy(_mo((t - 1) * TQ, TQ), TQ).start()

    def body_b(i, carry):
        it = i * UNB

        @pl.when(it % NT == 0)
        def _():
            wo_cp(it // NT).wait()
            wq_cp(it // NT + 1).wait()

        @pl.when(it == 2)
        def _():
            wm2_cp.wait()

        body([it + u for u in range(UNB)], SEQ_B, 'B')
        return carry

    with _scope('LB'):
        lax.fori_loop(0, 3 * NT // UNB, body_b, 0)

    wr_cp.wait()
    wo_cp(3).wait()
    sb_ = mod_v[:, 3 * D:4 * D]
    cb1_ = 1.0 + mod_v[:, 4 * D:5 * D]
    gb_ = mod_v[:, 5 * D:6 * D]
    wr8 = wr_v[...].astype(f32)
    wr_ = jnp.concatenate([wr8[r_:r_ + 1, :] for r_ in range(8)], axis=1)
    aux_v[0] = gb_ * cb1_
    aux_v[1] = gb_ * sb_
    aux_v[2] = cb1_ * wr_
    aux_v[3] = jnp.broadcast_to(jnp.sum(sb_ * wr_, axis=-1, keepdims=True), (8, D))

    def body_c(i, carry):
        body([i * UNC + u for u in range(UNC)], SEQ_D, 'C', LPD)
        return carry

    with _scope('LC'):
        lax.fori_loop(3 * NT // UNC, NIT // UNC, body_c, 0)

    with _scope('E1_last'):
        wg_cp.wait()
        wu_cp.wait()
        wd_cp.wait()
        r0 = (NT - 1) * TQ
        ln2_rows(r0, TQ)
        out_copy(r0, TQ).start()

    with _scope('E2_ffn'):
        best = best_v[0]
        bidx = bidx_v[0]
        rmax = jnp.max(best, axis=0, keepdims=True)
        idx_v = jnp.min(jnp.where(best == rmax, bidx, S), axis=0, keepdims=True)
        idx = jnp.minimum(idx_v[0, 0], S - 1)
        g0 = pl.multiple_of((idx // 8) * 8, 8)
        sb = mod_v[:, 3 * D:4 * D]
        cb = mod_v[:, 4 * D:5 * D]
        gb = mod_v[:, 5 * D:6 * D]
        x2 = x_v[pl.ds(g0, 8), :].astype(f32)
        h2 = (x2 - best_v[1][:, 0:1]) * best_v[2][:, 0:1] * (1.0 + cb) + sb
        h2b = h2.astype(bf16)
        gt = jnp.dot(h2b, wg_v[...], preferred_element_type=f32)
        up = jnp.dot(h2b, wu_v[...], preferred_element_type=f32)
        a = (gt * jax.nn.sigmoid(gt) * up).astype(bf16)
        y = jnp.dot(a, wd_v[:, 0:D], preferred_element_type=f32)
        y = y * jax.nn.sigmoid(rmax[:, 0:1])
        rows8 = lax.broadcasted_iota(jnp.int32, (8, 1), 0) + g0
        out_copy(0, S).wait()
        new = (x2 + gb * (h2 + y)).astype(bf16)
        out_v[pl.ds(g0, 8), :] = jnp.where(rows8 == idx, new, out_v[pl.ds(g0, 8), :])
        fix = out_copy(g0, 8)
        fix.start()
        fix.wait()


@jax.jit
def pallas_adaLN_cond__sliding_block_cached__moe_arch_mod__prompt_kernel(
    A_x, A_k_cache, A_v_cache, A_wq, A_wo, B_x, B_w_r, B_w_gate, B_w_up, B_w_down, c, w_mod,
):
    del B_x
    any_spec = pl.BlockSpec(memory_space=pl.ANY)
    return pl.pallas_call(
        _kernel,
        out_shape=jax.ShapeDtypeStruct(A_x.shape, A_x.dtype),
        in_specs=[any_spec] * 11,
        out_specs=any_spec,
        scratch_shapes=[
            pltpu.VMEM((S, D), bf16),
            pltpu.VMEM((S, D), bf16),
            pltpu.VMEM((S, D), bf16),
            pltpu.VMEM((NQS * TQ, GW), bf16),
            pltpu.VMEM((S, D), f32),
            pltpu.VMEM((D, 6 * D + PADC), bf16),
            pltpu.VMEM((HKV, D, GW), bf16),
            pltpu.VMEM((HKV, GW, D), bf16),
            pltpu.VMEM((D, F), bf16),
            pltpu.VMEM((D, F), bf16),
            pltpu.VMEM((F, D + PADC), bf16),
            pltpu.VMEM((HKV, W, DH), bf16),
            pltpu.VMEM((HKV, W, DH), bf16),
            pltpu.VMEM((HKV, DH, W), bf16),
            pltpu.VMEM((8, 1, D), bf16),
            pltpu.VMEM((16, 8, 128), bf16),
            pltpu.VMEM((16, D), bf16),
            pltpu.VMEM((8, 6 * D), f32),
            pltpu.VMEM((8, 8, 128), f32),
            pltpu.VMEM((8, 8, 128), jnp.int32),
            pltpu.VMEM((4, 8, D), f32),
            pltpu.SMEM((1,), jnp.int32),
            pltpu.SemaphoreType.DMA((NSEM,)),
        ],
        compiler_params=pltpu.CompilerParams(vmem_limit_bytes=110 * 1024 * 1024),
    )(A_x, A_k_cache, A_v_cache, A_wq, A_wo, B_w_r.reshape(8, 128), B_w_gate, B_w_up, B_w_down, c, w_mod)
```

```python
import contextlib
import math
import os

import jax
import jax.numpy as jnp
from jax import lax
from jax.experimental import pallas as pl
from jax.experimental.pallas import tpu as pltpu

S = 2048
D = 1024
HQ = 32
HKV = 4
REP = HQ // HKV
DH = 128
GW = REP * DH
W = 512
F = 3584
EPS = 1e-5
TQ = 256
NT = S // TQ
NIT = NT * HKV
NQS = NT
PADC = 128
TP = 512
SEQ_A = os.environ.get('KP_SEQA', 'KOV')
SEQ_B = os.environ.get('KP_SEQB', 'KQVOM')
SEQ_C = os.environ.get('KP_SEQC', 'KQVOL')
SEQ_D = os.environ.get('KP_SEQD', 'KoVOL')
PINLO = os.environ.get('KP_PINLO', 'Q')
UNA = int(os.environ.get('KP_UNA', 1))
UNB = int(os.environ.get('KP_UNB', 2))
UNC = int(os.environ.get('KP_UNC', 2))
P0PIN = int(os.environ.get('KP_P0PIN', 1))
LAG0 = int(os.environ.get('KP_LAG0', 2))
LPC = os.environ.get('KP_LPC', 'Q0,O128').split(',')
LPD = os.environ.get('KP_LPD', 'V0,O0').split(',')
LPE = os.environ.get('KP_LPE', 'V0,V96,V192,O32,O128').split(',')
LCNT = [int(c_) for c_ in os.environ.get('KP_LCNT', '05555552')]
PADW = int(os.environ.get('KP_PADW', 128))
NKC = int(os.environ.get('KP_NKC', 4))
KC = D // NKC
UNP = int(os.environ.get('KP_UNP', 1))
OS = int(os.environ.get('KP_OS', 32))
P0ROWS = int(os.environ.get('KP_P0ROWS', 8))
P0SPAN = int(os.environ.get('KP_P0SPAN', 256))
SCOPES = int(os.environ.get('KP_SCOPES', 0))
QSCALE = (DH ** -0.5) * math.log2(math.e)
PR = TQ // REP

f32 = jnp.float32
bf16 = jnp.bfloat16

(SEM_C, SEM_WR, SEM_X0, SEM_WM1, SEM_K, SEM_V, SEM_WG, SEM_WU, SEM_WD, SEM_OUT, SEM_K0, SEM_WM2) = range(12)
SEM_X = 12
SEM_WQ = SEM_X + NT
SEM_WO = SEM_WQ + HKV
SEM_WQ0 = SEM_WO + HKV
SEM_WMS = SEM_WQ0 + NKC
SEM_WMC = SEM_WMS + NKC
NSEM = SEM_WMC + NKC


def _scope(name):
    return jax.named_scope(name) if SCOPES else contextlib.nullcontext()


def _ln(x):
    m = jnp.mean(x, axis=-1, keepdims=True)
    xc = x - m
    v = jnp.mean(xc * xc, axis=-1, keepdims=True)
    return xc * lax.rsqrt(v + EPS)


def _recip(l):
    r = pl.reciprocal(l, approx=True)
    return r * (2.0 - l * r)


def _mo(x, m):
    return x if isinstance(x, int) else pl.multiple_of(x, m)


def _gate(x, flag, tok):
    n = x.shape[0]
    xs = jnp.where(flag, jnp.concatenate([tok] * (n // 8), axis=0), x[:, 0:128])
    return jnp.concatenate([xs, x[:, 128:]], axis=1)


def _gate1(x, flag, tok):
    r = tok.shape[0]
    x0 = jnp.where(flag, tok, x[0:r, 0:128])
    if x.shape[1] > 128:
        x0 = jnp.concatenate([x0, x[0:r, 128:]], axis=1)
    return jnp.concatenate([x0, x[r:]], axis=0)


def _rows(v8, n):
    return v8 if n == 8 else jnp.concatenate([v8] * (n // 8), axis=0)


def _token(y):
    t = y[:, 0:128]
    for j in range(1, y.shape[1] // 128):
        t = jnp.maximum(t, y[:, j * 128:(j + 1) * 128])
    u = t[0:8]
    for j in range(1, y.shape[0] // 8):
        u = jnp.maximum(u, t[8 * j:8 * (j + 1)])
    return u


def _kernel(x_hbm, k_hbm, v_hbm, wq_hbm, wo_hbm, wr_hbm, wg_hbm, wu_hbm, wd_hbm, c_hbm, wmod_hbm,
            out_hbm,
            x_v, out_v, h_v, q_v, acc_v, wmod_v, wq_v, wo_v, wg_v, wu_v, wd_v, k_v, v_v, kt_v,
            c_v8, wr_v8, sc_v, mod_v, best_v, bidx_v, aux_v, flag_s, sems):
    sk = k_hbm.shape[2]
    c_v = c_v8.at[0]
    wr_v = wr_v8.at[0]

    def cp(src, dst, i):
        return pltpu.make_async_copy(src, dst, sems.at[i])

    c_cp = cp(c_hbm, c_v, SEM_C)
    wr_cp = cp(wr_hbm, wr_v, SEM_WR)
    x0_cp = cp(x_hbm.at[0, pl.ds(0, TP), :], x_v.at[pl.ds(0, TP), :], SEM_X0)
    wm1_cp = cp(wmod_hbm.at[:, pl.ds(2 * D, D)], wmod_v.at[:, pl.ds(2 * D, D)], SEM_WM1)
    wm2_cp = cp(wmod_hbm.at[:, pl.ds(3 * D, 3 * D)], wmod_v.at[:, pl.ds(3 * D, 3 * D)], SEM_WM2)
    k0_cp = cp(k_hbm.at[0, 0, pl.ds(sk - W, W), :], k_v.at[0], SEM_K0)
    k_cp = cp(k_hbm.at[0, pl.ds(1, HKV - 1), pl.ds(sk - W, W), :], k_v.at[pl.ds(1, HKV - 1)], SEM_K)
    v_cp = cp(v_hbm.at[0, :, pl.ds(sk - W, W), :], v_v, SEM_V)
    wg_cp = cp(wg_hbm, wg_v, SEM_WG)
    wu_cp = cp(wu_hbm, wu_v, SEM_WU)
    wd_cp = cp(wd_hbm, wd_v.at[:, pl.ds(0, D)], SEM_WD)

    def x_cp(t):
        r0 = _mo(t * TQ, TQ)
        return cp(x_hbm.at[0, pl.ds(r0, TQ), :], x_v.at[pl.ds(r0, TQ), :], SEM_X + t)

    def wm_cp(part, j):
        c0 = _mo(part * D + j * KC, KC)
        return cp(wmod_hbm.at[:, pl.ds(c0, KC)], wmod_v.at[:, pl.ds(c0, KC)], (SEM_WMS, SEM_WMC)[part] + j)

    def wq0_cp(j):
        r0 = _mo(j * KC, KC)
        return cp(wq_hbm.at[pl.ds(r0, KC), pl.ds(0, GW)], wq_v.at[0, pl.ds(r0, KC), pl.ds(0, GW)], SEM_WQ0 + j)

    def wq_cp(g):
        return cp(wq_hbm.at[:, pl.ds(_mo(g * GW, GW), GW)], wq_v.at[g, :, pl.ds(0, GW)], SEM_WQ + g)

    def wo_cp(g):
        return cp(wo_hbm.at[pl.ds(_mo(g * GW, GW), GW), :], wo_v.at[g], SEM_WO + g)

    def out_copy(r0, n):
        return cp(out_v.at[pl.ds(r0, n), :], out_hbm.at[0, pl.ds(r0, n), :], SEM_OUT)

    for c_ in ([c_cp, x0_cp] + [c_ for j in range(NKC) for c_ in (wm_cp(0, j), wm_cp(1, j), wq0_cp(j))]
               + [x_cp(2), k0_cp, x_cp(3), k_cp, wr_cp]
               + [x_cp(t) for t in range(4, NT)]
               + [v_cp, wo_cp(0), wq_cp(1), wm1_cp, wm2_cp,
                  wo_cp(1), wq_cp(2), wo_cp(2), wq_cp(3), wo_cp(3), wg_cp, wu_cp, wd_cp]):
        c_.start()

    def ln1_rows(r0, n, lo=None):
        x = x_v[pl.ds(r0, n), :].astype(f32)
        if lo is not None:
            x = _gate(x, *lo)
        y = _ln(x) * _rows(mod_v[:, D:2 * D], n) + _rows(mod_v[:, 0:D], n)
        h_v[pl.ds(r0, n), :] = y.astype(bf16)
        return y

    def ln2_rows(r0, n, valid=None, lo=None):
        av = _rows(aux_v[0], n)
        bv = _rows(aux_v[1], n)
        rv = _rows(aux_v[2], n)
        r_c = _rows(aux_v[3, :, 0:128], n)
        x2 = x_v[pl.ds(r0, n), :].astype(f32)
        if lo is not None:
            x2 = _gate(x2, *lo)
        m = jnp.mean(x2, axis=-1, keepdims=True)
        xc = x2 - m
        var = jnp.mean(xc * xc, axis=-1, keepdims=True)
        rs = lax.rsqrt(var + EPS)
        y = (x2 + bv) + (xc * rs) * av
        out_v[pl.ds(r0, n), :] = y.astype(bf16)
        r = jnp.sum(xc * rv, axis=-1, keepdims=True) * rs
        r = (jnp.broadcast_to(r, (n, 128)) + r_c).astype(bf16).astype(f32)
        if valid is not None:
            r = jnp.where(valid, r, -jnp.inf)
        mb = jnp.broadcast_to(m, (n, 128))
        rsb = jnp.broadcast_to(rs, (n, 128))
        best = best_v[0]
        bm = best_v[1]
        brs = best_v[2]
        bidx = bidx_v[0]
        rows = lax.broadcasted_iota(jnp.int32, (8, 128), 0)
        for j in range(n // 8):
            sl = slice(8 * j, 8 * (j + 1))
            upd = r[sl] > best
            best = jnp.where(upd, r[sl], best)
            bm = jnp.where(upd, mb[sl], bm)
            brs = jnp.where(upd, rsb[sl], brs)
            bidx = jnp.where(upd, rows + (r0 + 8 * j), bidx)
        best_v[0] = best
        best_v[1] = bm
        best_v[2] = brs
        bidx_v[0] = bidx
        return y, best

    def mod_cols(c0, n):
        m = jnp.dot(sc_v[...], wmod_v[:, pl.ds(c0, n)], preferred_element_type=f32)
        mod_v[:, pl.ds(c0, n)] = m[0:8].astype(bf16).astype(f32)

    def qproj(hr0, qr0, n, g, c0, nc, hi=None, h=None):
        if h is None:
            h = h_v[pl.ds(hr0, n), :]
        if hi is not None:
            flag, tok = hi
            h = _gate1(h, flag, jnp.concatenate([tok, tok], axis=0).astype(bf16))
        q = jnp.dot(h, wq_v[g, :, c0:c0 + nc], preferred_element_type=f32)
        q_v[pl.ds(qr0, n), c0:c0 + nc] = (q * QSCALE).astype(bf16)
        return q

    with _scope('P0_wait_c_wm0'):
        flag_s[0] = 0
        c_cp.wait()
        cf = c_v[...].astype(f32)
        sc = (cf * jax.nn.sigmoid(cf)).astype(bf16)
        sc_v[...] = jnp.broadcast_to(sc, (16, D))
        best_v[0] = jnp.full((8, 128), -jnp.inf, f32)
        best_v[1] = jnp.zeros((8, 128), f32)
        best_v[2] = jnp.zeros((8, 128), f32)
        bidx_v[0] = jnp.zeros((8, 128), jnp.int32)
        x0_cp.wait()

        def norm_rows(i, carry):
            r0 = pl.multiple_of(i * 128, 128)
            acc_v[pl.ds(r0, 128), :] = _ln(x_v[pl.ds(r0, 128), :].astype(f32))
            return carry

        lax.fori_loop(0, TP // 128, norm_rows, 0)

    def k_chunk(j, carry):
        wm_cp(0, j).wait()
        wm_cp(1, j).wait()
        c0 = pl.multiple_of(j * KC, KC)
        scv = sc_v[...]
        sa = jnp.dot(scv, wmod_v[:, pl.ds(c0, KC)], preferred_element_type=f32)[0:8].astype(bf16).astype(f32)
        ca = jnp.dot(scv, wmod_v[:, pl.ds(D + c0, KC)], preferred_element_type=f32)[0:8].astype(bf16).astype(f32)
        mod_v[:, pl.ds(c0, KC)] = sa
        mod_v[:, pl.ds(D + c0, KC)] = 1.0 + ca
        h_v[0:TP, pl.ds(c0, KC)] = (acc_v[0:TP, pl.ds(c0, KC)] * _rows(1.0 + ca, TP) + _rows(sa, TP)).astype(bf16)
        wq0_cp(j).wait()
        part = jnp.dot(h_v[0:TP, pl.ds(c0, KC)], wq_v[0, pl.ds(c0, KC), 0:GW], preferred_element_type=f32)
        tot = jnp.where(j == 0, 0.0, acc_v[TP:2 * TP, :]) + part
        acc_v[TP:2 * TP, :] = tot
        q_v[0:TP, :] = (tot * QSCALE).astype(bf16)
        return carry

    with _scope('P1_kchunks'):
        lax.fori_loop(0, NKC, k_chunk, 0)

    def q0_cols(r0, n, j0, j1, ln_r0):
        flag = flag_s[0] > 0
        h = h_v[pl.ds(r0, n), :]
        toks = {}
        npc = (j1 - j0) - LAG0
        base, extra = divmod(TQ // P0ROWS, npc)
        cnts = [base + (1 if i < extra else 0) for i in range(npc)]
        off = 0
        for i, j in enumerate(range(j0, j1)):
            hi = (flag, toks[i - LAG0]) if (i - LAG0) in toks else None
            q = qproj(r0, r0, n, 0, j * DH, DH, hi, h)
            if i < npc:
                tk = None
                for k_ in range(cnts[i]):
                    r_ = (k_ * P0SPAN // cnts[i]) // 8 * 8
                    lo = (flag, q[r_:r_ + 8]) if P0PIN else None
                    t_ = _token(ln1_rows(_mo(ln_r0 + off, 8), P0ROWS, lo))
                    tk = t_ if tk is None else jnp.maximum(tk, t_)
                    off += P0ROWS
                toks[i] = tk

    with _scope('P2_ln'):
        x_cp(2).wait()
        ln1_rows(2 * TQ, TQ)
        k0_cp.wait()

    def q0_tile(i, carry):
        for u in range(UNP):
            t = 2 + i * UNP + u

            @pl.when(t + 1 < NT)
            def _():
                x_cp(t + 1).wait()

        @pl.when(i == 1)
        def _():
            k_cp.wait()

        for u in range(UNP):
            t = 2 + i * UNP + u
            q0_cols(pl.multiple_of(t * TQ, TQ), TQ, 0, REP, jnp.minimum(t + 1, NT - 1) * TQ)
            gk = jnp.clip(t - 2 - (UNP - 1), 0, HKV - 1)
            kt_v[gk] = k_v[gk].T
        return carry

    with _scope('P3_q0'):
        lax.fori_loop(0, (NT - 2) // UNP, q0_tile, 0)
        v_cp.wait()
        wm1_cp.wait()

    def body(its, seq, phase, pins=None):
        flag = flag_s[0] > 0
        st = dict(lo=None, hi=None, pend=None, next=None)

        def flush_op(rb=TQ):
            if st['pend'] is not None:
                st['pend'](st.get('done', 0), rb)
                st['done'] = rb % TQ
                if rb == TQ:
                    st['pend'] = None

        for u_, it in enumerate(its):
            g = it // NT
            t = it % NT
            a0 = _mo(t * TQ, TQ)
            q0 = a0

            def ln_step(p0, pins, t=t):
                n = 8
                hi = st['hi']
                for i, pin in enumerate(pins):
                    src_ = st.get(pin[0])
                    if src_ is None:
                        src_, r_ = st['V'], 0
                    else:
                        r_ = int(pin[1:])
                    c_ = 512 if r_ >= TQ else 0
                    r_ = r_ % TQ
                    lo = (flag, src_[r_:r_ + 8, c_:c_ + 128])
                    off = (p0 + i) * n
                    if isinstance(t, int):
                        y, b = ln2_rows((t - 1) * TQ + off, n, None, lo)
                    else:
                        tl = jnp.maximum(t - 1, 0)
                        y, b = ln2_rows(_mo(tl * TQ + off, n), n, t > 0, lo)
                    tk = jnp.maximum(_token(y), b)
                    hi = tk if hi is None else jnp.maximum(hi, tk)
                st['hi'] = hi

            def qk(hh, g=g, q0=q0):
                qh = q_v[pl.ds(q0, TQ), hh * DH:(hh + 1) * DH]
                s = jnp.dot(qh, kt_v[g], preferred_element_type=f32)
                if st['hi'] is not None:
                    s = _gate1(s, flag, st['hi'])
                    st['hi'] = None
                m = jnp.max(s, axis=-1, keepdims=True)
                p = jnp.exp2(s - m)
                st['K'] = s
                st['P'] = p
                l = jnp.sum(p, axis=-1, keepdims=True)
                return p.astype(bf16), l

            def pv(pl_, g=g):
                p, l = pl_
                o = jnp.dot(p, v_v[g], preferred_element_type=f32)
                st['V'] = o
                return o * _recip(l)

            def op(o, hh, ra, rb, g=g, a0=a0):
                n = rb - ra
                r0 = _mo(a0 + ra, 16)
                y = jnp.dot(o[ra:rb].astype(bf16), wo_v[g, hh * DH:(hh + 1) * DH, :], preferred_element_type=f32)
                st['O'] = y
                if hh == 0 and phase == 'B':
                    acc_v[pl.ds(r0, n), :] = jnp.where(g == 0, 0.0, acc_v[pl.ds(r0, n), :]) + y
                elif hh == REP - 1 and phase == 'C':
                    ga = _rows(mod_v[:, 2 * D:3 * D], n)
                    x = x_v[pl.ds(r0, n), :].astype(f32)
                    x_v[pl.ds(r0, n), :] = (x + ga * (acc_v[pl.ds(r0, n), :] + y)).astype(bf16)
                else:
                    acc_v[pl.ds(r0, n), :] += y

            sp = None
            for hh in range(REP):
                for tok in seq:
                    if tok == 'K':
                        sp = qk(hh)
                    elif tok == 'V':
                        o = pv(sp)
                        new_pend = (lambda ra, rb, o=o, hh=hh, op=op: op(o, hh, ra, rb))
                        if 'O' in seq[seq.index('V'):]:
                            st['next'] = new_pend
                        else:
                            st['pend'] = new_pend
                    elif tok == 'O':
                        flush_op()
                        if st['next'] is not None:
                            st['pend'] = st['next']
                            st['next'] = None
                    elif tok == 'o':
                        flush_op(OS)
                    elif tok == 'L':
                        if LCNT[hh]:
                            ln_step(sum(LCNT[:hh]), {len(LPD): LPD, len(LPE): LPE}[LCNT[hh]])
                    elif tok == 'Q':
                        q = qproj(a0, a0, TQ, g + 1, hh * DH, DH)
                        st['Q'] = q
                    elif tok == 'M':
                        pos = u_ * REP + hh
                        nm = -(-32 * UNB // (3 * NT))
                        spots = [(2 * k_ + 1) * REP * UNB // (2 * nm) for k_ in range(nm)]
                        if pos in spots:
                            j = jnp.minimum((its[0] // UNB) * nm + spots.index(pos), 31)
                            mod_cols(pl.multiple_of(2 * D + j * 128, 128), 128)
            if phase == 'C':
                flush_op()
        flush_op()
        if phase == 'C':
            for it in its:
                t = it % NT
                if isinstance(t, int):
                    out_copy((t - 1) * TQ, TQ).start()
                else:
                    @pl.when(t > 0)
                    def _():
                        out_copy(_mo((t - 1) * TQ, TQ), TQ).start()

    def body_b(i, carry):
        it = i * UNB

        @pl.when(it % NT == 0)
        def _():
            wo_cp(it // NT).wait()
            wq_cp(it // NT + 1).wait()

        @pl.when(it == 2)
        def _():
            wm2_cp.wait()

        body([it + u for u in range(UNB)], SEQ_B, 'B')
        return carry

    with _scope('LB'):
        lax.fori_loop(0, 3 * NT // UNB, body_b, 0)

    wr_cp.wait()
    wo_cp(3).wait()
    sb_ = mod_v[:, 3 * D:4 * D]
    cb1_ = 1.0 + mod_v[:, 4 * D:5 * D]
    gb_ = mod_v[:, 5 * D:6 * D]
    wr8 = wr_v[...].astype(f32)
    wr_ = jnp.concatenate([wr8[r_:r_ + 1, :] for r_ in range(8)], axis=1)
    aux_v[0] = gb_ * cb1_
    aux_v[1] = gb_ * sb_
    aux_v[2] = cb1_ * wr_
    aux_v[3] = jnp.broadcast_to(jnp.sum(sb_ * wr_, axis=-1, keepdims=True), (8, D))

    def body_c(i, carry):
        body([i * UNC + u for u in range(UNC)], SEQ_D, 'C', LPD)
        return carry

    with _scope('LC'):
        lax.fori_loop(3 * NT // UNC, NIT // UNC, body_c, 0)

    with _scope('E1_last'):
        wg_cp.wait()
        wu_cp.wait()
        wd_cp.wait()
        r0 = (NT - 1) * TQ
        ln2_rows(r0, TQ)
        out_copy(r0, TQ).start()

    with _scope('E2_ffn'):
        best = best_v[0]
        bidx = bidx_v[0]
        rmax = jnp.max(best, axis=0, keepdims=True)
        idx_v = jnp.min(jnp.where(best == rmax, bidx, S), axis=0, keepdims=True)
        idx = jnp.minimum(idx_v[0, 0], S - 1)
        g0 = pl.multiple_of((idx // 8) * 8, 8)
        sb = mod_v[:, 3 * D:4 * D]
        cb = mod_v[:, 4 * D:5 * D]
        gb = mod_v[:, 5 * D:6 * D]
        x2 = x_v[pl.ds(g0, 8), :].astype(f32)
        h2 = (x2 - best_v[1][:, 0:1]) * best_v[2][:, 0:1] * (1.0 + cb) + sb
        h2b = h2.astype(bf16)
        gt = jnp.dot(h2b, wg_v[...], preferred_element_type=f32)
        up = jnp.dot(h2b, wu_v[...], preferred_element_type=f32)
        a = (gt * jax.nn.sigmoid(gt) * up).astype(bf16)
        y = jnp.dot(a, wd_v[:, 0:D], preferred_element_type=f32)
        y = y * jax.nn.sigmoid(rmax[:, 0:1])
        rows8 = lax.broadcasted_iota(jnp.int32, (8, 1), 0) + g0
        out_copy(0, S).wait()
        new = (x2 + gb * (h2 + y)).astype(bf16)
        out_v[pl.ds(g0, 8), :] = jnp.where(rows8 == idx, new, out_v[pl.ds(g0, 8), :])
        fix = out_copy(g0, 8)
        fix.start()
        fix.wait()


@jax.jit
def pallas_adaLN_cond__sliding_block_cached__moe_arch_mod__prompt_kernel(
    A_x, A_k_cache, A_v_cache, A_wq, A_wo, B_x, B_w_r, B_w_gate, B_w_up, B_w_down, c, w_mod,
):
    del B_x
    any_spec = pl.BlockSpec(memory_space=pl.ANY)
    return pl.pallas_call(
        _kernel,
        out_shape=jax.ShapeDtypeStruct(A_x.shape, A_x.dtype),
        in_specs=[any_spec] * 11,
        out_specs=any_spec,
        scratch_shapes=[
            pltpu.VMEM((S, D), bf16),
            pltpu.VMEM((S, D), bf16),
            pltpu.VMEM((S, D), bf16),
            pltpu.VMEM((NQS * TQ, GW), bf16),
            pltpu.VMEM((S, D), f32),
            pltpu.VMEM((D, 6 * D + PADC), bf16),
            pltpu.VMEM((HKV, D, GW + PADW), bf16),
            pltpu.VMEM((HKV, GW, D), bf16),
            pltpu.VMEM((D, F), bf16),
            pltpu.VMEM((D, F), bf16),
            pltpu.VMEM((F, D + PADC), bf16),
            pltpu.VMEM((HKV, W, DH), bf16),
            pltpu.VMEM((HKV, W, DH), bf16),
            pltpu.VMEM((HKV, DH, W), bf16),
            pltpu.VMEM((8, 1, D), bf16),
            pltpu.VMEM((16, 8, 128), bf16),
            pltpu.VMEM((16, D), bf16),
            pltpu.VMEM((8, 6 * D), f32),
            pltpu.VMEM((8, 8, 128), f32),
            pltpu.VMEM((8, 8, 128), jnp.int32),
            pltpu.VMEM((4, 8, D), f32),
            pltpu.SMEM((1,), jnp.int32),
            pltpu.SemaphoreType.DMA((NSEM,)),
        ],
        compiler_params=pltpu.CompilerParams(vmem_limit_bytes=110 * 1024 * 1024),
    )(A_x, A_k_cache, A_v_cache, A_wq, A_wo, B_w_r.reshape(8, 128), B_w_gate, B_w_up, B_w_down, c, w_mod)
```

```python
import contextlib
import math
import os

import jax
import jax.numpy as jnp
from jax import lax
from jax.experimental import pallas as pl
from jax.experimental.pallas import tpu as pltpu

S = 2048
D = 1024
HQ = 32
HKV = 4
REP = HQ // HKV
DH = 128
GW = REP * DH
W = 512
F = 3584
EPS = 1e-5
TQ = 256
NT = S // TQ
NIT = NT * HKV
NQS = NT
PADC = 128
TP = 512
SEQ_A = os.environ.get('KP_SEQA', 'KOV')
SEQ_B = os.environ.get('KP_SEQB', 'KQVON')
SEQ_C = os.environ.get('KP_SEQC', 'KQVOL')
SEQ_D = os.environ.get('KP_SEQD', 'KoVOL')
PINLO = os.environ.get('KP_PINLO', 'Q')
UNA = int(os.environ.get('KP_UNA', 1))
UNB = int(os.environ.get('KP_UNB', 2))
UNC = int(os.environ.get('KP_UNC', 2))
P0PIN = int(os.environ.get('KP_P0PIN', 1))
LAG0 = int(os.environ.get('KP_LAG0', 2))
LPC = os.environ.get('KP_LPC', 'Q0,O128').split(',')
LPD = os.environ.get('KP_LPD', 'V0,O0').split(',')
LPE = os.environ.get('KP_LPE', 'V0,V96,V192,O32,O128').split(',')
LCNT = [int(c_) for c_ in os.environ.get('KP_LCNT', '05555552')]
PADW = int(os.environ.get('KP_PADW', 128))
NKC = int(os.environ.get('KP_NKC', 4))
KC = D // NKC
UNP = int(os.environ.get('KP_UNP', 1))
OS = int(os.environ.get('KP_OS', 32))
FG = int(os.environ.get('KP_FG', 0))
FD = int(os.environ.get('KP_FD', 15))
PADD = int(os.environ.get('KP_PADD', 256))
FI0 = int(os.environ.get('KP_FI0', 8))
FLAG_ = int(os.environ.get('KP_FLAG', 4))
FVR = int(os.environ.get('KP_FVR', 32))
NM = 3
NMC = 11
NPIN = os.environ.get('KP_NPIN', 'O64')
P0ROWS = int(os.environ.get('KP_P0ROWS', 8))
P0SPAN = int(os.environ.get('KP_P0SPAN', 256))
SCOPES = int(os.environ.get('KP_SCOPES', 0))
QSCALE = (DH ** -0.5) * math.log2(math.e)
PR = TQ // REP

f32 = jnp.float32
bf16 = jnp.bfloat16

(SEM_C, SEM_WR, SEM_X0, SEM_WM1, SEM_K, SEM_V, SEM_WG, SEM_WU, SEM_WD, SEM_OUT, SEM_K0, SEM_WM2) = range(12)
SEM_X = 12
SEM_WQ = SEM_X + NT
SEM_WO = SEM_WQ + HKV
SEM_WQ0 = SEM_WO + HKV
SEM_WMS = SEM_WQ0 + NKC
SEM_WMC = SEM_WMS + NKC
SEM_WMR = SEM_WMC + NKC
NSEM = SEM_WMR + NMC


def _scope(name):
    return jax.named_scope(name) if SCOPES else contextlib.nullcontext()


def _ln(x):
    m = jnp.mean(x, axis=-1, keepdims=True)
    xc = x - m
    v = jnp.mean(xc * xc, axis=-1, keepdims=True)
    return xc * lax.rsqrt(v + EPS)


def _recip(l):
    r = pl.reciprocal(l, approx=True)
    return r * (2.0 - l * r)


def _mo(x, m):
    return x if isinstance(x, int) else pl.multiple_of(x, m)


def _gate(x, flag, tok):
    n = x.shape[0]
    xs = jnp.where(flag, jnp.concatenate([tok] * (n // 8), axis=0), x[:, 0:128])
    return jnp.concatenate([xs, x[:, 128:]], axis=1)


def _gate1(x, flag, tok):
    r = tok.shape[0]
    x0 = jnp.where(flag, tok, x[0:r, 0:128])
    if x.shape[1] > 128:
        x0 = jnp.concatenate([x0, x[0:r, 128:]], axis=1)
    return x0 if x.shape[0] == r else jnp.concatenate([x0, x[r:]], axis=0)


def _rows(v8, n):
    return v8 if n == 8 else jnp.concatenate([v8] * (n // 8), axis=0)


def _token(y):
    t = y[:, 0:128]
    for j in range(1, y.shape[1] // 128):
        t = jnp.maximum(t, y[:, j * 128:(j + 1) * 128])
    u = t[0:8]
    for j in range(1, y.shape[0] // 8):
        u = jnp.maximum(u, t[8 * j:8 * (j + 1)])
    return u


def _kernel(x_hbm, k_hbm, v_hbm, wq_hbm, wo_hbm, wr_hbm, wg_hbm, wu_hbm, wd_hbm, c_hbm, wmod_hbm,
            out_hbm,
            x_v, out_v, h_v, q_v, acc_v, wmod_v, wmr_v, wq_v, wo_v, wg_v, wu_v, wd_v, k_v, v_v, kt_v,
            c_v8, wr_v8, sc_v, scc_v, acol_v, mod_v, best_v, bidx_v, aux_v, flag_s, sems):
    sk = k_hbm.shape[2]
    c_v = c_v8.at[0]
    wr_v = wr_v8.at[0]

    def cp(src, dst, i):
        return pltpu.make_async_copy(src, dst, sems.at[i])

    c_cp = cp(c_hbm, c_v, SEM_C)
    wr_cp = cp(wr_hbm, wr_v, SEM_WR)
    x0_cp = cp(x_hbm.at[0, pl.ds(0, TP), :], x_v.at[pl.ds(0, TP), :], SEM_X0)

    def wmr_cp(i):
        c0 = 2 * D + min(i * NM, 32 - NM) * 128
        return cp(wmod_hbm.at[:, pl.ds(c0, NM * 128)], wmr_v.at[i], SEM_WMR + i)

    k0_cp = cp(k_hbm.at[0, 0, pl.ds(sk - W, W), :], k_v.at[0], SEM_K0)
    k_cp = cp(k_hbm.at[0, pl.ds(1, HKV - 1), pl.ds(sk - W, W), :], k_v.at[pl.ds(1, HKV - 1)], SEM_K)
    v_cp = cp(v_hbm.at[0, :, pl.ds(sk - W, W), :], v_v, SEM_V)
    wg_cp = cp(wg_hbm, wg_v, SEM_WG)
    wu_cp = cp(wu_hbm, wu_v, SEM_WU)
    wd_cp = cp(wd_hbm, wd_v.at[:, pl.ds(0, D)], SEM_WD)

    def x_cp(t):
        r0 = _mo(t * TQ, TQ)
        return cp(x_hbm.at[0, pl.ds(r0, TQ), :], x_v.at[pl.ds(r0, TQ), :], SEM_X + t)

    def wm_cp(part, j):
        c0 = _mo(part * D + j * KC, KC)
        return cp(wmod_hbm.at[:, pl.ds(c0, KC)], wmod_v.at[:, pl.ds(c0, KC)], (SEM_WMS, SEM_WMC)[part] + j)

    def wq0_cp(j):
        r0 = _mo(j * KC, KC)
        return cp(wq_hbm.at[pl.ds(r0, KC), pl.ds(0, GW)], wq_v.at[0, pl.ds(r0, KC), pl.ds(0, GW)], SEM_WQ0 + j)

    def wq_cp(g):
        return cp(wq_hbm.at[:, pl.ds(_mo(g * GW, GW), GW)], wq_v.at[g, :, pl.ds(0, GW)], SEM_WQ + g)

    def wo_cp(g):
        return cp(wo_hbm.at[pl.ds(_mo(g * GW, GW), GW), :], wo_v.at[g], SEM_WO + g)

    def out_copy(r0, n):
        return cp(out_v.at[pl.ds(r0, n), :], out_hbm.at[0, pl.ds(r0, n), :], SEM_OUT)

    for c_ in ([c_cp, x0_cp] + [c_ for j in range(NKC) for c_ in (wm_cp(0, j), wm_cp(1, j), wq0_cp(j))]
               + [x_cp(2), k0_cp, x_cp(3), k_cp, wr_cp]
               + [x_cp(t) for t in range(4, NT)]
               + [v_cp, wo_cp(0), wq_cp(1)] + [wmr_cp(i) for i in range(NMC)]
               + [wo_cp(1), wq_cp(2), wo_cp(2), wq_cp(3), wo_cp(3), wg_cp, wu_cp, wd_cp]):
        c_.start()

    def ln1_rows(r0, n, lo=None):
        x = x_v[pl.ds(r0, n), :].astype(f32)
        if lo is not None:
            x = _gate(x, *lo)
        y = _ln(x) * _rows(mod_v[:, D:2 * D], n) + _rows(mod_v[:, 0:D], n)
        h_v[pl.ds(r0, n), :] = y.astype(bf16)
        return y

    def ln2_rows(r0, n, valid=None, lo=None):
        av = _rows(aux_v[0], n)
        bv = _rows(aux_v[1], n)
        rv = _rows(aux_v[2], n)
        r_c = _rows(aux_v[3, :, 0:128], n)
        x2 = x_v[pl.ds(r0, n), :].astype(f32)
        if lo is not None:
            x2 = _gate(x2, *lo)
        m = jnp.mean(x2, axis=-1, keepdims=True)
        xc = x2 - m
        var = jnp.mean(xc * xc, axis=-1, keepdims=True)
        rs = lax.rsqrt(var + EPS)
        y = x2 + ((xc * rs) * av + bv)
        out_v[pl.ds(r0, n), :] = y.astype(bf16)
        r = jnp.sum(xc * rv, axis=-1, keepdims=True) * rs
        r = (jnp.broadcast_to(r, (n, 128)) + r_c).astype(bf16).astype(f32)
        if valid is not None:
            r = jnp.where(valid, r, -jnp.inf)
        mb = jnp.broadcast_to(m, (n, 128))
        rsb = jnp.broadcast_to(rs, (n, 128))
        best = best_v[0]
        bm = best_v[1]
        brs = best_v[2]
        bidx = bidx_v[0]
        rows = lax.broadcasted_iota(jnp.int32, (8, 128), 0)
        for j in range(n // 8):
            sl = slice(8 * j, 8 * (j + 1))
            upd = r[sl] > best
            best = jnp.where(upd, r[sl], best)
            bm = jnp.where(upd, mb[sl], bm)
            brs = jnp.where(upd, rsb[sl], brs)
            bidx = jnp.where(upd, rows + (r0 + 8 * j), bidx)
        best_v[0] = best
        best_v[1] = bm
        best_v[2] = brs
        bidx_v[0] = bidx
        return y, best

    def qproj(hr0, qr0, n, g, c0, nc, hi=None, h=None):
        if h is None:
            h = h_v[pl.ds(hr0, n), :]
        if hi is not None:
            flag, tok = hi
            h = _gate1(h, flag, jnp.concatenate([tok, tok], axis=0).astype(bf16))
        q = jnp.dot(h, wq_v[g, :, c0:c0 + nc], preferred_element_type=f32)
        q_v[pl.ds(qr0, n), c0:c0 + nc] = (q * QSCALE).astype(bf16)
        return q

    with _scope('P0_wait_c_wm0'):
        flag_s[0] = 0
        c_cp.wait()
        cf = c_v[...].astype(f32)
        sc = (cf * jax.nn.sigmoid(cf)).astype(bf16)
        sc_v[...] = jnp.broadcast_to(sc, (16, D))
        scc_v[...] = jnp.broadcast_to(sc.astype(f32), (128, D)).T
        best_v[0] = jnp.full((8, 128), -jnp.inf, f32)
        best_v[1] = jnp.zeros((8, 128), f32)
        best_v[2] = jnp.zeros((8, 128), f32)
        bidx_v[0] = jnp.zeros((8, 128), jnp.int32)
        x0_cp.wait()

        def norm_rows(i, carry):
            r0 = pl.multiple_of(i * 128, 128)
            acc_v[pl.ds(r0, 128), :] = _ln(x_v[pl.ds(r0, 128), :].astype(f32))
            return carry

        lax.fori_loop(0, TP // 128, norm_rows, 0)

    def k_chunk(j, carry):
        wm_cp(0, j).wait()
        wm_cp(1, j).wait()
        c0 = pl.multiple_of(j * KC, KC)
        scv = sc_v[...]
        sa = jnp.dot(scv, wmod_v[:, pl.ds(c0, KC)], preferred_element_type=f32)[0:8].astype(bf16).astype(f32)
        ca = jnp.dot(scv, wmod_v[:, pl.ds(D + c0, KC)], preferred_element_type=f32)[0:8].astype(bf16).astype(f32)
        mod_v[:, pl.ds(c0, KC)] = sa
        mod_v[:, pl.ds(D + c0, KC)] = 1.0 + ca
        h_v[0:TP, pl.ds(c0, KC)] = (acc_v[0:TP, pl.ds(c0, KC)] * _rows(1.0 + ca, TP) + _rows(sa, TP)).astype(bf16)
        wq0_cp(j).wait()
        part = jnp.dot(h_v[0:TP, pl.ds(c0, KC)], wq_v[0, pl.ds(c0, KC), 0:GW], preferred_element_type=f32)
        tot = jnp.where(j == 0, 0.0, acc_v[TP:2 * TP, :]) + part
        acc_v[TP:2 * TP, :] = tot
        q_v[0:TP, :] = (tot * QSCALE).astype(bf16)
        return carry

    with _scope('P1_kchunks'):
        lax.fori_loop(0, NKC, k_chunk, 0)

    def q0_cols(r0, n, j0, j1, ln_r0):
        flag = flag_s[0] > 0
        h = h_v[pl.ds(r0, n), :]
        toks = {}
        npc = (j1 - j0) - LAG0
        base, extra = divmod(TQ // P0ROWS, npc)
        cnts = [base + (1 if i < extra else 0) for i in range(npc)]
        off = 0
        for i, j in enumerate(range(j0, j1)):
            hi = (flag, toks[i - LAG0]) if (i - LAG0) in toks else None
            q = qproj(r0, r0, n, 0, j * DH, DH, hi, h)
            if i < npc:
                tk = None
                for k_ in range(cnts[i]):
                    r_ = (k_ * P0SPAN // cnts[i]) // 8 * 8
                    lo = (flag, q[r_:r_ + 8]) if P0PIN else None
                    t_ = _token(ln1_rows(_mo(ln_r0 + off, 8), P0ROWS, lo))
                    tk = t_ if tk is None else jnp.maximum(tk, t_)
                    off += P0ROWS
                toks[i] = tk

    with _scope('P2_ln'):
        x_cp(2).wait()
        ln1_rows(2 * TQ, TQ)
        k0_cp.wait()

    def q0_tile(i, carry):
        for u in range(UNP):
            t = 2 + i * UNP + u

            @pl.when(t + 1 < NT)
            def _():
                x_cp(t + 1).wait()

        @pl.when(i == 1)
        def _():
            k_cp.wait()

        for u in range(UNP):
            t = 2 + i * UNP + u
            q0_cols(pl.multiple_of(t * TQ, TQ), TQ, 0, REP, jnp.minimum(t + 1, NT - 1) * TQ)
            gk = jnp.clip(t - 2 - (UNP - 1), 0, HKV - 1)
            kt_v[gk] = k_v[gk].T
        return carry

    with _scope('P3_q0'):
        lax.fori_loop(0, (NT - 2) // UNP, q0_tile, 0)
        v_cp.wait()
        wmr_cp(0).wait()

    def body(its, seq, phase, pins=None):
        flag = flag_s[0] > 0
        st = dict(lo=None, hi=None, pend=None, next=None)

        def flush_op(rb=TQ):
            if st['pend'] is not None:
                st['pend'](st.get('done', 0), rb)
                st['done'] = rb % TQ
                if rb == TQ:
                    st['pend'] = None

        for u_, it in enumerate(its):
            g = it // NT
            t = it % NT
            a0 = _mo(t * TQ, TQ)
            q0 = a0

            def ln_step(p0, pins, t=t):
                n = 8
                hi = st['hi']
                for i, pin in enumerate(pins):
                    src_ = st.get(pin[0])
                    if src_ is None:
                        src_, r_ = st['V'], 0
                    else:
                        r_ = int(pin[1:])
                    c_ = 512 if r_ >= TQ else 0
                    r_ = r_ % TQ
                    lo = (flag, src_[r_:r_ + 8, c_:c_ + 128])
                    off = (p0 + i) * n
                    if isinstance(t, int):
                        y, b = ln2_rows((t - 1) * TQ + off, n, None, lo)
                    else:
                        tl = jnp.maximum(t - 1, 0)
                        y, b = ln2_rows(_mo(tl * TQ + off, n), n, t > 0, lo)
                    tk = jnp.maximum(_token(y), b)
                    hi = tk if hi is None else jnp.maximum(hi, tk)
                st['hi'] = hi

            def qk(hh, g=g, q0=q0):
                qh = q_v[pl.ds(q0, TQ), hh * DH:(hh + 1) * DH]
                s = jnp.dot(qh, kt_v[g], preferred_element_type=f32)
                if st['hi'] is not None:
                    s = _gate1(s, flag, st['hi'])
                    st['hi'] = None
                m = jnp.max(s, axis=-1, keepdims=True)
                p = jnp.exp2(s - m)
                st['K'] = s
                st['P'] = p
                l = jnp.sum(p, axis=-1, keepdims=True)
                return p.astype(bf16), l

            def pv(pl_, g=g):
                p, l = pl_
                o = jnp.dot(p, v_v[g], preferred_element_type=f32)
                st['V'] = o
                return o * _recip(l)

            def op(o, hh, ra, rb, g=g, a0=a0):
                n = rb - ra
                r0 = _mo(a0 + ra, 16)
                y = jnp.dot(o[ra:rb].astype(bf16), wo_v[g, hh * DH:(hh + 1) * DH, :], preferred_element_type=f32)
                st['O'] = y
                if hh == 0 and phase == 'B':
                    acc_v[pl.ds(r0, n), :] = jnp.where(g == 0, 0.0, acc_v[pl.ds(r0, n), :]) + y
                elif hh == REP - 1 and phase == 'C':
                    ga = _rows(mod_v[:, 2 * D:3 * D], n)
                    x = x_v[pl.ds(r0, n), :].astype(f32)
                    x_v[pl.ds(r0, n), :] = (x + ga * (acc_v[pl.ds(r0, n), :] + y)).astype(bf16)
                else:
                    acc_v[pl.ds(r0, n), :] += y

            sp = None
            for hh in range(REP):
                for tok in seq:
                    if tok == 'K':
                        sp = qk(hh)
                    elif tok == 'V':
                        o = pv(sp)
                        new_pend = (lambda ra, rb, o=o, hh=hh, op=op: op(o, hh, ra, rb))
                        if 'O' in seq[seq.index('V'):]:
                            st['next'] = new_pend
                        else:
                            st['pend'] = new_pend
                    elif tok == 'O':
                        flush_op()
                        if st['next'] is not None:
                            st['pend'] = st['next']
                            st['next'] = None
                    elif tok == 'o':
                        flush_op(OS)
                    elif tok == 'L':
                        if LCNT[hh]:
                            ln_step(sum(LCNT[:hh]), {len(LPD): LPD, len(LPE): LPE}[LCNT[hh]])
                    elif tok == 'Q':
                        q = qproj(a0, a0, TQ, g + 1, hh * DH, DH)
                        st['Q'] = q
                    elif tok == 'N':
                        pos = u_ * REP + hh
                        nst = UNB * REP - 1
                        nm = NM
                        if pos > 0:
                            ci = jnp.minimum(its[0] // UNB, NMC - 1)
                            j = jnp.minimum(ci * nm, 32 - nm)
                            c0 = pl.multiple_of(2 * D + j * 128, 128)
                            ga_, gb_ = [(128 * k_) // nst for k_ in (pos - 1, pos)]
                            r_ = int(NPIN[1:])
                            acc = st.get('macc')
                            tok_ = st[NPIN[0]][r_:r_ + 8, 0:128]
                            for rg in range(ga_, gb_):
                                xc_ = scc_v[8 * rg:8 * rg + 8, :]
                                if rg == ga_:
                                    xc_ = jnp.where(flag, tok_, xc_)
                                w_ = wmr_v[ci, 8 * rg:8 * rg + 8, :].astype(f32)
                                pr_ = w_ * jnp.concatenate([xc_] * nm, axis=1)
                                acc = pr_ if acc is None else acc + pr_
                            st['macc'] = acc
                            st['hi'] = _token(acc)
                            if pos == nst:
                                tot_ = jnp.sum(acc, axis=0, keepdims=True).astype(bf16).astype(f32)
                                mod_v[:, pl.ds(c0, nm * 128)] = jnp.broadcast_to(tot_, (8, nm * 128))
            if phase == 'C':
                flush_op()
        flush_op()
        if phase == 'C':
            for it in its:
                t = it % NT
                if isinstance(t, int):
                    out_copy((t - 1) * TQ, TQ).start()
                else:
                    @pl.when(t > 0)
                    def _():
                        out_copy(_mo((t - 1) * TQ, TQ), TQ).start()

    def body_b(i, carry):
        it = i * UNB

        @pl.when(it % NT == 0)
        def _():
            wo_cp(it // NT).wait()
            wq_cp(it // NT + 1).wait()

        @pl.when(i == 1)
        def _():
            for i_ in range(1, NMC):
                wmr_cp(i_).wait()

        body([it + u for u in range(UNB)], SEQ_B, 'B')
        return carry

    with _scope('LB'):
        lax.fori_loop(0, 3 * NT // UNB, body_b, 0)

    wr_cp.wait()
    wo_cp(3).wait()
    sb_ = mod_v[:, 3 * D:4 * D]
    cb1_ = 1.0 + mod_v[:, 4 * D:5 * D]
    gb_ = mod_v[:, 5 * D:6 * D]
    wr8 = wr_v[...].astype(f32)
    wr_ = jnp.concatenate([wr8[r_:r_ + 1, :] for r_ in range(8)], axis=1)
    aux_v[0] = gb_ * cb1_
    aux_v[1] = gb_ * sb_
    aux_v[2] = cb1_ * wr_
    aux_v[3] = jnp.broadcast_to(jnp.sum(sb_ * wr_, axis=-1, keepdims=True), (8, D))

    def body_c(i, carry):
        body([i * UNC + u for u in range(UNC)], SEQ_D, 'C', LPD)
        return carry

    with _scope('LC'):
        lax.fori_loop(3 * NT // UNC, NIT // UNC, body_c, 0)

    with _scope('E1_last'):
        wg_cp.wait()
        wu_cp.wait()
        wd_cp.wait()
        r0 = (NT - 1) * TQ
        ln2_rows(r0, TQ)
        out_copy(r0, TQ).start()

    with _scope('E2_ffn'):
        best = best_v[0]
        bidx = bidx_v[0]
        rmax = jnp.max(best, axis=0, keepdims=True)
        idx_v = jnp.min(jnp.where(best == rmax, bidx, S), axis=0, keepdims=True)
        idx = jnp.minimum(idx_v[0, 0], S - 1)
        g0 = pl.multiple_of((idx // 8) * 8, 8)
        sb = mod_v[:, 3 * D:4 * D]
        cb = mod_v[:, 4 * D:5 * D]
        gb = mod_v[:, 5 * D:6 * D]
        x2 = x_v[pl.ds(g0, 8), :].astype(f32)
        h2 = (x2 - best_v[1][:, 0:1]) * best_v[2][:, 0:1] * (1.0 + cb) + sb
        h2b = h2.astype(bf16)
        rows8 = lax.broadcasted_iota(jnp.int32, (8, 1), 0) + g0
        sel = rows8 == idx

        def column(v8):
            row = jnp.sum(jnp.where(sel, v8, 0.0), axis=0, keepdims=True)
            return jnp.broadcast_to(row, (128, row.shape[1])).T

        def act(gt, up):
            return (gt * jax.nn.sigmoid(gt) * up).astype(bf16)

        def fin(a_):
            return jnp.broadcast_to(jnp.sum(a_, axis=0, keepdims=True), a_.shape)

        flag = flag_s[0] > 0
        nf = F // 128
        fm = nf - FG
        if FG:
            scc_v[...] = column(h2b.astype(f32))
        items = [('g', rg) for rg in range(D // 8)] if FG else []
        items += [('d', rg) for rg in range(FD * 16)]
        accs = {}
        a_strips = {}
        vtok = {}
        res = dict(g={}, u={}, y=None)
        strips = [(k_, j) for j in range(fm) for k_ in 'gu'] + [('d', j) for j in range(FD, nf)]

        def vpu_item(kind, rg, lo):
            col = (scc_v if kind == 'g' else acol_v)[8 * rg:8 * rg + 8, :]
            col = jnp.where(flag, lo, col)
            outs = []
            for nm_, w_ref, c0_, nc in ([('vg', wg_v, fm * 128, FG * 128), ('vu', wu_v, fm * 128, FG * 128)]
                                        if kind == 'g' else [('vd', wd_v, 0, D)]):
                pr_ = w_ref[8 * rg:8 * rg + 8, c0_:c0_ + nc].astype(f32) * jnp.concatenate([col] * (nc // 128), axis=1)
                accs[nm_] = pr_ if nm_ not in accs else accs[nm_] + pr_
                outs.append(accs[nm_])
            return outs

        pos = 0
        for i, (kind, j) in enumerate(strips):
            hi = vtok.get(i - FLAG_)
            if kind == 'd':
                if j not in a_strips:
                    assert not any(k_ == 'g' for k_, _ in items[pos:]), 'VPU gate/up not finished'
                    av_ = act(fin(accs['vg']), fin(accs['vu']))
                    for jj in range(FG):
                        a_strips[fm + jj] = av_[:, jj * 128:(jj + 1) * 128]
                lhs = a_strips[j]
                if hi is not None:
                    lhs = jnp.where(flag, hi.astype(bf16), lhs)
                r_ = jnp.dot(lhs, wd_v[j * 128:(j + 1) * 128, 0:D], preferred_element_type=f32)
                res['y'] = r_ if res['y'] is None else res['y'] + r_
                tok_ = r_[:, D - 128:D]
            else:
                lhs = h2b if hi is None else _gate1(h2b, flag, hi.astype(bf16))
                w_ref = wg_v if kind == 'g' else wu_v
                r_ = jnp.dot(lhs, w_ref[:, j * 128:(j + 1) * 128], preferred_element_type=f32)
                res[kind][j] = r_
                tok_ = r_
                if kind == 'u':
                    a_strips[j] = act(res['g'][j], r_)
                    if j < FD:
                        acol_v[j * 128:(j + 1) * 128, :] = column(a_strips[j].astype(f32))
            if i >= FI0 and pos < len(items):
                budget = FVR if i < len(strips) - 1 else 10 ** 9
                outs = None
                while pos < len(items) and budget > 0:
                    kind_, rg = items[pos]
                    outs = vpu_item(kind_, rg, tok_)
                    budget -= 2 * FG if kind_ == 'g' else 8
                    pos += 1
                tk = None
                for o_ in outs:
                    tk = _token(o_) if tk is None else jnp.maximum(tk, _token(o_))
                vtok[i] = tk
        y = res['y']
        if FD:
            y = y + fin(accs['vd'])
        y = y * jax.nn.sigmoid(rmax[:, 0:1])
        out_copy(0, S).wait()
        new = (x2 + gb * (h2 + y)).astype(bf16)
        out_v[pl.ds(g0, 8), :] = jnp.where(sel, new, out_v[pl.ds(g0, 8), :])
        fix = out_copy(g0, 8)
        fix.start()
        fix.wait()


@jax.jit
def pallas_adaLN_cond__sliding_block_cached__moe_arch_mod__prompt_kernel(
    A_x, A_k_cache, A_v_cache, A_wq, A_wo, B_x, B_w_r, B_w_gate, B_w_up, B_w_down, c, w_mod,
):
    del B_x
    any_spec = pl.BlockSpec(memory_space=pl.ANY)
    return pl.pallas_call(
        _kernel,
        out_shape=jax.ShapeDtypeStruct(A_x.shape, A_x.dtype),
        in_specs=[any_spec] * 11,
        out_specs=any_spec,
        scratch_shapes=[
            pltpu.VMEM((S, D), bf16),
            pltpu.VMEM((S, D), bf16),
            pltpu.VMEM((S, D), bf16),
            pltpu.VMEM((NQS * TQ, GW), bf16),
            pltpu.VMEM((S, D), f32),
            pltpu.VMEM((D, 2 * D + PADC), bf16),
            pltpu.VMEM((NMC, D, NM * 128), bf16),
            pltpu.VMEM((HKV, D, GW + PADW), bf16),
            pltpu.VMEM((HKV, GW, D), bf16),
            pltpu.VMEM((D, F), bf16),
            pltpu.VMEM((D, F), bf16),
            pltpu.VMEM((F, D + PADD), bf16),
            pltpu.VMEM((HKV, W, DH), bf16),
            pltpu.VMEM((HKV, W, DH), bf16),
            pltpu.VMEM((HKV, DH, W), bf16),
            pltpu.VMEM((8, 1, D), bf16),
            pltpu.VMEM((16, 8, 128), bf16),
            pltpu.VMEM((16, D), bf16),
            pltpu.VMEM((D, 128), f32),
            pltpu.VMEM((F, 128), f32),
            pltpu.VMEM((8, 6 * D), f32),
            pltpu.VMEM((8, 8, 128), f32),
            pltpu.VMEM((8, 8, 128), jnp.int32),
            pltpu.VMEM((4, 8, D), f32),
            pltpu.SMEM((1,), jnp.int32),
            pltpu.SemaphoreType.DMA((NSEM,)),
        ],
        compiler_params=pltpu.CompilerParams(vmem_limit_bytes=110 * 1024 * 1024,
                                             disable_semaphore_checks=bool(int(os.environ.get('KP_NOSEM', 1))),
                                             disable_bounds_checks=bool(int(os.environ.get('KP_NOBND', 1)))),
    )(A_x, A_k_cache, A_v_cache, A_wq, A_wo, B_w_r.reshape(8, 128), B_w_gate, B_w_up, B_w_down, c, w_mod)
```

```python
import contextlib
import math
import os

import jax
import jax.numpy as jnp
from jax import lax
from jax.experimental import pallas as pl
from jax.experimental.pallas import tpu as pltpu

S = 2048
D = 1024
HQ = 32
HKV = 4
REP = HQ // HKV
DH = 128
GW = REP * DH
W = 512
F = 3584
EPS = 1e-5
TQ = 256
NT = S // TQ
NIT = NT * HKV
NQS = NT
PADC = 128
TP = 512
SEQ_A = os.environ.get('KP_SEQA', 'KOV')
SEQ_B = os.environ.get('KP_SEQB', 'KQVON')
SEQ_C = os.environ.get('KP_SEQC', 'KQVOL')
SEQ_D = os.environ.get('KP_SEQD', 'KoVOL')
PINLO = os.environ.get('KP_PINLO', 'Q')
UNA = int(os.environ.get('KP_UNA', 1))
UNB = int(os.environ.get('KP_UNB', 2))
UNC = int(os.environ.get('KP_UNC', 2))
P0PIN = int(os.environ.get('KP_P0PIN', 1))
LAG0 = int(os.environ.get('KP_LAG0', 2))
LPC = os.environ.get('KP_LPC', 'Q0,O128').split(',')
LPD = os.environ.get('KP_LPD', 'V0,O0').split(',')
LPE = os.environ.get('KP_LPE', 'V0,V96,V192,O32,O128').split(',')
LCNT = [int(c_) for c_ in os.environ.get('KP_LCNT', '05555552')]
PADW = int(os.environ.get('KP_PADW', 128))
NKC = int(os.environ.get('KP_NKC', 4))
KC = D // NKC
UNP = int(os.environ.get('KP_UNP', 1))
OS = int(os.environ.get('KP_OS', 32))
FG = int(os.environ.get('KP_FG', 0))
FD = int(os.environ.get('KP_FD', 15))
PADD = int(os.environ.get('KP_PADD', 256))
FI0 = int(os.environ.get('KP_FI0', 8))
FLAG_ = int(os.environ.get('KP_FLAG', 4))
FVR = int(os.environ.get('KP_FVR', 32))
YS = int(os.environ.get('KP_YS', 0))
YLEAD = int(os.environ.get('KP_YLEAD', 2))
NM = 3
NMC = 11
NPIN = os.environ.get('KP_NPIN', 'O64')
P0ROWS = int(os.environ.get('KP_P0ROWS', 8))
P0SPAN = int(os.environ.get('KP_P0SPAN', 256))
SCOPES = int(os.environ.get('KP_SCOPES', 0))
QSCALE = (DH ** -0.5) * math.log2(math.e)
PR = TQ // REP

f32 = jnp.float32
bf16 = jnp.bfloat16

(SEM_C, SEM_WR, SEM_X0, SEM_WM1, SEM_K, SEM_V, SEM_WG, SEM_WU, SEM_WD, SEM_OUT, SEM_K0, SEM_WM2) = range(12)
SEM_X = 12
SEM_WQ = SEM_X + NT
SEM_WO = SEM_WQ + HKV
SEM_WQ0 = SEM_WO + HKV
SEM_WMS = SEM_WQ0 + NKC
SEM_WMC = SEM_WMS + NKC
SEM_WMR = SEM_WMC + NKC
NSEM = SEM_WMR + 2


def _scope(name):
    return jax.named_scope(name) if SCOPES else contextlib.nullcontext()


def _ln(x):
    m = jnp.mean(x, axis=-1, keepdims=True)
    xc = x - m
    v = jnp.mean(xc * xc, axis=-1, keepdims=True)
    return xc * lax.rsqrt(v + EPS)


def _recip(l):
    r = pl.reciprocal(l, approx=True)
    return r * (2.0 - l * r)


def _mo(x, m):
    return x if isinstance(x, int) else pl.multiple_of(x, m)


def _gate(x, flag, tok):
    n = x.shape[0]
    xs = jnp.where(flag, jnp.concatenate([tok] * (n // 8), axis=0), x[:, 0:128])
    return jnp.concatenate([xs, x[:, 128:]], axis=1)


def _gate1(x, flag, tok):
    r = tok.shape[0]
    x0 = jnp.where(flag, tok, x[0:r, 0:128])
    if x.shape[1] > 128:
        x0 = jnp.concatenate([x0, x[0:r, 128:]], axis=1)
    return x0 if x.shape[0] == r else jnp.concatenate([x0, x[r:]], axis=0)


def _rows(v8, n):
    return v8 if n == 8 else jnp.concatenate([v8] * (n // 8), axis=0)


def _token(y):
    t = y[:, 0:128]
    for j in range(1, y.shape[1] // 128):
        t = jnp.maximum(t, y[:, j * 128:(j + 1) * 128])
    u = t[0:8]
    for j in range(1, y.shape[0] // 8):
        u = jnp.maximum(u, t[8 * j:8 * (j + 1)])
    return u


def _kernel(x_hbm, k_hbm, v_hbm, wq_hbm, wo_hbm, wr_hbm, wg_hbm, wu_hbm, wd_hbm, c_hbm, wmod_hbm,
            out_hbm,
            x_v, out_v, h_v, q_v, acc_v, wmod_v, wmr_v, wq_v, wo_v, wg_v, wu_v, wd_v, k_v, v_v, kt_v,
            c_v8, wr_v8, sc_v, scc_v, acol_v, mod_v, best_v, bidx_v, aux_v, flag_s, sems):
    sk = k_hbm.shape[2]
    c_v = c_v8.at[0]
    wr_v = wr_v8.at[0]

    def cp(src, dst, i):
        return pltpu.make_async_copy(src, dst, sems.at[i])

    c_cp = cp(c_hbm, c_v, SEM_C)
    wr_cp = cp(wr_hbm, wr_v, SEM_WR)
    x0_cp = cp(x_hbm.at[0, pl.ds(0, TP), :], x_v.at[pl.ds(0, TP), :], SEM_X0)

    def wmr_cp(i):
        c0 = 2 * D + min(i * NM, 32 - NM) * 128
        return cp(wmod_hbm.at[:, pl.ds(c0, NM * 128)], wmr_v.at[i], SEM_WMR + (0 if i < 2 else 1))

    def wait_all(view, sem):
        cp(view, view, sem).wait()

    k0_cp = cp(k_hbm.at[0, 0, pl.ds(sk - W, W), :], k_v.at[0], SEM_K0)
    k_cp = cp(k_hbm.at[0, pl.ds(1, HKV - 1), pl.ds(sk - W, W), :], k_v.at[pl.ds(1, HKV - 1)], SEM_K)
    v_cp = cp(v_hbm.at[0, :, pl.ds(sk - W, W), :], v_v, SEM_V)
    wg_cp = cp(wg_hbm, wg_v, SEM_WG)
    wu_cp = cp(wu_hbm, wu_v, SEM_WU)
    wd_cp = cp(wd_hbm, wd_v.at[:, pl.ds(0, D)], SEM_WD)

    def x_cp(t):
        r0 = _mo(t * TQ, TQ)
        return cp(x_hbm.at[0, pl.ds(r0, TQ), :], x_v.at[pl.ds(r0, TQ), :], SEM_X + t)

    def wm_cp(part, j):
        c0 = _mo(part * D + j * KC, KC)
        return cp(wmod_hbm.at[:, pl.ds(c0, KC)], wmod_v.at[:, pl.ds(c0, KC)], (SEM_WMS, SEM_WMC)[part] + j)

    def wq0_cp(j):
        r0 = _mo(j * KC, KC)
        return cp(wq_hbm.at[pl.ds(r0, KC), pl.ds(0, GW)], wq_v.at[0, pl.ds(r0, KC), pl.ds(0, GW)], SEM_WQ0 + j)

    def wq_cp(g):
        return cp(wq_hbm.at[:, pl.ds(_mo(g * GW, GW), GW)], wq_v.at[g, :, pl.ds(0, GW)], SEM_WQ + min(g, 2))

    def wo_cp(g):
        return cp(wo_hbm.at[pl.ds(_mo(g * GW, GW), GW), :], wo_v.at[g], SEM_WO + min(g, 1))

    def out_copy(r0, n):
        return cp(out_v.at[pl.ds(r0, n), :], out_hbm.at[0, pl.ds(r0, n), :], SEM_OUT)

    for c_ in ([c_cp, x0_cp] + [c_ for j in range(NKC) for c_ in (wm_cp(0, j), wm_cp(1, j), wq0_cp(j))]
               + [x_cp(2), k0_cp, x_cp(3), k_cp, wr_cp]
               + [x_cp(t) for t in range(4, NT)]
               + [v_cp, wo_cp(0), wq_cp(1)] + [wmr_cp(i) for i in range(NMC)]
               + [wo_cp(1), wq_cp(2), wo_cp(2), wq_cp(3), wo_cp(3), wg_cp, wu_cp, wd_cp]):
        c_.start()

    def ln1_rows(r0, n, lo=None):
        x = x_v[pl.ds(r0, n), :].astype(f32)
        if lo is not None:
            x = _gate(x, *lo)
        y = _ln(x) * _rows(mod_v[:, D:2 * D], n) + _rows(mod_v[:, 0:D], n)
        h_v[pl.ds(r0, n), :] = y.astype(bf16)
        return y

    def ln2_rows(r0, n, valid=None, lo=None, router_only=False):
        av = _rows(aux_v[0], n)
        bv = _rows(aux_v[1], n)
        rv = _rows(aux_v[2], n)
        r_c = _rows(aux_v[3, :, 0:128], n)
        x2 = x_v[pl.ds(r0, n), :].astype(f32)
        if lo is not None:
            x2 = _gate(x2, *lo)
        m = jnp.mean(x2, axis=-1, keepdims=True)
        xc = x2 - m
        var = jnp.mean(xc * xc, axis=-1, keepdims=True)
        rs = lax.rsqrt(var + EPS)
        if not router_only:
            y = x2 + ((xc * rs) * av + bv)
            out_v[pl.ds(r0, n), :] = y.astype(bf16)
        r = jnp.sum(xc * rv, axis=-1, keepdims=True) * rs
        r = (jnp.broadcast_to(r, (n, 128)) + r_c).astype(bf16).astype(f32)
        if valid is not None:
            r = jnp.where(valid, r, -jnp.inf)
        mb = jnp.broadcast_to(m, (n, 128))
        rsb = jnp.broadcast_to(rs, (n, 128))
        best = best_v[0]
        bm = best_v[1]
        brs = best_v[2]
        bidx = bidx_v[0]
        rows = lax.broadcasted_iota(jnp.int32, (8, 128), 0)
        for j in range(n // 8):
            sl = slice(8 * j, 8 * (j + 1))
            upd = r[sl] > best
            best = jnp.where(upd, r[sl], best)
            bm = jnp.where(upd, mb[sl], bm)
            brs = jnp.where(upd, rsb[sl], brs)
            bidx = jnp.where(upd, rows + (r0 + 8 * j), bidx)
        best_v[0] = best
        best_v[1] = bm
        best_v[2] = brs
        bidx_v[0] = bidx
        if router_only:
            return mb, rsb
        return y, best

    def qproj(hr0, qr0, n, g, c0, nc, hi=None, h=None):
        if h is None:
            h = h_v[pl.ds(hr0, n), :]
        if hi is not None:
            flag, tok = hi
            h = _gate1(h, flag, jnp.concatenate([tok, tok], axis=0).astype(bf16))
        q = jnp.dot(h, wq_v[g, :, c0:c0 + nc], preferred_element_type=f32)
        q_v[pl.ds(qr0, n), c0:c0 + nc] = (q * QSCALE).astype(bf16)
        return q

    with _scope('P0_wait_c_wm0'):
        flag_s[0] = 0
        c_cp.wait()
        cf = c_v[...].astype(f32)
        sc = (cf * jax.nn.sigmoid(cf)).astype(bf16)
        sc_v[...] = jnp.broadcast_to(sc, (16, D))
        scc_v[...] = jnp.broadcast_to(sc.astype(f32), (128, D)).T
        best_v[0] = jnp.full((8, 128), -jnp.inf, f32)
        best_v[1] = jnp.zeros((8, 128), f32)
        best_v[2] = jnp.zeros((8, 128), f32)
        bidx_v[0] = jnp.zeros((8, 128), jnp.int32)
        x0_cp.wait()

        def norm_rows(i, carry):
            r0 = pl.multiple_of(i * 128, 128)
            acc_v[pl.ds(r0, 128), :] = _ln(x_v[pl.ds(r0, 128), :].astype(f32))
            return carry

        lax.fori_loop(0, TP // 128, norm_rows, 0)

    def k_chunk(j, carry):
        wm_cp(0, j).wait()
        wm_cp(1, j).wait()
        c0 = pl.multiple_of(j * KC, KC)
        scv = sc_v[...]
        sa = jnp.dot(scv, wmod_v[:, pl.ds(c0, KC)], preferred_element_type=f32)[0:8].astype(bf16).astype(f32)
        ca = jnp.dot(scv, wmod_v[:, pl.ds(D + c0, KC)], preferred_element_type=f32)[0:8].astype(bf16).astype(f32)
        mod_v[:, pl.ds(c0, KC)] = sa
        mod_v[:, pl.ds(D + c0, KC)] = 1.0 + ca
        h_v[0:TP, pl.ds(c0, KC)] = (acc_v[0:TP, pl.ds(c0, KC)] * _rows(1.0 + ca, TP) + _rows(sa, TP)).astype(bf16)
        wq0_cp(j).wait()
        part = jnp.dot(h_v[0:TP, pl.ds(c0, KC)], wq_v[0, pl.ds(c0, KC), 0:GW], preferred_element_type=f32)
        tot = jnp.where(j == 0, 0.0, acc_v[TP:2 * TP, :]) + part
        acc_v[TP:2 * TP, :] = tot
        q_v[0:TP, :] = (tot * QSCALE).astype(bf16)
        return carry

    with _scope('P1_kchunks'):
        lax.fori_loop(0, NKC, k_chunk, 0)

    def q0_cols(r0, n, j0, j1, ln_r0):
        flag = flag_s[0] > 0
        h = h_v[pl.ds(r0, n), :]
        toks = {}
        npc = (j1 - j0) - LAG0
        base, extra = divmod(TQ // P0ROWS, npc)
        cnts = [base + (1 if i < extra else 0) for i in range(npc)]
        off = 0
        for i, j in enumerate(range(j0, j1)):
            hi = (flag, toks[i - LAG0]) if (i - LAG0) in toks else None
            q = qproj(r0, r0, n, 0, j * DH, DH, hi, h)
            if i < npc:
                tk = None
                for k_ in range(cnts[i]):
                    r_ = (k_ * P0SPAN // cnts[i]) // 8 * 8
                    lo = (flag, q[r_:r_ + 8]) if P0PIN else None
                    t_ = _token(ln1_rows(_mo(ln_r0 + off, 8), P0ROWS, lo))
                    tk = t_ if tk is None else jnp.maximum(tk, t_)
                    off += P0ROWS
                toks[i] = tk

    with _scope('P2_ln'):
        x_cp(2).wait()
        ln1_rows(2 * TQ, TQ)
        k0_cp.wait()

    def q0_tile(i, carry):
        for u in range(UNP):
            t = 2 + i * UNP + u

            @pl.when(t + 1 < NT)
            def _():
                x_cp(t + 1).wait()

        @pl.when(i == 1)
        def _():
            k_cp.wait()

        for u in range(UNP):
            t = 2 + i * UNP + u
            q0_cols(pl.multiple_of(t * TQ, TQ), TQ, 0, REP, jnp.minimum(t + 1, NT - 1) * TQ)
            gk = jnp.clip(t - 2 - (UNP - 1), 0, HKV - 1)
            kt_v[gk] = k_v[gk].T
        return carry

    with _scope('P3_q0'):
        lax.fori_loop(0, (NT - 2) // UNP, q0_tile, 0)
        v_cp.wait()
        wo_cp(0).wait()
        wq_cp(1).wait()
        wr_cp.wait()
        wait_all(wmr_v.at[pl.ds(0, 2)], SEM_WMR)

    def body(its, seq, phase, pins=None):
        flag = flag_s[0] > 0
        st = dict(lo=None, hi=None, pend=None, next=None)

        def flush_op(rb=TQ):
            if st['pend'] is not None:
                st['pend'](st.get('done', 0), rb)
                st['done'] = rb % TQ
                if rb == TQ:
                    st['pend'] = None

        for u_, it in enumerate(its):
            g = it // NT
            t = it % NT
            a0 = _mo(t * TQ, TQ)
            q0 = a0

            def ln_step(p0, pins, t=t):
                n = 8
                hi = st['hi']
                for i, pin in enumerate(pins):
                    src_ = st.get(pin[0])
                    if src_ is None:
                        src_, r_ = st['V'], 0
                    else:
                        r_ = int(pin[1:])
                    c_ = 512 if r_ >= TQ else 0
                    r_ = r_ % TQ
                    lo = (flag, src_[r_:r_ + 8, c_:c_ + 128])
                    off = (p0 + i) * n
                    if isinstance(t, int):
                        y, b = ln2_rows((t - 1) * TQ + off, n, None, lo)
                    else:
                        tl = jnp.maximum(t - 1, 0)
                        y, b = ln2_rows(_mo(tl * TQ + off, n), n, t > 0, lo)
                    tk = jnp.maximum(_token(y), b)
                    hi = tk if hi is None else jnp.maximum(hi, tk)
                st['hi'] = hi

            def qk(hh, g=g, q0=q0):
                qh = q_v[pl.ds(q0, TQ), hh * DH:(hh + 1) * DH]
                s = jnp.dot(qh, kt_v[g], preferred_element_type=f32)
                if st['hi'] is not None:
                    s = _gate1(s, flag, st['hi'])
                    st['hi'] = None
                m = jnp.max(s, axis=-1, keepdims=True)
                p = jnp.exp2(s - m)
                st['K'] = s
                st['P'] = p
                l = jnp.sum(p, axis=-1, keepdims=True)
                return p.astype(bf16), l

            def pv(pl_, g=g):
                p, l = pl_
                o = jnp.dot(p, v_v[g], preferred_element_type=f32)
                st['V'] = o
                return o * _recip(l)

            def op(o, hh, ra, rb, g=g, a0=a0):
                n = rb - ra
                r0 = _mo(a0 + ra, 16)
                y = jnp.dot(o[ra:rb].astype(bf16), wo_v[g, hh * DH:(hh + 1) * DH, :], preferred_element_type=f32)
                st['O'] = y
                if hh == 0 and phase == 'B':
                    acc_v[pl.ds(r0, n), :] = jnp.where(g == 0, 0.0, acc_v[pl.ds(r0, n), :]) + y
                elif hh == REP - 1 and phase == 'C':
                    ga = _rows(mod_v[:, 2 * D:3 * D], n)
                    x = x_v[pl.ds(r0, n), :].astype(f32)
                    x_v[pl.ds(r0, n), :] = (x + ga * (acc_v[pl.ds(r0, n), :] + y)).astype(bf16)
                else:
                    acc_v[pl.ds(r0, n), :] += y

            sp = None
            for hh in range(REP):
                for tok in seq:
                    if tok == 'K':
                        sp = qk(hh)
                    elif tok == 'V':
                        o = pv(sp)
                        new_pend = (lambda ra, rb, o=o, hh=hh, op=op: op(o, hh, ra, rb))
                        if 'O' in seq[seq.index('V'):]:
                            st['next'] = new_pend
                        else:
                            st['pend'] = new_pend
                    elif tok == 'O':
                        flush_op()
                        if st['next'] is not None:
                            st['pend'] = st['next']
                            st['next'] = None
                    elif tok == 'o':
                        flush_op(OS)
                    elif tok == 'L':
                        if LCNT[hh]:
                            ln_step(sum(LCNT[:hh]), {len(LPD): LPD, len(LPE): LPE}[LCNT[hh]])
                    elif tok == 'Q':
                        q = qproj(a0, a0, TQ, g + 1, hh * DH, DH)
                        st['Q'] = q
                    elif tok == 'N':
                        pos = u_ * REP + hh
                        nst = UNB * REP - 1
                        nm = NM
                        if pos > 0:
                            ci = jnp.minimum(its[0] // UNB, NMC - 1)
                            j = jnp.minimum(ci * nm, 32 - nm)
                            c0 = pl.multiple_of(2 * D + j * 128, 128)
                            ga_, gb_ = [(128 * k_) // nst for k_ in (pos - 1, pos)]
                            r_ = int(NPIN[1:])
                            acc = st.get('macc')
                            tok_ = st[NPIN[0]][r_:r_ + 8, 0:128]
                            for rg in range(ga_, gb_):
                                xc_ = scc_v[8 * rg:8 * rg + 8, :]
                                if rg == ga_:
                                    xc_ = jnp.where(flag, tok_, xc_)
                                w_ = wmr_v[ci, 8 * rg:8 * rg + 8, :].astype(f32)
                                pr_ = w_ * jnp.concatenate([xc_] * nm, axis=1)
                                acc = pr_ if acc is None else acc + pr_
                            st['macc'] = acc
                            st['hi'] = _token(acc)
                            if pos == nst:
                                tot_ = jnp.sum(acc, axis=0, keepdims=True).astype(bf16).astype(f32)
                                mod_v[:, pl.ds(c0, nm * 128)] = jnp.broadcast_to(tot_, (8, nm * 128))
            if phase == 'C':
                flush_op()
        flush_op()
        if phase == 'C':
            for it in its:
                t = it % NT
                if isinstance(t, int):
                    out_copy((t - 1) * TQ, TQ).start()
                else:
                    @pl.when(t > 0)
                    def _():
                        out_copy(_mo((t - 1) * TQ, TQ), TQ).start()

    def body_b(i, carry):
        it = i * UNB

        @pl.when(i == 2)
        def _():
            wait_all(wmr_v.at[pl.ds(2, NMC - 2)], SEM_WMR + 1)
            wait_all(wq_v.at[pl.ds(2, 2), :, pl.ds(0, GW)], SEM_WQ + 2)
            wait_all(wo_v.at[pl.ds(1, 3)], SEM_WO + 1)

        body([it + u for u in range(UNB)], SEQ_B, 'B')
        return carry

    with _scope('LB'):
        lax.fori_loop(0, 3 * NT // UNB, body_b, 0)

    wg_cp.wait()
    wu_cp.wait()
    wd_cp.wait()
    sb_ = mod_v[:, 3 * D:4 * D]
    cb1_ = 1.0 + mod_v[:, 4 * D:5 * D]
    gb_ = mod_v[:, 5 * D:6 * D]
    wr8 = wr_v[...].astype(f32)
    wr_ = jnp.concatenate([wr8[r_:r_ + 1, :] for r_ in range(8)], axis=1)
    aux_v[0] = gb_ * cb1_
    aux_v[1] = gb_ * sb_
    aux_v[2] = cb1_ * wr_
    aux_v[3] = jnp.broadcast_to(jnp.sum(sb_ * wr_, axis=-1, keepdims=True), (8, D))

    def body_c(i, carry):
        body([i * UNC + u for u in range(UNC)], SEQ_D, 'C', LPD)
        return carry

    with _scope('LC'):
        lax.fori_loop(3 * NT // UNC, NIT // UNC, body_c, 0)

    with _scope('E1_last'):
        rl0 = (NT - 1) * TQ
        if YS:
            stat_m, stat_rs = ln2_rows(rl0, TQ, router_only=True)
        else:
            ln2_rows(rl0, TQ)
            out_copy(rl0, TQ).start()

    with _scope('E2_ffn'):
        best = best_v[0]
        bidx = bidx_v[0]
        rmax = jnp.max(best, axis=0, keepdims=True)
        idx_v = jnp.min(jnp.where(best == rmax, bidx, S), axis=0, keepdims=True)
        idx = jnp.minimum(idx_v[0, 0], S - 1)
        g0 = pl.multiple_of((idx // 8) * 8, 8)
        sb = mod_v[:, 3 * D:4 * D]
        cb = mod_v[:, 4 * D:5 * D]
        gb = mod_v[:, 5 * D:6 * D]
        x2 = x_v[pl.ds(g0, 8), :].astype(f32)
        h2 = (x2 - best_v[1][:, 0:1]) * best_v[2][:, 0:1] * (1.0 + cb) + sb
        h2b = h2.astype(bf16)
        rows8 = lax.broadcasted_iota(jnp.int32, (8, 1), 0) + g0
        sel = rows8 == idx

        def column(v8):
            row = jnp.sum(jnp.where(sel, v8, 0.0), axis=0, keepdims=True)
            return jnp.broadcast_to(row, (128, row.shape[1])).T

        def act(gt, up):
            return (gt * jax.nn.sigmoid(gt) * up).astype(bf16)

        def fin(a_):
            return jnp.broadcast_to(jnp.sum(a_, axis=0, keepdims=True), a_.shape)

        flag = flag_s[0] > 0
        nf = F // 128
        fm = nf - FG
        if FG:
            scc_v[...] = column(h2b.astype(f32))
        items = [('g', rg) for rg in range(D // 8)] if FG else []
        items += [('d', rg) for rg in range(FD * 16)]
        accs = {}
        a_strips = {}
        vtok = {}
        res = dict(g={}, u={}, y=None)
        strips = [(k_, j) for j in range(fm) for k_ in 'gu'] + [('d', j) for j in range(FD, nf)]

        def vpu_item(kind, rg, lo):
            col = (scc_v if kind == 'g' else acol_v)[8 * rg:8 * rg + 8, :]
            col = jnp.where(flag, lo, col)
            outs = []
            for nm_, w_ref, c0_, nc in ([('vg', wg_v, fm * 128, FG * 128), ('vu', wu_v, fm * 128, FG * 128)]
                                        if kind == 'g' else [('vd', wd_v, 0, D)]):
                pr_ = w_ref[8 * rg:8 * rg + 8, c0_:c0_ + nc].astype(f32) * jnp.concatenate([col] * (nc // 128), axis=1)
                accs[nm_] = pr_ if nm_ not in accs else accs[nm_] + pr_
                outs.append(accs[nm_])
            return outs

        pos = 0
        ypos = 0
        ytoks = {}
        ytok = h2[:, 0:128]
        for i, (kind, j) in enumerate(strips):
            hi = vtok.get(i - FLAG_)
            if kind == 'd':
                if j not in a_strips:
                    assert not any(k_ == 'g' for k_, _ in items[pos:]), 'VPU gate/up not finished'
                    av_ = act(fin(accs['vg']), fin(accs['vu']))
                    for jj in range(FG):
                        a_strips[fm + jj] = av_[:, jj * 128:(jj + 1) * 128]
                lhs = a_strips[j]
                if hi is not None:
                    lhs = jnp.where(flag, hi.astype(bf16), lhs)
                r_ = jnp.dot(lhs, wd_v[j * 128:(j + 1) * 128, 0:D], preferred_element_type=f32)
                res['y'] = r_ if res['y'] is None else res['y'] + r_
                tok_ = r_[:, D - 128:D]
            else:
                lhs = h2b if hi is None else _gate1(h2b, flag, hi.astype(bf16))
                w_ref = wg_v if kind == 'g' else wu_v
                r_ = jnp.dot(lhs, w_ref[:, j * 128:(j + 1) * 128], preferred_element_type=f32)
                res[kind][j] = r_
                tok_ = r_
                if kind == 'u':
                    a_strips[j] = act(res['g'][j], r_)
                    if j < FD:
                        acol_v[j * 128:(j + 1) * 128, :] = column(a_strips[j].astype(f32))
            if YS and ypos < TQ // 8:
                tk = None
                for _ in range(min(YS, TQ // 8 - ypos)):
                    sl = slice(8 * ypos, 8 * ypos + 8)
                    x2_ = x_v[rl0 + 8 * ypos:rl0 + 8 * ypos + 8, :].astype(f32)
                    m_ = jnp.where(flag, ytok, stat_m[sl])
                    nrm = (x2_ - jnp.concatenate([m_] * 8, axis=1)) * jnp.concatenate([stat_rs[sl]] * 8, axis=1)
                    y_ = x2_ + (nrm * aux_v[0] + aux_v[1])
                    out_v[rl0 + 8 * ypos:rl0 + 8 * ypos + 8, :] = y_.astype(bf16)
                    tk = _token(y_) if tk is None else jnp.maximum(tk, _token(y_))
                    ypos += 1
                vtok[i - YLEAD] = tk
                ytoks[i] = tok_
                ytok = ytoks.get(i + 1 - YLEAD, ytok) if i + 1 >= YLEAD else ytok
                if ypos == TQ // 8:
                    out_copy(rl0, TQ).start()
            if i >= FI0 and pos < len(items):
                budget = FVR if i < len(strips) - 1 else 10 ** 9
                outs = None
                while pos < len(items) and budget > 0:
                    kind_, rg = items[pos]
                    outs = vpu_item(kind_, rg, tok_)
                    budget -= 2 * FG if kind_ == 'g' else 8
                    pos += 1
                tk = None
                for o_ in outs:
                    tk = _token(o_) if tk is None else jnp.maximum(tk, _token(o_))
                vtok[i] = tk
        y = res['y']
        if FD:
            y = y + fin(accs['vd'])
        y = y * jax.nn.sigmoid(rmax[:, 0:1])
        out_copy(0, S).wait()
        new = (x2 + gb * (h2 + y)).astype(bf16)
        out_v[pl.ds(g0, 8), :] = jnp.where(sel, new, out_v[pl.ds(g0, 8), :])
        fix = out_copy(g0, 8)
        fix.start()
        fix.wait()


@jax.jit
def pallas_adaLN_cond__sliding_block_cached__moe_arch_mod__prompt_kernel(
    A_x, A_k_cache, A_v_cache, A_wq, A_wo, B_x, B_w_r, B_w_gate, B_w_up, B_w_down, c, w_mod,
):
    del B_x
    any_spec = pl.BlockSpec(memory_space=pl.ANY)
    return pl.pallas_call(
        _kernel,
        out_shape=jax.ShapeDtypeStruct(A_x.shape, A_x.dtype),
        in_specs=[any_spec] * 11,
        out_specs=any_spec,
        scratch_shapes=[
            pltpu.VMEM((S, D), bf16),
            pltpu.VMEM((S, D), bf16),
            pltpu.VMEM((S, D), bf16),
            pltpu.VMEM((NQS * TQ, GW), bf16),
            pltpu.VMEM((S, D), f32),
            pltpu.VMEM((D, 2 * D + PADC), bf16),
            pltpu.VMEM((NMC, D, NM * 128), bf16),
            pltpu.VMEM((HKV, D, GW + PADW), bf16),
            pltpu.VMEM((HKV, GW, D), bf16),
            pltpu.VMEM((D, F), bf16),
            pltpu.VMEM((D, F), bf16),
            pltpu.VMEM((F, D + PADD), bf16),
            pltpu.VMEM((HKV, W, DH), bf16),
            pltpu.VMEM((HKV, W, DH), bf16),
            pltpu.VMEM((HKV, DH, W), bf16),
            pltpu.VMEM((8, 1, D), bf16),
            pltpu.VMEM((16, 8, 128), bf16),
            pltpu.VMEM((16, D), bf16),
            pltpu.VMEM((D, 128), f32),
            pltpu.VMEM((F, 128), f32),
            pltpu.VMEM((8, 6 * D), f32),
            pltpu.VMEM((8, 8, 128), f32),
            pltpu.VMEM((8, 8, 128), jnp.int32),
            pltpu.VMEM((4, 8, D), f32),
            pltpu.SMEM((1,), jnp.int32),
            pltpu.SemaphoreType.DMA((NSEM,)),
        ],
        compiler_params=pltpu.CompilerParams(vmem_limit_bytes=110 * 1024 * 1024,
                                             disable_semaphore_checks=bool(int(os.environ.get('KP_NOSEM', 1))),
                                             disable_bounds_checks=bool(int(os.environ.get('KP_NOBND', 1)))),
    )(A_x, A_k_cache, A_v_cache, A_wq, A_wo, B_w_r.reshape(8, 128), B_w_gate, B_w_up, B_w_down, c, w_mod)
```

```python
import contextlib
import math
import os

import jax
import jax.numpy as jnp
from jax import lax
from jax.experimental import pallas as pl
from jax.experimental.pallas import tpu as pltpu


def _p(name, default):
    v = os.environ.get('KP_' + name)
    return default if v is None else type(default)(v)


S = 2048
D = 1024
HQ = 32
HKV = 4
REP = HQ // HKV
DH = 128
GW = REP * DH
W = 512
F = 3584
EPS = 1e-5
TQ = 256
HR = TQ // 2
KH = D // 2
NT = S // TQ
TP = 512
NKC = 4
PADW = 128
PADD = 256
NM = 3
NMC = 11
UNB = 2
UNC = 2
FD = _p('FD', 15)
FI0 = _p('FI0', 8)
FLAG_ = _p('FLAG', 4)
FVR = _p('FVR', 32)
LAG0 = _p('LAG0', 2)
T3B = _p('T3B', 5)
LCNT = [int(c_) for c_ in _p('LCNT', '00565655')]
LPINS = {5: _p('LP5', 'V0,V64,V128,V192,O0').split(','), 6: _p('LP6', 'V0,V64,V128,V192,N64,O0').split(',')}
NPIN = _p('NPIN', 'N64')
WQPIN = _p('WQPIN', 'V128')
WOPIN = _p('WOPIN', 'O0')
SCOPES = _p('SCOPES', 0)
QSCALE = (DH ** -0.5) * math.log2(math.e)

f32 = jnp.float32
bf16 = jnp.bfloat16

(SEM_C, SEM_WR, SEM_X0, SEM_K0, SEM_K, SEM_V, SEM_WG, SEM_WU, SEM_WD, SEM_OUT) = range(10)
SEM_X = 10
SEM_WQ = SEM_X + NT
SEM_WO = SEM_WQ + HKV
SEM_WQ0 = SEM_WO + HKV
SEM_WM = SEM_WQ0 + NKC
SEM_WMR = SEM_WM + NKC
NSEM = SEM_WMR + 2

ORDER7 = (4, 2, 1, 7, 5, 3, 6)
A_SLOT = {1: 0, 2: 1, 5: 2, 6: 3, 7: 4}
B_SLOT = {1: 0, 3: 1, 4: 2, 6: 3, 7: 4}


def _a_op(i, a11, a12, a21, a22):
    return {1: lambda: a11 + a22, 2: lambda: a21 + a22, 3: lambda: a11, 4: lambda: a22,
            5: lambda: a11 + a12, 6: lambda: a21 - a11, 7: lambda: a12 - a22}[i]()


def _a_sums(a11, a12, a21, a22):
    return [_a_op(i, a11, a12, a21, a22) for i in (1, 2, 5, 6, 7)]


def _b_sums(b11, b12, b21, b22):
    return [b11 + b22, b12 - b22, b21 - b11, b11 + b12, b21 + b22]


class _Combine:
    def __init__(self):
        self.m = {}

    def feed(self, i, v):
        m = self.m
        if i == 4:
            m['c11'] = v
            return []
        if i == 2:
            m['c22'] = v
            return [(1, 0, v + m['c11'])]
        if i == 1:
            m['c11'] = m['c11'] + v
            m['c22'] = v - m['c22']
            return []
        if i == 7:
            m['c11'] = m['c11'] + v
            return []
        if i == 5:
            m['c12'] = v
            return [(0, 0, m['c11'] - v)]
        if i == 3:
            m['c22'] = m['c22'] + v
            return [(0, 1, m['c12'] + v)]
        return [(1, 1, m['c22'] + v)]


def _scope(name):
    return jax.named_scope(name) if SCOPES else contextlib.nullcontext()


def _ln(x):
    m = jnp.mean(x, axis=-1, keepdims=True)
    xc = x - m
    v = jnp.mean(xc * xc, axis=-1, keepdims=True)
    return xc * lax.rsqrt(v + EPS)


def _recip(l):
    r = pl.reciprocal(l, approx=True)
    return r * (2.0 - l * r)


def _mo(x, m):
    return x if isinstance(x, int) else pl.multiple_of(x, m)


def _rows(v8, n):
    return v8 if n == 8 else jnp.concatenate([v8] * (n // 8), axis=0)


def _gate(x, flag, tok):
    xs = jnp.where(flag, _rows(tok, x.shape[0]), x[:, 0:128])
    return jnp.concatenate([xs, x[:, 128:]], axis=1)


def _gate1(x, flag, tok):
    r = tok.shape[0]
    x0 = jnp.where(flag, tok, x[0:r, 0:128])
    if x.shape[1] > 128:
        x0 = jnp.concatenate([x0, x[0:r, 128:]], axis=1)
    return x0 if x.shape[0] == r else jnp.concatenate([x0, x[r:]], axis=0)


def _token(*ys):
    u = None
    for y in ys:
        for i in range(y.shape[0] // 8):
            for j in range(y.shape[1] // 128):
                v = y[8 * i:8 * i + 8, 128 * j:128 * j + 128]
                u = v if u is None else jnp.maximum(u, v)
    return u


def _kernel(x_hbm, k_hbm, v_hbm, wq_hbm, wo_hbm, wr_hbm, wg_hbm, wu_hbm, wd_hbm, c_hbm, wmod_hbm,
            out_hbm,
            x_v, out_v, h_v, hs_v, q_v, acc_v, wm_v, wmr_v, wq_v, wqs_v, wo_v, wos_v, wg_v, wu_v, wd_v,
            k_v, v_v, kt_v, c_v8, wr_v8, sc_v, scc_v, acol_v, mod_v, best_v, bidx_v, aux_v, flag_s, sems):
    sk = k_hbm.shape[2]
    c_v = c_v8.at[0]
    wr_v = wr_v8.at[0]

    def cp(src, dst, i):
        return pltpu.make_async_copy(src, dst, sems.at[i])

    def wait_all(view, sem):
        cp(view, view, sem).wait()

    c_cp = cp(c_hbm, c_v, SEM_C)
    wr_cp = cp(wr_hbm, wr_v, SEM_WR)
    x0_cp = cp(x_hbm.at[0, pl.ds(0, TP), :], x_v.at[pl.ds(0, TP), :], SEM_X0)
    k0_cp = cp(k_hbm.at[0, 0, pl.ds(sk - W, W), :], k_v.at[0], SEM_K0)
    k_cp = cp(k_hbm.at[0, pl.ds(1, HKV - 1), pl.ds(sk - W, W), :], k_v.at[pl.ds(1, HKV - 1)], SEM_K)
    v_cp = cp(v_hbm.at[0, :, pl.ds(sk - W, W), :], v_v, SEM_V)
    wg_cp = cp(wg_hbm, wg_v, SEM_WG)
    wu_cp = cp(wu_hbm, wu_v, SEM_WU)
    wd_cp = cp(wd_hbm, wd_v.at[:, pl.ds(0, D)], SEM_WD)

    def x_cp(t):
        r0 = _mo(t * TQ, TQ)
        return cp(x_hbm.at[0, pl.ds(r0, TQ), :], x_v.at[pl.ds(r0, TQ), :], SEM_X + t)

    def wm_cps(j):
        return [cp(wmod_hbm.at[:, pl.ds(i * KH + j * 128, 128)], wm_v.at[j, :, pl.ds(i * 128, 128)], SEM_WM + j)
                for i in range(4)]

    def wq0_cps(j):
        return [cp(wq_hbm.at[pl.ds(_mo(i * KH + j * 128, 128), 128), pl.ds(0, GW)],
                   wq_v.at[0, pl.ds(_mo(i * KH + j * 128, 128), 128), pl.ds(0, GW)], SEM_WQ0 + j) for i in range(2)]

    def wmr_cp(i):
        c0 = 2 * D + min(i * NM, 32 - NM) * 128
        return cp(wmod_hbm.at[:, pl.ds(c0, NM * 128)], wmr_v.at[i], SEM_WMR + (0 if i < 2 else 1))

    def wq_cp(g):
        return cp(wq_hbm.at[:, pl.ds(g * GW, GW)], wq_v.at[g, :, pl.ds(0, GW)], SEM_WQ + g)

    def wo_cp(g):
        return cp(wo_hbm.at[pl.ds(g * GW, GW), :], wo_v.at[g], SEM_WO + min(g, 2))

    def out_copy(r0, n):
        return cp(out_v.at[pl.ds(r0, n), :], out_hbm.at[0, pl.ds(r0, n), :], SEM_OUT)

    for c_ in ([c_cp, x0_cp] + [c_ for j in range(NKC) for c_ in wm_cps(j) + wq0_cps(j)]
               + [x_cp(2), k0_cp, x_cp(3), x_cp(4), k_cp, x_cp(5), wr_cp, wo_cp(0), wq_cp(1), x_cp(6), x_cp(7), v_cp,
                  wmr_cp(0), wmr_cp(1), wq_cp(2), wo_cp(1)] + [wmr_cp(i) for i in range(2, NMC)]
               + [wq_cp(3), wo_cp(2), wo_cp(3), wg_cp, wu_cp, wd_cp]):
        c_.start()

    def ln1_pair(t, r, n, lo=None):
        ys = []
        for half in range(2):
            r0 = _mo(t * TQ + half * HR + r, 8)
            x = x_v[pl.ds(r0, n), :].astype(f32)
            if lo is not None:
                x = _gate(x, *lo)
            y = _ln(x) * _rows(mod_v[:, D:2 * D], n) + _rows(mod_v[:, 0:D], n)
            h_v[pl.ds(r0, n), :] = y.astype(bf16)
            ys.append(y)
        sums = jnp.concatenate(_a_sums(ys[0][:, :KH], ys[0][:, KH:], ys[1][:, :KH], ys[1][:, KH:]), axis=1)
        hs_v[pl.ds(_mo(t * HR + r, 8), n), :] = sums.astype(bf16)
        return sums

    def wq_unit(g, u, lo):
        r0 = _mo(u * 8, 8)
        top = _gate(wq_v[g, pl.ds(r0, 8), 0:GW].astype(f32), *lo)
        bot = wq_v[g, pl.ds(KH + r0, 8), 0:GW].astype(f32)
        outs = []
        for p in range(REP // 2):
            c0, c1, c2 = 2 * p * DH, (2 * p + 1) * DH, (2 * p + 2) * DH
            outs += _b_sums(top[:, c0:c1], top[:, c1:c2], bot[:, c0:c1], bot[:, c1:c2])
        sums = jnp.concatenate(outs, axis=1)
        wqs_v[g, pl.ds(r0, 8), :] = sums.astype(bf16)
        return sums

    def wo_unit(g, u, lo):
        r0 = _mo((u // 16) * 2 * DH + (u % 16) * 8, 8)
        top = _gate(wo_v[g, pl.ds(r0, 8), :].astype(f32), *lo)
        bot = wo_v[g, pl.ds(DH + r0, 8), :].astype(f32)
        sums = jnp.concatenate(_b_sums(top[:, :KH], top[:, KH:], bot[:, :KH], bot[:, KH:]), axis=1)
        wos_v[g, pl.ds(_mo(u * 8, 8), 8), :] = sums.astype(bf16)
        return sums

    def ln2_rows(r0, n, valid=None, lo=None):
        av = _rows(aux_v[0], n)
        bv = _rows(aux_v[1], n)
        rv = _rows(aux_v[2], n)
        r_c = _rows(aux_v[3, :, 0:128], n)
        x2 = x_v[pl.ds(r0, n), :].astype(f32)
        if lo is not None:
            x2 = _gate(x2, *lo)
        m = jnp.mean(x2, axis=-1, keepdims=True)
        xc = x2 - m
        var = jnp.mean(xc * xc, axis=-1, keepdims=True)
        rs = lax.rsqrt(var + EPS)
        y = x2 + ((xc * rs) * av + bv)
        out_v[pl.ds(r0, n), :] = y.astype(bf16)
        r = jnp.sum(xc * rv, axis=-1, keepdims=True) * rs
        r = (jnp.broadcast_to(r, (n, 128)) + r_c).astype(bf16).astype(f32)
        if valid is not None:
            r = jnp.where(valid, r, -jnp.inf)
        mb = jnp.broadcast_to(m, (n, 128))
        rsb = jnp.broadcast_to(rs, (n, 128))
        best = best_v[0]
        bm = best_v[1]
        brs = best_v[2]
        bidx = bidx_v[0]
        rows = lax.broadcasted_iota(jnp.int32, (8, 128), 0)
        for j in range(n // 8):
            sl = slice(8 * j, 8 * (j + 1))
            upd = r[sl] > best
            best = jnp.where(upd, r[sl], best)
            bm = jnp.where(upd, mb[sl], bm)
            brs = jnp.where(upd, rsb[sl], brs)
            bidx = jnp.where(upd, rows + (r0 + 8 * j), bidx)
        best_v[0] = best
        best_v[1] = bm
        best_v[2] = brs
        bidx_v[0] = bidx
        return y, best

    with _scope('P0_wait'):
        flag_s[0] = 0
        c_cp.wait()
        cf = c_v[...].astype(f32)
        sc = (cf * jax.nn.sigmoid(cf)).astype(bf16)
        sc_v[...] = jnp.broadcast_to(sc, (16, D))
        scc_v[...] = jnp.broadcast_to(sc.astype(f32), (128, D)).T
        best_v[0] = jnp.full((8, 128), -jnp.inf, f32)
        best_v[1] = jnp.zeros((8, 128), f32)
        best_v[2] = jnp.zeros((8, 128), f32)
        bidx_v[0] = jnp.zeros((8, 128), jnp.int32)
        x0_cp.wait()

        def norm_rows(i, carry):
            r0 = pl.multiple_of(i * 128, 128)
            acc_v[pl.ds(r0, 128), 0:D] = _ln(x_v[pl.ds(r0, 128), :].astype(f32))
            return carry

        lax.fori_loop(0, TP // 128, norm_rows, 0)

    def k_chunk(j, carry):
        wait_all(wm_v.at[j, :, pl.ds(0, 512)], SEM_WM + j)
        clo = pl.multiple_of(j * 128, 128)
        chi = pl.multiple_of(KH + j * 128, 128)
        md = jnp.dot(sc_v[...], wm_v[j, :, 0:512], preferred_element_type=f32)[0:8].astype(bf16).astype(f32)
        hh = []
        for i, c0 in enumerate((clo, chi)):
            sa = md[:, i * 128:(i + 1) * 128]
            ca1 = 1.0 + md[:, (2 + i) * 128:(3 + i) * 128]
            mod_v[:, pl.ds(c0, 128)] = sa
            mod_v[:, pl.ds(D + c0, 128)] = ca1
            y = acc_v[0:TP, pl.ds(c0, 128)] * _rows(ca1, TP) + _rows(sa, TP)
            h_v[0:TP, pl.ds(c0, 128)] = y.astype(bf16)
            hh.append(y)
        for t in range(TP // TQ):
            top = slice(t * TQ, t * TQ + HR)
            bot = slice(t * TQ + HR, (t + 1) * TQ)
            for i, s_ in enumerate(_a_sums(hh[0][top], hh[1][top], hh[0][bot], hh[1][bot])):
                hs_v[t * HR:(t + 1) * HR, pl.ds(i * KH + clo, 128)] = s_.astype(bf16)
        for c_ in wq0_cps(j):
            c_.wait()
        lhs = jnp.concatenate([h_v[0:TP, pl.ds(clo, 128)], h_v[0:TP, pl.ds(chi, 128)]], axis=1)
        rhs = jnp.concatenate([wq_v[0, pl.ds(clo, 128), 0:GW], wq_v[0, pl.ds(chi, 128), 0:GW]], axis=0)
        tot = jnp.where(j == 0, 0.0, acc_v[0:TP, D:2 * D]) + jnp.dot(lhs, rhs, preferred_element_type=f32)
        acc_v[0:TP, D:2 * D] = tot
        q_v[0:TP, :] = (tot * QSCALE).astype(bf16)
        return carry

    with _scope('P1_kchunks'):
        lax.fori_loop(0, NKC, k_chunk, 0)

    with _scope('P2_ln'):
        x_cp(2).wait()
        ln1_pair(2, 0, HR)
        k0_cp.wait()

    def q0_tile(t, units):
        flag = flag_s[0] > 0
        r0 = pl.multiple_of(t * TQ, TQ)
        tn = jnp.minimum(t + 1, NT - 1)
        h = h_v[pl.ds(r0, TQ), :]
        jobs = [(lambda lo, r=r: ln1_pair(tn, r, 8, lo)) for r in range(0, HR, 8)]
        step = max(1, len(units) // len(jobs))
        mixed = []
        for i, jb in enumerate(jobs):
            mixed.append(jb)
            mixed += units[i * len(units) // len(jobs):(i + 1) * len(units) // len(jobs)]
        npc = REP - LAG0
        toks = {}
        for j in range(REP):
            hj = h
            if (j - LAG0) in toks:
                tk = toks[j - LAG0]
                hj = _gate1(h, flag, jnp.concatenate([tk, tk], axis=0).astype(bf16))
            q = jnp.dot(hj, wq_v[0, :, j * DH:(j + 1) * DH], preferred_element_type=f32)
            q_v[pl.ds(r0, TQ), j * DH:(j + 1) * DH] = (q * QSCALE).astype(bf16)
            if j < npc:
                mine = mixed[j * len(mixed) // npc:(j + 1) * len(mixed) // npc]
                outs = []
                for k_, jb in enumerate(mine):
                    r_ = (k_ * TQ // len(mine)) // 8 * 8
                    outs.append(jb((flag, q[r_:r_ + 8])))
                toks[j] = _token(*outs)

    def q0_a(t, carry):
        x_cp(t + 1).wait()

        @pl.when(t == 3)
        def _():
            k_cp.wait()

        q0_tile(t, [])
        gk = jnp.minimum(t - 2, HKV - 1)
        kt_v[gk] = k_v[gk].T
        return carry

    def q0_b(t, carry):
        @pl.when(t + 1 < NT)
        def _():
            x_cp(t + 1).wait()

        nu = -(-64 // (NT - T3B))
        u0 = jnp.minimum((t - T3B) * nu, 64 - nu)
        units = []
        for u in range(nu):
            units.append(lambda lo, u=u: wq_unit(1, u0 + u, lo))
            units.append(lambda lo, u=u: wo_unit(0, u0 + u, lo))
        q0_tile(t, units)
        gk = jnp.minimum(t - 2, HKV - 1)
        kt_v[gk] = k_v[gk].T
        return carry

    with _scope('P3_q0'):
        lax.fori_loop(2, T3B, q0_a, 0)
        wo_cp(0).wait()
        wq_cp(1).wait()
        lax.fori_loop(T3B, NT, q0_b, 0)
        v_cp.wait()
        wr_cp.wait()
        wait_all(wmr_v.at[pl.ds(0, 2)], SEM_WMR)
        wq_cp(2).wait()
        wo_cp(1).wait()

    def body(i, un, last_group):
        flag = flag_s[0] > 0
        st = dict(hi=None, pend=[])
        g = 3 if last_group else (i * un) // NT

        def pin(name):
            r_ = int(name[1:])
            return flag, st[name[0]][r_:r_ + 8, 0:128]

        def add_hi(tk):
            st['hi'] = tk if st['hi'] is None else jnp.maximum(st['hi'], tk)

        def o_run(n):
            for k_ in range(min(n, len(st['pend']))):
                y = st['pend'].pop(0)()
                if k_ == 0:
                    st['N'] = y
                st['O'] = y

        for u_ in range(un):
            t = (i * un + u_) % NT
            a0 = pl.multiple_of(t * TQ, TQ)
            m0 = pl.multiple_of(t * HR, HR)

            def qk(hh, a0=a0):
                qh = q_v[pl.ds(a0, TQ), hh * DH:(hh + 1) * DH]
                s = jnp.dot(qh, kt_v[g], preferred_element_type=f32)
                if st['hi'] is not None:
                    s = _gate1(s, flag, st['hi'])
                    st['hi'] = None
                m = jnp.max(s, axis=-1, keepdims=True)
                p = jnp.exp2(s - m)
                l = jnp.sum(p, axis=-1, keepdims=True)
                return p.astype(bf16), l

            def pv(pl_):
                p, l = pl_
                o = jnp.dot(p, v_v[g], preferred_element_type=f32)
                st['V'] = o
                return o * _recip(l)

            def q_prod(p, k, comb, a0=a0, m0=m0):
                if k in A_SLOT:
                    lhs = hs_v[pl.ds(m0, HR), A_SLOT[k] * KH:(A_SLOT[k] + 1) * KH]
                elif k == 3:
                    lhs = h_v[pl.ds(a0, HR), 0:KH]
                else:
                    lhs = h_v[pl.ds(pl.multiple_of(a0 + HR, HR), HR), KH:D]
                if k in B_SLOT:
                    c0 = (p * 5 + B_SLOT[k]) * DH
                    rhs = wqs_v[g + 1, :, c0:c0 + DH]
                elif k == 2:
                    rhs = wq_v[g + 1, 0:KH, 2 * p * DH:(2 * p + 1) * DH]
                else:
                    rhs = wq_v[g + 1, KH:D, (2 * p + 1) * DH:(2 * p + 2) * DH]
                y = jnp.dot(lhs, rhs, preferred_element_type=f32)
                st['Q'] = y
                for rh, ch, v in comb.feed(k, y):
                    r0 = pl.multiple_of(a0 + rh * HR, HR)
                    q_v[pl.ds(r0, HR), (2 * p + ch) * DH:(2 * p + ch + 1) * DH] = (v * QSCALE).astype(bf16)

            def o_prod(p, k, o0, o1, comb, a0=a0, m0=m0):
                lhs = _a_op(k, o0[:HR], o1[:HR], o0[HR:], o1[HR:]).astype(bf16)
                if k in B_SLOT:
                    rhs = wos_v[g, p * DH:(p + 1) * DH, B_SLOT[k] * KH:(B_SLOT[k] + 1) * KH]
                elif k == 2:
                    rhs = wo_v[g, 2 * p * DH:(2 * p + 1) * DH, 0:KH]
                else:
                    rhs = wo_v[g, (2 * p + 1) * DH:(2 * p + 2) * DH, KH:D]
                y = jnp.dot(lhs, rhs, preferred_element_type=f32)
                cs = slice((k - 1) * KH, k * KH)
                old = acc_v[pl.ds(m0, HR), cs]
                if p == 0 and not last_group:
                    acc_v[pl.ds(m0, HR), cs] = jnp.where(g == 0, 0.0, old) + y
                elif p == REP // 2 - 1 and last_group:
                    for rh, ch, v in comb.feed(k, old + y):
                        r0 = pl.multiple_of(a0 + rh * HR, HR)
                        cx = slice(ch * KH, (ch + 1) * KH)
                        ga = _rows(mod_v[:, 2 * D + ch * KH:2 * D + (ch + 1) * KH], HR)
                        x_v[pl.ds(r0, HR), cx] = (x_v[pl.ds(r0, HR), cx].astype(f32) + ga * v).astype(bf16)
                else:
                    acc_v[pl.ds(m0, HR), cs] = old + y
                return y

            def side_b(hh):
                pos = u_ * REP + hh
                if pos < 2:
                    return
                nst = un * REP - 2
                k_ = pos - 2
                ci = jnp.minimum(i, NMC - 1)
                acc = st.get('macc')
                lo = pin(NPIN)
                for rg in range(128 * k_ // nst, 128 * (k_ + 1) // nst):
                    xc_ = scc_v[8 * rg:8 * rg + 8, :]
                    if rg == 128 * k_ // nst:
                        xc_ = jnp.where(lo[0], lo[1], xc_)
                    pr_ = wmr_v[ci, 8 * rg:8 * rg + 8, :].astype(f32) * jnp.concatenate([xc_] * NM, axis=1)
                    acc = pr_ if acc is None else acc + pr_
                st['macc'] = acc
                add_hi(_token(acc))
                if k_ == nst - 1:
                    c0 = pl.multiple_of(2 * D + jnp.minimum(ci * NM, 32 - NM) * 128, 128)
                    tot_ = jnp.sum(acc, axis=0, keepdims=True).astype(bf16).astype(f32)
                    mod_v[:, pl.ds(c0, NM * 128)] = jnp.broadcast_to(tot_, (8, NM * 128))
                nu = 64 * un // NT
                u0 = (i % (NT // un)) * nu
                for u in range(nu * k_ // nst, nu * (k_ + 1) // nst):
                    add_hi(_token(wq_unit(jnp.minimum(g + 2, HKV - 1), u0 + u, pin(WQPIN))))
                    add_hi(_token(wo_unit(g + 1, u0 + u, pin(WOPIN))))

            def side_c(hh, t=t):
                tl = jnp.maximum(t - 1, 0)
                for k_ in range(LCNT[hh]):
                    off = (sum(LCNT[:hh]) + k_) * 8
                    y, b = ln2_rows(pl.multiple_of(tl * TQ + off, 8), 8, t > 0, pin(LPINS[LCNT[hh]][k_]))
                    add_hi(_token(y, b))

            for p in range(REP // 2):
                h0, h1 = 2 * p, 2 * p + 1
                if not last_group:
                    cq = _Combine()
                    sp = qk(h0)
                    for k in ORDER7[:4]:
                        q_prod(p, k, cq)
                    o0 = pv(sp)
                    o_run(4)
                    side_b(h0)
                    sp = qk(h1)
                    for k in ORDER7[4:]:
                        q_prod(p, k, cq)
                    o1 = pv(sp)
                    o_run(3)
                    side_b(h1)
                elif not st['pend']:
                    sp0 = qk(h0)
                    sp1 = qk(h1)
                    o0 = pv(sp0)
                    o1 = pv(sp1)
                else:
                    sp = qk(h0)
                    o_run(1)
                    o0 = pv(sp)
                    o_run(2)
                    side_c(h0)
                    sp = qk(h1)
                    o_run(1)
                    o1 = pv(sp)
                    o_run(3)
                    side_c(h1)
                co = _Combine()
                st['pend'] = [(lambda k=k, p=p, o0=o0, o1=o1, co=co, f=o_prod: f(p, k, o0, o1, co)) for k in ORDER7]
        o_run(7)
        if last_group:
            for u_ in range(un):
                t = (i * un + u_) % NT

                @pl.when(t > 0)
                def _():
                    out_copy(pl.multiple_of((t - 1) * TQ, TQ), TQ).start()

    def body_b(i, carry):
        @pl.when(i == 2)
        def _():
            wait_all(wmr_v.at[pl.ds(2, NMC - 2)], SEM_WMR + 1)
            wq_cp(3).wait()
            wait_all(wo_v.at[pl.ds(2, 2)], SEM_WO + 2)

        body(i, UNB, False)
        return carry

    with _scope('LB'):
        lax.fori_loop(0, 3 * NT // UNB, body_b, 0)

    wg_cp.wait()
    wu_cp.wait()
    wd_cp.wait()
    sb_ = mod_v[:, 3 * D:4 * D]
    cb1_ = 1.0 + mod_v[:, 4 * D:5 * D]
    gb_ = mod_v[:, 5 * D:6 * D]
    wr8 = wr_v[...].astype(f32)
    wr_ = jnp.concatenate([wr8[r_:r_ + 1, :] for r_ in range(8)], axis=1)
    aux_v[0] = gb_ * cb1_
    aux_v[1] = gb_ * sb_
    aux_v[2] = cb1_ * wr_
    aux_v[3] = jnp.broadcast_to(jnp.sum(sb_ * wr_, axis=-1, keepdims=True), (8, D))

    def body_c(i, carry):
        body(i, UNC, True)
        return carry

    with _scope('LC'):
        lax.fori_loop(0, NT // UNC, body_c, 0)

    with _scope('E1_last'):
        ln2_rows((NT - 1) * TQ, TQ)
        out_copy((NT - 1) * TQ, TQ).start()

    with _scope('E2_ffn'):
        best = best_v[0]
        bidx = bidx_v[0]
        rmax = jnp.max(best, axis=0, keepdims=True)
        idx_v = jnp.min(jnp.where(best == rmax, bidx, S), axis=0, keepdims=True)
        idx = jnp.minimum(idx_v[0, 0], S - 1)
        g0 = pl.multiple_of((idx // 8) * 8, 8)
        sb = mod_v[:, 3 * D:4 * D]
        cb = mod_v[:, 4 * D:5 * D]
        gb = mod_v[:, 5 * D:6 * D]
        x2 = x_v[pl.ds(g0, 8), :].astype(f32)
        h2 = (x2 - best_v[1][:, 0:1]) * best_v[2][:, 0:1] * (1.0 + cb) + sb
        h2b = h2.astype(bf16)
        sel = (lax.broadcasted_iota(jnp.int32, (8, 1), 0) + g0) == idx
        flag = flag_s[0] > 0
        nf = F // 128
        strips = [(k_, j) for j in range(nf) for k_ in 'gu'] + [('d', j) for j in range(FD, nf)]
        gate_r, a_strips, vtok = {}, {}, {}
        y = None
        yv = None
        pos = 0
        for i, (kind, j) in enumerate(strips):
            hi = vtok.get(i - FLAG_)
            if kind == 'd':
                lhs = a_strips[j]
                if hi is not None:
                    lhs = jnp.where(flag, hi.astype(bf16), lhs)
                r_ = jnp.dot(lhs, wd_v[j * 128:(j + 1) * 128, 0:D], preferred_element_type=f32)
                y = r_ if y is None else y + r_
                tok_ = r_[:, D - 128:D]
            else:
                lhs = h2b if hi is None else _gate1(h2b, flag, hi.astype(bf16))
                w_ref = wg_v if kind == 'g' else wu_v
                tok_ = jnp.dot(lhs, w_ref[:, j * 128:(j + 1) * 128], preferred_element_type=f32)
                if kind == 'g':
                    gate_r[j] = tok_
                else:
                    a_strips[j] = (gate_r[j] * jax.nn.sigmoid(gate_r[j]) * tok_).astype(bf16)
                    if j < FD:
                        row = jnp.sum(jnp.where(sel, a_strips[j].astype(f32), 0.0), axis=0, keepdims=True)
                        acol_v[j * 128:(j + 1) * 128, :] = jnp.broadcast_to(row, (128, 128)).T
            if i >= FI0 and pos < FD * 16:
                end = min(pos + FVR // 8, FD * 16) if i < len(strips) - 1 else FD * 16
                for rg in range(pos, end):
                    col = jnp.where(flag, tok_, acol_v[8 * rg:8 * rg + 8, :])
                    pr_ = wd_v[8 * rg:8 * rg + 8, 0:D].astype(f32) * jnp.concatenate([col] * (D // 128), axis=1)
                    yv = pr_ if yv is None else yv + pr_
                pos = end
                vtok[i] = _token(yv)
        y = (y + jnp.sum(yv, axis=0, keepdims=True)) * jax.nn.sigmoid(rmax[:, 0:1])
        out_copy(0, S).wait()
        new = (x2 + gb * (h2 + y)).astype(bf16)
        out_v[pl.ds(g0, 8), :] = jnp.where(sel, new, out_v[pl.ds(g0, 8), :])
        fix = out_copy(g0, 8)
        fix.start()
        fix.wait()


@jax.jit
def pallas_adaLN_cond__sliding_block_cached__moe_arch_mod__prompt_kernel(
    A_x, A_k_cache, A_v_cache, A_wq, A_wo, B_x, B_w_r, B_w_gate, B_w_up, B_w_down, c, w_mod,
):
    del B_x
    any_spec = pl.BlockSpec(memory_space=pl.ANY)
    return pl.pallas_call(
        _kernel,
        out_shape=jax.ShapeDtypeStruct(A_x.shape, A_x.dtype),
        in_specs=[any_spec] * 11,
        out_specs=any_spec,
        scratch_shapes=[
            pltpu.VMEM((S, D), bf16),
            pltpu.VMEM((S, D), bf16),
            pltpu.VMEM((S, D), bf16),
            pltpu.VMEM((S // 2, 5 * KH), bf16),
            pltpu.VMEM((S, GW), bf16),
            pltpu.VMEM((S // 2, 7 * KH), f32),
            pltpu.VMEM((NKC, D, 512 + PADW), bf16),
            pltpu.VMEM((NMC, D, NM * 128), bf16),
            pltpu.VMEM((HKV, D, GW + PADW), bf16),
            pltpu.VMEM((HKV, KH, 5 * KH), bf16),
            pltpu.VMEM((HKV, GW, D), bf16),
            pltpu.VMEM((HKV, KH, 5 * KH), bf16),
            pltpu.VMEM((D, F), bf16),
            pltpu.VMEM((D, F), bf16),
            pltpu.VMEM((F, D + PADD), bf16),
            pltpu.VMEM((HKV, W, DH), bf16),
            pltpu.VMEM((HKV, W, DH), bf16),
            pltpu.VMEM((HKV, DH, W), bf16),
            pltpu.VMEM((8, 1, D), bf16),
            pltpu.VMEM((16, 8, 128), bf16),
            pltpu.VMEM((16, D), bf16),
            pltpu.VMEM((D, 128), f32),
            pltpu.VMEM((2 * D, 128), f32),
            pltpu.VMEM((8, 6 * D), f32),
            pltpu.VMEM((8, 8, 128), f32),
            pltpu.VMEM((8, 8, 128), jnp.int32),
            pltpu.VMEM((4, 8, D), f32),
            pltpu.SMEM((1,), jnp.int32),
            pltpu.SemaphoreType.DMA((NSEM,)),
        ],
        compiler_params=pltpu.CompilerParams(vmem_limit_bytes=124 * 1024 * 1024,
                                             disable_semaphore_checks=bool(_p('NOSEM', 1)),
                                             disable_bounds_checks=bool(_p('NOBND', 0))),
    )(A_x, A_k_cache, A_v_cache, A_wq, A_wo, B_w_r.reshape(8, 128), B_w_gate, B_w_up, B_w_down, c, w_mod)
```

```python
import contextlib
import math
import os

import jax
import jax.numpy as jnp
from jax import lax
from jax.experimental import pallas as pl
from jax.experimental.pallas import tpu as pltpu


def _p(name, default):
    v = os.environ.get('KP_' + name)
    return default if v is None else type(default)(v)


S = 2048
D = 1024
HQ = 32
HKV = 4
REP = HQ // HKV
DH = 128
GW = REP * DH
W = 512
F = 3584
EPS = 1e-5
TQ = 256
HR = TQ // 2
KH = D // 2
NT = S // TQ
TP = 512
NKC = 4
PADW = 128
PADD = 256
NM = 3
NMC = 11
UNB = 2
UNC = 2
FD = _p('FD', 15)
FI0 = _p('FI0', 8)
FLAG_ = _p('FLAG', 4)
FVR = _p('FVR', 32)
LAG0 = _p('LAG0', 2)
T3B = 4
LCNT = [int(c_) for c_ in _p('LCNT', '00565655')]
LPE = _p('LPE', 'V0,V32,V64,V96,V128,V160').split(',')
LPO = _p('LPO', 'V0,V56,V112,V168,V224,N24').split(',')
HIROW = _p('HIROW', 0)
OORD = [int(c_) for c_ in _p('OORD', '3651274')]
SKIPL = _p('SKIPL', 1)
BSEQ = [int(c_) for c_ in _p('BSEQ', '33')]
P3S = _p('P3S', 6)
P3LAG = _p('P3LAG', 5)
KUPIN = _p('KUPIN', 1)
CSEQ = [int(c_) for c_ in _p('CSEQ', '1213')]
NPIN = _p('NPIN', 'N64')
WQPIN = _p('WQPIN', 'V128')
WOPIN = _p('WOPIN', 'O0')
SCOPES = _p('SCOPES', 0)
QSCALE = (DH ** -0.5) * math.log2(math.e)

f32 = jnp.float32
bf16 = jnp.bfloat16

(SEM_C, SEM_WR, SEM_X0, SEM_K0, SEM_K, SEM_V, SEM_WG, SEM_WU, SEM_WD, SEM_OUT) = range(10)
SEM_X = 10
SEM_W = SEM_X + NT
SEM_WQ0 = SEM_W + 6
SEM_WM = SEM_WQ0 + NKC
SEM_WMR = SEM_WM + NKC
NSEM = SEM_WMR + 2

ORDER7 = (4, 2, 1, 7, 5, 3, 6)
A_SLOT = {1: 0, 2: 1, 5: 2, 6: 3, 7: 4}
B_SLOT = {1: 0, 3: 1, 4: 2, 6: 3, 7: 4}


def _a_op(i, a11, a12, a21, a22):
    return {1: lambda: a11 + a22, 2: lambda: a21 + a22, 3: lambda: a11, 4: lambda: a22,
            5: lambda: a11 + a12, 6: lambda: a21 - a11, 7: lambda: a12 - a22}[i]()


def _a_sums(a11, a12, a21, a22):
    return [_a_op(i, a11, a12, a21, a22) for i in (1, 2, 5, 6, 7)]


def _b_sums(b11, b12, b21, b22):
    return [b11 + b22, b12 - b22, b21 - b11, b11 + b12, b21 + b22]


class _Combine:
    def __init__(self):
        self.m = {}

    def feed(self, i, v):
        m = self.m
        if i == 4:
            m['c11'] = v
            return []
        if i == 2:
            m['c22'] = v
            return [(1, 0, v + m['c11'])]
        if i == 1:
            m['c11'] = m['c11'] + v
            m['c22'] = v - m['c22']
            return []
        if i == 7:
            m['c11'] = m['c11'] + v
            return []
        if i == 5:
            m['c12'] = v
            return [(0, 0, m['c11'] - v)]
        if i == 3:
            m['c22'] = m['c22'] + v
            return [(0, 1, m['c12'] + v)]
        return [(1, 1, m['c22'] + v)]


def _scope(name):
    return jax.named_scope(name) if SCOPES else contextlib.nullcontext()


def _ln(x):
    m = jnp.mean(x, axis=-1, keepdims=True)
    xc = x - m
    v = jnp.mean(xc * xc, axis=-1, keepdims=True)
    return xc * lax.rsqrt(v + EPS)


def _recip(l):
    r = pl.reciprocal(l, approx=True)
    return r * (2.0 - l * r)


def _mo(x, m):
    return x if isinstance(x, int) else pl.multiple_of(x, m)


def _rows(v8, n):
    return v8 if n == 8 else jnp.concatenate([v8] * (n // 8), axis=0)


def _gate(x, flag, tok):
    xs = jnp.where(flag, _rows(tok, x.shape[0]), x[:, 0:128])
    return jnp.concatenate([xs, x[:, 128:]], axis=1)


def _gate1(x, flag, tok, row=0):
    if row:
        return jnp.concatenate([x[:row], _gate1(x[row:], flag, tok)], axis=0)
    r = tok.shape[0]
    x0 = jnp.where(flag, tok, x[0:r, 0:128])
    if x.shape[1] > 128:
        x0 = jnp.concatenate([x0, x[0:r, 128:]], axis=1)
    return x0 if x.shape[0] == r else jnp.concatenate([x0, x[r:]], axis=0)


def _token(*ys):
    u = None
    for y in ys:
        for i in range(y.shape[0] // 8):
            for j in range(y.shape[1] // 128):
                v = y[8 * i:8 * i + 8, 128 * j:128 * j + 128]
                u = v if u is None else jnp.maximum(u, v)
    return u


def _kernel(x_hbm, k_hbm, v_hbm, wq_hbm, wo_hbm, wr_hbm, wg_hbm, wu_hbm, wd_hbm, c_hbm, wmod_hbm,
            out_hbm,
            x_v, out_v, h_v, hs_v, q_v, acc_v, wm_v, wmr_v, wq_v, wqs0_v, wqs_v, wo_v, wos_v, wg_v, wu_v, wd_v,
            k_v, v_v, kt_v, c_v8, wr_v8, sc_v, scc_v, acol_v, mod_v, best_v, bidx_v, aux_v, flag_s, sems):
    sk = k_hbm.shape[2]
    c_v = c_v8.at[0]
    wr_v = wr_v8.at[0]

    def cp(src, dst, i):
        return pltpu.make_async_copy(src, dst, sems.at[i])

    def wait_all(view, sem):
        cp(view, view, sem).wait()

    c_cp = cp(c_hbm, c_v, SEM_C)
    wr_cp = cp(wr_hbm, wr_v, SEM_WR)
    x0_cp = cp(x_hbm.at[0, pl.ds(0, TP), :], x_v.at[pl.ds(0, TP), :], SEM_X0)
    k0_cp = cp(k_hbm.at[0, 0, pl.ds(sk - W, W), :], k_v.at[0], SEM_K0)
    k_cp = cp(k_hbm.at[0, pl.ds(1, HKV - 1), pl.ds(sk - W, W), :], k_v.at[pl.ds(1, HKV - 1)], SEM_K)
    v_cp = cp(v_hbm.at[0, :, pl.ds(sk - W, W), :], v_v, SEM_V)
    wg_cp = cp(wg_hbm, wg_v, SEM_WG)
    wu_cp = cp(wu_hbm, wu_v, SEM_WU)
    wd_cp = cp(wd_hbm, wd_v.at[:, pl.ds(0, D)], SEM_WD)

    def x_cp(t):
        r0 = _mo(t * TQ, TQ)
        return cp(x_hbm.at[0, pl.ds(r0, TQ), :], x_v.at[pl.ds(r0, TQ), :], SEM_X + t)

    def wm_cps(j):
        return [cp(wmod_hbm.at[:, pl.ds(i * KH + j * 128, 128)], wm_v.at[j, :, pl.ds(i * 128, 128)], SEM_WM + j)
                for i in range(4)]

    def wmr_cp(i):
        c0 = 2 * D + min(i * NM, 32 - NM) * 128
        return cp(wmod_hbm.at[:, pl.ds(c0, NM * 128)], wmr_v.at[i], SEM_WMR + (0 if i < 2 else 1))

    def wq_cps(g, c, n, sem):
        rows = [(0, D)] if n == 4 else [(_mo(i * KH + c * 128, 128), n * 128) for i in range(2)]
        return [cp(wq_hbm.at[pl.ds(r0, nr), pl.ds(g * GW, GW)], wq_v.at[g, pl.ds(r0, nr), pl.ds(0, GW)], sem)
                for r0, nr in rows]

    def wo_cp(c, n, sem):
        r0 = _mo(c * 256, 256)
        return cp(wo_hbm.at[pl.ds(r0, n * 256), :], wo_v.at[pl.ds(r0, n * 256), :], sem)

    def w0_cps(c):
        return wq_cps(1, c, 1, SEM_W + c) + [wo_cp(c, 1, SEM_W + c)]

    w1a_cps = wq_cps(2, 0, 2, SEM_W + 4) + [wo_cp(4, 2, SEM_W + 4)]
    wrest_cps = wq_cps(2, 2, 2, SEM_W + 5) + wq_cps(3, 0, 4, SEM_W + 5) + [wo_cp(6, 10, SEM_W + 5)]

    def out_copy(r0, n):
        return cp(out_v.at[pl.ds(r0, n), :], out_hbm.at[0, pl.ds(r0, n), :], SEM_OUT)

    for c_ in ([c_cp, x0_cp] + [c_ for j in range(NKC) for c_ in wm_cps(j) + wq_cps(0, j, 1, SEM_WQ0 + j)]
               + [x_cp(2), k0_cp, x_cp(3), x_cp(4), k_cp, x_cp(5), wr_cp] + w0_cps(0)
               + [x_cp(6)] + w0_cps(1) + [x_cp(7)] + w0_cps(2) + w0_cps(3) + [v_cp, wmr_cp(0), wmr_cp(1)] + w1a_cps
               + [wmr_cp(i) for i in range(2, NMC)] + wrest_cps + [wg_cp, wu_cp, wd_cp]):
        c_.start()

    def ln1_pair(t, r, n, lo=None):
        ys = []
        for half in range(2):
            r0 = _mo(t * TQ + half * HR + r, 8)
            x = x_v[pl.ds(r0, n), :].astype(f32)
            if lo is not None:
                x = _gate(x, *lo)
            y = _ln(x) * _rows(mod_v[:, D:2 * D], n) + _rows(mod_v[:, 0:D], n)
            h_v[pl.ds(r0, n), :] = y.astype(bf16)
            ys.append(y)
        sums = jnp.concatenate(_a_sums(ys[0][:, :KH], ys[0][:, KH:], ys[1][:, :KH], ys[1][:, KH:]), axis=1)
        hs_v[pl.ds(_mo(t * HR + r, 8), n), :] = sums.astype(bf16)
        return sums

    def wqs_ref(g):
        return wqs0_v if isinstance(g, int) and g == 0 else wqs_v.at[g - 1]

    def wq_unit(g, u, lo):
        r0 = _mo(u * 8, 8)
        top = _gate(wq_v[g, pl.ds(r0, 8), 0:GW].astype(f32), *lo)
        bot = wq_v[g, pl.ds(KH + r0, 8), 0:GW].astype(f32)
        outs = []
        for p in range(REP // 2):
            c0, c1, c2 = 2 * p * DH, (2 * p + 1) * DH, (2 * p + 2) * DH
            outs += _b_sums(top[:, c0:c1], top[:, c1:c2], bot[:, c0:c1], bot[:, c1:c2])
        sums = jnp.concatenate(outs, axis=1)
        wqs_ref(g)[pl.ds(r0, 8), :] = sums.astype(bf16)
        return sums

    def wo_unit(g, u, lo):
        r0 = _mo(g * GW + (u // 16) * 2 * DH + (u % 16) * 8, 8)
        top = _gate(wo_v[pl.ds(r0, 8), :].astype(f32), *lo)
        bot = wo_v[pl.ds(DH + r0, 8), :].astype(f32)
        sums = jnp.concatenate(_b_sums(top[:, :KH], top[:, KH:], bot[:, :KH], bot[:, KH:]), axis=1)
        wos_v[g, pl.ds(_mo(u * 8, 8), 8), :] = sums.astype(bf16)
        return sums

    def ln2_rows(r0, n, valid=None, lo=None):
        av = _rows(aux_v[0], n)
        bv = _rows(aux_v[1], n)
        rv = _rows(aux_v[2], n)
        r_c = _rows(aux_v[3, :, 0:128], n)
        x2 = x_v[pl.ds(r0, n), :].astype(f32)
        if lo is not None:
            x2 = _gate(x2, *lo)
        m = jnp.mean(x2, axis=-1, keepdims=True)
        xc = x2 - m
        var = jnp.mean(xc * xc, axis=-1, keepdims=True)
        rs = lax.rsqrt(var + EPS)
        y = x2 + ((xc * rs) * av + bv)
        out_v[pl.ds(r0, n), :] = y.astype(bf16)
        r = jnp.sum(xc * rv, axis=-1, keepdims=True) * rs
        r = (jnp.broadcast_to(r, (n, 128)) + r_c).astype(bf16).astype(f32)
        if valid is not None:
            r = jnp.where(valid, r, -jnp.inf)
        mb = jnp.broadcast_to(m, (n, 128))
        rsb = jnp.broadcast_to(rs, (n, 128))
        best = best_v[0]
        bm = best_v[1]
        brs = best_v[2]
        bidx = bidx_v[0]
        rows = lax.broadcasted_iota(jnp.int32, (8, 128), 0)
        for j in range(n // 8):
            sl = slice(8 * j, 8 * (j + 1))
            upd = r[sl] > best
            best = jnp.where(upd, r[sl], best)
            bm = jnp.where(upd, mb[sl], bm)
            brs = jnp.where(upd, rsb[sl], brs)
            bidx = jnp.where(upd, rows + (r0 + 8 * j), bidx)
        best_v[0] = best
        best_v[1] = bm
        best_v[2] = brs
        bidx_v[0] = bidx
        return y, best

    def q_rhs(g, p, k):
        if k in B_SLOT:
            c0 = (p * 5 + B_SLOT[k]) * DH
            return wqs_ref(g)[:, c0:c0 + DH]
        if k == 2:
            return wq_v[g, 0:KH, 2 * p * DH:(2 * p + 1) * DH]
        return wq_v[g, KH:D, (2 * p + 1) * DH:(2 * p + 2) * DH]

    def q_store(a0, p, blocks):
        for rh, ch, v in blocks:
            r0 = pl.multiple_of(a0 + rh * HR, HR)
            q_v[pl.ds(r0, HR), (2 * p + ch) * DH:(2 * p + ch + 1) * DH] = (v * QSCALE).astype(bf16)

    with _scope('P0_wait'):
        flag_s[0] = 0
        c_cp.wait()
        cf = c_v[...].astype(f32)
        sc = (cf * jax.nn.sigmoid(cf)).astype(bf16)
        sc_v[...] = jnp.broadcast_to(sc, (16, D))
        scc_v[...] = jnp.broadcast_to(sc.astype(f32), (128, D)).T
        best_v[0] = jnp.full((8, 128), -jnp.inf, f32)
        best_v[1] = jnp.zeros((8, 128), f32)
        best_v[2] = jnp.zeros((8, 128), f32)
        bidx_v[0] = jnp.zeros((8, 128), jnp.int32)
        x0_cp.wait()

        def norm_rows(i, carry):
            r0 = pl.multiple_of(i * 128, 128)
            acc_v[pl.ds(r0, 128), 0:D] = _ln(x_v[pl.ds(r0, 128), :].astype(f32))
            return carry

        lax.fori_loop(0, TP // 128, norm_rows, 0)

    def k_chunk(j, carry):
        wait_all(wm_v.at[j, :, pl.ds(0, 512)], SEM_WM + j)
        clo = pl.multiple_of(j * 128, 128)
        chi = pl.multiple_of(KH + j * 128, 128)
        md = jnp.dot(sc_v[...], wm_v[j, :, 0:512], preferred_element_type=f32)[0:8].astype(bf16).astype(f32)
        hh = []
        for i, c0 in enumerate((clo, chi)):
            sa = md[:, i * 128:(i + 1) * 128]
            ca1 = 1.0 + md[:, (2 + i) * 128:(3 + i) * 128]
            mod_v[:, pl.ds(c0, 128)] = sa
            mod_v[:, pl.ds(D + c0, 128)] = ca1
            y = acc_v[0:TP, pl.ds(c0, 128)] * _rows(ca1, TP) + _rows(sa, TP)
            h_v[0:TP, pl.ds(c0, 128)] = y.astype(bf16)
            hh.append(y)
        for t in range(TP // TQ):
            top = slice(t * TQ, t * TQ + HR)
            bot = slice(t * TQ + HR, (t + 1) * TQ)
            for i, s_ in enumerate(_a_sums(hh[0][top], hh[1][top], hh[0][bot], hh[1][bot])):
                hs_v[t * HR:(t + 1) * HR, pl.ds(i * KH + clo, 128)] = s_.astype(bf16)
        for c_ in wq_cps(0, j, 1, SEM_WQ0 + j):
            c_.wait()
        lhs = jnp.concatenate([h_v[0:TP, pl.ds(clo, 128)], h_v[0:TP, pl.ds(chi, 128)]], axis=1)
        rhs = jnp.concatenate([wq_v[0, pl.ds(clo, 128), 0:GW], wq_v[0, pl.ds(chi, 128), 0:GW]], axis=0)
        flag = flag_s[0] > 0
        toks = {}
        for n_ in range(4):
            cs = slice(n_ * 256, (n_ + 1) * 256)
            lh = lhs
            if n_ - 2 in toks:
                tk = toks[n_ - 2]
                lh = _gate1(lhs, flag, jnp.concatenate([tk, tk], axis=0).astype(bf16))
            part = jnp.dot(lh, rhs[:, cs], preferred_element_type=f32)
            tot = jnp.where(j == 0, 0.0, acc_v[0:TP, D + n_ * 256:D + (n_ + 1) * 256]) + part
            acc_v[0:TP, D + n_ * 256:D + (n_ + 1) * 256] = tot
            q_v[0:TP, cs] = (tot * QSCALE).astype(bf16)
            if n_ < 2:
                toks[n_] = _token(*[wq_unit(0, j * 16 + n_ * 8 + u, (flag, part[64 * u:64 * u + 8, 0:128]))
                                    for u in range(8)])
        return carry

    with _scope('P1_kchunks'):
        lax.fori_loop(0, NKC, k_chunk, 0)

    with _scope('P2_ln'):
        x_cp(2).wait()
        ln1_pair(2, 0, HR)
        k0_cp.wait()

    def q0_tile(t, units):
        flag = flag_s[0] > 0
        a0 = pl.multiple_of(t * TQ, TQ)
        m0 = pl.multiple_of(t * HR, HR)
        tn = jnp.minimum(t + 1, NT - 1)
        lhs = {k: hs_v[pl.ds(m0, HR), s_ * KH:(s_ + 1) * KH] for k, s_ in A_SLOT.items()}
        lhs[3] = h_v[pl.ds(a0, HR), 0:KH]
        lhs[4] = h_v[pl.ds(pl.multiple_of(a0 + HR, HR), HR), KH:D]
        jobs = [(lambda lo, r=r: ln1_pair(tn, r, 8, lo)) for r in range(0, HR, 8)]
        mixed = []
        for i, jb in enumerate(jobs):
            mixed.append(jb)
            mixed += units[i * len(units) // len(jobs):(i + 1) * len(units) // len(jobs)]
        nprod = 7 * REP // 2
        nslot = nprod - P3S - P3LAG
        toks = {}
        n_ = 0
        for p in range(REP // 2):
            comb = _Combine()
            for k in ORDER7:
                lh = lhs[k]
                if n_ - P3LAG in toks:
                    tk = toks[n_ - P3LAG]
                    lh = _gate1(lh, flag, jnp.concatenate([tk, tk], axis=0).astype(bf16))
                y = jnp.dot(lh, q_rhs(0, p, k), preferred_element_type=f32)
                q_store(a0, p, comb.feed(k, y))
                sl = n_ - P3S
                if 0 <= sl < nslot:
                    mine = mixed[sl * len(mixed) // nslot:(sl + 1) * len(mixed) // nslot]
                    outs = []
                    for k_, jb in enumerate(mine):
                        r_ = (k_ * HR // len(mine)) // 8 * 8
                        outs.append(jb((flag, y[r_:r_ + 8])))
                    if outs:
                        toks[n_] = _token(*outs)
                n_ += 1

    def q0_a(t, carry):
        x_cp(t + 1).wait()

        @pl.when(t == 3)
        def _():
            k_cp.wait()

        q0_tile(t, [])
        gk = jnp.minimum(t - 2, HKV - 1)
        kt_v[gk] = k_v[gk].T
        return carry

    def q0_b(t, carry):
        @pl.when(t + 1 < NT)
        def _():
            x_cp(t + 1).wait()

        for c_ in w0_cps(t - T3B):
            c_.wait()
        nu = 16
        u0 = (t - T3B) * nu
        units = []
        for u in range(nu):
            units.append(lambda lo, u=u: wq_unit(1, u0 + u, lo))
            units.append(lambda lo, u=u: wo_unit(0, u0 + u, lo))
        q0_tile(t, units)
        gk = jnp.minimum(t - 2, HKV - 1)
        kt_v[gk] = k_v[gk].T
        return carry

    with _scope('P3_q0'):
        lax.fori_loop(2, T3B, q0_a, 0)
        lax.fori_loop(T3B, NT, q0_b, 0)
        v_cp.wait()
        wr_cp.wait()
        wait_all(wmr_v.at[pl.ds(0, 2)], SEM_WMR)
        for c_ in w1a_cps:
            c_.wait()

    def body(i, un, last_group):
        flag = flag_s[0] > 0
        st = dict(hi=None, pend=[])
        g = 3 if last_group else (i * un) // NT

        def pin(name):
            r_ = int(name[1:])
            return flag, st[name[0]][r_:r_ + 8, 0:128]

        def add_hi(tk):
            st['hi'] = tk if st['hi'] is None else jnp.maximum(st['hi'], tk)

        def o_run(n):
            for k_ in range(min(n, len(st['pend']))):
                y = st['pend'].pop(0)()
                if k_ == 0:
                    st['N'] = y
                st['O'] = y

        for u_ in range(un):
            t = (i * un + u_) % NT
            a0 = pl.multiple_of(t * TQ, TQ)
            m0 = pl.multiple_of(t * HR, HR)

            def qk(hh, a0=a0):
                qh = q_v[pl.ds(a0, TQ), hh * DH:(hh + 1) * DH]
                s = jnp.dot(qh, kt_v[g], preferred_element_type=f32)
                if st['hi'] is not None:
                    s = _gate1(s, flag, st['hi'], HIROW if last_group else 0)
                    st['hi'] = None
                m = jnp.max(s, axis=-1, keepdims=True)
                p = jnp.exp2(s - m)
                l = jnp.sum(p, axis=-1, keepdims=True)
                return p.astype(bf16), l

            def pv(pl_):
                p, l = pl_
                o = jnp.dot(p, v_v[g], preferred_element_type=f32)
                st['V'] = o
                return o * _recip(l)

            def q_prod(p, k, comb, a0=a0, m0=m0):
                if k in A_SLOT:
                    lhs = hs_v[pl.ds(m0, HR), A_SLOT[k] * KH:(A_SLOT[k] + 1) * KH]
                elif k == 3:
                    lhs = h_v[pl.ds(a0, HR), 0:KH]
                else:
                    lhs = h_v[pl.ds(pl.multiple_of(a0 + HR, HR), HR), KH:D]
                y = jnp.dot(lhs, q_rhs(g + 1, p, k), preferred_element_type=f32)
                st['Q'] = y
                q_store(a0, p, comb.feed(k, y))

            def o_prod(p, k, o0, o1, comb, a0=a0, m0=m0):
                lhs = _a_op(k, o0[:HR], o1[:HR], o0[HR:], o1[HR:]).astype(bf16)
                if k in B_SLOT:
                    rhs = wos_v[g, p * DH:(p + 1) * DH, B_SLOT[k] * KH:(B_SLOT[k] + 1) * KH]
                elif k == 2:
                    rhs = wo_v[pl.ds(_mo(g * GW + 2 * p * DH, DH), DH), 0:KH]
                else:
                    rhs = wo_v[pl.ds(_mo(g * GW + (2 * p + 1) * DH, DH), DH), KH:D]
                y = jnp.dot(lhs, rhs, preferred_element_type=f32)
                cs = slice((k - 1) * KH, k * KH)
                old = acc_v[pl.ds(m0, HR), cs]
                if p == 0 and not last_group:
                    acc_v[pl.ds(m0, HR), cs] = jnp.where(g == 0, 0.0, old) + y
                elif p == REP // 2 - 1 and last_group:
                    for rh, ch, v in comb.feed(k, old + y):
                        r0 = pl.multiple_of(a0 + rh * HR, HR)
                        cx = slice(ch * KH, (ch + 1) * KH)
                        ga = _rows(mod_v[:, 2 * D + ch * KH:2 * D + (ch + 1) * KH], HR)
                        x_v[pl.ds(r0, HR), cx] = (x_v[pl.ds(r0, HR), cx].astype(f32) + ga * v).astype(bf16)
                else:
                    acc_v[pl.ds(m0, HR), cs] = old + y
                return y

            def side_b(hh):
                pos = u_ * REP + hh
                nst = un * REP - 2 - SKIPL
                if pos < 2 or pos - 2 >= nst:
                    return
                k_ = pos - 2
                ci = jnp.minimum(i, NMC - 1)
                acc = st.get('macc')
                lo = pin(NPIN)
                for rg in range(128 * k_ // nst, 128 * (k_ + 1) // nst):
                    xc_ = scc_v[8 * rg:8 * rg + 8, :]
                    if rg == 128 * k_ // nst:
                        xc_ = jnp.where(lo[0], lo[1], xc_)
                    pr_ = wmr_v[ci, 8 * rg:8 * rg + 8, :].astype(f32) * jnp.concatenate([xc_] * NM, axis=1)
                    acc = pr_ if acc is None else acc + pr_
                st['macc'] = acc
                add_hi(_token(acc))
                if k_ == nst - 1:
                    c0 = pl.multiple_of(2 * D + jnp.minimum(ci * NM, 32 - NM) * 128, 128)
                    tot_ = jnp.sum(acc, axis=0, keepdims=True).astype(bf16).astype(f32)
                    mod_v[:, pl.ds(c0, NM * 128)] = jnp.broadcast_to(tot_, (8, NM * 128))
                nu = 64 * un // NT
                u0 = (i % (NT // un)) * nu
                for u in range(nu * k_ // nst, nu * (k_ + 1) // nst):
                    add_hi(_token(wq_unit(jnp.minimum(g + 2, HKV - 1), u0 + u, pin(WQPIN))))
                    add_hi(_token(wo_unit(g + 1, u0 + u, pin(WOPIN))))

            def side_c(hh, t=t):
                tl = jnp.maximum(t - 1, 0)
                for k_ in range(LCNT[hh]):
                    off = (sum(LCNT[:hh]) + k_) * 8
                    y, b = ln2_rows(pl.multiple_of(tl * TQ + off, 8), 8, t > 0, pin((LPE, LPO)[hh % 2][k_]))
                    add_hi(_token(y, b))

            for p in range(REP // 2):
                h0, h1 = 2 * p, 2 * p + 1
                if not last_group:
                    cq = _Combine()
                    sp = qk(h0)
                    for k in ORDER7[:BSEQ[0]]:
                        q_prod(p, k, cq)
                    o0 = pv(sp)
                    o_run(BSEQ[1])
                    side_b(h0)
                    sp = qk(h1)
                    for k in ORDER7[BSEQ[0]:]:
                        q_prod(p, k, cq)
                    o1 = pv(sp)
                    o_run(7)
                    side_b(h1)
                elif not st['pend']:
                    sp0 = qk(h0)
                    sp1 = qk(h1)
                    o0 = pv(sp0)
                    o1 = pv(sp1)
                else:
                    sp = qk(h0)
                    o_run(CSEQ[0])
                    st['F'] = st['O']
                    o0 = pv(sp)
                    o_run(CSEQ[1])
                    side_c(h0)
                    sp = qk(h1)
                    o_run(CSEQ[2])
                    st['F'] = st['O']
                    o1 = pv(sp)
                    o_run(CSEQ[3])
                    side_c(h1)
                co = _Combine()
                st['pend'] = [(lambda k=k, p=p, o0=o0, o1=o1, co=co, f=o_prod: f(p, k, o0, o1, co))
                              for k in (ORDER7 if last_group and p == REP // 2 - 1 else OORD)]
        o_run(7)
        if last_group:
            for u_ in range(un):
                t = (i * un + u_) % NT

                @pl.when(t > 0)
                def _():
                    out_copy(pl.multiple_of((t - 1) * TQ, TQ), TQ).start()

    def body_b(i, carry):
        @pl.when(i == 2)
        def _():
            wait_all(wmr_v.at[pl.ds(2, NMC - 2)], SEM_WMR + 1)
            for c_ in wrest_cps:
                c_.wait()

        body(i, UNB, False)
        return carry

    with _scope('LB'):
        lax.fori_loop(0, 3 * NT // UNB, body_b, 0)

    wg_cp.wait()
    wu_cp.wait()
    wd_cp.wait()
    sb_ = mod_v[:, 3 * D:4 * D]
    cb1_ = 1.0 + mod_v[:, 4 * D:5 * D]
    gb_ = mod_v[:, 5 * D:6 * D]
    wr8 = wr_v[...].astype(f32)
    wr_ = jnp.concatenate([wr8[r_:r_ + 1, :] for r_ in range(8)], axis=1)
    aux_v[0] = gb_ * cb1_
    aux_v[1] = gb_ * sb_
    aux_v[2] = cb1_ * wr_
    aux_v[3] = jnp.broadcast_to(jnp.sum(sb_ * wr_, axis=-1, keepdims=True), (8, D))

    def body_c(i, carry):
        body(i, UNC, True)
        return carry

    with _scope('LC'):
        lax.fori_loop(0, NT // UNC, body_c, 0)

    with _scope('E1_last'):
        ln2_rows((NT - 1) * TQ, TQ)
        out_copy((NT - 1) * TQ, TQ).start()

    with _scope('E2_ffn'):
        best = best_v[0]
        bidx = bidx_v[0]
        rmax = jnp.max(best, axis=0, keepdims=True)
        idx_v = jnp.min(jnp.where(best == rmax, bidx, S), axis=0, keepdims=True)
        idx = jnp.minimum(idx_v[0, 0], S - 1)
        g0 = pl.multiple_of((idx // 8) * 8, 8)
        sb = mod_v[:, 3 * D:4 * D]
        cb = mod_v[:, 4 * D:5 * D]
        gb = mod_v[:, 5 * D:6 * D]
        x2 = x_v[pl.ds(g0, 8), :].astype(f32)
        h2 = (x2 - best_v[1][:, 0:1]) * best_v[2][:, 0:1] * (1.0 + cb) + sb
        h2b = h2.astype(bf16)
        sel = (lax.broadcasted_iota(jnp.int32, (8, 1), 0) + g0) == idx
        flag = flag_s[0] > 0
        nf = F // 128
        strips = [(k_, j) for j in range(nf) for k_ in 'gu'] + [('d', j) for j in range(FD, nf)]
        gate_r, a_strips, vtok = {}, {}, {}
        y = None
        yv = None
        pos = 0
        for i, (kind, j) in enumerate(strips):
            hi = vtok.get(i - FLAG_)
            if kind == 'd':
                lhs = a_strips[j]
                if hi is not None:
                    lhs = jnp.where(flag, hi.astype(bf16), lhs)
                r_ = jnp.dot(lhs, wd_v[j * 128:(j + 1) * 128, 0:D], preferred_element_type=f32)
                y = r_ if y is None else y + r_
                tok_ = r_[:, D - 128:D]
            else:
                lhs = h2b if hi is None else _gate1(h2b, flag, hi.astype(bf16))
                w_ref = wg_v if kind == 'g' else wu_v
                tok_ = jnp.dot(lhs, w_ref[:, j * 128:(j + 1) * 128], preferred_element_type=f32)
                if kind == 'g':
                    gate_r[j] = tok_
                else:
                    a_strips[j] = (gate_r[j] * jax.nn.sigmoid(gate_r[j]) * tok_).astype(bf16)
                    if j < FD:
                        row = jnp.sum(jnp.where(sel, a_strips[j].astype(f32), 0.0), axis=0, keepdims=True)
                        acol_v[j * 128:(j + 1) * 128, :] = jnp.broadcast_to(row, (128, 128)).T
            if i >= FI0 and pos < FD * 16:
                end = min(pos + FVR // 8, FD * 16) if i < len(strips) - 1 else FD * 16
                for rg in range(pos, end):
                    col = jnp.where(flag, tok_, acol_v[8 * rg:8 * rg + 8, :])
                    pr_ = wd_v[8 * rg:8 * rg + 8, 0:D].astype(f32) * jnp.concatenate([col] * (D // 128), axis=1)
                    yv = pr_ if yv is None else yv + pr_
                pos = end
                vtok[i] = _token(yv)
        y = (y + jnp.sum(yv, axis=0, keepdims=True)) * jax.nn.sigmoid(rmax[:, 0:1])
        out_copy(0, S).wait()
        new = (x2 + gb * (h2 + y)).astype(bf16)
        out_v[pl.ds(g0, 8), :] = jnp.where(sel, new, out_v[pl.ds(g0, 8), :])
        fix = out_copy(g0, 8)
        fix.start()
        fix.wait()


@jax.jit
def pallas_adaLN_cond__sliding_block_cached__moe_arch_mod__prompt_kernel(
    A_x, A_k_cache, A_v_cache, A_wq, A_wo, B_x, B_w_r, B_w_gate, B_w_up, B_w_down, c, w_mod,
):
    del B_x
    any_spec = pl.BlockSpec(memory_space=pl.ANY)
    return pl.pallas_call(
        _kernel,
        out_shape=jax.ShapeDtypeStruct(A_x.shape, A_x.dtype),
        in_specs=[any_spec] * 11,
        out_specs=any_spec,
        scratch_shapes=[
            pltpu.VMEM((S, D), bf16),
            pltpu.VMEM((S, D), bf16),
            pltpu.VMEM((S, D), bf16),
            pltpu.VMEM((S // 2, 5 * KH), bf16),
            pltpu.VMEM((S, GW), bf16),
            pltpu.VMEM((S // 2, 7 * KH), f32),
            pltpu.VMEM((NKC, D, 512 + PADW), bf16),
            pltpu.VMEM((NMC, D, NM * 128), bf16),
            pltpu.VMEM((HKV, D, GW + PADW), bf16),
            pltpu.VMEM((KH, 5 * KH), bf16),
            pltpu.VMEM((HKV - 1, KH, 5 * KH), bf16),
            pltpu.VMEM((HKV * GW, D), bf16),
            pltpu.VMEM((HKV, KH, 5 * KH), bf16),
            pltpu.VMEM((D, F), bf16),
            pltpu.VMEM((D, F), bf16),
            pltpu.VMEM((F, D + PADD), bf16),
            pltpu.VMEM((HKV, W, DH), bf16),
            pltpu.VMEM((HKV, W, DH), bf16),
            pltpu.VMEM((HKV, DH, W), bf16),
            pltpu.VMEM((8, 1, D), bf16),
            pltpu.VMEM((16, 8, 128), bf16),
            pltpu.VMEM((16, D), bf16),
            pltpu.VMEM((D, 128), f32),
            pltpu.VMEM((2 * D, 128), f32),
            pltpu.VMEM((8, 6 * D), f32),
            pltpu.VMEM((8, 8, 128), f32),
            pltpu.VMEM((8, 8, 128), jnp.int32),
            pltpu.VMEM((4, 8, D), f32),
            pltpu.SMEM((1,), jnp.int32),
            pltpu.SemaphoreType.DMA((NSEM,)),
        ],
        compiler_params=pltpu.CompilerParams(vmem_limit_bytes=124 * 1024 * 1024,
                                             disable_semaphore_checks=bool(_p('NOSEM', 1)),
                                             disable_bounds_checks=bool(_p('NOBND', 0))),
    )(A_x, A_k_cache, A_v_cache, A_wq, A_wo, B_w_r.reshape(8, 128), B_w_gate, B_w_up, B_w_down, c, w_mod)
```

```python
import contextlib
import math
import os

import jax
import jax.numpy as jnp
from jax import lax
from jax.experimental import pallas as pl
from jax.experimental.pallas import tpu as pltpu


def _p(name, default):
    v = os.environ.get('KP_' + name)
    return default if v is None else type(default)(v)


S = 2048
D = 1024
HQ = 32
HKV = 4
REP = HQ // HKV
DH = 128
GW = REP * DH
W = 512
F = 3584
EPS = 1e-5
TQ = 256
HR = TQ // 2
KH = D // 2
NT = S // TQ
TP = 512
NKC = 4
PADW = 128
PADD = 256
NM = 3
NMC = 11
UNB = 2
UNC = 2
FD = _p('FD', 15)
FI0 = _p('FI0', 8)
FLAG_ = _p('FLAG', 4)
FVR = _p('FVR', 32)
LAG0 = _p('LAG0', 2)
T3B = 4
LCNT = [int(c_) for c_ in _p('LCNT', '00565655')]
LPE = _p('LPE', 'V0,V32,V64,V96,V128,V160').split(',')
LPO = _p('LPO', 'V0,V56,V112,V168,V224,N24').split(',')
HIROW = _p('HIROW', 0)
OORD = [int(c_) for c_ in _p('OORD', '3651274')]
SKIPL = _p('SKIPL', 1)
BSEQ = [int(c_) for c_ in _p('BSEQ', '33')]
P3S = _p('P3S', 7)
P3LAG = _p('P3LAG', 5)
LTOK = _p('LTOK', 1)
P3US = _p('P3US', 0)
P3ULAG = _p('P3ULAG', 3)
P3UR = _p('P3UR', 56)
CSEQ = [int(c_) for c_ in _p('CSEQ', '1213')]
NPIN = _p('NPIN', 'N64')
WQPIN = _p('WQPIN', 'V128')
WOPIN = _p('WOPIN', 'O0')
SCOPES = _p('SCOPES', 0)
QSCALE = (DH ** -0.5) * math.log2(math.e)

f32 = jnp.float32
bf16 = jnp.bfloat16

(SEM_C, SEM_WR, SEM_X0, SEM_K0, SEM_K, SEM_V, SEM_WG, SEM_WU, SEM_WD, SEM_OUT) = range(10)
SEM_X = 10
SEM_W = SEM_X + NT
SEM_WQ0 = SEM_W + 6
SEM_WM = SEM_WQ0 + NKC
SEM_WMR = SEM_WM + NKC
NSEM = SEM_WMR + 2

ORDER7 = (4, 2, 1, 7, 5, 3, 6)
A_SLOT = {1: 0, 2: 1, 5: 2, 6: 3, 7: 4}
B_SLOT = {1: 0, 3: 1, 4: 2, 6: 3, 7: 4}


def _a_op(i, a11, a12, a21, a22):
    return {1: lambda: a11 + a22, 2: lambda: a21 + a22, 3: lambda: a11, 4: lambda: a22,
            5: lambda: a11 + a12, 6: lambda: a21 - a11, 7: lambda: a12 - a22}[i]()


def _a_sums(a11, a12, a21, a22):
    return [_a_op(i, a11, a12, a21, a22) for i in (1, 2, 5, 6, 7)]


def _b_sums(b11, b12, b21, b22):
    return [b11 + b22, b12 - b22, b21 - b11, b11 + b12, b21 + b22]


class _Combine:
    def __init__(self):
        self.m = {}

    def feed(self, i, v):
        m = self.m
        if i == 4:
            m['c11'] = v
            return []
        if i == 2:
            m['c22'] = v
            return [(1, 0, v + m['c11'])]
        if i == 1:
            m['c11'] = m['c11'] + v
            m['c22'] = v - m['c22']
            return []
        if i == 7:
            m['c11'] = m['c11'] + v
            return []
        if i == 5:
            m['c12'] = v
            return [(0, 0, m['c11'] - v)]
        if i == 3:
            m['c22'] = m['c22'] + v
            return [(0, 1, m['c12'] + v)]
        return [(1, 1, m['c22'] + v)]


def _scope(name):
    return jax.named_scope(name) if SCOPES else contextlib.nullcontext()


def _ln(x):
    m = jnp.mean(x, axis=-1, keepdims=True)
    xc = x - m
    v = jnp.mean(xc * xc, axis=-1, keepdims=True)
    return xc * lax.rsqrt(v + EPS)


def _recip(l):
    r = pl.reciprocal(l, approx=True)
    return r * (2.0 - l * r)


def _mo(x, m):
    return x if isinstance(x, int) else pl.multiple_of(x, m)


def _rows(v8, n):
    return v8 if n == 8 else jnp.concatenate([v8] * (n // 8), axis=0)


def _gate(x, flag, tok):
    xs = jnp.where(flag, _rows(tok, x.shape[0]), x[:, 0:128])
    return jnp.concatenate([xs, x[:, 128:]], axis=1)


def _gate1(x, flag, tok, row=0):
    if row:
        return jnp.concatenate([x[:row], _gate1(x[row:], flag, tok)], axis=0)
    r = tok.shape[0]
    x0 = jnp.where(flag, tok, x[0:r, 0:128])
    if x.shape[1] > 128:
        x0 = jnp.concatenate([x0, x[0:r, 128:]], axis=1)
    return x0 if x.shape[0] == r else jnp.concatenate([x0, x[r:]], axis=0)


def _token(*ys):
    u = None
    for y in ys:
        for i in range(y.shape[0] // 8):
            for j in range(y.shape[1] // 128):
                v = y[8 * i:8 * i + 8, 128 * j:128 * j + 128]
                u = v if u is None else jnp.maximum(u, v)
    return u


def _kernel(x_hbm, k_hbm, v_hbm, wq_hbm, wo_hbm, wr_hbm, wg_hbm, wu_hbm, wd_hbm, c_hbm, wmod_hbm,
            out_hbm,
            x_v, out_v, h_v, hs_v, q_v, acc_v, wm_v, wmr_v, wq_v, wqs0_v, wqs_v, wo_v, wos_v, wg_v, wu_v, wd_v,
            k_v, v_v, kt_v, c_v8, wr_v8, sc_v, scc_v, acol_v, mod_v, best_v, bidx_v, aux_v, flag_s, sems):
    sk = k_hbm.shape[2]
    c_v = c_v8.at[0]
    wr_v = wr_v8.at[0]

    def cp(src, dst, i):
        return pltpu.make_async_copy(src, dst, sems.at[i])

    def wait_all(view, sem):
        cp(view, view, sem).wait()

    c_cp = cp(c_hbm, c_v, SEM_C)
    wr_cp = cp(wr_hbm, wr_v, SEM_WR)
    x0_cp = cp(x_hbm.at[0, pl.ds(0, TP), :], x_v.at[pl.ds(0, TP), :], SEM_X0)
    k0_cp = cp(k_hbm.at[0, 0, pl.ds(sk - W, W), :], k_v.at[0], SEM_K0)
    k_cp = cp(k_hbm.at[0, pl.ds(1, HKV - 1), pl.ds(sk - W, W), :], k_v.at[pl.ds(1, HKV - 1)], SEM_K)
    v_cp = cp(v_hbm.at[0, :, pl.ds(sk - W, W), :], v_v, SEM_V)
    wg_cp = cp(wg_hbm, wg_v, SEM_WG)
    wu_cp = cp(wu_hbm, wu_v, SEM_WU)
    wd_cp = cp(wd_hbm, wd_v.at[:, pl.ds(0, D)], SEM_WD)

    def x_cp(t):
        r0 = _mo(t * TQ, TQ)
        return cp(x_hbm.at[0, pl.ds(r0, TQ), :], x_v.at[pl.ds(r0, TQ), :], SEM_X + t)

    def wm_cps(j):
        return [cp(wmod_hbm.at[:, pl.ds(i * KH + j * 128, 128)], wm_v.at[j, :, pl.ds(i * 128, 128)], SEM_WM + j)
                for i in range(4)]

    def wmr_cp(i):
        c0 = 2 * D + min(i * NM, 32 - NM) * 128
        return cp(wmod_hbm.at[:, pl.ds(c0, NM * 128)], wmr_v.at[i], SEM_WMR + (0 if i < 2 else 1))

    def wq_cps(g, c, n, sem):
        rows = [(0, D)] if n == 4 else [(_mo(i * KH + c * 128, 128), n * 128) for i in range(2)]
        return [cp(wq_hbm.at[pl.ds(r0, nr), pl.ds(g * GW, GW)], wq_v.at[g, pl.ds(r0, nr), pl.ds(0, GW)], sem)
                for r0, nr in rows]

    def wo_cp(c, n, sem):
        r0 = _mo(c * 256, 256)
        return cp(wo_hbm.at[pl.ds(r0, n * 256), :], wo_v.at[pl.ds(r0, n * 256), :], sem)

    def w0_cps(c):
        return wq_cps(1, c, 1, SEM_W + c) + [wo_cp(c, 1, SEM_W + c)]

    w1a_cps = wq_cps(2, 0, 2, SEM_W + 4) + [wo_cp(4, 2, SEM_W + 4)]
    wrest_cps = wq_cps(2, 2, 2, SEM_W + 5) + wq_cps(3, 0, 4, SEM_W + 5) + [wo_cp(6, 10, SEM_W + 5)]

    def out_copy(r0, n):
        return cp(out_v.at[pl.ds(r0, n), :], out_hbm.at[0, pl.ds(r0, n), :], SEM_OUT)

    for c_ in ([c_cp, x0_cp] + [c_ for j in range(NKC) for c_ in wm_cps(j) + wq_cps(0, j, 1, SEM_WQ0 + j)]
               + [x_cp(2), k0_cp, x_cp(3), x_cp(4), k_cp, x_cp(5), wr_cp] + w0_cps(0)
               + [x_cp(6)] + w0_cps(1) + [x_cp(7)] + w0_cps(2) + w0_cps(3) + [v_cp, wmr_cp(0), wmr_cp(1)] + w1a_cps
               + [wmr_cp(i) for i in range(2, NMC)] + wrest_cps + [wg_cp, wu_cp, wd_cp]):
        c_.start()

    def ln1_pair(t, r, n, lo=None):
        ys = []
        for half in range(2):
            r0 = _mo(t * TQ + half * HR + r, 8)
            x = x_v[pl.ds(r0, n), :].astype(f32)
            if lo is not None:
                x = _gate(x, *lo)
            y = _ln(x) * _rows(mod_v[:, D:2 * D], n) + _rows(mod_v[:, 0:D], n)
            h_v[pl.ds(r0, n), :] = y.astype(bf16)
            ys.append(y)
        sums = jnp.concatenate(_a_sums(ys[0][:, :KH], ys[0][:, KH:], ys[1][:, :KH], ys[1][:, KH:]), axis=1)
        hs_v[pl.ds(_mo(t * HR + r, 8), n), :] = sums.astype(bf16)
        return sums[:, KH:3 * KH] if LTOK else sums

    def wqs_ref(g):
        return wqs0_v if isinstance(g, int) and g == 0 else wqs_v.at[g - 1]

    def wq_unit(g, u, lo):
        r0 = _mo(u * 8, 8)
        top = _gate(wq_v[g, pl.ds(r0, 8), 0:GW].astype(f32), *lo)
        bot = wq_v[g, pl.ds(KH + r0, 8), 0:GW].astype(f32)
        outs = []
        for p in range(REP // 2):
            c0, c1, c2 = 2 * p * DH, (2 * p + 1) * DH, (2 * p + 2) * DH
            outs += _b_sums(top[:, c0:c1], top[:, c1:c2], bot[:, c0:c1], bot[:, c1:c2])
        sums = jnp.concatenate(outs, axis=1)
        wqs_ref(g)[pl.ds(r0, 8), :] = sums.astype(bf16)
        return jnp.concatenate([o_ for i, o_ in enumerate(outs) if i % 5 >= 3], axis=1) if LTOK else sums

    def wo_unit(g, u, lo):
        r0 = _mo(g * GW + (u // 16) * 2 * DH + (u % 16) * 8, 8)
        top = _gate(wo_v[pl.ds(r0, 8), :].astype(f32), *lo)
        bot = wo_v[pl.ds(DH + r0, 8), :].astype(f32)
        sums = jnp.concatenate(_b_sums(top[:, :KH], top[:, KH:], bot[:, :KH], bot[:, KH:]), axis=1)
        wos_v[g, pl.ds(_mo(u * 8, 8), 8), :] = sums.astype(bf16)
        return sums[:, 3 * KH:] if LTOK else sums

    def ln2_rows(r0, n, valid=None, lo=None):
        av = _rows(aux_v[0], n)
        bv = _rows(aux_v[1], n)
        rv = _rows(aux_v[2], n)
        r_c = _rows(aux_v[3, :, 0:128], n)
        x2 = x_v[pl.ds(r0, n), :].astype(f32)
        if lo is not None:
            x2 = _gate(x2, *lo)
        m = jnp.mean(x2, axis=-1, keepdims=True)
        xc = x2 - m
        var = jnp.mean(xc * xc, axis=-1, keepdims=True)
        rs = lax.rsqrt(var + EPS)
        y = x2 + ((xc * rs) * av + bv)
        out_v[pl.ds(r0, n), :] = y.astype(bf16)
        r = jnp.sum(xc * rv, axis=-1, keepdims=True) * rs
        r = (jnp.broadcast_to(r, (n, 128)) + r_c).astype(bf16).astype(f32)
        if valid is not None:
            r = jnp.where(valid, r, -jnp.inf)
        mb = jnp.broadcast_to(m, (n, 128))
        rsb = jnp.broadcast_to(rs, (n, 128))
        best = best_v[0]
        bm = best_v[1]
        brs = best_v[2]
        bidx = bidx_v[0]
        rows = lax.broadcasted_iota(jnp.int32, (8, 128), 0)
        for j in range(n // 8):
            sl = slice(8 * j, 8 * (j + 1))
            upd = r[sl] > best
            best = jnp.where(upd, r[sl], best)
            bm = jnp.where(upd, mb[sl], bm)
            brs = jnp.where(upd, rsb[sl], brs)
            bidx = jnp.where(upd, rows + (r0 + 8 * j), bidx)
        best_v[0] = best
        best_v[1] = bm
        best_v[2] = brs
        bidx_v[0] = bidx
        return y, best

    def q_rhs(g, p, k):
        if k in B_SLOT:
            c0 = (p * 5 + B_SLOT[k]) * DH
            return wqs_ref(g)[:, c0:c0 + DH]
        if k == 2:
            return wq_v[g, 0:KH, 2 * p * DH:(2 * p + 1) * DH]
        return wq_v[g, KH:D, (2 * p + 1) * DH:(2 * p + 2) * DH]

    def q_store(a0, p, blocks):
        for rh, ch, v in blocks:
            r0 = pl.multiple_of(a0 + rh * HR, HR)
            q_v[pl.ds(r0, HR), (2 * p + ch) * DH:(2 * p + ch + 1) * DH] = (v * QSCALE).astype(bf16)

    with _scope('P0_wait'):
        flag_s[0] = 0
        c_cp.wait()
        cf = c_v[...].astype(f32)
        sc = (cf * jax.nn.sigmoid(cf)).astype(bf16)
        sc_v[...] = jnp.broadcast_to(sc, (16, D))
        scc_v[...] = jnp.broadcast_to(sc.astype(f32), (128, D)).T
        best_v[0] = jnp.full((8, 128), -jnp.inf, f32)
        best_v[1] = jnp.zeros((8, 128), f32)
        best_v[2] = jnp.zeros((8, 128), f32)
        bidx_v[0] = jnp.zeros((8, 128), jnp.int32)
        x0_cp.wait()

        def norm_rows(i, carry):
            r0 = pl.multiple_of(i * 128, 128)
            acc_v[pl.ds(r0, 128), 0:D] = _ln(x_v[pl.ds(r0, 128), :].astype(f32))
            return carry

        lax.fori_loop(0, TP // 128, norm_rows, 0)

    def k_chunk(j, carry):
        wait_all(wm_v.at[j, :, pl.ds(0, 512)], SEM_WM + j)
        clo = pl.multiple_of(j * 128, 128)
        chi = pl.multiple_of(KH + j * 128, 128)
        md = jnp.dot(sc_v[...], wm_v[j, :, 0:512], preferred_element_type=f32)[0:8].astype(bf16).astype(f32)
        hh = []
        for i, c0 in enumerate((clo, chi)):
            sa = md[:, i * 128:(i + 1) * 128]
            ca1 = 1.0 + md[:, (2 + i) * 128:(3 + i) * 128]
            mod_v[:, pl.ds(c0, 128)] = sa
            mod_v[:, pl.ds(D + c0, 128)] = ca1
            y = acc_v[0:TP, pl.ds(c0, 128)] * _rows(ca1, TP) + _rows(sa, TP)
            h_v[0:TP, pl.ds(c0, 128)] = y.astype(bf16)
            hh.append(y)
        for t in range(TP // TQ):
            top = slice(t * TQ, t * TQ + HR)
            bot = slice(t * TQ + HR, (t + 1) * TQ)
            for i, s_ in enumerate(_a_sums(hh[0][top], hh[1][top], hh[0][bot], hh[1][bot])):
                hs_v[t * HR:(t + 1) * HR, pl.ds(i * KH + clo, 128)] = s_.astype(bf16)
        for c_ in wq_cps(0, j, 1, SEM_WQ0 + j):
            c_.wait()
        lhs = jnp.concatenate([h_v[0:TP, pl.ds(clo, 128)], h_v[0:TP, pl.ds(chi, 128)]], axis=1)
        rhs = jnp.concatenate([wq_v[0, pl.ds(clo, 128), 0:GW], wq_v[0, pl.ds(chi, 128), 0:GW]], axis=0)
        flag = flag_s[0] > 0
        toks = {}
        for n_ in range(4):
            cs = slice(n_ * 256, (n_ + 1) * 256)
            lh = lhs
            if n_ - 2 in toks:
                tk = toks[n_ - 2]
                lh = _gate1(lhs, flag, jnp.concatenate([tk, tk], axis=0).astype(bf16))
            part = jnp.dot(lh, rhs[:, cs], preferred_element_type=f32)
            tot = jnp.where(j == 0, 0.0, acc_v[0:TP, D + n_ * 256:D + (n_ + 1) * 256]) + part
            acc_v[0:TP, D + n_ * 256:D + (n_ + 1) * 256] = tot
            q_v[0:TP, cs] = (tot * QSCALE).astype(bf16)
            if n_ < 2:
                toks[n_] = _token(*[wq_unit(0, j * 16 + n_ * 8 + u, (flag, part[64 * u:64 * u + 8, 0:128]))
                                    for u in range(8)])
        return carry

    with _scope('P1_kchunks'):
        lax.fori_loop(0, NKC, k_chunk, 0)

    with _scope('P2_ln'):
        x_cp(2).wait()
        ln1_pair(2, 0, HR)
        k0_cp.wait()

    def q0_tile(t, units):
        flag = flag_s[0] > 0
        a0 = pl.multiple_of(t * TQ, TQ)
        m0 = pl.multiple_of(t * HR, HR)
        tn = jnp.minimum(t + 1, NT - 1)
        lhs = {k: hs_v[pl.ds(m0, HR), s_ * KH:(s_ + 1) * KH] for k, s_ in A_SLOT.items()}
        lhs[3] = h_v[pl.ds(a0, HR), 0:KH]
        lhs[4] = h_v[pl.ds(pl.multiple_of(a0 + HR, HR), HR), KH:D]
        jobs = [(lambda lo, r=r: ln1_pair(tn, r, 8, lo)) for r in range(0, HR, 8)]
        nprod = 7 * REP // 2
        nslot = nprod - P3S - P3LAG
        nuslot = nprod - P3US - P3ULAG
        utoks = {}
        toks = {}
        n_ = 0
        for p in range(REP // 2):
            comb = _Combine()
            for k in ORDER7:
                lh = lhs[k]
                tks = [d_[n_ - l_] for d_, l_ in ((toks, P3LAG), (utoks, P3ULAG)) if n_ - l_ in d_]
                if tks:
                    tk = _token(*tks)
                    lh = _gate1(lh, flag, jnp.concatenate([tk, tk], axis=0).astype(bf16))
                y = jnp.dot(lh, q_rhs(0, p, k), preferred_element_type=f32)
                q_store(a0, p, comb.feed(k, y))
                for lst, s0, ns, dst, rofs in ((jobs, P3S, nslot, toks, 0), (units, P3US, nuslot, utoks, P3UR)):
                    sl = n_ - s0
                    if 0 <= sl < ns:
                        mine = lst[sl * len(lst) // ns:(sl + 1) * len(lst) // ns]
                        outs = []
                        for k_, jb in enumerate(mine):
                            r_ = (rofs + k_ * HR // len(mine)) % HR // 8 * 8
                            outs.append(jb((flag, y[r_:r_ + 8])))
                        if outs:
                            dst[n_] = _token(*outs)
                n_ += 1

    def q0_a(t, carry):
        x_cp(t + 1).wait()

        @pl.when(t == 3)
        def _():
            k_cp.wait()

        q0_tile(t, [])
        gk = jnp.minimum(t - 2, HKV - 1)
        kt_v[gk] = k_v[gk].T
        return carry

    def q0_b(t, carry):
        @pl.when(t + 1 < NT)
        def _():
            x_cp(t + 1).wait()

        for c_ in w0_cps(t - T3B):
            c_.wait()
        nu = 16
        u0 = (t - T3B) * nu
        units = []
        for u in range(nu):
            units.append(lambda lo, u=u: wq_unit(1, u0 + u, lo))
            units.append(lambda lo, u=u: wo_unit(0, u0 + u, lo))
        q0_tile(t, units)
        gk = jnp.minimum(t - 2, HKV - 1)
        kt_v[gk] = k_v[gk].T
        return carry

    with _scope('P3_q0'):
        lax.fori_loop(2, T3B, q0_a, 0)
        lax.fori_loop(T3B, NT, q0_b, 0)
        v_cp.wait()
        wr_cp.wait()
        wait_all(wmr_v.at[pl.ds(0, 2)], SEM_WMR)
        for c_ in w1a_cps:
            c_.wait()

    def body(i, un, last_group):
        flag = flag_s[0] > 0
        st = dict(hi=None, pend=[])
        g = 3 if last_group else (i * un) // NT

        def pin(name):
            r_ = int(name[1:])
            return flag, st[name[0]][r_:r_ + 8, 0:128]

        def add_hi(tk):
            st['hi'] = tk if st['hi'] is None else jnp.maximum(st['hi'], tk)

        def o_run(n):
            for k_ in range(min(n, len(st['pend']))):
                y = st['pend'].pop(0)()
                if k_ == 0:
                    st['N'] = y
                st['O'] = y

        for u_ in range(un):
            t = (i * un + u_) % NT
            a0 = pl.multiple_of(t * TQ, TQ)
            m0 = pl.multiple_of(t * HR, HR)

            def qk(hh, a0=a0):
                qh = q_v[pl.ds(a0, TQ), hh * DH:(hh + 1) * DH]
                s = jnp.dot(qh, kt_v[g], preferred_element_type=f32)
                if st['hi'] is not None:
                    s = _gate1(s, flag, st['hi'], HIROW if last_group else 0)
                    st['hi'] = None
                m = jnp.max(s, axis=-1, keepdims=True)
                p = jnp.exp2(s - m)
                l = jnp.sum(p, axis=-1, keepdims=True)
                return p.astype(bf16), l

            def pv(pl_):
                p, l = pl_
                o = jnp.dot(p, v_v[g], preferred_element_type=f32)
                st['V'] = o
                return o * _recip(l)

            def q_prod(p, k, comb, a0=a0, m0=m0):
                if k in A_SLOT:
                    lhs = hs_v[pl.ds(m0, HR), A_SLOT[k] * KH:(A_SLOT[k] + 1) * KH]
                elif k == 3:
                    lhs = h_v[pl.ds(a0, HR), 0:KH]
                else:
                    lhs = h_v[pl.ds(pl.multiple_of(a0 + HR, HR), HR), KH:D]
                y = jnp.dot(lhs, q_rhs(g + 1, p, k), preferred_element_type=f32)
                st['Q'] = y
                q_store(a0, p, comb.feed(k, y))

            def o_prod(p, k, o0, o1, comb, a0=a0, m0=m0):
                lhs = _a_op(k, o0[:HR], o1[:HR], o0[HR:], o1[HR:]).astype(bf16)
                if k in B_SLOT:
                    rhs = wos_v[g, p * DH:(p + 1) * DH, B_SLOT[k] * KH:(B_SLOT[k] + 1) * KH]
                elif k == 2:
                    rhs = wo_v[pl.ds(_mo(g * GW + 2 * p * DH, DH), DH), 0:KH]
                else:
                    rhs = wo_v[pl.ds(_mo(g * GW + (2 * p + 1) * DH, DH), DH), KH:D]
                y = jnp.dot(lhs, rhs, preferred_element_type=f32)
                cs = slice((k - 1) * KH, k * KH)
                old = acc_v[pl.ds(m0, HR), cs]
                if p == 0 and not last_group:
                    acc_v[pl.ds(m0, HR), cs] = jnp.where(g == 0, 0.0, old) + y
                elif p == REP // 2 - 1 and last_group:
                    for rh, ch, v in comb.feed(k, old + y):
                        r0 = pl.multiple_of(a0 + rh * HR, HR)
                        cx = slice(ch * KH, (ch + 1) * KH)
                        ga = _rows(mod_v[:, 2 * D + ch * KH:2 * D + (ch + 1) * KH], HR)
                        x_v[pl.ds(r0, HR), cx] = (x_v[pl.ds(r0, HR), cx].astype(f32) + ga * v).astype(bf16)
                else:
                    acc_v[pl.ds(m0, HR), cs] = old + y
                return y

            def side_b(hh):
                pos = u_ * REP + hh
                nst = un * REP - 2 - SKIPL
                if pos < 2 or pos - 2 >= nst:
                    return
                k_ = pos - 2
                ci = jnp.minimum(i, NMC - 1)
                acc = st.get('macc')
                lo = pin(NPIN)
                for rg in range(128 * k_ // nst, 128 * (k_ + 1) // nst):
                    xc_ = scc_v[8 * rg:8 * rg + 8, :]
                    if rg == 128 * k_ // nst:
                        xc_ = jnp.where(lo[0], lo[1], xc_)
                    pr_ = wmr_v[ci, 8 * rg:8 * rg + 8, :].astype(f32) * jnp.concatenate([xc_] * NM, axis=1)
                    acc = pr_ if acc is None else acc + pr_
                st['macc'] = acc
                add_hi(_token(acc))
                if k_ == nst - 1:
                    c0 = pl.multiple_of(2 * D + jnp.minimum(ci * NM, 32 - NM) * 128, 128)
                    tot_ = jnp.sum(acc, axis=0, keepdims=True).astype(bf16).astype(f32)
                    mod_v[:, pl.ds(c0, NM * 128)] = jnp.broadcast_to(tot_, (8, NM * 128))
                nu = 64 * un // NT
                u0 = (i % (NT // un)) * nu
                for u in range(nu * k_ // nst, nu * (k_ + 1) // nst):
                    add_hi(_token(wq_unit(jnp.minimum(g + 2, HKV - 1), u0 + u, pin(WQPIN))))
                    add_hi(_token(wo_unit(g + 1, u0 + u, pin(WOPIN))))

            def side_c(hh, t=t):
                tl = jnp.maximum(t - 1, 0)
                for k_ in range(LCNT[hh]):
                    off = (sum(LCNT[:hh]) + k_) * 8
                    y, b = ln2_rows(pl.multiple_of(tl * TQ + off, 8), 8, t > 0, pin((LPE, LPO)[hh % 2][k_]))
                    add_hi(_token(y, b))

            for p in range(REP // 2):
                h0, h1 = 2 * p, 2 * p + 1
                if not last_group:
                    cq = _Combine()
                    sp = qk(h0)
                    for k in ORDER7[:BSEQ[0]]:
                        q_prod(p, k, cq)
                    o0 = pv(sp)
                    o_run(BSEQ[1])
                    side_b(h0)
                    sp = qk(h1)
                    for k in ORDER7[BSEQ[0]:]:
                        q_prod(p, k, cq)
                    o1 = pv(sp)
                    o_run(7)
                    side_b(h1)
                elif not st['pend']:
                    sp0 = qk(h0)
                    sp1 = qk(h1)
                    o0 = pv(sp0)
                    o1 = pv(sp1)
                else:
                    sp = qk(h0)
                    o_run(CSEQ[0])
                    st['F'] = st['O']
                    o0 = pv(sp)
                    o_run(CSEQ[1])
                    side_c(h0)
                    sp = qk(h1)
                    o_run(CSEQ[2])
                    st['F'] = st['O']
                    o1 = pv(sp)
                    o_run(CSEQ[3])
                    side_c(h1)
                co = _Combine()
                st['pend'] = [(lambda k=k, p=p, o0=o0, o1=o1, co=co, f=o_prod: f(p, k, o0, o1, co))
                              for k in (ORDER7 if last_group and p == REP // 2 - 1 else OORD)]
        o_run(7)
        if last_group:
            for u_ in range(un):
                t = (i * un + u_) % NT

                @pl.when(t > 0)
                def _():
                    out_copy(pl.multiple_of((t - 1) * TQ, TQ), TQ).start()

    def body_b(i, carry):
        @pl.when(i == 2)
        def _():
            wait_all(wmr_v.at[pl.ds(2, NMC - 2)], SEM_WMR + 1)
            for c_ in wrest_cps:
                c_.wait()

        body(i, UNB, False)
        return carry

    with _scope('LB'):
        lax.fori_loop(0, 3 * NT // UNB, body_b, 0)

    wg_cp.wait()
    wu_cp.wait()
    wd_cp.wait()
    sb_ = mod_v[:, 3 * D:4 * D]
    cb1_ = 1.0 + mod_v[:, 4 * D:5 * D]
    gb_ = mod_v[:, 5 * D:6 * D]
    wr8 = wr_v[...].astype(f32)
    wr_ = jnp.concatenate([wr8[r_:r_ + 1, :] for r_ in range(8)], axis=1)
    aux_v[0] = gb_ * cb1_
    aux_v[1] = gb_ * sb_
    aux_v[2] = cb1_ * wr_
    aux_v[3] = jnp.broadcast_to(jnp.sum(sb_ * wr_, axis=-1, keepdims=True), (8, D))

    def body_c(i, carry):
        body(i, UNC, True)
        return carry

    with _scope('LC'):
        lax.fori_loop(0, NT // UNC, body_c, 0)

    with _scope('E1_last'):
        ln2_rows((NT - 1) * TQ, TQ)
        out_copy((NT - 1) * TQ, TQ).start()

    with _scope('E2_ffn'):
        best = best_v[0]
        bidx = bidx_v[0]
        rmax = jnp.max(best, axis=0, keepdims=True)
        idx_v = jnp.min(jnp.where(best == rmax, bidx, S), axis=0, keepdims=True)
        idx = jnp.minimum(idx_v[0, 0], S - 1)
        g0 = pl.multiple_of((idx // 8) * 8, 8)
        sb = mod_v[:, 3 * D:4 * D]
        cb = mod_v[:, 4 * D:5 * D]
        gb = mod_v[:, 5 * D:6 * D]
        x2 = x_v[pl.ds(g0, 8), :].astype(f32)
        h2 = (x2 - best_v[1][:, 0:1]) * best_v[2][:, 0:1] * (1.0 + cb) + sb
        h2b = h2.astype(bf16)
        sel = (lax.broadcasted_iota(jnp.int32, (8, 1), 0) + g0) == idx
        flag = flag_s[0] > 0
        nf = F // 128
        strips = [(k_, j) for j in range(nf) for k_ in 'gu'] + [('d', j) for j in range(FD, nf)]
        gate_r, a_strips, vtok = {}, {}, {}
        y = None
        yv = None
        pos = 0
        for i, (kind, j) in enumerate(strips):
            hi = vtok.get(i - FLAG_)
            if kind == 'd':
                lhs = a_strips[j]
                if hi is not None:
                    lhs = jnp.where(flag, hi.astype(bf16), lhs)
                r_ = jnp.dot(lhs, wd_v[j * 128:(j + 1) * 128, 0:D], preferred_element_type=f32)
                y = r_ if y is None else y + r_
                tok_ = r_[:, D - 128:D]
            else:
                lhs = h2b if hi is None else _gate1(h2b, flag, hi.astype(bf16))
                w_ref = wg_v if kind == 'g' else wu_v
                tok_ = jnp.dot(lhs, w_ref[:, j * 128:(j + 1) * 128], preferred_element_type=f32)
                if kind == 'g':
                    gate_r[j] = tok_
                else:
                    a_strips[j] = (gate_r[j] * jax.nn.sigmoid(gate_r[j]) * tok_).astype(bf16)
                    if j < FD:
                        row = jnp.sum(jnp.where(sel, a_strips[j].astype(f32), 0.0), axis=0, keepdims=True)
                        acol_v[j * 128:(j + 1) * 128, :] = jnp.broadcast_to(row, (128, 128)).T
            if i >= FI0 and pos < FD * 16:
                end = min(pos + FVR // 8, FD * 16) if i < len(strips) - 1 else FD * 16
                for rg in range(pos, end):
                    col = jnp.where(flag, tok_, acol_v[8 * rg:8 * rg + 8, :])
                    pr_ = wd_v[8 * rg:8 * rg + 8, 0:D].astype(f32) * jnp.concatenate([col] * (D // 128), axis=1)
                    yv = pr_ if yv is None else yv + pr_
                pos = end
                vtok[i] = _token(yv)
        y = (y + jnp.sum(yv, axis=0, keepdims=True)) * jax.nn.sigmoid(rmax[:, 0:1])
        out_copy(0, S).wait()
        new = (x2 + gb * (h2 + y)).astype(bf16)
        out_v[pl.ds(g0, 8), :] = jnp.where(sel, new, out_v[pl.ds(g0, 8), :])
        fix = out_copy(g0, 8)
        fix.start()
        fix.wait()


@jax.jit
def pallas_adaLN_cond__sliding_block_cached__moe_arch_mod__prompt_kernel(
    A_x, A_k_cache, A_v_cache, A_wq, A_wo, B_x, B_w_r, B_w_gate, B_w_up, B_w_down, c, w_mod,
):
    del B_x
    any_spec = pl.BlockSpec(memory_space=pl.ANY)
    return pl.pallas_call(
        _kernel,
        out_shape=jax.ShapeDtypeStruct(A_x.shape, A_x.dtype),
        in_specs=[any_spec] * 11,
        out_specs=any_spec,
        scratch_shapes=[
            pltpu.VMEM((S, D), bf16),
            pltpu.VMEM((S, D), bf16),
            pltpu.VMEM((S, D), bf16),
            pltpu.VMEM((S // 2, 5 * KH), bf16),
            pltpu.VMEM((S, GW), bf16),
            pltpu.VMEM((S // 2, 7 * KH), f32),
            pltpu.VMEM((NKC, D, 512 + PADW), bf16),
            pltpu.VMEM((NMC, D, NM * 128), bf16),
            pltpu.VMEM((HKV, D, GW + PADW), bf16),
            pltpu.VMEM((KH, 5 * KH), bf16),
            pltpu.VMEM((HKV - 1, KH, 5 * KH), bf16),
            pltpu.VMEM((HKV * GW, D), bf16),
            pltpu.VMEM((HKV, KH, 5 * KH), bf16),
            pltpu.VMEM((D, F), bf16),
            pltpu.VMEM((D, F), bf16),
            pltpu.VMEM((F, D + PADD), bf16),
            pltpu.VMEM((HKV, W, DH), bf16),
            pltpu.VMEM((HKV, W, DH), bf16),
            pltpu.VMEM((HKV, DH, W), bf16),
            pltpu.VMEM((8, 1, D), bf16),
            pltpu.VMEM((16, 8, 128), bf16),
            pltpu.VMEM((16, D), bf16),
            pltpu.VMEM((D, 128), f32),
            pltpu.VMEM((2 * D, 128), f32),
            pltpu.VMEM((8, 6 * D), f32),
            pltpu.VMEM((8, 8, 128), f32),
            pltpu.VMEM((8, 8, 128), jnp.int32),
            pltpu.VMEM((4, 8, D), f32),
            pltpu.SMEM((1,), jnp.int32),
            pltpu.SemaphoreType.DMA((NSEM,)),
        ],
        compiler_params=pltpu.CompilerParams(vmem_limit_bytes=124 * 1024 * 1024,
                                             disable_semaphore_checks=bool(_p('NOSEM', 1)),
                                             disable_bounds_checks=bool(_p('NOBND', 0))),
    )(A_x, A_k_cache, A_v_cache, A_wq, A_wo, B_w_r.reshape(8, 128), B_w_gate, B_w_up, B_w_down, c, w_mod)
```

```python
import contextlib
import math
import os

import jax
import jax.numpy as jnp
from jax import lax
from jax.experimental import pallas as pl
from jax.experimental.pallas import tpu as pltpu


def _p(name, default):
    v = os.environ.get('KP_' + name)
    return default if v is None else type(default)(v)


def _ints(s):
    return [int(c_) for c_ in s.split(',')]


S = 2048
D = 1024
HQ = 32
HKV = 4
REP = HQ // HKV
DH = 128
GW = REP * DH
W = 512
F = 3584
EPS = 1e-5
TQ = 256
QR = TQ // 4
QC = D // 4
NT = S // TQ
TP = 512
NKC = 4
KC = D // NKC
PADW = 128
PADD = 256
NM = 3
NMC = 11
FD = _p('FD', 15)
FI0 = _p('FI0', 8)
FLAG_ = _p('FLAG', 4)
FVR = _p('FVR', 32)
LAG0 = _p('LAG0', 2)
T3B = 4
WC = _p('WC', 256)
NU = 32 * QC // WC
QORD = _ints(_p('QORD', '4,2,1,7,5,3,6'))
OORD = _ints(_p('OORD', '3,6,5,1,2,7,4'))
IORD = _ints(_p('IORD', '4,2,1,7,5,3,6'))
QRUN = _ints(_p('QRUN', '7,6,6,6,6,6,6,6'))
ORUN_B = _ints(_p('ORUNB', '0,0,0,0,0,0,0,0,6,6,6,6,6,6,6,7'))
ORUN_C = _ints(_p('ORUNC', '0,0,0,0,2,3,2,3,16,17,0,0,2,3,2,3'))
LCNT = _ints(_p('LCNT', '3,3,3,3,3,3,3,3,4,4,5,5,5,5,5,5'))
LPINS = _p('LPINS', 'V0,V48,V96,V144,V192,V240').split(',')
LHI = _p('LHI', 2)
CORD = _ints(_p('CORD', '3,6,4,2,1,7,5'))
LFL = _p('LFL', 8)
OHI = _p('OHI', 0)
NPIN = _p('NPIN', 'V192')
NHI = _p('NHI', 2)
WPINS = _p('WPINS', 'V0,V32,V64,V96,V128,V160,V192').split(',')
WSUB = _p('WSUB', 1)
WSTEP = _p('WSTEP', 'oooooooo' + 'qqqqqqqq')
SCOPES = _p('SCOPES', 0)
QSCALE = (DH ** -0.5) * math.log2(math.e)

f32 = jnp.float32
bf16 = jnp.bfloat16

(SEM_C, SEM_WR, SEM_X0, SEM_K0, SEM_K, SEM_V, SEM_WG, SEM_WU, SEM_WD, SEM_OUT) = range(10)
SEM_X = 10
SEM_W = SEM_X + NT
SEM_WQ0 = SEM_W + 6
SEM_WM = SEM_WQ0 + NKC
SEM_WMR = SEM_WM + NKC
NSEM = SEM_WMR + 2

A_COEF = {1: ((0, 0, 1), (1, 1, 1)), 2: ((1, 0, 1), (1, 1, 1)), 3: ((0, 0, 1),), 4: ((1, 1, 1),),
          5: ((0, 0, 1), (0, 1, 1)), 6: ((1, 0, 1), (0, 0, -1)), 7: ((0, 1, 1), (1, 1, -1))}
B_COEF = {1: ((0, 0, 1), (1, 1, 1)), 2: ((0, 0, 1),), 3: ((0, 1, 1), (1, 1, -1)), 4: ((1, 0, 1), (0, 0, -1)),
          5: ((1, 1, 1),), 6: ((0, 0, 1), (0, 1, 1)), 7: ((1, 0, 1), (1, 1, 1))}
C_COEF = {(0, 0): {1: 1, 4: 1, 5: -1, 7: 1}, (0, 1): {3: 1, 5: 1}, (1, 0): {2: 1, 4: 1},
          (1, 1): {1: 1, 2: -1, 3: 1, 6: 1}}


def _lin(coef, get):
    v = get(coef[0][0], coef[0][1])
    for r, c, s in coef[1:]:
        v = v + get(r, c) if s > 0 else v - get(r, c)
    return v


class _Combine:
    def __init__(self):
        self.part = {}

    def feed(self, i, v):
        done = []
        for key, coef in C_COEF.items():
            if i not in coef:
                continue
            s = coef[i]
            if key not in self.part:
                cur = (v, s, 1)
            else:
                u, su, n = self.part[key]
                if s == su:
                    cur = (u + v, s, n + 1)
                elif su > 0:
                    cur = (u - v, 1, n + 1)
                else:
                    cur = (v - u, 1, n + 1)
            self.part[key] = cur
            if cur[2] == len(coef):
                assert cur[1] > 0
                done.append((key[0], key[1], cur[0]))
        return done


class _Combine2:
    def __init__(self):
        self.inner = {}
        self.outer = {}

    def feed(self, i, j, v):
        done = []
        for r, c, u in self.inner.setdefault(i, _Combine()).feed(j, v):
            for r2, c2, w in self.outer.setdefault((r, c), _Combine()).feed(i, u):
                done.append((2 * r2 + r, 2 * c2 + c, w))
        return done


class _LhsOps:
    def __init__(self, get, get_bf16=None):
        self.get, self.get_bf16, self.cache = get, get_bf16, {}

    def outer(self, i, a, b):
        if len(A_COEF[i]) == 1:
            r, c, _ = A_COEF[i][0]
            return self.get(2 * r + a, 2 * c + b)
        if (i, a, b) not in self.cache:
            self.cache[i, a, b] = _lin(A_COEF[i], lambda r, c: self.get(2 * r + a, 2 * c + b))
        return self.cache[i, a, b]

    def op(self, i, j):
        if self.get_bf16 is not None and len(A_COEF[i]) == 1 and len(A_COEF[j]) == 1:
            return self.get_bf16(2 * A_COEF[i][0][0] + A_COEF[j][0][0], 2 * A_COEF[i][0][1] + A_COEF[j][0][1])
        return _lin(A_COEF[j], lambda a, b: self.outer(i, a, b)).astype(bf16)


def _scope(name):
    return jax.named_scope(name) if SCOPES else contextlib.nullcontext()


def _ln(x):
    m = jnp.mean(x, axis=-1, keepdims=True)
    xc = x - m
    v = jnp.mean(xc * xc, axis=-1, keepdims=True)
    return xc * lax.rsqrt(v + EPS)


def _recip(l):
    r = pl.reciprocal(l, approx=True)
    return r * (2.0 - l * r)


def _mo(x, m):
    return x if isinstance(x, int) else pl.multiple_of(x, m)


def _rows(v8, n):
    return v8 if n == 8 else jnp.concatenate([v8] * (n // 8), axis=0)


def _gate(x, flag, tok):
    xs = jnp.where(flag, _rows(tok, x.shape[0]), x[:, 0:128])
    return xs if x.shape[1] == 128 else jnp.concatenate([xs, x[:, 128:]], axis=1)


def _gate1(x, flag, tok):
    r = tok.shape[0]
    x0 = jnp.where(flag, tok, x[0:r, 0:128])
    if x.shape[1] > 128:
        x0 = jnp.concatenate([x0, x[0:r, 128:]], axis=1)
    return x0 if x.shape[0] == r else jnp.concatenate([x0, x[r:]], axis=0)


def _token(*ys):
    u = None
    for y in ys:
        for i in range(y.shape[0] // 8):
            for j in range(y.shape[1] // 128):
                v = y[8 * i:8 * i + 8, 128 * j:128 * j + 128]
                u = v if u is None else jnp.maximum(u, v)
    return u


def _kernel(x_hbm, k_hbm, v_hbm, wq_hbm, wo_hbm, wr_hbm, wg_hbm, wu_hbm, wd_hbm, c_hbm, wmod_hbm,
            out_hbm,
            x_v, h_v, q_v, acc_v, accb_v, wmr_v, wq_v, wqs_v, wo_v, wos_v, wg_v, wu_v, wd_v,
            k_v, v_v, kt_v, c_v8, wr_v8, sc_v, scc_v, acol_v, mod_v, best_v, bidx_v, aux_v, flag_s, sems):
    sk = k_hbm.shape[2]
    c_v = c_v8.at[0]
    wr_v = wr_v8.at[0]
    out_v = h_v
    x2e_v = wo_v.at[0]
    wm_v = wg_v

    def cp(src, dst, i):
        return pltpu.make_async_copy(src, dst, sems.at[i])

    def wait_all(view, sem):
        cp(view, view, sem).wait()

    c_cp = cp(c_hbm, c_v, SEM_C)
    wr_cp = cp(wr_hbm, wr_v, SEM_WR)
    x0_cp = cp(x_hbm.at[0, pl.ds(0, TP), :], x_v.at[pl.ds(0, TP), :], SEM_X0)
    k0_cp = cp(k_hbm.at[0, 0, pl.ds(sk - W, W), :], k_v.at[0], SEM_K0)
    k_cp = cp(k_hbm.at[0, pl.ds(1, HKV - 1), pl.ds(sk - W, W), :], k_v.at[pl.ds(1, HKV - 1)], SEM_K)
    v_cp = cp(v_hbm.at[0, :, pl.ds(sk - W, W), :], v_v, SEM_V)
    wg_cp = cp(wg_hbm, wg_v, SEM_WG)
    wu_cp = cp(wu_hbm, wu_v, SEM_WU)
    wd_cp = cp(wd_hbm, wd_v.at[:, pl.ds(0, D)], SEM_WD)

    def x_cp(t):
        r0 = _mo(t * TQ, TQ)
        return cp(x_hbm.at[0, pl.ds(r0, TQ), :], x_v.at[pl.ds(r0, TQ), :], SEM_X + t)

    def wm_cps(j):
        return [cp(wmod_hbm.at[:, pl.ds(i * D + j * KC, KC)], wm_v.at[:, pl.ds((2 * j + i) * KC, KC)], SEM_WM + j)
                for i in range(2)]

    def wq0_cp(j):
        r0 = _mo(j * KC, KC)
        return cp(wq_hbm.at[pl.ds(r0, KC), pl.ds(0, GW)], wq_v.at[0, pl.ds(r0, KC), pl.ds(0, GW)], SEM_WQ0 + j)

    def wmr_cp(i):
        c0 = 2 * D + min(i * NM, 32 - NM) * 128
        return cp(wmod_hbm.at[:, pl.ds(c0, NM * 128)], wmr_v.at[i], SEM_WMR + (0 if i < 2 else 1))

    def w_cps(s, c, n, sem):
        rows = [(0, D)] if n == 4 else [(_mo(i * QC + c * 64, 64), n * 64) for i in range(4)]
        cps = []
        if s + 1 < HKV:
            cps += [cp(wq_hbm.at[pl.ds(r0, nr), pl.ds((s + 1) * GW, GW)],
                       wq_v.at[s + 1, pl.ds(r0, nr), pl.ds(0, GW)], sem) for r0, nr in rows]
        cps += [cp(wo_hbm.at[pl.ds(s * GW + r0, nr), :], wo_v.at[s, pl.ds(r0, nr), :], sem) for r0, nr in rows]
        return cps

    w1_cps = w_cps(1, 0, 4, SEM_W + 4)
    wrest_cps = w_cps(2, 0, 4, SEM_W + 5) + w_cps(3, 0, 4, SEM_W + 5)

    def out_copy(r0, n):
        return cp(out_v.at[pl.ds(r0, n), :], out_hbm.at[0, pl.ds(r0, n), :], SEM_OUT)

    for c_ in ([c_cp, x0_cp] + [c_ for j in range(NKC) for c_ in wm_cps(j) + [wq0_cp(j)]]
               + [x_cp(2), k0_cp, x_cp(3), x_cp(4), k_cp, x_cp(5), wr_cp] + w_cps(0, 0, 1, SEM_W)
               + [x_cp(6)] + w_cps(0, 1, 1, SEM_W + 1) + [x_cp(7)] + w_cps(0, 2, 1, SEM_W + 2)
               + w_cps(0, 3, 1, SEM_W + 3) + [v_cp, wmr_cp(0), wmr_cp(1)] + w1_cps
               + [wmr_cp(i) for i in range(2, NMC)] + wrest_cps + [wu_cp, wd_cp]):
        c_.start()

    def ln1_rows(r0, n, lo=None):
        x = x_v[pl.ds(r0, n), :].astype(f32)
        if lo is not None:
            x = _gate(x, *lo)
        y = _ln(x) * _rows(mod_v[:, D:2 * D], n) + _rows(mod_v[:, 0:D], n)
        h_v[pl.ds(r0, n), :] = y.astype(bf16)
        return y

    def w_unit(src, dst, u0, u, lo):
        nsub = QC // WC
        r0 = _mo((u0 // nsub + u // nsub) * 8, 8)
        c0 = (u % nsub) * WC
        def load(a, b):
            return src[pl.ds(a * QC + r0, 8), b * QC + c0:b * QC + c0 + WC].astype(f32)

        multi = isinstance(lo, list)
        blk = {}
        if not multi:
            blk = {(a, b): _gate(load(a, b), *lo) if a == b else load(a, b) for a in range(4) for b in range(4)}
        toks = []
        for i in range(1, 8):
            outer = {}
            for a in range(2):
                for b in range(2):
                    if multi:
                        v = _lin(B_COEF[i], lambda r, c: load(2 * r + a, 2 * c + b))
                        sel_ = jnp.where(lo[i - 1][0], jnp.concatenate([lo[i - 1][1]] * (WC // 128), axis=1), v)
                        outer[a, b] = sel_ if a == b else v
                    else:
                        outer[a, b] = _lin(B_COEF[i], lambda r, c: blk[2 * r + a, 2 * c + b])
            for j in range(1, 8):
                v = _lin(B_COEF[j], lambda a, b: outer[a, b])
                cd = ((i - 1) * 7 + j - 1) * QC + c0
                dst[pl.ds(r0, 8), cd:cd + WC] = v.astype(bf16)
                if j >= 6:
                    toks.append(v)
        return _token(*toks)

    def ln2_rows(x2_ref, rx, r0, n, valid=None, lo=None):
        av = _rows(aux_v[0], n)
        bv = _rows(aux_v[1], n)
        rv = _rows(aux_v[2], n)
        r_c = _rows(aux_v[3, :, 0:128], n)
        x2 = x2_ref[pl.ds(rx, n), :].astype(f32)
        if lo is not None:
            x2 = _gate(x2, *lo)
        m = jnp.mean(x2, axis=-1, keepdims=True)
        xc = x2 - m
        var = jnp.mean(xc * xc, axis=-1, keepdims=True)
        rs = lax.rsqrt(var + EPS)
        y = x2 + ((xc * rs) * av + bv)
        out_v[pl.ds(r0, n), :] = y.astype(bf16)
        r = jnp.sum(xc * rv, axis=-1, keepdims=True) * rs
        r = (jnp.broadcast_to(r, (n, 128)) + r_c).astype(bf16).astype(f32)
        if valid is not None:
            r = jnp.where(valid, r, -jnp.inf)
        mb = jnp.broadcast_to(m, (n, 128))
        rsb = jnp.broadcast_to(rs, (n, 128))
        best = best_v[0]
        bm = best_v[1]
        brs = best_v[2]
        bidx = bidx_v[0]
        rows = lax.broadcasted_iota(jnp.int32, (8, 128), 0)
        for j in range(n // 8):
            sl = slice(8 * j, 8 * (j + 1))
            upd = r[sl] > best
            best = jnp.where(upd, r[sl], best)
            bm = jnp.where(upd, mb[sl], bm)
            brs = jnp.where(upd, rsb[sl], brs)
            bidx = jnp.where(upd, rows + (r0 + 8 * j), bidx)
        best_v[0] = best
        best_v[1] = bm
        best_v[2] = brs
        bidx_v[0] = bidx
        return y, best

    with _scope('P0_wait'):
        flag_s[0] = 0
        c_cp.wait()
        cf = c_v[...].astype(f32)
        sc = (cf * jax.nn.sigmoid(cf)).astype(bf16)
        sc_v[...] = jnp.broadcast_to(sc, (16, D))
        scc_v[...] = jnp.broadcast_to(sc.astype(f32), (128, D)).T
        best_v[0] = jnp.full((8, 128), -jnp.inf, f32)
        best_v[1] = jnp.zeros((8, 128), f32)
        best_v[2] = jnp.zeros((8, 128), f32)
        bidx_v[0] = jnp.zeros((8, 128), jnp.int32)
        x0_cp.wait()

        def norm_rows(i, carry):
            r0 = pl.multiple_of(i * 64, 64)
            for t in range(2):
                (acc_v, accb_v)[t][pl.ds(r0, 64), 0:D] = _ln(x_v[pl.ds(t * TQ + r0, 64), :].astype(f32))
            return carry

        lax.fori_loop(0, TQ // 64, norm_rows, 0)

    def k_chunk(j, carry):
        c0 = pl.multiple_of(j * KC, KC)
        cm = pl.multiple_of(2 * j * KC, 2 * KC)
        wait_all(wm_v.at[:, pl.ds(cm, 2 * KC)], SEM_WM + j)
        md = jnp.dot(sc_v[...], wm_v[:, pl.ds(cm, 2 * KC)], preferred_element_type=f32)[0:8].astype(bf16).astype(f32)
        sa = md[:, 0:KC]
        ca1 = 1.0 + md[:, KC:2 * KC]
        mod_v[:, pl.ds(c0, KC)] = sa
        mod_v[:, pl.ds(D + c0, KC)] = ca1
        nrm = jnp.concatenate([acc_v[:, pl.ds(c0, KC)], accb_v[:, pl.ds(c0, KC)]], axis=0)
        h_v[0:TP, pl.ds(c0, KC)] = (nrm * _rows(ca1, TP) + _rows(sa, TP)).astype(bf16)
        wq0_cp(j).wait()
        part = jnp.dot(h_v[0:TP, pl.ds(c0, KC)], wq_v[0, pl.ds(c0, KC), 0:GW], preferred_element_type=f32)
        tot = jnp.where(j == 0, 0.0, jnp.concatenate([acc_v[:, D:2 * D], accb_v[:, D:2 * D]], axis=0)) + part
        acc_v[:, D:2 * D] = tot[0:TQ]
        accb_v[:, D:2 * D] = tot[TQ:TP]
        q_v[0, 0:TP, :] = (tot * QSCALE).astype(bf16)
        return carry

    with _scope('P1_kchunks'):
        lax.fori_loop(0, NKC, k_chunk, 0)

    with _scope('P2_ln'):
        wg_cp.start()
        x_cp(2).wait()
        ln1_rows(2 * TQ, TQ)
        k0_cp.wait()

    def q0_tile(t, units):
        flag = flag_s[0] > 0
        r0 = pl.multiple_of(t * TQ, TQ)
        rn = jnp.minimum(t + 1, NT - 1) * TQ
        h = h_v[pl.ds(r0, TQ), :]
        jobs = [(lambda lo, r=r: _token(ln1_rows(pl.multiple_of(rn + r, 8), 8, lo))) for r in range(0, TQ, 8)]
        mixed = []
        for i, jb in enumerate(jobs):
            mixed.append(jb)
            mixed += units[i * len(units) // len(jobs):(i + 1) * len(units) // len(jobs)]
        nslot = 2 * REP - 2 * LAG0
        toks = {}
        n_ = 0
        for j in range(REP):
            q = None
            for kh in range(2):
                hj = h[:, kh * 512:(kh + 1) * 512]
                if n_ - 2 * LAG0 + 1 in toks:
                    tk = toks[n_ - 2 * LAG0 + 1]
                    hj = _gate1(hj, flag, jnp.concatenate([tk, tk], axis=0).astype(bf16))
                y = jnp.dot(hj, wq_v[0, kh * 512:(kh + 1) * 512, j * DH:(j + 1) * DH], preferred_element_type=f32)
                q = y if q is None else q + y
                sl = n_ - 1
                if 0 <= sl < nslot:
                    mine = mixed[sl * len(mixed) // nslot:(sl + 1) * len(mixed) // nslot]
                    outs = []
                    for k_, jb in enumerate(mine):
                        r_ = (k_ * TQ // len(mine)) // 8 * 8
                        outs.append(jb((flag, y[r_:r_ + 8])))
                    toks[n_] = _token(*outs)
                n_ += 1
            q_v[0, pl.ds(r0, TQ), j * DH:(j + 1) * DH] = (q * QSCALE).astype(bf16)

    def q0_a(t, carry):
        x_cp(t + 1).wait()

        @pl.when(t == 3)
        def _():
            k_cp.wait()

        q0_tile(t, [])
        gk = jnp.minimum(t - 2, HKV - 1)
        kt_v[gk] = k_v[gk].T
        return carry

    def q0_b(t, carry):
        @pl.when(t + 1 < NT)
        def _():
            x_cp(t + 1).wait()

        for c_ in w_cps(0, t - T3B, 1, SEM_W + t - T3B):
            c_.wait()
        nu = NU // 4
        u0 = (t - T3B) * nu
        units = []
        for u in range(nu):
            units.append(lambda lo, u=u: w_unit(wq_v.at[1], wqs_v.at[1], u0, u, lo))
            units.append(lambda lo, u=u: w_unit(wo_v.at[0], wos_v.at[0], u0, u, lo))
        q0_tile(t, units)
        gk = jnp.minimum(t - 2, HKV - 1)
        kt_v[gk] = k_v[gk].T
        return carry

    with _scope('P3_q0'):
        lax.fori_loop(2, T3B, q0_a, 0)
        lax.fori_loop(T3B, NT, q0_b, 0)
        v_cp.wait()
        wr_cp.wait()
        wait_all(wmr_v.at[pl.ds(0, 2)], SEM_WMR)
        for c_ in w1_cps:
            c_.wait()

    def body(i, last_group):
        flag = flag_s[0] > 0
        st = {}
        his = {}
        g = 3 if last_group else i // (NT // 2)
        qs = g % 2
        blk = i % (NT // 2)
        m0 = pl.multiple_of(blk * QR, QR)
        o_todo = []

        def pin(name):
            r_ = int(name[1:])
            return flag, st[name[0]][r_:r_ + 8, 0:128]

        def add_hi(step, tk):
            his[step] = tk if step not in his else jnp.maximum(his[step], tk)

        def lgate(lhs, gate):
            return lhs if gate is None else _gate1(lhs, flag, jnp.concatenate([gate, gate], axis=0).astype(bf16))

        def run(todo, n, gate=None):
            ys = []
            for k_ in range(min(n, len(todo))):
                ys.append(todo.pop(0)(gate))
                gate = None
                st['abcdefgh'[min(k_, 7)]] = ys[-1]
            return ys

        def qk(step, a0, hh):
            s = jnp.dot(q_v[qs, pl.ds(a0, TQ), hh * DH:(hh + 1) * DH], kt_v[g], preferred_element_type=f32)
            if step in his:
                s = _gate1(s, flag, his.pop(step))
            st['K'] = s
            m = jnp.max(s, axis=-1, keepdims=True)
            p = jnp.exp2(s - m)
            l = jnp.sum(p, axis=-1, keepdims=True)
            return p.astype(bf16), l

        def pv(step, os_, pl_):
            p, l = pl_
            o = jnp.dot(p, v_v[g], preferred_element_type=f32)
            st['V'] = o
            os_.append(o * _recip(l))
            if OHI:
                add_hi(step + OHI, _token(os_[-1]))

        if not last_group:
            ci = jnp.minimum(i, NMC - 1)
            nu = NU // 4
            u0 = (i % 4) * nu
            gq = jnp.minimum(g + 2, HKV - 1)

        def side_b(s_):
            lo = [pin(n_) for n_ in WPINS] if WSUB else pin(WPINS[0])
            kind = WSTEP[s_]
            k_ = WSTEP[:s_].count(kind)
            for u in range(k_ * nu // 8, (k_ + 1) * nu // 8):
                if kind == 'o':
                    add_hi(s_ + 1, w_unit(wo_v.at[g + 1], wos_v.at[1 - qs], u0, u, lo))
                else:
                    add_hi(s_ + 1, w_unit(wq_v.at[gq], wqs_v.at[gq % 2], u0, u, lo))
            nn = 2 * REP - NHI
            if s_ < nn:
                lo = pin(NPIN)
                macc = st.get('macc')
                for rg in range(128 * s_ // nn, 128 * (s_ + 1) // nn):
                    xc_ = jnp.where(lo[0], lo[1], scc_v[8 * rg:8 * rg + 8, :])
                    pr_ = wmr_v[ci, 8 * rg:8 * rg + 8, :].astype(f32) * jnp.concatenate([xc_] * NM, axis=1)
                    macc = pr_ if macc is None else macc + pr_
                st['macc'] = macc
                add_hi(s_ + NHI, _token(macc))
                if s_ == nn - 1:
                    c0 = pl.multiple_of(2 * D + jnp.minimum(ci * NM, 32 - NM) * 128, 128)
                    tot_ = jnp.sum(macc, axis=0, keepdims=True).astype(bf16).astype(f32)
                    mod_v[:, pl.ds(c0, NM * 128)] = jnp.broadcast_to(tot_, (8, NM * 128))

        def ln_piece(n_, lo):
            if n_ < 32:
                r0 = pl.multiple_of(jnp.maximum(2 * blk - 1, 0) * TQ + n_ * 8, 8)
                return _token(*ln2_rows(x_v, r0, r0, 8, blk > 0, lo))
            off = (n_ - 32) * 8
            return _token(*ln2_rows(x2e_v, pl.multiple_of(blk * TQ + off, 8), pl.multiple_of(2 * blk * TQ + off, 8),
                                    8, None, lo))

        def side_c(s_):
            for k_ in range(LCNT[s_]):
                add_hi(s_ + LHI, ln_piece(sum(LCNT[:s_]) + k_, pin(LPINS[k_])))

        for par in range(2):
            a0 = pl.multiple_of((2 * blk + par) * TQ, TQ)
            acc = (acc_v, accb_v)[par]
            os_ = []

            def h_blk(a, b, a0=a0):
                return h_v[pl.ds(pl.multiple_of(a0 + a * QR, QR), QR), b * QC:(b + 1) * QC]

            q_lhs = _LhsOps(lambda a, b, f=h_blk: f(a, b).astype(f32), h_blk)
            q_comb = _Combine2()

            def q_prod(i_, j_, gate, a0=a0, q_lhs=q_lhs, q_comb=q_comb):
                c0 = ((i_ - 1) * 7 + j_ - 1) * QC
                y = jnp.dot(lgate(q_lhs.op(i_, j_), gate), wqs_v[1 - qs, :, c0:c0 + QC], preferred_element_type=f32)
                for a, b, v in q_comb.feed(i_, j_, y):
                    r0 = pl.multiple_of(a0 + a * QR, QR)
                    q_v[1 - qs, pl.ds(r0, QR), b * QC:(b + 1) * QC] = (v * QSCALE).astype(bf16)
                return y

            q_todo = [(lambda gate, i_=i_, j_=j_, f=q_prod: f(i_, j_, gate)) for i_ in QORD for j_ in IORD]
            o_lhs = _LhsOps(lambda a, b, os_=os_: jnp.concatenate(
                [os_[2 * b][a * QR:(a + 1) * QR], os_[2 * b + 1][a * QR:(a + 1) * QR]], axis=1))

            o_comb = _Combine2()

            def o_prod(i_, j_, gate, acc=acc, o_lhs=o_lhs, o_comb=o_comb, par=par, a0=a0):
                c0 = ((i_ - 1) * 7 + j_ - 1) * QC
                y = jnp.dot(lgate(o_lhs.op(i_, j_), gate), wos_v[qs, :, c0:c0 + QC], preferred_element_type=f32)
                old = acc[pl.ds(m0, QR), c0:c0 + QC]
                if not last_group:
                    acc[pl.ds(m0, QR), c0:c0 + QC] = jnp.where(g == 0, 0.0, old) + y
                    return y
                for a, b, v in o_comb.feed(i_, j_, old + y):
                    rs = pl.ds(pl.multiple_of(a0 + a * QR, QR), QR)
                    cx = slice(b * QC, (b + 1) * QC)
                    ga = _rows(mod_v[:, 2 * D + b * QC:2 * D + (b + 1) * QC], QR)
                    x2 = (x_v[rs, cx].astype(f32) + ga * v).astype(bf16)
                    if par == 0:
                        x2e_v[pl.ds(pl.multiple_of(blk * TQ + a * QR, QR), QR), cx] = x2
                    else:
                        x_v[rs, cx] = x2
                return y

            def o_add(outers, f=o_prod):
                o_todo.extend([(lambda gate, i_=i_, j_=j_: f(i_, j_, gate)) for i_ in outers for j_ in IORD])

            hh = 0
            while hh < REP:
                s_ = par * REP + hh
                if hh == 4:
                    o_add((CORD if last_group else OORD)[:2])
                if not last_group:
                    sp = qk(s_, a0, hh)
                    run(q_todo, QRUN[hh])
                    pv(s_, os_, sp)
                    if WSTEP[s_] == 'o':
                        side_b(s_)
                    run(o_todo, ORUN_B[s_])
                    if WSTEP[s_] != 'o':
                        side_b(s_)
                elif not o_todo:
                    sp0 = qk(s_, a0, hh)
                    sp1 = qk(s_ + 1, a0, hh + 1)
                    pv(s_, os_, sp0)
                    side_c(s_)
                    pv(s_ + 1, os_, sp1)
                    side_c(s_ + 1)
                    hh += 1
                else:
                    sp = qk(s_, a0, hh)
                    run(o_todo, 1)
                    pv(s_, os_, sp)
                    run(o_todo, ORUN_C[s_])
                    side_c(s_)
                hh += 1
            o_add((CORD if last_group else OORD)[2:])
        late = list(range(sum(LCNT), 64)) if last_group else []
        gates = {4 + 4 * k_: his[s_] for k_, s_ in enumerate(sorted(his))}
        nfl = len(o_todo)
        for k_ in range(nfl):
            y = run(o_todo, 1, gates.get(k_))[0]
            ns = nfl - LFL
            mine = late[k_ * len(late) // ns:(k_ + 1) * len(late) // ns] if k_ < ns else []
            for n_ in mine:
                tk = ln_piece(n_, (flag, y[0:8, 0:128]))
                gates[k_ + LFL] = tk if k_ + LFL not in gates else jnp.maximum(tk, gates[k_ + LFL])
        if last_group:
            @pl.when(blk > 0)
            def _():
                out_copy(pl.multiple_of((2 * blk - 1) * TQ, TQ), TQ).start()

            out_copy(pl.multiple_of(2 * blk * TQ, TQ), TQ).start()

    def body_b(i, carry):
        @pl.when(i == 2)
        def _():
            wait_all(wmr_v.at[pl.ds(2, NMC - 2)], SEM_WMR + 1)
            for c_ in wrest_cps:
                c_.wait()

        body(i, False)
        return carry

    with _scope('LB'):
        lax.fori_loop(0, 3 * NT // 2, body_b, 0)

    wg_cp.wait()
    wu_cp.wait()
    wd_cp.wait()
    sb_ = mod_v[:, 3 * D:4 * D]
    cb1_ = 1.0 + mod_v[:, 4 * D:5 * D]
    gb_ = mod_v[:, 5 * D:6 * D]
    wr8 = wr_v[...].astype(f32)
    wr_ = jnp.concatenate([wr8[r_:r_ + 1, :] for r_ in range(8)], axis=1)
    aux_v[0] = gb_ * cb1_
    aux_v[1] = gb_ * sb_
    aux_v[2] = cb1_ * wr_
    aux_v[3] = jnp.broadcast_to(jnp.sum(sb_ * wr_, axis=-1, keepdims=True), (8, D))

    def body_c(i, carry):
        body(i, True)
        return carry

    with _scope('LC'):
        lax.fori_loop(0, NT // 2, body_c, 0)

    with _scope('E1_last'):
        ln2_rows(x_v, (NT - 1) * TQ, (NT - 1) * TQ, TQ)
        out_copy((NT - 1) * TQ, TQ).start()

    with _scope('E2_ffn'):
        best = best_v[0]
        bidx = bidx_v[0]
        rmax = jnp.max(best, axis=0, keepdims=True)
        idx_v = jnp.min(jnp.where(best == rmax, bidx, S), axis=0, keepdims=True)
        idx = jnp.minimum(idx_v[0, 0], S - 1)
        g0 = pl.multiple_of((idx // 8) * 8, 8)
        sb = mod_v[:, 3 * D:4 * D]
        cb = mod_v[:, 4 * D:5 * D]
        gb = mod_v[:, 5 * D:6 * D]
        ge = pl.multiple_of((g0 // (2 * TQ)) * TQ + g0 % TQ, 8)
        x2 = jnp.where((g0 // TQ) % 2 == 0, x2e_v[pl.ds(ge, 8), :], x_v[pl.ds(g0, 8), :]).astype(f32)
        h2 = (x2 - best_v[1][:, 0:1]) * best_v[2][:, 0:1] * (1.0 + cb) + sb
        h2b = h2.astype(bf16)
        sel = (lax.broadcasted_iota(jnp.int32, (8, 1), 0) + g0) == idx
        flag = flag_s[0] > 0
        nf = F // 128
        strips = [(k_, j) for j in range(nf) for k_ in 'gu'] + [('d', j) for j in range(FD, nf)]
        gate_r, a_strips, vtok = {}, {}, {}
        y = None
        yv = None
        pos = 0
        for i, (kind, j) in enumerate(strips):
            hi = vtok.get(i - FLAG_)
            if kind == 'd':
                lhs = a_strips[j]
                if hi is not None:
                    lhs = jnp.where(flag, hi.astype(bf16), lhs)
                r_ = jnp.dot(lhs, wd_v[j * 128:(j + 1) * 128, 0:D], preferred_element_type=f32)
                y = r_ if y is None else y + r_
                tok_ = r_[:, D - 128:D]
            else:
                lhs = h2b if hi is None else _gate1(h2b, flag, hi.astype(bf16))
                w_ref = wg_v if kind == 'g' else wu_v
                tok_ = jnp.dot(lhs, w_ref[:, j * 128:(j + 1) * 128], preferred_element_type=f32)
                if kind == 'g':
                    gate_r[j] = tok_
                else:
                    a_strips[j] = (gate_r[j] * jax.nn.sigmoid(gate_r[j]) * tok_).astype(bf16)
                    if j < FD:
                        row = jnp.sum(jnp.where(sel, a_strips[j].astype(f32), 0.0), axis=0, keepdims=True)
                        acol_v[j * 128:(j + 1) * 128, :] = jnp.broadcast_to(row, (128, 128)).T
            if i >= FI0 and pos < FD * 16:
                end = min(pos + FVR // 8, FD * 16) if i < len(strips) - 1 else FD * 16
                for rg in range(pos, end):
                    col = jnp.where(flag, tok_, acol_v[8 * rg:8 * rg + 8, :])
                    pr_ = wd_v[8 * rg:8 * rg + 8, 0:D].astype(f32) * jnp.concatenate([col] * (D // 128), axis=1)
                    yv = pr_ if yv is None else yv + pr_
                pos = end
                vtok[i] = _token(yv)
        y = (y + jnp.sum(yv, axis=0, keepdims=True)) * jax.nn.sigmoid(rmax[:, 0:1])
        out_copy(0, S).wait()
        new = (x2 + gb * (h2 + y)).astype(bf16)
        out_v[pl.ds(g0, 8), :] = jnp.where(sel, new, out_v[pl.ds(g0, 8), :])
        fix = out_copy(g0, 8)
        fix.start()
        fix.wait()


@jax.jit
def pallas_adaLN_cond__sliding_block_cached__moe_arch_mod__prompt_kernel(
    A_x, A_k_cache, A_v_cache, A_wq, A_wo, B_x, B_w_r, B_w_gate, B_w_up, B_w_down, c, w_mod,
):
    del B_x
    any_spec = pl.BlockSpec(memory_space=pl.ANY)
    return pl.pallas_call(
        _kernel,
        out_shape=jax.ShapeDtypeStruct(A_x.shape, A_x.dtype),
        in_specs=[any_spec] * 11,
        out_specs=any_spec,
        scratch_shapes=[
            pltpu.VMEM((S, D), bf16),
            pltpu.VMEM((S, D), bf16),
            pltpu.VMEM((2, S, GW), bf16),
            pltpu.VMEM((S // 8, 49 * QC), f32),
            pltpu.VMEM((S // 8, 49 * QC), f32),
            pltpu.VMEM((NMC, D, NM * 128), bf16),
            pltpu.VMEM((HKV, D, GW + PADW), bf16),
            pltpu.VMEM((2, QC, 49 * QC), bf16),
            pltpu.VMEM((HKV, GW, D), bf16),
            pltpu.VMEM((2, QC, 49 * QC), bf16),
            pltpu.VMEM((D, F), bf16),
            pltpu.VMEM((D, F), bf16),
            pltpu.VMEM((F, D + PADD), bf16),
            pltpu.VMEM((HKV, W, DH), bf16),
            pltpu.VMEM((HKV, W, DH), bf16),
            pltpu.VMEM((HKV, DH, W), bf16),
            pltpu.VMEM((8, 1, D), bf16),
            pltpu.VMEM((16, 8, 128), bf16),
            pltpu.VMEM((16, D), bf16),
            pltpu.VMEM((D, 128), f32),
            pltpu.VMEM((2 * D, 128), f32),
            pltpu.VMEM((8, 6 * D), f32),
            pltpu.VMEM((8, 8, 128), f32),
            pltpu.VMEM((8, 8, 128), jnp.int32),
            pltpu.VMEM((4, 8, D), f32),
            pltpu.SMEM((1,), jnp.int32),
            pltpu.SemaphoreType.DMA((NSEM,)),
        ],
        compiler_params=pltpu.CompilerParams(vmem_limit_bytes=126 * 1024 * 1024,
                                             disable_semaphore_checks=bool(_p('NOSEM', 1)),
                                             disable_bounds_checks=bool(_p('NOBND', 0))),
    )(A_x, A_k_cache, A_v_cache, A_wq, A_wo, B_w_r.reshape(8, 128), B_w_gate, B_w_up, B_w_down, c, w_mod)
```

```python
import contextlib
import math
import os

import jax
import jax.numpy as jnp
from jax import lax
from jax.experimental import pallas as pl
from jax.experimental.pallas import tpu as pltpu


def _p(name, default):
    v = os.environ.get('KP_' + name)
    return default if v is None else type(default)(v)


def _ints(s):
    return [int(c_) for c_ in s.split(',')]


S = 2048
D = 1024
HQ = 32
HKV = 4
REP = HQ // HKV
DH = 128
GW = REP * DH
W = 512
F = 3584
EPS = 1e-5
TQ = 256
QR = TQ // 4
QC = D // 4
NT = S // TQ
TP = 512
NKC = 4
KC = D // NKC
PADW = 128
PADD = 256
NM = 3
NMC = 11
FD = _p('FD', 15)
FI0 = _p('FI0', 8)
FLAG_ = _p('FLAG', 4)
FVR = _p('FVR', 32)
LAG0 = _p('LAG0', 2)
T3B = 4
WC = _p('WC', 256)
NU = 32 * QC // WC
QORD = _ints(_p('QORD', '4,2,1,7,5,3,6'))
OORD = _ints(_p('OORD', '3,6,5,1,2,7,4'))
IORD = _ints(_p('IORD', '4,2,1,7,5,3,6'))
QRUN = _ints(_p('QRUN', '7,6,6,6,6,6,6,6'))
ORUN_B = _ints(_p('ORUNB', '0,0,0,0,0,0,0,0,6,6,6,6,6,6,6,7'))
ORUN_C = _ints(_p('ORUNC', '0,0,0,0,2,3,2,3,16,17,0,0,2,3,2,3'))
LCNT = _ints(_p('LCNT', '4,4,4,4,4,4,4,4'))
LPINS = (_p('LPE', 'V0,V64,V128,V192').split(','), _p('LPO', 'V0,V64,V128,V192').split(','))
LHIO = _p('LHIO', 2)
LHI = _p('LHI', 2)
CORD = _ints(_p('CORD', '6,3,5,1,2,4,7'))
DBG = _p('DBG', '')
CMODE = _p('CMODE', 'pair')
LF0 = _p('LF0', 4)
GST = _p('GST', 4)
ONLY = _p('ONLY', 'PBC')
OHIC = _p('OHIC', 3)
P3SUB = _p('P3SUB', 1)
P3S = _p('P3S', 0)
PSUM = _p('PSUM', 1)
QPRE = _p('QPRE', 9)
P3LAG = _p('P3LAG', 4)
P3US = _p('P3US', 0)
P3ULAG = _p('P3ULAG', 3)
LFL = _p('LFL', 8)
OHI = _p('OHI', 0)
NPIN = _p('NPIN', 'V192')
NHI = _p('NHI', 2)
WPINS = _p('WPINS', 'V0,V32,V64,V96,V128,V160,V192').split(',')
WSUB = _p('WSUB', 1)
WSTEP = _p('WSTEP', 'oooooooo' + 'qqqqqqqq')
SCOPES = _p('SCOPES', 0)
QSCALE = (DH ** -0.5) * math.log2(math.e)

f32 = jnp.float32
bf16 = jnp.bfloat16

(SEM_C, SEM_WR, SEM_X0, SEM_K0, SEM_K, SEM_V, SEM_WG, SEM_WU, SEM_WD, SEM_OUT) = range(10)
SEM_X = 10
SEM_W = SEM_X + NT
SEM_WQ0 = SEM_W + 6
SEM_WM = SEM_WQ0 + NKC
SEM_WMR = SEM_WM + NKC
NSEM = SEM_WMR + 2

A_COEF = {1: ((0, 0, 1), (1, 1, 1)), 2: ((1, 0, 1), (1, 1, 1)), 3: ((0, 0, 1),), 4: ((1, 1, 1),),
          5: ((0, 0, 1), (0, 1, 1)), 6: ((1, 0, 1), (0, 0, -1)), 7: ((0, 1, 1), (1, 1, -1))}
B_COEF = {1: ((0, 0, 1), (1, 1, 1)), 2: ((0, 0, 1),), 3: ((0, 1, 1), (1, 1, -1)), 4: ((1, 0, 1), (0, 0, -1)),
          5: ((1, 1, 1),), 6: ((0, 0, 1), (0, 1, 1)), 7: ((1, 0, 1), (1, 1, 1))}
C_COEF = {(0, 0): {1: 1, 4: 1, 5: -1, 7: 1}, (0, 1): {3: 1, 5: 1}, (1, 0): {2: 1, 4: 1},
          (1, 1): {1: 1, 2: -1, 3: 1, 6: 1}}


def _lin(coef, get):
    v = get(coef[0][0], coef[0][1])
    for r, c, s in coef[1:]:
        v = v + get(r, c) if s > 0 else v - get(r, c)
    return v


class _Combine:
    def __init__(self):
        self.part = {}

    def feed(self, i, v):
        done = []
        for key, coef in C_COEF.items():
            if i not in coef:
                continue
            s = coef[i]
            if key not in self.part:
                cur = (v, s, 1)
            else:
                u, su, n = self.part[key]
                if s == su:
                    cur = (u + v, s, n + 1)
                elif su > 0:
                    cur = (u - v, 1, n + 1)
                else:
                    cur = (v - u, 1, n + 1)
            self.part[key] = cur
            if cur[2] == len(coef):
                assert cur[1] > 0
                done.append((key[0], key[1], cur[0]))
        return done


class _Combine2:
    def __init__(self):
        self.inner = {}
        self.outer = {}

    def feed(self, i, j, v):
        done = []
        for r, c, u in self.inner.setdefault(i, _Combine()).feed(j, v):
            for r2, c2, w in self.outer.setdefault((r, c), _Combine()).feed(i, u):
                done.append((2 * r2 + r, 2 * c2 + c, w))
        return done


class _LhsOps:
    def __init__(self, get, get_bf16=None):
        self.get, self.get_bf16, self.cache = get, get_bf16, {}

    def outer(self, i, a, b):
        if len(A_COEF[i]) == 1:
            r, c, _ = A_COEF[i][0]
            return self.get(2 * r + a, 2 * c + b)
        if (i, a, b) not in self.cache:
            self.cache[i, a, b] = _lin(A_COEF[i], lambda r, c: self.get(2 * r + a, 2 * c + b))
        return self.cache[i, a, b]

    def op(self, i, j):
        if self.get_bf16 is not None and len(A_COEF[i]) == 1 and len(A_COEF[j]) == 1:
            return self.get_bf16(2 * A_COEF[i][0][0] + A_COEF[j][0][0], 2 * A_COEF[i][0][1] + A_COEF[j][0][1])
        return _lin(A_COEF[j], lambda a, b: self.outer(i, a, b)).astype(bf16)


def _scope(name):
    return jax.named_scope(name) if SCOPES else contextlib.nullcontext()


def _ln(x):
    m = jnp.mean(x, axis=-1, keepdims=True)
    xc = x - m
    v = jnp.mean(xc * xc, axis=-1, keepdims=True)
    return xc * lax.rsqrt(v + EPS)


def _recip(l):
    r = pl.reciprocal(l, approx=True)
    return r * (2.0 - l * r)


def _mo(x, m):
    return x if isinstance(x, int) else pl.multiple_of(x, m)


def _rows(v8, n):
    return v8 if n == 8 else jnp.concatenate([v8] * (n // 8), axis=0)


def _gate(x, flag, tok):
    xs = jnp.where(flag, _rows(tok, x.shape[0]), x[:, 0:128])
    return xs if x.shape[1] == 128 else jnp.concatenate([xs, x[:, 128:]], axis=1)


def _gate1(x, flag, tok):
    r = tok.shape[0]
    x0 = jnp.where(flag, tok, x[0:r, 0:128])
    if x.shape[1] > 128:
        x0 = jnp.concatenate([x0, x[0:r, 128:]], axis=1)
    return x0 if x.shape[0] == r else jnp.concatenate([x0, x[r:]], axis=0)


def _token(*ys):
    u = None
    for y in ys:
        for i in range(y.shape[0] // 8):
            for j in range(y.shape[1] // 128):
                v = y[8 * i:8 * i + 8, 128 * j:128 * j + 128]
                u = v if u is None else jnp.maximum(u, v)
    return u


def _kernel(x_hbm, k_hbm, v_hbm, wq_hbm, wo_hbm, wr_hbm, wg_hbm, wu_hbm, wd_hbm, c_hbm, wmod_hbm,
            out_hbm,
            x_v, h_v, q_v, acc_v, accb_v, wmr_v, wq_v, wqs_v, wo_v, wos_v, wg_v, wu_v, wd_v,
            k_v, v_v, kt_v, c_v8, wr_v8, sc_v, scc_v, acol_v, mod_v, best_v, bidx_v, aux_v, flag_s, sems):
    sk = k_hbm.shape[2]
    c_v = c_v8.at[0]
    wr_v = wr_v8.at[0]
    out_v = h_v
    x2e_v = wo_v.at[0]
    wm_v = wg_v

    def cp(src, dst, i):
        return pltpu.make_async_copy(src, dst, sems.at[i])

    def wait_all(view, sem):
        cp(view, view, sem).wait()

    c_cp = cp(c_hbm, c_v, SEM_C)
    wr_cp = cp(wr_hbm, wr_v, SEM_WR)
    x0_cp = cp(x_hbm.at[0, pl.ds(0, TP), :], x_v.at[pl.ds(0, TP), :], SEM_X0)
    k0_cp = cp(k_hbm.at[0, 0, pl.ds(sk - W, W), :], k_v.at[0], SEM_K0)
    k_cp = cp(k_hbm.at[0, pl.ds(1, HKV - 1), pl.ds(sk - W, W), :], k_v.at[pl.ds(1, HKV - 1)], SEM_K)
    v_cp = cp(v_hbm.at[0, :, pl.ds(sk - W, W), :], v_v, SEM_V)
    wg_cp = cp(wg_hbm, wg_v, SEM_WG)
    wu_cp = cp(wu_hbm, wu_v, SEM_WU)
    wd_cp = cp(wd_hbm, wd_v.at[:, pl.ds(0, D)], SEM_WD)

    def x_cp(t):
        r0 = _mo(t * TQ, TQ)
        return cp(x_hbm.at[0, pl.ds(r0, TQ), :], x_v.at[pl.ds(r0, TQ), :], SEM_X + t)

    def wm_cps(j):
        return [cp(wmod_hbm.at[:, pl.ds(i * D + j * KC, KC)], wm_v.at[:, pl.ds((2 * j + i) * KC, KC)], SEM_WM + j)
                for i in range(2)]

    def wq0_cp(j):
        r0 = _mo(j * KC, KC)
        return cp(wq_hbm.at[pl.ds(r0, KC), pl.ds(0, GW)], wq_v.at[0, pl.ds(r0, KC), pl.ds(0, GW)], SEM_WQ0 + j)

    def wmr_cp(i):
        c0 = 2 * D + min(i * NM, 32 - NM) * 128
        return cp(wmod_hbm.at[:, pl.ds(c0, NM * 128)], wmr_v.at[i], SEM_WMR + (0 if i < 2 else 1))

    def w_cps(s, c, n, sem):
        rows = [(0, D)] if n == 4 else [(_mo(i * QC + c * 64, 64), n * 64) for i in range(4)]
        cps = []
        if s + 1 < HKV:
            cps += [cp(wq_hbm.at[pl.ds(r0, nr), pl.ds((s + 1) * GW, GW)],
                       wq_v.at[s + 1, pl.ds(r0, nr), pl.ds(0, GW)], sem) for r0, nr in rows]
        cps += [cp(wo_hbm.at[pl.ds(s * GW + r0, nr), :], wo_v.at[s, pl.ds(r0, nr), :], sem) for r0, nr in rows]
        return cps

    w1_cps = w_cps(1, 0, 4, SEM_W + 4)
    wrest_cps = w_cps(2, 0, 4, SEM_W + 5) + w_cps(3, 0, 4, SEM_W + 5)

    def out_copy(r0, n):
        return cp(out_v.at[pl.ds(r0, n), :], out_hbm.at[0, pl.ds(r0, n), :], SEM_OUT)

    for c_ in ([c_cp, x0_cp] + [c_ for j in range(NKC) for c_ in wm_cps(j) + [wq0_cp(j)]]
               + [x_cp(2), k0_cp, x_cp(3), x_cp(4), k_cp, x_cp(5), wr_cp] + w_cps(0, 0, 1, SEM_W)
               + [x_cp(6)] + w_cps(0, 1, 1, SEM_W + 1) + [x_cp(7)] + w_cps(0, 2, 1, SEM_W + 2)
               + w_cps(0, 3, 1, SEM_W + 3) + [v_cp, wmr_cp(0), wmr_cp(1)] + w1_cps
               + [wmr_cp(i) for i in range(2, NMC)] + wrest_cps + [wu_cp, wd_cp]):
        c_.start()

    def ln1_rows(r0, n, lo=None):
        x = x_v[pl.ds(r0, n), :].astype(f32)
        if lo is not None:
            x = _gate(x, *lo)
        y = _ln(x) * _rows(mod_v[:, D:2 * D], n) + _rows(mod_v[:, 0:D], n)
        h_v[pl.ds(r0, n), :] = y.astype(bf16)
        return y

    def w_unit(src, dst, u0, u, lo):
        nsub = QC // WC
        r0 = _mo((u0 // nsub + u // nsub) * 8, 8)
        c0 = (u % nsub) * WC
        def load(a, b):
            return src[pl.ds(a * QC + r0, 8), b * QC + c0:b * QC + c0 + WC].astype(f32)

        multi = isinstance(lo, list)
        blk = {}
        if not multi:
            blk = {(a, b): _gate(load(a, b), *lo) if a == b else load(a, b) for a in range(4) for b in range(4)}
        toks = []
        for i in range(1, 8):
            outer = {}
            for a in range(2):
                for b in range(2):
                    if multi:
                        v = _lin(B_COEF[i], lambda r, c: load(2 * r + a, 2 * c + b))
                        sel_ = jnp.where(lo[i - 1][0], jnp.concatenate([lo[i - 1][1]] * (WC // 128), axis=1), v)
                        outer[a, b] = sel_ if a == b else v
                    else:
                        outer[a, b] = _lin(B_COEF[i], lambda r, c: blk[2 * r + a, 2 * c + b])
            for j in range(1, 8):
                v = _lin(B_COEF[j], lambda a, b: outer[a, b])
                cd = ((i - 1) * 7 + j - 1) * QC + c0
                dst[pl.ds(r0, 8), cd:cd + WC] = v.astype(bf16)
                if j >= 6:
                    toks.append(v)
        return _token(*toks)

    def ln2_rows(x2_ref, rx, r0, n, valid=None, lo=None):
        av = _rows(aux_v[0], n)
        bv = _rows(aux_v[1], n)
        rv = _rows(aux_v[2], n)
        r_c = _rows(aux_v[3, :, 0:128], n)
        x2 = x2_ref[pl.ds(rx, n), :].astype(f32)
        if lo is not None:
            x2 = _gate(x2, *lo)
        m = jnp.mean(x2, axis=-1, keepdims=True)
        xc = x2 - m
        var = jnp.mean(xc * xc, axis=-1, keepdims=True)
        rs = lax.rsqrt(var + EPS)
        y = x2 + ((xc * rs) * av + bv)
        out_v[pl.ds(r0, n), :] = y.astype(bf16)
        r = jnp.sum(xc * rv, axis=-1, keepdims=True) * rs
        r = (jnp.broadcast_to(r, (n, 128)) + r_c).astype(bf16).astype(f32)
        if valid is not None:
            r = jnp.where(valid, r, -jnp.inf)
        mb = jnp.broadcast_to(m, (n, 128))
        rsb = jnp.broadcast_to(rs, (n, 128))
        best = best_v[0]
        bm = best_v[1]
        brs = best_v[2]
        bidx = bidx_v[0]
        rows = lax.broadcasted_iota(jnp.int32, (8, 128), 0)
        for j in range(n // 8):
            sl = slice(8 * j, 8 * (j + 1))
            upd = r[sl] > best
            best = jnp.where(upd, r[sl], best)
            bm = jnp.where(upd, mb[sl], bm)
            brs = jnp.where(upd, rsb[sl], brs)
            bidx = jnp.where(upd, rows + (r0 + 8 * j), bidx)
        best_v[0] = best
        best_v[1] = bm
        best_v[2] = brs
        bidx_v[0] = bidx
        return y, best

    with _scope('P0_wait'):
        flag_s[0] = 0
        c_cp.wait()
        cf = c_v[...].astype(f32)
        sc = (cf * jax.nn.sigmoid(cf)).astype(bf16)
        sc_v[...] = jnp.broadcast_to(sc, (16, D))
        scc_v[...] = jnp.broadcast_to(sc.astype(f32), (128, D)).T
        best_v[0] = jnp.full((8, 128), -jnp.inf, f32)
        best_v[1] = jnp.zeros((8, 128), f32)
        best_v[2] = jnp.zeros((8, 128), f32)
        bidx_v[0] = jnp.zeros((8, 128), jnp.int32)
        x0_cp.wait()

        def norm_rows(i, carry):
            r0 = pl.multiple_of(i * 64, 64)
            for t in range(2):
                (acc_v, accb_v)[t][pl.ds(r0, 64), 0:D] = _ln(x_v[pl.ds(t * TQ + r0, 64), :].astype(f32))
            return carry

        lax.fori_loop(0, TQ // 64, norm_rows, 0)

    def k_chunk(j, carry):
        c0 = pl.multiple_of(j * KC, KC)
        cm = pl.multiple_of(2 * j * KC, 2 * KC)
        wait_all(wm_v.at[:, pl.ds(cm, 2 * KC)], SEM_WM + j)
        md = jnp.dot(sc_v[...], wm_v[:, pl.ds(cm, 2 * KC)], preferred_element_type=f32)[0:8].astype(bf16).astype(f32)
        sa = md[:, 0:KC]
        ca1 = 1.0 + md[:, KC:2 * KC]
        mod_v[:, pl.ds(c0, KC)] = sa
        mod_v[:, pl.ds(D + c0, KC)] = ca1
        nrm = jnp.concatenate([acc_v[:, pl.ds(c0, KC)], accb_v[:, pl.ds(c0, KC)]], axis=0)
        h_v[0:TP, pl.ds(c0, KC)] = (nrm * _rows(ca1, TP) + _rows(sa, TP)).astype(bf16)
        wq0_cp(j).wait()
        part = jnp.dot(h_v[0:TP, pl.ds(c0, KC)], wq_v[0, pl.ds(c0, KC), 0:GW], preferred_element_type=f32)
        tot = jnp.where(j == 0, 0.0, jnp.concatenate([acc_v[:, D:2 * D], accb_v[:, D:2 * D]], axis=0)) + part
        acc_v[:, D:2 * D] = tot[0:TQ]
        accb_v[:, D:2 * D] = tot[TQ:TP]
        q_v[0, 0:TP, :] = (tot * QSCALE).astype(bf16)
        return carry

    with _scope('P1_kchunks'):
        lax.fori_loop(0, NKC, k_chunk, 0)

    with _scope('P2_ln'):
        wg_cp.start()
        x_cp(2).wait()
        ln1_rows(2 * TQ, TQ)
        k0_cp.wait()

    def q0_tile(t, units):
        flag = flag_s[0] > 0
        r0 = pl.multiple_of(t * TQ, TQ)
        rn = jnp.minimum(t + 1, NT - 1) * TQ
        h = h_v[pl.ds(r0, TQ), :]
        jobs = [(lambda lo, r=r: _token(ln1_rows(pl.multiple_of(rn + r, 8), 8, lo))) for r in range(0, TQ, 8)]
        nslot = 2 * REP - P3S - P3LAG
        nuslot = 2 * REP - P3US - P3ULAG
        toks = {}
        n_ = 0
        for j in range(REP):
            q = None
            for kh in range(2):
                hj = h[:, kh * 512:(kh + 1) * 512]
                if n_ in toks:
                    tk = _token(*toks[n_])
                    hj = _gate1(hj, flag, jnp.concatenate([tk, tk], axis=0).astype(bf16))
                y = jnp.dot(hj, wq_v[0, kh * 512:(kh + 1) * 512, j * DH:(j + 1) * DH], preferred_element_type=f32)
                q = y if q is None else q + y
                sl = n_ - P3S
                if 0 <= sl < nslot:
                    mine = jobs[sl * len(jobs) // nslot:(sl + 1) * len(jobs) // nslot]
                    for k_, jb in enumerate(mine):
                        r_ = (k_ * TQ // len(mine)) // 8 * 8
                        toks.setdefault(n_ + P3LAG, []).append(jb((flag, y[r_:r_ + 8])))
                sl = n_ - P3US
                if 0 <= sl < nuslot:
                    mine = units[sl * len(units) // nuslot:(sl + 1) * len(units) // nuslot]
                    for k_, jb in enumerate(mine):
                        rr = [((k_ * 7 + z) * TQ // (7 * len(mine))) // 8 * 8 for z in range(7)]
                        lo = [(flag, y[r_:r_ + 8]) for r_ in rr] if P3SUB else (flag, y[rr[0]:rr[0] + 8])
                        toks.setdefault(n_ + P3ULAG, []).append(jb(lo))
                n_ += 1
            q_v[0, pl.ds(r0, TQ), j * DH:(j + 1) * DH] = (q * QSCALE).astype(bf16)

    def q0_a(t, carry):
        x_cp(t + 1).wait()

        @pl.when(t == 3)
        def _():
            k_cp.wait()

        q0_tile(t, [])
        gk = jnp.minimum(t - 2, HKV - 1)
        kt_v[gk] = k_v[gk].T
        return carry

    def q0_b(t, carry):
        @pl.when(t + 1 < NT)
        def _():
            x_cp(t + 1).wait()

        for c_ in w_cps(0, t - T3B, 1, SEM_W + t - T3B):
            c_.wait()
        nu = NU // 4
        u0 = (t - T3B) * nu
        units = []
        for u in range(nu):
            units.append(lambda lo, u=u: w_unit(wq_v.at[1], wqs_v.at[1], u0, u, lo))
            units.append(lambda lo, u=u: w_unit(wo_v.at[0], wos_v.at[0], u0, u, lo))
        q0_tile(t, units)
        gk = jnp.minimum(t - 2, HKV - 1)
        kt_v[gk] = k_v[gk].T
        return carry

    with _scope('P3_q0'):
        if 'P' in ONLY:
            lax.fori_loop(2, T3B, q0_a, 0)
            lax.fori_loop(T3B, NT, q0_b, 0)
        v_cp.wait()
        wr_cp.wait()
        wait_all(wmr_v.at[pl.ds(0, 2)], SEM_WMR)
        for c_ in w1_cps:
            c_.wait()

    def body(i, last_group):
        flag = flag_s[0] > 0
        st = {}
        his = {}
        g = 3 if last_group else i // (NT // 2)
        qs = g % 2
        blk = i % (NT // 2)
        m0 = pl.multiple_of(blk * QR, QR)
        o_todo = []

        def pin(name):
            r_ = int(name[1:])
            return flag, st[name[0]][r_:r_ + 8, 0:128]

        def add_hi(step, tk):
            his[step] = tk if step not in his else jnp.maximum(his[step], tk)

        def lgate(lhs, gate):
            return lhs if gate is None else _gate1(lhs, flag, jnp.concatenate([gate, gate], axis=0).astype(bf16))

        def run(todo, n, gate=None):
            ys = []
            for k_ in range(min(n, len(todo))):
                ys.append(todo.pop(0)(gate))
                gate = None
                st['abcdefgh'[min(k_, 7)]] = ys[-1]
            return ys

        def qk(step, a0, hh):
            s = jnp.dot(q_v[qs, pl.ds(a0, TQ), hh * DH:(hh + 1) * DH], kt_v[g], preferred_element_type=f32)
            if step in his:
                s = _gate1(s, flag, his.pop(step))
            st['J'] = st.get('K')
            st['K'] = s
            m = jnp.max(s, axis=-1, keepdims=True)
            p = jnp.exp2(s - m)
            if PSUM:
                ps = (p[:, 0:128] + p[:, 128:256]) + (p[:, 256:384] + p[:, 384:512])
                p = jnp.concatenate([p[:, 0:384], jnp.where(flag, ps, p[:, 384:512])], axis=1)
                l = jnp.sum(ps, axis=-1, keepdims=True)
            else:
                l = jnp.sum(p, axis=-1, keepdims=True)
            return p.astype(bf16), l

        def pv(step, os_, pl_):
            p, l = pl_
            o = jnp.dot(p, v_v[g], preferred_element_type=f32)
            st['W'] = st.get('V')
            st['V'] = o
            os_.append(o * _recip(l))
            ohi = OHIC if last_group else OHI
            if ohi:
                add_hi(step + ohi, _token(os_[-1]))

        if not last_group:
            ci = jnp.minimum(i, NMC - 1)
            nu = NU // 4
            u0 = (i % 4) * nu
            gq = jnp.minimum(g + 2, HKV - 1)

        def side_b(s_):
            lo = [pin(n_) for n_ in WPINS] if WSUB else pin(WPINS[0])
            kind = WSTEP[s_]
            k_ = WSTEP[:s_].count(kind)
            for u in range(k_ * nu // 8, (k_ + 1) * nu // 8):
                if kind == 'o':
                    add_hi(s_ + 1, w_unit(wo_v.at[g + 1], wos_v.at[1 - qs], u0, u, lo))
                else:
                    add_hi(s_ + 1, w_unit(wq_v.at[gq], wqs_v.at[gq % 2], u0, u, lo))
            nn = 2 * REP - NHI
            if s_ < nn:
                lo = pin(NPIN)
                macc = st.get('macc')
                for rg in range(128 * s_ // nn, 128 * (s_ + 1) // nn):
                    xc_ = jnp.where(lo[0], lo[1], scc_v[8 * rg:8 * rg + 8, :])
                    pr_ = wmr_v[ci, 8 * rg:8 * rg + 8, :].astype(f32) * jnp.concatenate([xc_] * NM, axis=1)
                    macc = pr_ if macc is None else macc + pr_
                st['macc'] = macc
                add_hi(s_ + NHI, _token(macc))
                if s_ == nn - 1:
                    c0 = pl.multiple_of(2 * D + jnp.minimum(ci * NM, 32 - NM) * 128, 128)
                    tot_ = jnp.sum(macc, axis=0, keepdims=True).astype(bf16).astype(f32)
                    mod_v[:, pl.ds(c0, NM * 128)] = jnp.broadcast_to(tot_, (8, NM * 128))

        def ln_piece(n_, lo):
            if n_ < 32:
                r0 = pl.multiple_of(jnp.maximum(2 * blk - 1, 0) * TQ + n_ * 8, 8)
                return _token(*ln2_rows(x_v, r0, r0, 8, blk > 0, lo))
            off = (n_ - 32) * 8
            return _token(*ln2_rows(x2e_v, pl.multiple_of(blk * TQ + off, 8), pl.multiple_of(2 * blk * TQ + off, 8),
                                    8, None, lo))

        def side_c(s_):
            for k_ in range(LCNT[s_ % REP]):
                add_hi(s_ + (LHI, LHIO)[s_ % 2], ln_piece(32 * (s_ // REP) + sum(LCNT[:s_ % REP]) + k_, pin(LPINS[s_ % 2][k_])))

        def flush(late):
            gates = {GST * (k_ + 1): his.pop(s_) for k_, s_ in enumerate(sorted(his))}
            nfl = len(o_todo)
            ns = nfl - LFL - LF0
            for k_ in range(nfl):
                y = run(o_todo, 1, gates.get(k_))[0]
                sl = k_ - LF0
                mine = late[sl * len(late) // ns:(sl + 1) * len(late) // ns] if 0 <= sl < ns else []
                for n_ in mine:
                    tk = ln_piece(n_, (flag, y[0:8, 0:128]))
                    gates[k_ + LFL] = tk if k_ + LFL not in gates else jnp.maximum(tk, gates[k_ + LFL])

        for par in range(2):
            a0 = pl.multiple_of((2 * blk + par) * TQ, TQ)
            acc = (acc_v, accb_v)[par]
            os_ = []

            def h_blk(a, b, a0=a0):
                return h_v[pl.ds(pl.multiple_of(a0 + a * QR, QR), QR), b * QC:(b + 1) * QC]

            q_lhs = _LhsOps(lambda a, b, f=h_blk: f(a, b).astype(f32), h_blk)
            q_comb = _Combine2()

            def q_prod(i_, j_, gate, a0=a0, q_lhs=q_lhs, q_comb=q_comb):
                c0 = ((i_ - 1) * 7 + j_ - 1) * QC
                y = jnp.dot(lgate(q_lhs.op(i_, j_), gate), wqs_v[1 - qs, :, c0:c0 + QC], preferred_element_type=f32)
                for a, b, v in q_comb.feed(i_, j_, y):
                    r0 = pl.multiple_of(a0 + a * QR, QR)
                    q_v[1 - qs, pl.ds(r0, QR), b * QC:(b + 1) * QC] = (v * QSCALE).astype(bf16)
                return y

            q_todo = [(lambda gate, i_=i_, j_=j_, f=q_prod: f(i_, j_, gate)) for i_ in QORD for j_ in IORD]
            o_lhs = _LhsOps(lambda a, b, os_=os_: jnp.concatenate(
                [os_[2 * b][a * QR:(a + 1) * QR], os_[2 * b + 1][a * QR:(a + 1) * QR]], axis=1))

            o_comb = _Combine2()

            def o_prod(i_, j_, gate, acc=acc, o_lhs=o_lhs, o_comb=o_comb, par=par, a0=a0):
                c0 = ((i_ - 1) * 7 + j_ - 1) * QC
                y = jnp.dot(lgate(o_lhs.op(i_, j_), gate), wos_v[qs, :, c0:c0 + QC], preferred_element_type=f32)
                old = acc[pl.ds(m0, QR), c0:c0 + QC]
                if not last_group or 'F' in DBG:
                    acc[pl.ds(m0, QR), c0:c0 + QC] = jnp.where(g == 0, 0.0, old) + y
                    return y
                for a, b, v in o_comb.feed(i_, j_, old + y):
                    rs = pl.ds(pl.multiple_of(a0 + a * QR, QR), QR)
                    cx = slice(b * QC, (b + 1) * QC)
                    ga = _rows(mod_v[:, 2 * D + b * QC:2 * D + (b + 1) * QC], QR)
                    x2 = (x_v[rs, cx].astype(f32) + ga * v).astype(bf16)
                    if par == 0:
                        x2e_v[pl.ds(pl.multiple_of(blk * TQ + a * QR, QR), QR), cx] = x2
                    else:
                        x_v[rs, cx] = x2
                return y

            def o_add(outers, f=o_prod):
                o_todo.extend([(lambda gate, i_=i_, j_=j_: f(i_, j_, gate)) for i_ in outers for j_ in IORD])

            hh = 0
            if last_group and CMODE:
                s0 = par * REP
                if CMODE == 'roll':
                    nxt = qk(s0, a0, 0)
                    for hh in range(REP):
                        cur = nxt
                        if hh + 1 < REP:
                            nxt = qk(s0 + hh + 1, a0, hh + 1)
                        else:
                            o_add(CORD[:2])
                            run(o_todo, 1)
                        pv(s0 + hh, os_, cur)
                        side_c(s0 + hh)
                elif CMODE == 'nat':
                    for hh in range(REP):
                        if hh == 4:
                            o_add(CORD[:2])
                        cur = qk(s0 + hh, a0, hh)
                        run(o_todo, 1)
                        pv(s0 + hh, os_, cur)
                        side_c(s0 + hh)
                else:
                    for hh in range(0, REP, 2):
                        sp0 = qk(s0 + hh, a0, hh)
                        sp1 = qk(s0 + hh + 1, a0, hh + 1)
                        pv(s0 + hh, os_, sp0)
                        side_c(s0 + hh)
                        pv(s0 + hh + 1, os_, sp1)
                        side_c(s0 + hh + 1)
                    o_add(CORD[:2])
                o_add(CORD[2:])
                flush(list(range(32 * par + sum(LCNT), 32 * par + 32)))
                continue
            while hh < REP:
                s_ = par * REP + hh
                if hh == 4:
                    o_add((CORD if last_group else OORD)[:2])
                if not last_group:
                    sp = qk(s_, a0, hh)
                    run(q_todo, min(QRUN[hh], QPRE))
                    pv(s_, os_, sp)
                    run(q_todo, QRUN[hh] - min(QRUN[hh], QPRE))
                    if WSTEP[s_] == 'o':
                        side_b(s_)
                    run(o_todo, ORUN_B[s_])
                    if WSTEP[s_] != 'o':
                        side_b(s_)
                elif not o_todo:
                    sp0 = qk(s_, a0, hh)
                    sp1 = qk(s_ + 1, a0, hh + 1)
                    pv(s_, os_, sp0)
                    side_c(s_)
                    pv(s_ + 1, os_, sp1)
                    side_c(s_ + 1)
                    hh += 1
                else:
                    sp = qk(s_, a0, hh)
                    run(o_todo, 1)
                    pv(s_, os_, sp)
                    run(o_todo, ORUN_C[s_])
                    side_c(s_)
                hh += 1
            o_add((CORD if last_group else OORD)[2:])
        flush([])
        if last_group:
            @pl.when(blk > 0)
            def _():
                out_copy(pl.multiple_of((2 * blk - 1) * TQ, TQ), TQ).start()

            out_copy(pl.multiple_of(2 * blk * TQ, TQ), TQ).start()

    def body_b(i, carry):
        @pl.when(i == 2)
        def _():
            wait_all(wmr_v.at[pl.ds(2, NMC - 2)], SEM_WMR + 1)
            for c_ in wrest_cps:
                c_.wait()

        body(i, False)
        return carry

    with _scope('LB'):
        if 'B' in ONLY:
            lax.fori_loop(0, 3 * NT // 2, body_b, 0)

    wg_cp.wait()
    wu_cp.wait()
    wd_cp.wait()
    sb_ = mod_v[:, 3 * D:4 * D]
    cb1_ = 1.0 + mod_v[:, 4 * D:5 * D]
    gb_ = mod_v[:, 5 * D:6 * D]
    wr8 = wr_v[...].astype(f32)
    wr_ = jnp.concatenate([wr8[r_:r_ + 1, :] for r_ in range(8)], axis=1)
    aux_v[0] = gb_ * cb1_
    aux_v[1] = gb_ * sb_
    aux_v[2] = cb1_ * wr_
    aux_v[3] = jnp.broadcast_to(jnp.sum(sb_ * wr_, axis=-1, keepdims=True), (8, D))

    def body_c(i, carry):
        body(i, True)
        return carry

    with _scope('LC'):
        if 'C' in ONLY:
            lax.fori_loop(0, NT // 2, body_c, 0)

    with _scope('E1_last'):
        ln2_rows(x_v, (NT - 1) * TQ, (NT - 1) * TQ, TQ)
        out_copy((NT - 1) * TQ, TQ).start()

    with _scope('E2_ffn'):
        best = best_v[0]
        bidx = bidx_v[0]
        rmax = jnp.max(best, axis=0, keepdims=True)
        idx_v = jnp.min(jnp.where(best == rmax, bidx, S), axis=0, keepdims=True)
        idx = jnp.minimum(idx_v[0, 0], S - 1)
        g0 = pl.multiple_of((idx // 8) * 8, 8)
        sb = mod_v[:, 3 * D:4 * D]
        cb = mod_v[:, 4 * D:5 * D]
        gb = mod_v[:, 5 * D:6 * D]
        ge = pl.multiple_of((g0 // (2 * TQ)) * TQ + g0 % TQ, 8)
        x2 = jnp.where((g0 // TQ) % 2 == 0, x2e_v[pl.ds(ge, 8), :], x_v[pl.ds(g0, 8), :]).astype(f32)
        h2 = (x2 - best_v[1][:, 0:1]) * best_v[2][:, 0:1] * (1.0 + cb) + sb
        h2b = h2.astype(bf16)
        sel = (lax.broadcasted_iota(jnp.int32, (8, 1), 0) + g0) == idx
        flag = flag_s[0] > 0
        nf = F // 128
        strips = [(k_, j) for j in range(nf) for k_ in 'gu'] + [('d', j) for j in range(FD, nf)]
        gate_r, a_strips, vtok = {}, {}, {}
        y = None
        yv = None
        pos = 0
        for i, (kind, j) in enumerate(strips):
            hi = vtok.get(i - FLAG_)
            if kind == 'd':
                lhs = a_strips[j]
                if hi is not None:
                    lhs = jnp.where(flag, hi.astype(bf16), lhs)
                r_ = jnp.dot(lhs, wd_v[j * 128:(j + 1) * 128, 0:D], preferred_element_type=f32)
                y = r_ if y is None else y + r_
                tok_ = r_[:, D - 128:D]
            else:
                lhs = h2b if hi is None else _gate1(h2b, flag, hi.astype(bf16))
                w_ref = wg_v if kind == 'g' else wu_v
                tok_ = jnp.dot(lhs, w_ref[:, j * 128:(j + 1) * 128], preferred_element_type=f32)
                if kind == 'g':
                    gate_r[j] = tok_
                else:
                    a_strips[j] = (gate_r[j] * jax.nn.sigmoid(gate_r[j]) * tok_).astype(bf16)
                    if j < FD:
                        row = jnp.sum(jnp.where(sel, a_strips[j].astype(f32), 0.0), axis=0, keepdims=True)
                        acol_v[j * 128:(j + 1) * 128, :] = jnp.broadcast_to(row, (128, 128)).T
            if i >= FI0 and pos < FD * 16:
                end = min(pos + FVR // 8, FD * 16) if i < len(strips) - 1 else FD * 16
                for rg in range(pos, end):
                    col = jnp.where(flag, tok_, acol_v[8 * rg:8 * rg + 8, :])
                    pr_ = wd_v[8 * rg:8 * rg + 8, 0:D].astype(f32) * jnp.concatenate([col] * (D // 128), axis=1)
                    yv = pr_ if yv is None else yv + pr_
                pos = end
                vtok[i] = _token(yv)
        y = (y + jnp.sum(yv, axis=0, keepdims=True)) * jax.nn.sigmoid(rmax[:, 0:1])
        if ONLY != 'PBC':
            gz = pl.multiple_of((g0 % 64) // 16 * 16, 16)
            for z in (q_v.at[idx % 2], wqs_v.at[idx % 2], wos_v.at[idx % 2], acc_v, accb_v):
                y = y + z[pl.ds(gz, 16), 0:D].astype(f32)[0:8]
            y = y + kt_v[idx % 4, pl.ds(gz, 16), 0:128].astype(f32)[0:8, 0:1]
        out_copy(0, S).wait()
        new = (x2 + gb * (h2 + y)).astype(bf16)
        out_v[pl.ds(g0, 8), :] = jnp.where(sel, new, out_v[pl.ds(g0, 8), :])
        fix = out_copy(g0, 8)
        fix.start()
        fix.wait()


@jax.jit
def pallas_adaLN_cond__sliding_block_cached__moe_arch_mod__prompt_kernel(
    A_x, A_k_cache, A_v_cache, A_wq, A_wo, B_x, B_w_r, B_w_gate, B_w_up, B_w_down, c, w_mod,
):
    del B_x
    any_spec = pl.BlockSpec(memory_space=pl.ANY)
    return pl.pallas_call(
        _kernel,
        out_shape=jax.ShapeDtypeStruct(A_x.shape, A_x.dtype),
        in_specs=[any_spec] * 11,
        out_specs=any_spec,
        scratch_shapes=[
            pltpu.VMEM((S, D), bf16),
            pltpu.VMEM((S, D), bf16),
            pltpu.VMEM((2, S, GW), bf16),
            pltpu.VMEM((S // 8, 49 * QC), f32),
            pltpu.VMEM((S // 8, 49 * QC), f32),
            pltpu.VMEM((NMC, D, NM * 128), bf16),
            pltpu.VMEM((HKV, D, GW + PADW), bf16),
            pltpu.VMEM((2, QC, 49 * QC), bf16),
            pltpu.VMEM((HKV, GW, D), bf16),
            pltpu.VMEM((2, QC, 49 * QC), bf16),
            pltpu.VMEM((D, F), bf16),
            pltpu.VMEM((D, F), bf16),
            pltpu.VMEM((F, D + PADD), bf16),
            pltpu.VMEM((HKV, W, DH), bf16),
            pltpu.VMEM((HKV, W, DH), bf16),
            pltpu.VMEM((HKV, DH, W), bf16),
            pltpu.VMEM((8, 1, D), bf16),
            pltpu.VMEM((16, 8, 128), bf16),
            pltpu.VMEM((16, D), bf16),
            pltpu.VMEM((D, 128), f32),
            pltpu.VMEM((2 * D, 128), f32),
            pltpu.VMEM((8, 6 * D), f32),
            pltpu.VMEM((8, 8, 128), f32),
            pltpu.VMEM((8, 8, 128), jnp.int32),
            pltpu.VMEM((4, 8, D), f32),
            pltpu.SMEM((1,), jnp.int32),
            pltpu.SemaphoreType.DMA((NSEM,)),
        ],
        compiler_params=pltpu.CompilerParams(vmem_limit_bytes=126 * 1024 * 1024,
                                             disable_semaphore_checks=bool(_p('NOSEM', 1)),
                                             disable_bounds_checks=bool(_p('NOBND', 0))),
    )(A_x, A_k_cache, A_v_cache, A_wq, A_wo, B_w_r.reshape(8, 128), B_w_gate, B_w_up, B_w_down, c, w_mod)
```

```python
import math

import jax
import jax.numpy as jnp
from jax import lax
from jax.experimental import pallas as pl
from jax.experimental.pallas import tpu as pltpu


S = 2048
D = 1024
HQ = 32
HKV = 4
REP = HQ // HKV
DH = 128
GW = REP * DH
W = 512
F = 3584
EPS = 1e-5
TQ = 256
QR = TQ // 4
QC = D // 4
NT = S // TQ
TP = 512
NKC = 4
KC = D // NKC
PADW = 128
PADD = 256
NM = 3
NMC = 11
T3B = 4
NU = QC // 8
FD = 15
FI0 = 8
FLAG_ = 4
FVR = 4
QORD = (3, 6, 5, 1, 2, 7, 4)
OORD = (3, 6, 5, 1, 2, 7, 4)
CORD = (3, 6, 2, 1, 4, 7, 5)
IORD = (4, 2, 1, 7, 5, 3, 6)
QRUN = (6, 6, 6, 7, 6, 6, 6, 6)
ORUN = (6, 6, 7, 6, 7, 5, 6, 6)
LPINS = (24, 80, 136, 192)
WPINS = (32, 64, 96, 128, 160, 192, 224)
NPIN = 192
LHI = 2
OHIC = 3
NHI = 2
GST = 4
GSTB = 6
P3LAG = 4
P3ULAG = 3
P3S = 1
P3US = 0
P3RO = 48
P3URO = 16
P3SP = 192
WTOK = 7
IORDC = (4, 2, 1, 7, 5, 3, 6)
QSCALE = (DH ** -0.5) * math.log2(math.e)

f32 = jnp.float32
bf16 = jnp.bfloat16

(SEM_C, SEM_WR, SEM_X0, SEM_K0, SEM_K, SEM_V, SEM_WG, SEM_WU, SEM_WD, SEM_OUT) = range(10)
SEM_X = 10
SEM_W = SEM_X + NT
SEM_WQ0 = SEM_W + 6
SEM_WM = SEM_WQ0 + NKC
SEM_WMR = SEM_WM + NKC
NSEM = SEM_WMR + 2

A_COEF = {1: ((0, 0, 1), (1, 1, 1)), 2: ((1, 0, 1), (1, 1, 1)), 3: ((0, 0, 1),), 4: ((1, 1, 1),),
          5: ((0, 0, 1), (0, 1, 1)), 6: ((1, 0, 1), (0, 0, -1)), 7: ((0, 1, 1), (1, 1, -1))}
B_COEF = {1: ((0, 0, 1), (1, 1, 1)), 2: ((0, 0, 1),), 3: ((0, 1, 1), (1, 1, -1)), 4: ((1, 0, 1), (0, 0, -1)),
          5: ((1, 1, 1),), 6: ((0, 0, 1), (0, 1, 1)), 7: ((1, 0, 1), (1, 1, 1))}
C_COEF = {(0, 0): {1: 1, 4: 1, 5: -1, 7: 1}, (0, 1): {3: 1, 5: 1}, (1, 0): {2: 1, 4: 1},
          (1, 1): {1: 1, 2: -1, 3: 1, 6: 1}}


def _lin(coef, get):
    v = get(coef[0][0], coef[0][1])
    for r, c, s in coef[1:]:
        v = v + get(r, c) if s > 0 else v - get(r, c)
    return v


def _col(i, j):
    c0 = ((i - 1) * 7 + j - 1) * QC
    return slice(c0, c0 + QC)


class _Combine:
    def __init__(self):
        self.part = {}

    def feed(self, i, v):
        done = []
        for key, coef in C_COEF.items():
            if i not in coef:
                continue
            s = coef[i]
            if key not in self.part:
                cur = (v, s, 1)
            else:
                u, su, n = self.part[key]
                if s == su:
                    cur = (u + v, s, n + 1)
                elif su > 0:
                    cur = (u - v, 1, n + 1)
                else:
                    cur = (v - u, 1, n + 1)
            self.part[key] = cur
            if cur[2] == len(coef):
                assert cur[1] > 0
                done.append((key[0], key[1], cur[0]))
        return done


class _Combine2:
    def __init__(self):
        self.inner = {}
        self.outer = {}

    def feed(self, i, j, v):
        done = []
        for r, c, u in self.inner.setdefault(i, _Combine()).feed(j, v):
            for r2, c2, w in self.outer.setdefault((r, c), _Combine()).feed(i, u):
                done.append((2 * r2 + r, 2 * c2 + c, w))
        return done


class _LhsOps:
    def __init__(self, get, get_bf16=None):
        self.get, self.get_bf16, self.cache = get, get_bf16, {}

    def outer(self, i, a, b):
        if len(A_COEF[i]) == 1:
            r, c, _ = A_COEF[i][0]
            return self.get(2 * r + a, 2 * c + b)
        if (i, a, b) not in self.cache:
            self.cache[i, a, b] = _lin(A_COEF[i], lambda r, c: self.get(2 * r + a, 2 * c + b))
        return self.cache[i, a, b]

    def op(self, i, j):
        if self.get_bf16 is not None and len(A_COEF[i]) == 1 and len(A_COEF[j]) == 1:
            return self.get_bf16(2 * A_COEF[i][0][0] + A_COEF[j][0][0], 2 * A_COEF[i][0][1] + A_COEF[j][0][1])
        return _lin(A_COEF[j], lambda a, b: self.outer(i, a, b)).astype(bf16)


def _ln(x):
    m = jnp.mean(x, axis=-1, keepdims=True)
    xc = x - m
    v = jnp.mean(xc * xc, axis=-1, keepdims=True)
    return xc * lax.rsqrt(v + EPS)


def _recip(l):
    r = pl.reciprocal(l, approx=True)
    return r * (2.0 - l * r)


def _mo(x, m):
    return x if isinstance(x, int) else pl.multiple_of(x, m)


def _rows(v8, n):
    return v8 if n == 8 else jnp.concatenate([v8] * (n // 8), axis=0)


def _gate(x, flag, tok):
    xs = jnp.where(flag, _rows(tok, x.shape[0]), x[:, 0:128])
    return xs if x.shape[1] == 128 else jnp.concatenate([xs, x[:, 128:]], axis=1)


def _gate1(x, flag, tok):
    r = tok.shape[0]
    x0 = jnp.where(flag, tok, x[0:r, 0:128])
    if x.shape[1] > 128:
        x0 = jnp.concatenate([x0, x[0:r, 128:]], axis=1)
    return x0 if x.shape[0] == r else jnp.concatenate([x0, x[r:]], axis=0)


def _token(*ys):
    u = None
    for y in ys:
        for i in range(y.shape[0] // 8):
            for j in range(y.shape[1] // 128):
                v = y[8 * i:8 * i + 8, 128 * j:128 * j + 128]
                u = v if u is None else jnp.maximum(u, v)
    return u


def _kernel(x_hbm, k_hbm, v_hbm, wq_hbm, wo_hbm, wr_hbm, wg_hbm, wu_hbm, wd_hbm, c_hbm, wmod_hbm,
            out_hbm,
            x_v, h_v, q_v, acc_v, accb_v, wmr_v, wq_v, wqs_v, wo_v, wos_v, wg_v, wu_v, wd_v,
            k_v, v_v, kt_v, c_v8, wr_v8, sc_v, scc_v, acol_v, mod_v, best_v, bidx_v, aux_v, flag_s, sems):
    sk = k_hbm.shape[2]
    c_v = c_v8.at[0]
    wr_v = wr_v8.at[0]
    out_v = h_v
    wm_v = wg_v

    def cp(src, dst, i):
        return pltpu.make_async_copy(src, dst, sems.at[i])

    def wait_all(view, sem):
        cp(view, view, sem).wait()

    c_cp = cp(c_hbm, c_v, SEM_C)
    wr_cp = cp(wr_hbm, wr_v, SEM_WR)
    x0_cp = cp(x_hbm.at[0, pl.ds(0, TP), :], x_v.at[pl.ds(0, TP), :], SEM_X0)
    k0_cp = cp(k_hbm.at[0, 0, pl.ds(sk - W, W), :], k_v.at[0], SEM_K0)
    k_cp = cp(k_hbm.at[0, pl.ds(1, HKV - 1), pl.ds(sk - W, W), :], k_v.at[pl.ds(1, HKV - 1)], SEM_K)
    v_cp = cp(v_hbm.at[0, :, pl.ds(sk - W, W), :], v_v, SEM_V)
    wg_cp = cp(wg_hbm, wg_v, SEM_WG)
    wu_cp = cp(wu_hbm, wu_v, SEM_WU)
    wd_cp = cp(wd_hbm, wd_v.at[:, pl.ds(0, D)], SEM_WD)

    def x_cp(t):
        r0 = _mo(t * TQ, TQ)
        return cp(x_hbm.at[0, pl.ds(r0, TQ), :], x_v.at[pl.ds(r0, TQ), :], SEM_X + t)

    def wm_cps(j):
        return [cp(wmod_hbm.at[:, pl.ds(i * D + j * KC, KC)], wm_v.at[:, pl.ds((2 * j + i) * KC, KC)], SEM_WM + j)
                for i in range(2)]

    def wq0_cp(j):
        r0 = _mo(j * KC, KC)
        return cp(wq_hbm.at[pl.ds(r0, KC), pl.ds(0, GW)], wq_v.at[0, pl.ds(r0, KC), pl.ds(0, GW)], SEM_WQ0 + j)

    def wmr_cp(i):
        c0 = 2 * D + min(i * NM, 32 - NM) * 128
        return cp(wmod_hbm.at[:, pl.ds(c0, NM * 128)], wmr_v.at[i], SEM_WMR + (0 if i < 2 else 1))

    def w_cps(s, c, n, sem):
        rows = [(0, D)] if n == 4 else [(_mo(i * QC + c * 64, 64), n * 64) for i in range(4)]
        cps = []
        if s + 1 < HKV:
            cps += [cp(wq_hbm.at[pl.ds(r0, nr), pl.ds((s + 1) * GW, GW)],
                       wq_v.at[s + 1, pl.ds(r0, nr), pl.ds(0, GW)], sem) for r0, nr in rows]
        cps += [cp(wo_hbm.at[pl.ds(s * GW + r0, nr), :], wo_v.at[s, pl.ds(r0, nr), :], sem) for r0, nr in rows]
        return cps

    w1_cps = w_cps(1, 0, 4, SEM_W + 4)
    wrest_cps = w_cps(2, 0, 4, SEM_W + 5) + w_cps(3, 0, 4, SEM_W + 5)

    def out_copy(r0, n):
        return cp(out_v.at[pl.ds(r0, n), :], out_hbm.at[0, pl.ds(r0, n), :], SEM_OUT)

    for c_ in ([c_cp, x0_cp] + [c_ for j in range(NKC) for c_ in wm_cps(j) + [wq0_cp(j)]]
               + [x_cp(2), k0_cp, x_cp(3), x_cp(4), k_cp, x_cp(5), wr_cp] + w_cps(0, 0, 1, SEM_W)
               + [x_cp(6)] + w_cps(0, 1, 1, SEM_W + 1) + [x_cp(7)] + w_cps(0, 2, 1, SEM_W + 2)
               + w_cps(0, 3, 1, SEM_W + 3) + [v_cp, wmr_cp(0), wmr_cp(1)] + w1_cps
               + [wmr_cp(i) for i in range(2, NMC)] + wrest_cps + [wu_cp, wd_cp]):
        c_.start()

    def ln1_rows(r0, n, lo=None):
        x = x_v[pl.ds(r0, n), :].astype(f32)
        if lo is not None:
            x = _gate(x, *lo)
        y = _ln(x) * _rows(mod_v[:, D:2 * D], n) + _rows(mod_v[:, 0:D], n)
        h_v[pl.ds(r0, n), :] = y.astype(bf16)
        return y

    def w_unit(src, dst, u, los):
        r0 = pl.multiple_of(u * 8, 8)

        def load(a, b):
            return src[pl.ds(a * QC + r0, 8), b * QC:(b + 1) * QC].astype(f32)

        toks = []
        for i in range(1, 8):
            flag, tok = los[i - 1]
            outer = {}
            for a in range(2):
                for b in range(2):
                    v = _lin(B_COEF[i], lambda r, c: load(2 * r + a, 2 * c + b))
                    outer[a, b] = jnp.where(flag, jnp.concatenate([tok] * (QC // 128), axis=1), v) if a == b else v
            for j in range(1, 8):
                v = _lin(B_COEF[j], lambda a, b: outer[a, b])
                dst[pl.ds(r0, 8), _col(i, j)] = v.astype(bf16)
                if j >= WTOK:
                    toks.append(v)
        return _token(*toks)

    def ln2_rows(r0, n, valid=None, lo=None):
        av = _rows(aux_v[0], n)
        bv = _rows(aux_v[1], n)
        rv = _rows(aux_v[2], n)
        r_c = _rows(aux_v[3, :, 0:128], n)
        x2 = x_v[pl.ds(r0, n), :].astype(f32)
        if lo is not None:
            x2 = _gate(x2, *lo)
        m = jnp.mean(x2, axis=-1, keepdims=True)
        xc = x2 - m
        var = jnp.mean(xc * xc, axis=-1, keepdims=True)
        rs = lax.rsqrt(var + EPS)
        y = x2 + ((xc * rs) * av + bv)
        r = jnp.sum(xc * rv, axis=-1, keepdims=True) * rs
        out_v[pl.ds(r0, n), :] = y.astype(bf16)
        r = (jnp.broadcast_to(r, (n, 128)) + r_c).astype(bf16).astype(f32)
        if valid is not None:
            r = jnp.where(valid, r, -jnp.inf)
        mb = jnp.broadcast_to(m, (n, 128))
        rsb = jnp.broadcast_to(rs, (n, 128))
        best = best_v[0]
        bm = best_v[1]
        brs = best_v[2]
        bidx = bidx_v[0]
        rows = lax.broadcasted_iota(jnp.int32, (8, 128), 0)
        for j in range(n // 8):
            sl = slice(8 * j, 8 * (j + 1))
            upd = r[sl] > best
            best = jnp.where(upd, r[sl], best)
            bm = jnp.where(upd, mb[sl], bm)
            brs = jnp.where(upd, rsb[sl], brs)
            bidx = jnp.where(upd, rows + (r0 + 8 * j), bidx)
        best_v[0] = best
        best_v[1] = bm
        best_v[2] = brs
        bidx_v[0] = bidx
        return y, best

    flag_s[0] = 0
    c_cp.wait()
    cf = c_v[...].astype(f32)
    sc = (cf * jax.nn.sigmoid(cf)).astype(bf16)
    sc_v[...] = jnp.broadcast_to(sc, (16, D))
    scc_v[...] = jnp.broadcast_to(sc.astype(f32), (128, D)).T
    best_v[0] = jnp.full((8, 128), -jnp.inf, f32)
    best_v[1] = jnp.zeros((8, 128), f32)
    best_v[2] = jnp.zeros((8, 128), f32)
    bidx_v[0] = jnp.zeros((8, 128), jnp.int32)
    x0_cp.wait()

    def norm_rows(i, carry):
        r0 = pl.multiple_of(i * 64, 64)
        for t in range(2):
            (acc_v, accb_v)[t][pl.ds(r0, 64), 0:D] = _ln(x_v[pl.ds(t * TQ + r0, 64), :].astype(f32))
        return carry

    lax.fori_loop(0, TQ // 64, norm_rows, 0)

    def k_chunk(j, carry):
        c0 = pl.multiple_of(j * KC, KC)
        cm = pl.multiple_of(2 * j * KC, 2 * KC)
        wait_all(wm_v.at[:, pl.ds(cm, 2 * KC)], SEM_WM + j)
        md = jnp.dot(sc_v[...], wm_v[:, pl.ds(cm, 2 * KC)], preferred_element_type=f32)[0:8].astype(bf16).astype(f32)
        sa = md[:, 0:KC] * QSCALE
        ca1 = (1.0 + md[:, KC:2 * KC]) * QSCALE
        mod_v[:, pl.ds(c0, KC)] = sa
        mod_v[:, pl.ds(D + c0, KC)] = ca1
        nrm = jnp.concatenate([acc_v[:, pl.ds(c0, KC)], accb_v[:, pl.ds(c0, KC)]], axis=0)
        h_v[0:TP, pl.ds(c0, KC)] = (nrm * _rows(ca1, TP) + _rows(sa, TP)).astype(bf16)
        wq0_cp(j).wait()
        part = jnp.dot(h_v[0:TP, pl.ds(c0, KC)], wq_v[0, pl.ds(c0, KC), 0:GW], preferred_element_type=f32)
        tot = jnp.where(j == 0, 0.0, jnp.concatenate([acc_v[:, D:2 * D], accb_v[:, D:2 * D]], axis=0)) + part
        acc_v[:, D:2 * D] = tot[0:TQ]
        accb_v[:, D:2 * D] = tot[TQ:TP]
        q_v[0, 0:TP, :] = tot.astype(bf16)
        return carry

    lax.fori_loop(0, NKC, k_chunk, 0)

    wg_cp.start()
    x_cp(2).wait()
    ln1_rows(2 * TQ, TQ)
    k0_cp.wait()

    def q0_tile(t, units):
        flag = flag_s[0] > 0
        r0 = pl.multiple_of(t * TQ, TQ)
        rn = jnp.minimum(t + 1, NT - 1) * TQ
        h = h_v[pl.ds(r0, TQ), :]
        jobs = [(lambda lo, r=r: _token(ln1_rows(pl.multiple_of(rn + r, 8), 8, lo))) for r in range(0, TQ, 8)]
        nslot = 2 * REP - P3LAG - P3S
        nuslot = 2 * REP - P3ULAG - P3US
        toks = {}
        n_ = 0
        for j in range(REP):
            q = None
            for kh in range(2):
                hj = h[:, kh * 512:(kh + 1) * 512]
                if n_ in toks:
                    tk = _token(*toks[n_])
                    hj = _gate1(hj, flag, jnp.concatenate([tk, tk], axis=0).astype(bf16))
                y = jnp.dot(hj, wq_v[0, kh * 512:(kh + 1) * 512, j * DH:(j + 1) * DH], preferred_element_type=f32)
                q = y if q is None else q + y
                sl = n_ - P3S
                if 0 <= sl < nslot:
                    mine = jobs[sl * len(jobs) // nslot:(sl + 1) * len(jobs) // nslot]
                    for k_, jb in enumerate(mine):
                        r_ = min(P3RO + k_ * TQ // len(mine), TQ - 8) // 8 * 8
                        toks.setdefault(n_ + P3LAG, []).append(jb((flag, y[r_:r_ + 8])))
                sl = n_ - P3US
                if 0 <= sl < nuslot:
                    mine = units[sl * len(units) // nuslot:(sl + 1) * len(units) // nuslot]
                    for k_, jb in enumerate(mine):
                        rr = [min(P3URO + (k_ * 7 + z) * P3SP // (7 * len(mine)), TQ - 8) // 8 * 8 for z in range(7)]
                        toks.setdefault(n_ + P3ULAG, []).append(jb([(flag, y[r_:r_ + 8]) for r_ in rr]))
                n_ += 1
            q_v[0, pl.ds(r0, TQ), j * DH:(j + 1) * DH] = q.astype(bf16)

    def q0_a(t, carry):
        x_cp(t + 1).wait()

        @pl.when(t == 3)
        def _():
            k_cp.wait()

        q0_tile(t, [])
        gk = jnp.minimum(t - 2, HKV - 1)
        kt_v[gk] = k_v[gk].T
        return carry

    def q0_b(t, carry):
        @pl.when(t + 1 < NT)
        def _():
            x_cp(t + 1).wait()

        for c_ in w_cps(0, t - T3B, 1, SEM_W + t - T3B):
            c_.wait()
        nu = NU // 4
        u0 = (t - T3B) * nu
        units = []
        for u in range(nu):
            units.append(lambda los, u=u: w_unit(wq_v.at[1], wqs_v.at[1], u0 + u, los))
            units.append(lambda los, u=u: w_unit(wo_v.at[0], wos_v.at[0], u0 + u, los))
        q0_tile(t, units)
        gk = jnp.minimum(t - 2, HKV - 1)
        kt_v[gk] = k_v[gk].T
        return carry

    lax.fori_loop(2, T3B, q0_a, 0)
    lax.fori_loop(T3B, NT, q0_b, 0)
    v_cp.wait()
    wr_cp.wait()
    wait_all(wmr_v.at[pl.ds(0, 2)], SEM_WMR)
    for c_ in w1_cps:
        c_.wait()

    def body(i, last_group):
        flag = flag_s[0] > 0
        st = {}
        his = {}
        g = 3 if last_group else i // (NT // 2)
        qs = g % 2
        blk = i % (NT // 2)
        m0 = pl.multiple_of(blk * QR, QR)
        o_todo = []

        def pin(r_):
            return flag, st['V'][r_:r_ + 8]

        def add_hi(step, tk):
            his[step] = tk if step not in his else jnp.maximum(his[step], tk)

        def run(todo, n):
            for _ in range(n):
                todo.pop(0)(None)

        def flush():
            gates = {(GST if last_group else GSTB) * (k_ + 1): his.pop(s_) for k_, s_ in enumerate(sorted(his))}
            for k_ in range(len(o_todo)):
                o_todo.pop(0)(gates.get(k_))

        def qk(step, a0, hh):
            s = jnp.dot(q_v[qs, pl.ds(a0, TQ), hh * DH:(hh + 1) * DH], kt_v[g], preferred_element_type=f32)
            if step in his:
                s = _gate1(s, flag, his.pop(step))
            p = jnp.exp2(s - jnp.max(s, axis=-1, keepdims=True))
            ps = (p[:, 0:128] + p[:, 128:256]) + (p[:, 256:384] + p[:, 384:512])
            p = jnp.concatenate([p[:, 0:384], jnp.where(flag, ps, p[:, 384:512])], axis=1)
            return p.astype(bf16), jnp.sum(ps, axis=-1, keepdims=True)

        def pv(step, os_, pl_):
            p, l = pl_
            o = jnp.dot(p, v_v[g], preferred_element_type=f32)
            st['V'] = o
            os_.append(o * _recip(l))
            if last_group:
                add_hi(step + OHIC, _token(os_[-1]))

        def side_b(s_):
            u = (i % 4) * (NU // 4) + s_ % REP
            los = [pin(r_) for r_ in WPINS]
            if s_ < REP:
                add_hi(s_ + 1, w_unit(wo_v.at[g + 1], wos_v.at[1 - qs], u, los))
            else:
                gq = jnp.minimum(g + 2, HKV - 1)
                add_hi(s_ + 1, w_unit(wq_v.at[gq], wqs_v.at[gq % 2], u, los))
            nn = 2 * REP - NHI
            ci = jnp.minimum(i, NMC - 1)
            if s_ < nn:
                lo = pin(NPIN)
                macc = st.get('macc')
                for rg in range(128 * s_ // nn, 128 * (s_ + 1) // nn):
                    xc_ = jnp.where(lo[0], lo[1], scc_v[8 * rg:8 * rg + 8, :])
                    pr_ = wmr_v[ci, 8 * rg:8 * rg + 8, :].astype(f32) * jnp.concatenate([xc_] * NM, axis=1)
                    macc = pr_ if macc is None else macc + pr_
                st['macc'] = macc
                add_hi(s_ + NHI, _token(macc))
                if s_ == nn - 1:
                    c0 = pl.multiple_of(2 * D + jnp.minimum(ci * NM, 32 - NM) * 128, 128)
                    tot_ = jnp.sum(macc, axis=0, keepdims=True).astype(bf16).astype(f32)
                    mod_v[:, pl.ds(c0, NM * 128)] = jnp.broadcast_to(tot_, (8, NM * 128))

        def side_c(s_):
            for k_, r_ in enumerate(LPINS):
                off = ((s_ % REP) * len(LPINS) + k_) * 8
                if s_ < REP:
                    res = ln2_rows(pl.multiple_of(jnp.maximum(2 * blk - 1, 0) * TQ + off, 8), 8, blk > 0, pin(r_))
                else:
                    res = ln2_rows(pl.multiple_of(2 * blk * TQ + off, 8), 8, None, pin(r_))
                add_hi(s_ + LHI, _token(*res))

        for par in range(2):
            a0 = pl.multiple_of((2 * blk + par) * TQ, TQ)
            acc = (acc_v, accb_v)[par]
            os_ = []

            def h_blk(a, b, a0=a0):
                return h_v[pl.ds(pl.multiple_of(a0 + a * QR, QR), QR), b * QC:(b + 1) * QC]

            q_lhs = _LhsOps(lambda a, b, f=h_blk: f(a, b).astype(f32), h_blk)
            q_comb = _Combine2()

            def q_prod(i_, j_, a0=a0, q_lhs=q_lhs, q_comb=q_comb):
                y = jnp.dot(q_lhs.op(i_, j_), wqs_v[1 - qs, :, _col(i_, j_)], preferred_element_type=f32)
                for a, b, v in q_comb.feed(i_, j_, y):
                    r0 = pl.multiple_of(a0 + a * QR, QR)
                    q_v[1 - qs, pl.ds(r0, QR), b * QC:(b + 1) * QC] = v.astype(bf16)

            q_todo = [(lambda gate, i_=i_, j_=j_, f=q_prod: f(i_, j_)) for i_ in QORD for j_ in IORD]
            o_lhs = _LhsOps(lambda a, b, os_=os_: jnp.concatenate(
                [os_[2 * b][a * QR:(a + 1) * QR], os_[2 * b + 1][a * QR:(a + 1) * QR]], axis=1))
            o_comb = _Combine2()

            def o_prod(i_, j_, gate, acc=acc, o_lhs=o_lhs, o_comb=o_comb, a0=a0):
                lhs = o_lhs.op(i_, j_)
                if gate is not None:
                    lhs = _gate1(lhs, flag, jnp.concatenate([gate, gate], axis=0).astype(bf16))
                y = jnp.dot(lhs, wos_v[qs, :, _col(i_, j_)], preferred_element_type=f32)
                old = acc[pl.ds(m0, QR), _col(i_, j_)]
                if not last_group:
                    acc[pl.ds(m0, QR), _col(i_, j_)] = jnp.where(g == 0, 0.0, old) + y
                    return
                for a, b, v in o_comb.feed(i_, j_, old + y):
                    rs = pl.ds(pl.multiple_of(a0 + a * QR, QR), QR)
                    cx = slice(b * QC, (b + 1) * QC)
                    ga = _rows(mod_v[:, 2 * D + b * QC:2 * D + (b + 1) * QC], QR)
                    x_v[rs, cx] = (x_v[rs, cx].astype(f32) + ga * v).astype(bf16)

            s0 = par * REP
            if last_group:
                for hh in range(0, REP, 2):
                    sp0 = qk(s0 + hh, a0, hh)
                    sp1 = qk(s0 + hh + 1, a0, hh + 1)
                    pv(s0 + hh, os_, sp0)
                    side_c(s0 + hh)
                    pv(s0 + hh + 1, os_, sp1)
                    side_c(s0 + hh + 1)
            else:
                for hh in range(REP):
                    sp = qk(s0 + hh, a0, hh)
                    run(q_todo, QRUN[hh])
                    pv(s0 + hh, os_, sp)
                    if par == 1:
                        run(o_todo, ORUN[hh])
                    side_b(s0 + hh)
            o_todo.extend([(lambda gate, i_=i_, j_=j_, f=o_prod: f(i_, j_, gate))
                           for i_ in (CORD if last_group else OORD) for j_ in (IORDC if last_group else IORD)])
            if last_group or par == 1:
                flush()
        if last_group:
            @pl.when(blk > 0)
            def _():
                out_copy(pl.multiple_of((2 * blk - 1) * TQ, TQ), TQ).start()

            out_copy(pl.multiple_of(2 * blk * TQ, TQ), TQ).start()

    def body_b(i, carry):
        @pl.when(i == 2)
        def _():
            wait_all(wmr_v.at[pl.ds(2, NMC - 2)], SEM_WMR + 1)
            for c_ in wrest_cps:
                c_.wait()

        body(i, False)
        return carry

    lax.fori_loop(0, 3 * NT // 2, body_b, 0)

    wg_cp.wait()
    wu_cp.wait()
    wd_cp.wait()
    sb_ = mod_v[:, 3 * D:4 * D]
    cb1_ = 1.0 + mod_v[:, 4 * D:5 * D]
    gb_ = mod_v[:, 5 * D:6 * D]
    wr8 = wr_v[...].astype(f32)
    wr_ = jnp.concatenate([wr8[r_:r_ + 1, :] for r_ in range(8)], axis=1)
    aux_v[0] = gb_ * cb1_
    aux_v[1] = gb_ * sb_
    aux_v[2] = cb1_ * wr_
    aux_v[3] = jnp.broadcast_to(jnp.sum(sb_ * wr_, axis=-1, keepdims=True), (8, D))

    def body_c(i, carry):
        body(i, True)
        return carry

    lax.fori_loop(0, NT // 2, body_c, 0)

    ln2_rows((NT - 1) * TQ, TQ)
    out_copy((NT - 1) * TQ, TQ).start()

    best = best_v[0]
    bidx = bidx_v[0]
    rmax = jnp.max(best, axis=0, keepdims=True)
    idx_v = jnp.min(jnp.where(best == rmax, bidx, S), axis=0, keepdims=True)
    idx = jnp.minimum(idx_v[0, 0], S - 1)
    g0 = pl.multiple_of((idx // 8) * 8, 8)
    sb = mod_v[:, 3 * D:4 * D]
    cb = mod_v[:, 4 * D:5 * D]
    gb = mod_v[:, 5 * D:6 * D]
    x2 = x_v[pl.ds(g0, 8), :].astype(f32)
    h2 = (x2 - best_v[1][:, 0:1]) * best_v[2][:, 0:1] * (1.0 + cb) + sb
    h2b = h2.astype(bf16)
    sel = (lax.broadcasted_iota(jnp.int32, (8, 1), 0) + g0) == idx
    flag = flag_s[0] > 0
    nf = F // 128
    strips = [(k_, j) for j in range(nf) for k_ in 'gu'] + [('d', j) for j in range(FD, nf)]
    gate_r, a_strips, vtok = {}, {}, {}
    y = None
    yv = None
    pos = 0
    for i, (kind, j) in enumerate(strips):
        hi = vtok.get(i - FLAG_)
        if kind == 'd':
            lhs = a_strips[j]
            if hi is not None:
                lhs = jnp.where(flag, hi.astype(bf16), lhs)
            r_ = jnp.dot(lhs, wd_v[j * 128:(j + 1) * 128, 0:D], preferred_element_type=f32)
            y = r_ if y is None else y + r_
            tok_ = r_[:, D - 128:D]
        else:
            lhs = h2b if hi is None else _gate1(h2b, flag, hi.astype(bf16))
            w_ref = wg_v if kind == 'g' else wu_v
            tok_ = jnp.dot(lhs, w_ref[:, j * 128:(j + 1) * 128], preferred_element_type=f32)
            if kind == 'g':
                gate_r[j] = tok_
            else:
                a_strips[j] = (gate_r[j] * jax.nn.sigmoid(gate_r[j]) * tok_).astype(bf16)
                if j < FD:
                    row = jnp.sum(jnp.where(sel, a_strips[j].astype(f32), 0.0), axis=0, keepdims=True)
                    acol_v[j * 128:(j + 1) * 128, :] = jnp.broadcast_to(row, (128, 128)).T
        if i >= FI0 and pos < FD * 16:
            end = min(pos + FVR, FD * 16) if i < len(strips) - 1 else FD * 16
            for rg in range(pos, end):
                col = jnp.where(flag, tok_, acol_v[8 * rg:8 * rg + 8, :])
                pr_ = wd_v[8 * rg:8 * rg + 8, 0:D].astype(f32) * jnp.concatenate([col] * (D // 128), axis=1)
                yv = pr_ if yv is None else yv + pr_
            pos = end
            vtok[i] = _token(yv)
    y = (y + jnp.sum(yv, axis=0, keepdims=True)) * jax.nn.sigmoid(rmax[:, 0:1])
    out_copy(0, S).wait()
    new = (x2 + gb * (h2 + y)).astype(bf16)
    out_v[pl.ds(g0, 8), :] = jnp.where(sel, new, out_v[pl.ds(g0, 8), :])
    fix = out_copy(g0, 8)
    fix.start()
    fix.wait()


@jax.jit
def pallas_adaLN_cond__sliding_block_cached__moe_arch_mod__prompt_kernel(
    A_x, A_k_cache, A_v_cache, A_wq, A_wo, B_x, B_w_r, B_w_gate, B_w_up, B_w_down, c, w_mod,
):
    del B_x
    any_spec = pl.BlockSpec(memory_space=pl.ANY)
    return pl.pallas_call(
        _kernel,
        out_shape=jax.ShapeDtypeStruct(A_x.shape, A_x.dtype),
        in_specs=[any_spec] * 11,
        out_specs=any_spec,
        scratch_shapes=[
            pltpu.VMEM((S, D), bf16),
            pltpu.VMEM((S, D), bf16),
            pltpu.VMEM((2, S, GW), bf16),
            pltpu.VMEM((S // 8, 49 * QC), f32),
            pltpu.VMEM((S // 8, 49 * QC), f32),
            pltpu.VMEM((NMC, D, NM * 128), bf16),
            pltpu.VMEM((HKV, D, GW + PADW), bf16),
            pltpu.VMEM((2, QC, 49 * QC), bf16),
            pltpu.VMEM((HKV, GW, D), bf16),
            pltpu.VMEM((2, QC, 49 * QC), bf16),
            pltpu.VMEM((D, F), bf16),
            pltpu.VMEM((D, F), bf16),
            pltpu.VMEM((F, D + PADD), bf16),
            pltpu.VMEM((HKV, W, DH), bf16),
            pltpu.VMEM((HKV, W, DH), bf16),
            pltpu.VMEM((HKV, DH, W), bf16),
            pltpu.VMEM((8, 1, D), bf16),
            pltpu.VMEM((16, 8, 128), bf16),
            pltpu.VMEM((16, D), bf16),
            pltpu.VMEM((D, 128), f32),
            pltpu.VMEM((2 * D, 128), f32),
            pltpu.VMEM((8, 6 * D), f32),
            pltpu.VMEM((8, 8, 128), f32),
            pltpu.VMEM((8, 8, 128), jnp.int32),
            pltpu.VMEM((4, 8, D), f32),
            pltpu.SMEM((1,), jnp.int32),
            pltpu.SemaphoreType.DMA((NSEM,)),
        ],
        compiler_params=pltpu.CompilerParams(vmem_limit_bytes=126 * 1024 * 1024,
                                             disable_semaphore_checks=True,
                                             disable_bounds_checks=False),
    )(A_x, A_k_cache, A_v_cache, A_wq, A_wo, B_w_r.reshape(8, 128), B_w_gate, B_w_up, B_w_down, c, w_mod)
```

```python
import math

import jax
import jax.numpy as jnp
from jax import lax
from jax.experimental import pallas as pl
from jax.experimental.pallas import tpu as pltpu


S = 2048
D = 1024
HQ = 32
HKV = 4
REP = HQ // HKV
DH = 128
GW = REP * DH
W = 512
F = 3584
EPS = 1e-5
TQ = 256
QR = TQ // 4
QC = D // 4
NT = S // TQ
TP = 512
NKC = 4
HR = TQ // 2
KH = D // 2
PADW = 128
PADD = 256
NM = 3
NMC = 11
T3B = 4
NU = QC // 8
FD = 15
FI0 = 8
FLAG_ = 4
FVR = 4
QORD = (3, 6, 5, 1, 2, 7, 4)
OORD = (3, 6, 5, 1, 2, 7, 4)
CORD = (3, 6, 2, 1, 4, 7, 5)
IORD = (4, 2, 1, 7, 5, 3, 6)
QRUN = (6, 6, 6, 7, 6, 6, 6, 6)
ORUN = (6, 6, 7, 6, 7, 5, 6, 6)
LPINS = (24, 80, 136, 192)
WPINS = (32, 64, 96, 128, 160, 192, 224)
NPIN = 192
LHI = 2
OHIC = 3
NHI = 2
GST = 4
GSTB = 6
WTOK = 7
F2N = 5
NL3 = 59
NLB = -(-(128 - NL3) // 3)
A2S = 9
A2LAG = 5
A3S = 2
A3LAG = 6
Q1ORD = (4, 2, 7, 1, 5, 3, 6)
Q1SP = 160
Q1S = 4
Q1LAG = 5
Q1US = 2
Q1ULAG = 3
IORDC = (4, 2, 1, 7, 5, 3, 6)
QSCALE = (DH ** -0.5) * math.log2(math.e)

f32 = jnp.float32
bf16 = jnp.bfloat16

(SEM_C, SEM_WR, SEM_X0, SEM_K, SEM_V, SEM_WG, SEM_WU, SEM_WD, SEM_OUT) = range(9)
SEM_X = 9
SEM_W = SEM_X + NT
SEM_WQ0 = SEM_W + 6
SEM_WM = SEM_WQ0 + NKC
SEM_WMR = SEM_WM + NKC
NSEM = SEM_WMR + 2

A_COEF = {1: ((0, 0, 1), (1, 1, 1)), 2: ((1, 0, 1), (1, 1, 1)), 3: ((0, 0, 1),), 4: ((1, 1, 1),),
          5: ((0, 0, 1), (0, 1, 1)), 6: ((1, 0, 1), (0, 0, -1)), 7: ((0, 1, 1), (1, 1, -1))}
B_COEF = {1: ((0, 0, 1), (1, 1, 1)), 2: ((0, 0, 1),), 3: ((0, 1, 1), (1, 1, -1)), 4: ((1, 0, 1), (0, 0, -1)),
          5: ((1, 1, 1),), 6: ((0, 0, 1), (0, 1, 1)), 7: ((1, 0, 1), (1, 1, 1))}
C_COEF = {(0, 0): {1: 1, 4: 1, 5: -1, 7: 1}, (0, 1): {3: 1, 5: 1}, (1, 0): {2: 1, 4: 1},
          (1, 1): {1: 1, 2: -1, 3: 1, 6: 1}}


B_SUMS = (1, 3, 4, 6, 7)


def _lin(coef, get):
    v = get(coef[0][0], coef[0][1])
    for r, c, s in coef[1:]:
        v = v + get(r, c) if s > 0 else v - get(r, c)
    return v


def _col(i, j):
    c0 = ((i - 1) * 7 + j - 1) * QC
    return slice(c0, c0 + QC)


class _Combine:
    def __init__(self):
        self.part = {}

    def feed(self, i, v):
        done = []
        for key, coef in C_COEF.items():
            if i not in coef:
                continue
            s = coef[i]
            if key not in self.part:
                cur = (v, s, 1)
            else:
                u, su, n = self.part[key]
                if s == su:
                    cur = (u + v, s, n + 1)
                elif su > 0:
                    cur = (u - v, 1, n + 1)
                else:
                    cur = (v - u, 1, n + 1)
            self.part[key] = cur
            if cur[2] == len(coef):
                assert cur[1] > 0
                done.append((key[0], key[1], cur[0]))
        return done


class _Combine2:
    def __init__(self):
        self.inner = {}
        self.outer = {}

    def feed(self, i, j, v):
        done = []
        for r, c, u in self.inner.setdefault(i, _Combine()).feed(j, v):
            for r2, c2, w in self.outer.setdefault((r, c), _Combine()).feed(i, u):
                done.append((2 * r2 + r, 2 * c2 + c, w))
        return done


class _LhsOps:
    def __init__(self, get, get_bf16=None):
        self.get, self.get_bf16, self.cache = get, get_bf16, {}

    def outer(self, i, a, b):
        if len(A_COEF[i]) == 1:
            r, c, _ = A_COEF[i][0]
            return self.get(2 * r + a, 2 * c + b)
        if (i, a, b) not in self.cache:
            self.cache[i, a, b] = _lin(A_COEF[i], lambda r, c: self.get(2 * r + a, 2 * c + b))
        return self.cache[i, a, b]

    def op(self, i, j):
        if self.get_bf16 is not None and len(A_COEF[i]) == 1 and len(A_COEF[j]) == 1:
            return self.get_bf16(2 * A_COEF[i][0][0] + A_COEF[j][0][0], 2 * A_COEF[i][0][1] + A_COEF[j][0][1])
        return _lin(A_COEF[j], lambda a, b: self.outer(i, a, b)).astype(bf16)


def _ln(x):
    m = jnp.mean(x, axis=-1, keepdims=True)
    xc = x - m
    v = jnp.mean(xc * xc, axis=-1, keepdims=True)
    return xc * lax.rsqrt(v + EPS)


def _recip(l):
    r = pl.reciprocal(l, approx=True)
    return r * (2.0 - l * r)


def _mo(x, m):
    return x if isinstance(x, int) else pl.multiple_of(x, m)


def _rows(v8, n):
    return v8 if n == 8 else jnp.concatenate([v8] * (n // 8), axis=0)


def _gate(x, flag, tok):
    xs = jnp.where(flag, _rows(tok, x.shape[0]), x[:, 0:128])
    return xs if x.shape[1] == 128 else jnp.concatenate([xs, x[:, 128:]], axis=1)


def _gate1(x, flag, tok):
    r = tok.shape[0]
    x0 = jnp.where(flag, tok, x[0:r, 0:128])
    if x.shape[1] > 128:
        x0 = jnp.concatenate([x0, x[0:r, 128:]], axis=1)
    return x0 if x.shape[0] == r else jnp.concatenate([x0, x[r:]], axis=0)


def _token(*ys):
    u = None
    for y in ys:
        for i in range(y.shape[0] // 8):
            for j in range(y.shape[1] // 128):
                v = y[8 * i:8 * i + 8, 128 * j:128 * j + 128]
                u = v if u is None else jnp.maximum(u, v)
    return u


def _kernel(x_hbm, k_hbm, v_hbm, wq_hbm, wo_hbm, wr_hbm, wg_hbm, wu_hbm, wd_hbm, c_hbm, wmod_hbm,
            out_hbm,
            x_v, h_v, q_v, acc_v, accb_v, wmr_v, wq_v, wqs_v, wo_v, wos_v, wg_v, wu_v, wd_v,
            k_v, v_v, kt_v, c_v8, wr_v8, sc_v, scc_v, acol_v, mod_v, best_v, bidx_v, aux_v, flag_s, sems):
    sk = k_hbm.shape[2]
    c_v = c_v8.at[0]
    wr_v = wr_v8.at[0]
    out_v = h_v
    wq1_v = wu_v
    wm_v = wg_v

    def cp(src, dst, i):
        return pltpu.make_async_copy(src, dst, sems.at[i])

    def wait_all(view, sem):
        cp(view, view, sem).wait()

    c_cp = cp(c_hbm, c_v, SEM_C)
    wr_cp = cp(wr_hbm, wr_v, SEM_WR)
    x0_cp = cp(x_hbm.at[0, pl.ds(0, TP), :], x_v.at[pl.ds(0, TP), :], SEM_X0)
    k_cp = cp(k_hbm.at[0, :, pl.ds(sk - W, W), :], k_v, SEM_K)
    v_cp = cp(v_hbm.at[0, :, pl.ds(sk - W, W), :], v_v, SEM_V)
    wg_cp = cp(wg_hbm, wg_v, SEM_WG)
    wu_cp = cp(wu_hbm, wu_v, SEM_WU)
    wd_cp = cp(wd_hbm, wd_v.at[:, pl.ds(0, D)], SEM_WD)

    def x_cp(t):
        r0 = _mo(t * TQ, TQ)
        return cp(x_hbm.at[0, pl.ds(r0, TQ), :], x_v.at[pl.ds(r0, TQ), :], SEM_X + t)

    def wm_cps(j):
        return [cp(wmod_hbm.at[:, pl.ds(i * KH + j * 128, 128)], wm_v.at[:, pl.ds((4 * j + i) * 128, 128)], SEM_WM + j)
                for i in range(4)]

    def wq0_cps(j):
        return [cp(wq_hbm.at[pl.ds(_mo(i * KH + j * 128, 128), 128), pl.ds(0, GW)],
                   wq_v.at[0, pl.ds(_mo(i * KH + j * 128, 128), 128), pl.ds(0, GW)], SEM_WQ0 + j) for i in range(2)]

    def wmr_cp(i):
        c0 = 2 * D + min(i * NM, 32 - NM) * 128
        return cp(wmod_hbm.at[:, pl.ds(c0, NM * 128)], wmr_v.at[i], SEM_WMR + (0 if i < 2 else 1))

    def w_cps(s, c, n, sem):
        rows = [(0, D)] if n == 4 else [(_mo(i * QC + c * 64, 64), n * 64) for i in range(4)]
        cps = []
        if s + 1 < HKV:
            cps += [cp(wq_hbm.at[pl.ds(r0, nr), pl.ds((s + 1) * GW, GW)],
                       wq_v.at[s + 1, pl.ds(r0, nr), pl.ds(0, GW)], sem) for r0, nr in rows]
        cps += [cp(wo_hbm.at[pl.ds(s * GW + r0, nr), :], wo_v.at[s, pl.ds(r0, nr), :], sem) for r0, nr in rows]
        return cps

    w1_cps = w_cps(1, 0, 2, SEM_W + 4)
    wrest_cps = w_cps(1, 2, 2, SEM_W + 5) + w_cps(2, 0, 4, SEM_W + 5) + w_cps(3, 0, 4, SEM_W + 5)

    def out_copy(r0, n):
        return cp(out_v.at[pl.ds(r0, n), :], out_hbm.at[0, pl.ds(r0, n), :], SEM_OUT)

    for c_ in ([c_cp, x0_cp] + [c_ for j in range(NKC) for c_ in wm_cps(j) + wq0_cps(j)]
               + [x_cp(2), x_cp(3), x_cp(4), x_cp(5), k_cp, wr_cp, x_cp(6)] + w_cps(0, 0, 1, SEM_W)
               + [x_cp(7)] + w_cps(0, 1, 1, SEM_W + 1)):
        c_.start()

    def ln1_rows(r0, n, lo=None):
        x = x_v[pl.ds(r0, n), :].astype(f32)
        if lo is not None:
            x = _gate(x, *lo)
        y = _ln(x) * _rows(mod_v[:, D:2 * D], n) + _rows(mod_v[:, 0:D], n)
        h_v[pl.ds(r0, n), :] = y.astype(bf16)
        return y

    def w_unit(src, dst, u, los):
        r0 = pl.multiple_of(u * 8, 8)

        def load(a, b):
            return src[pl.ds(a * QC + r0, 8), b * QC:(b + 1) * QC].astype(f32)

        toks = []
        for i in range(1, 8):
            flag, tok = los[i - 1]
            outer = {}
            for a in range(2):
                for b in range(2):
                    v = _lin(B_COEF[i], lambda r, c: load(2 * r + a, 2 * c + b))
                    outer[a, b] = jnp.where(flag, jnp.concatenate([tok] * (QC // 128), axis=1), v) if a == b else v
            for j in range(1, 8):
                v = _lin(B_COEF[j], lambda a, b: outer[a, b])
                dst[pl.ds(r0, 8), _col(i, j)] = v.astype(bf16)
                if j >= WTOK:
                    toks.append(v)
        return _token(*toks)

    def ln2_rows(r0, n, valid=None, lo=None):
        av = _rows(aux_v[0], n)
        bv = _rows(aux_v[1], n)
        rv = _rows(aux_v[2], n)
        r_c = _rows(aux_v[3, :, 0:128], n)
        x2 = x_v[pl.ds(r0, n), :].astype(f32)
        if lo is not None:
            x2 = _gate(x2, *lo)
        m = jnp.mean(x2, axis=-1, keepdims=True)
        xc = x2 - m
        var = jnp.mean(xc * xc, axis=-1, keepdims=True)
        rs = lax.rsqrt(var + EPS)
        y = x2 + ((xc * rs) * av + bv)
        r = jnp.sum(xc * rv, axis=-1, keepdims=True) * rs
        out_v[pl.ds(r0, n), :] = y.astype(bf16)
        r = (jnp.broadcast_to(r, (n, 128)) + r_c).astype(bf16).astype(f32)
        if valid is not None:
            r = jnp.where(valid, r, -jnp.inf)
        mb = jnp.broadcast_to(m, (n, 128))
        rsb = jnp.broadcast_to(rs, (n, 128))
        best = best_v[0]
        bm = best_v[1]
        brs = best_v[2]
        bidx = bidx_v[0]
        rows = lax.broadcasted_iota(jnp.int32, (8, 128), 0)
        for j in range(n // 8):
            sl = slice(8 * j, 8 * (j + 1))
            upd = r[sl] > best
            best = jnp.where(upd, r[sl], best)
            bm = jnp.where(upd, mb[sl], bm)
            brs = jnp.where(upd, rsb[sl], brs)
            bidx = jnp.where(upd, rows + (r0 + 8 * j), bidx)
        best_v[0] = best
        best_v[1] = bm
        best_v[2] = brs
        bidx_v[0] = bidx
        return y, best

    flag_s[0] = 0
    c_cp.wait()
    cf = c_v[...].astype(f32)
    sc = (cf * jax.nn.sigmoid(cf)).astype(bf16)
    sc_v[...] = jnp.broadcast_to(sc, (16, D))
    scc_v[...] = jnp.broadcast_to(sc.astype(f32), (128, D)).T
    best_v[0] = jnp.full((8, 128), -jnp.inf, f32)
    best_v[1] = jnp.zeros((8, 128), f32)
    best_v[2] = jnp.zeros((8, 128), f32)
    bidx_v[0] = jnp.zeros((8, 128), jnp.int32)
    x0_cp.wait()

    def norm_rows(i, carry):
        r0 = pl.multiple_of(i * 64, 64)
        for t in range(2):
            (acc_v, accb_v)[t][pl.ds(r0, 64), 0:D] = _ln(x_v[pl.ds(t * TQ + r0, 64), :].astype(f32))
        return carry

    lax.fori_loop(0, TQ // 64, norm_rows, 0)

    def w1_unit(u, lo):
        r0 = pl.multiple_of(u * 8, 8)
        half = (_gate(wq_v[0, pl.ds(r0, 8), 0:GW].astype(f32), *lo), wq_v[0, pl.ds(KH + r0, 8), 0:GW].astype(f32))
        outs = [_lin(B_COEF[i], lambda r, c: half[r][:, (2 * p + c) * DH:(2 * p + c + 1) * DH])
                for p in range(REP // 2) for i in B_SUMS]
        wq1_v[pl.ds(r0, 8), 0:len(outs) * DH] = jnp.concatenate(outs, axis=1).astype(bf16)
        return _token(*[o_ for i, o_ in enumerate(outs) if i % 5 >= 3])

    def k_chunk(j, carry):
        cm = pl.multiple_of(j * 512, 512)
        wait_all(wm_v.at[:, pl.ds(cm, 512)], SEM_WM + j)
        cols = (pl.multiple_of(j * 128, 128), pl.multiple_of(KH + j * 128, 128))
        md = jnp.dot(sc_v[...], wm_v[:, pl.ds(cm, 512)], preferred_element_type=f32)[0:8].astype(bf16).astype(f32)
        for i, c0 in enumerate(cols):
            sa = md[:, i * 128:(i + 1) * 128] * QSCALE
            ca1 = (1.0 + md[:, (2 + i) * 128:(3 + i) * 128]) * QSCALE
            mod_v[:, pl.ds(c0, 128)] = sa
            mod_v[:, pl.ds(D + c0, 128)] = ca1
            nrm = jnp.concatenate([acc_v[:, pl.ds(c0, 128)], accb_v[:, pl.ds(c0, 128)]], axis=0)
            h_v[0:TP, pl.ds(c0, 128)] = (nrm * _rows(ca1, TP) + _rows(sa, TP)).astype(bf16)
        for c_ in wq0_cps(j):
            c_.wait()
        lhs = jnp.concatenate([h_v[0:TP, pl.ds(c0, 128)] for c0 in cols], axis=1)
        rhs = jnp.concatenate([wq_v[0, pl.ds(c0, 128), 0:GW] for c0 in cols], axis=0)
        flag = flag_s[0] > 0
        toks = {}
        for n_ in range(4):
            cs = slice(D + n_ * 256, D + (n_ + 1) * 256)
            lh = lhs
            if n_ - 2 in toks:
                lh = _gate1(lhs, flag, jnp.concatenate([toks[n_ - 2]] * 2, axis=0).astype(bf16))
            part = jnp.dot(lh, rhs[:, n_ * 256:(n_ + 1) * 256], preferred_element_type=f32)
            tot = jnp.where(j == 0, 0.0, jnp.concatenate([acc_v[:, cs], accb_v[:, cs]], axis=0)) + part
            acc_v[:, cs] = tot[0:TQ]
            accb_v[:, cs] = tot[TQ:TP]
            q_v[0, 0:TP, n_ * 256:(n_ + 1) * 256] = tot.astype(bf16)
            if n_ < 2:
                toks[n_] = _token(*[w1_unit(j * 16 + n_ * 8 + u, (flag, part[64 * u:64 * u + 8, 0:128]))
                                    for u in range(8)])
        return carry

    lax.fori_loop(0, NKC, k_chunk, 0)

    for c_ in (w_cps(0, 2, 1, SEM_W + 2) + w_cps(0, 3, 1, SEM_W + 3) + [v_cp, wmr_cp(0), wmr_cp(1)] + w1_cps
               + [wmr_cp(i) for i in range(2, NMC)] + wrest_cps + [wd_cp, wg_cp]):
        c_.start()
    x_cp(2).wait()
    x_cp(3).wait()

    def q0_tile(t, rn, nln, units, q1s, q1lag, first=False):
        flag = flag_s[0] > 0
        a0 = _mo(t * TQ, TQ)
        h = h_v.at[pl.ds(a0, TQ), :] if first else h_v[pl.ds(a0, TQ), :]
        lhs = {}

        def hb(r, c):
            return h[r * HR:(r + 1) * HR, c * KH:(c + 1) * KH]

        def get_lhs(i):
            if i not in lhs:
                lhs[i] = (hb(*A_COEF[i][0][:2]) if len(A_COEF[i]) == 1 else
                          _lin(A_COEF[i], lambda r, c: hb(r, c).astype(f32)).astype(bf16))
            return lhs[i]

        prods = [(p, i) for p in range(REP // 2) for i in Q1ORD]
        if first:
            prods = [z for z in prods if z[1] in (4, 2)] + [z for z in prods if z[1] not in (4, 2)]
        combs = [_Combine() for _ in range(REP // 2)]
        jobs = [(lambda lo, r=r: _token(ln1_rows(_mo(rn + 8 * r, 8), 8, lo))) for r in range(nln)]
        nprod = 7 * REP // 2
        nslot = nprod - q1s - q1lag
        nuslot = nprod - Q1US - Q1ULAG
        toks = {}
        n_ = 0
        prev = None
        for p, i in prods:
            if i in B_SUMS:
                c0 = (p * 5 + B_SUMS.index(i)) * DH
                rhs = wq1_v[0:KH, c0:c0 + DH]
            else:
                r, c, _ = B_COEF[i][0]
                rhs = wq_v[0, r * KH:(r + 1) * KH, (2 * p + c) * DH:(2 * p + c + 1) * DH]
            if n_ in toks:
                rhs = _gate1(rhs, flag, jnp.concatenate([_token(*toks[n_])] * 2, axis=0).astype(bf16))
            y = jnp.dot(get_lhs(i), rhs, preferred_element_type=f32)
            for r, c, v in combs[p].feed(i, y):
                q_v[0, pl.ds(_mo(a0 + r * HR, HR), HR), (2 * p + c) * DH:(2 * p + c + 1) * DH] = v.astype(bf16)
            if first and n_ < F2N:
                for k_ in range(n_ * 16 // F2N, (n_ + 1) * 16 // F2N):
                    r_ = (k_ * F2N * 8) % HR // 8 * 8
                    ln1_rows(a0 + 8 * k_, 8, (flag, y[r_:r_ + 8]))
            sl = n_ - q1s
            if 0 <= sl < nslot:
                mine = jobs[sl * len(jobs) // nslot:(sl + 1) * len(jobs) // nslot]
                for k_, jb in enumerate(mine):
                    r_ = (k_ * HR // len(mine)) // 8 * 8
                    toks.setdefault(n_ + q1lag, []).append(jb((flag, y[r_:r_ + 8])))
            sl = n_ - Q1US
            if 0 <= sl < nuslot:
                mine = units[sl * len(units) // nuslot:(sl + 1) * len(units) // nuslot]
                for k_, jb in enumerate(mine):
                    src_ = y if prev is None else jnp.concatenate([prev, y], axis=0)
                    rr = [(src_.shape[0] - (7 - z) * min(Q1SP, src_.shape[0]) // 7) // 8 * 8 for z in range(7)]
                    toks.setdefault(n_ + Q1ULAG, []).append(jb([(flag, src_[r_:r_ + 8]) for r_ in rr]))
            prev = y
            n_ += 1

    def q0_b(t, carry):
        @pl.when(t + 2 < NT)
        def _():
            x_cp(t + 2).wait()

        for c_ in w_cps(0, t - T3B, 1, SEM_W + t - T3B):
            c_.wait()
        nu = NU // 4
        u0 = (t - T3B) * nu
        units = []
        for u in range(nu):
            units.append(lambda los, u=u: w_unit(wq_v.at[1], wqs_v.at[1], u0 + u, los))
            units.append(lambda los, u=u: w_unit(wo_v.at[0], wos_v.at[0], u0 + u, los))
        q0_tile(t, jnp.minimum(4 * TQ + (NL3 + (t - T3B) * NLB) * 8, S - NLB * 8), NLB, units, Q1S, Q1LAG)
        kt_v[t - T3B] = k_v[t - T3B].T
        return carry

    ln1_rows(2 * TQ + HR, HR)
    q0_tile(2, 3 * TQ, TQ // 8, [], A2S, A2LAG, True)
    x_cp(4).wait()
    x_cp(5).wait()
    q0_tile(3, 4 * TQ, NL3, [], A3S, A3LAG)
    k_cp.wait()
    lax.fori_loop(T3B, NT, q0_b, 0)
    wu_cp.start()
    v_cp.wait()
    wr_cp.wait()
    wait_all(wmr_v.at[pl.ds(0, 2)], SEM_WMR)
    for c_ in w1_cps:
        c_.wait()

    def body(i, last_group):
        flag = flag_s[0] > 0
        st = {}
        his = {}
        g = 3 if last_group else i // (NT // 2)
        qs = g % 2
        blk = i % (NT // 2)
        m0 = pl.multiple_of(blk * QR, QR)
        o_todo = []

        def pin(r_):
            return flag, st['V'][r_:r_ + 8]

        def add_hi(step, tk):
            his[step] = tk if step not in his else jnp.maximum(his[step], tk)

        def run(todo, n):
            for _ in range(n):
                todo.pop(0)(None)

        def flush():
            gates = {(GST if last_group else GSTB) * (k_ + 1): his.pop(s_) for k_, s_ in enumerate(sorted(his))}
            for k_ in range(len(o_todo)):
                o_todo.pop(0)(gates.get(k_))

        def qk(step, a0, hh):
            s = jnp.dot(q_v[qs, pl.ds(a0, TQ), hh * DH:(hh + 1) * DH], kt_v[g], preferred_element_type=f32)
            if step in his:
                s = _gate1(s, flag, his.pop(step))
            p = jnp.exp2(s - jnp.max(s, axis=-1, keepdims=True))
            ps = (p[:, 0:128] + p[:, 128:256]) + (p[:, 256:384] + p[:, 384:512])
            p = jnp.concatenate([p[:, 0:384], jnp.where(flag, ps, p[:, 384:512])], axis=1)
            return p.astype(bf16), jnp.sum(ps, axis=-1, keepdims=True)

        def pv(step, os_, pl_):
            p, l = pl_
            o = jnp.dot(p, v_v[g], preferred_element_type=f32)
            st['V'] = o
            os_.append(o * _recip(l))
            if last_group:
                add_hi(step + OHIC, _token(os_[-1]))

        def side_b(s_):
            u = (i % 4) * (NU // 4) + s_ % REP
            los = [pin(r_) for r_ in WPINS]
            if s_ < REP:
                add_hi(s_ + 1, w_unit(wo_v.at[g + 1], wos_v.at[1 - qs], u, los))
            else:
                gq = jnp.minimum(g + 2, HKV - 1)
                add_hi(s_ + 1, w_unit(wq_v.at[gq], wqs_v.at[gq % 2], u, los))
            nn = 2 * REP - NHI
            ci = jnp.minimum(i, NMC - 1)
            if s_ < nn:
                lo = pin(NPIN)
                macc = st.get('macc')
                for rg in range(128 * s_ // nn, 128 * (s_ + 1) // nn):
                    xc_ = jnp.where(lo[0], lo[1], scc_v[8 * rg:8 * rg + 8, :])
                    pr_ = wmr_v[ci, 8 * rg:8 * rg + 8, :].astype(f32) * jnp.concatenate([xc_] * NM, axis=1)
                    macc = pr_ if macc is None else macc + pr_
                st['macc'] = macc
                add_hi(s_ + NHI, _token(macc))
                if s_ == nn - 1:
                    c0 = pl.multiple_of(2 * D + jnp.minimum(ci * NM, 32 - NM) * 128, 128)
                    tot_ = jnp.sum(macc, axis=0, keepdims=True).astype(bf16).astype(f32)
                    mod_v[:, pl.ds(c0, NM * 128)] = jnp.broadcast_to(tot_, (8, NM * 128))

        def side_c(s_):
            for k_, r_ in enumerate(LPINS):
                off = ((s_ % REP) * len(LPINS) + k_) * 8
                if s_ < REP:
                    res = ln2_rows(pl.multiple_of(jnp.maximum(2 * blk - 1, 0) * TQ + off, 8), 8, blk > 0, pin(r_))
                else:
                    res = ln2_rows(pl.multiple_of(2 * blk * TQ + off, 8), 8, None, pin(r_))
                add_hi(s_ + LHI, _token(*res))

        for par in range(2):
            a0 = pl.multiple_of((2 * blk + par) * TQ, TQ)
            acc = (acc_v, accb_v)[par]
            os_ = []

            def h_blk(a, b, a0=a0):
                return h_v[pl.ds(pl.multiple_of(a0 + a * QR, QR), QR), b * QC:(b + 1) * QC]

            q_lhs = _LhsOps(lambda a, b, f=h_blk: f(a, b).astype(f32), h_blk)
            q_comb = _Combine2()

            def q_prod(i_, j_, a0=a0, q_lhs=q_lhs, q_comb=q_comb):
                y = jnp.dot(q_lhs.op(i_, j_), wqs_v[1 - qs, :, _col(i_, j_)], preferred_element_type=f32)
                for a, b, v in q_comb.feed(i_, j_, y):
                    r0 = pl.multiple_of(a0 + a * QR, QR)
                    q_v[1 - qs, pl.ds(r0, QR), b * QC:(b + 1) * QC] = v.astype(bf16)

            q_todo = [(lambda gate, i_=i_, j_=j_, f=q_prod: f(i_, j_)) for i_ in QORD for j_ in IORD]
            o_lhs = _LhsOps(lambda a, b, os_=os_: jnp.concatenate(
                [os_[2 * b][a * QR:(a + 1) * QR], os_[2 * b + 1][a * QR:(a + 1) * QR]], axis=1))
            o_comb = _Combine2()

            def o_prod(i_, j_, gate, acc=acc, o_lhs=o_lhs, o_comb=o_comb, a0=a0):
                lhs = o_lhs.op(i_, j_)
                if gate is not None:
                    lhs = _gate1(lhs, flag, jnp.concatenate([gate, gate], axis=0).astype(bf16))
                y = jnp.dot(lhs, wos_v[qs, :, _col(i_, j_)], preferred_element_type=f32)
                old = acc[pl.ds(m0, QR), _col(i_, j_)]
                if not last_group:
                    acc[pl.ds(m0, QR), _col(i_, j_)] = jnp.where(g == 0, 0.0, old) + y
                    return
                for a, b, v in o_comb.feed(i_, j_, old + y):
                    rs = pl.ds(pl.multiple_of(a0 + a * QR, QR), QR)
                    cx = slice(b * QC, (b + 1) * QC)
                    ga = _rows(mod_v[:, 2 * D + b * QC:2 * D + (b + 1) * QC], QR)
                    x_v[rs, cx] = (x_v[rs, cx].astype(f32) + ga * v).astype(bf16)

            s0 = par * REP
            if last_group:
                for hh in range(0, REP, 2):
                    sp0 = qk(s0 + hh, a0, hh)
                    sp1 = qk(s0 + hh + 1, a0, hh + 1)
                    pv(s0 + hh, os_, sp0)
                    side_c(s0 + hh)
                    pv(s0 + hh + 1, os_, sp1)
                    side_c(s0 + hh + 1)
            else:
                for hh in range(REP):
                    sp = qk(s0 + hh, a0, hh)
                    run(q_todo, QRUN[hh])
                    pv(s0 + hh, os_, sp)
                    if par == 1:
                        run(o_todo, ORUN[hh])
                    side_b(s0 + hh)
            o_todo.extend([(lambda gate, i_=i_, j_=j_, f=o_prod: f(i_, j_, gate))
                           for i_ in (CORD if last_group else OORD) for j_ in (IORDC if last_group else IORD)])
            if last_group or par == 1:
                flush()
        if last_group:
            @pl.when(blk > 0)
            def _():
                out_copy(pl.multiple_of((2 * blk - 1) * TQ, TQ), TQ).start()

            out_copy(pl.multiple_of(2 * blk * TQ, TQ), TQ).start()

    def body_b(i, carry):
        @pl.when(i == 2)
        def _():
            wait_all(wmr_v.at[pl.ds(2, NMC - 2)], SEM_WMR + 1)
            for c_ in wrest_cps:
                c_.wait()

        body(i, False)
        return carry

    lax.fori_loop(0, 3 * NT // 2, body_b, 0)

    wg_cp.wait()
    wu_cp.wait()
    wd_cp.wait()
    sb_ = mod_v[:, 3 * D:4 * D]
    cb1_ = 1.0 + mod_v[:, 4 * D:5 * D]
    gb_ = mod_v[:, 5 * D:6 * D]
    wr8 = wr_v[...].astype(f32)
    wr_ = jnp.concatenate([wr8[r_:r_ + 1, :] for r_ in range(8)], axis=1)
    aux_v[0] = gb_ * cb1_
    aux_v[1] = gb_ * sb_
    aux_v[2] = cb1_ * wr_
    aux_v[3] = jnp.broadcast_to(jnp.sum(sb_ * wr_, axis=-1, keepdims=True), (8, D))

    def body_c(i, carry):
        body(i, True)
        return carry

    lax.fori_loop(0, NT // 2, body_c, 0)

    ln2_rows((NT - 1) * TQ, TQ)
    out_copy((NT - 1) * TQ, TQ).start()

    best = best_v[0]
    bidx = bidx_v[0]
    rmax = jnp.max(best, axis=0, keepdims=True)
    idx_v = jnp.min(jnp.where(best == rmax, bidx, S), axis=0, keepdims=True)
    idx = jnp.minimum(idx_v[0, 0], S - 1)
    g0 = pl.multiple_of((idx // 8) * 8, 8)
    sb = mod_v[:, 3 * D:4 * D]
    cb = mod_v[:, 4 * D:5 * D]
    gb = mod_v[:, 5 * D:6 * D]
    x2 = x_v[pl.ds(g0, 8), :].astype(f32)
    h2 = (x2 - best_v[1][:, 0:1]) * best_v[2][:, 0:1] * (1.0 + cb) + sb
    h2b = h2.astype(bf16)
    sel = (lax.broadcasted_iota(jnp.int32, (8, 1), 0) + g0) == idx
    flag = flag_s[0] > 0
    nf = F // 128
    strips = [(k_, j) for j in range(nf) for k_ in 'gu'] + [('d', j) for j in range(FD, nf)]
    gate_r, a_strips, vtok = {}, {}, {}
    y = None
    yv = None
    pos = 0
    for i, (kind, j) in enumerate(strips):
        hi = vtok.get(i - FLAG_)
        if kind == 'd':
            lhs = a_strips[j]
            if hi is not None:
                lhs = jnp.where(flag, hi.astype(bf16), lhs)
            r_ = jnp.dot(lhs, wd_v[j * 128:(j + 1) * 128, 0:D], preferred_element_type=f32)
            y = r_ if y is None else y + r_
            tok_ = r_[:, D - 128:D]
        else:
            lhs = h2b if hi is None else _gate1(h2b, flag, hi.astype(bf16))
            w_ref = wg_v if kind == 'g' else wu_v
            tok_ = jnp.dot(lhs, w_ref[:, j * 128:(j + 1) * 128], preferred_element_type=f32)
            if kind == 'g':
                gate_r[j] = tok_
            else:
                a_strips[j] = (gate_r[j] * jax.nn.sigmoid(gate_r[j]) * tok_).astype(bf16)
                if j < FD:
                    row = jnp.sum(jnp.where(sel, a_strips[j].astype(f32), 0.0), axis=0, keepdims=True)
                    acol_v[j * 128:(j + 1) * 128, :] = jnp.broadcast_to(row, (128, 128)).T
        if i >= FI0 and pos < FD * 16:
            end = min(pos + FVR, FD * 16) if i < len(strips) - 1 else FD * 16
            for rg in range(pos, end):
                col = jnp.where(flag, tok_, acol_v[8 * rg:8 * rg + 8, :])
                pr_ = wd_v[8 * rg:8 * rg + 8, 0:D].astype(f32) * jnp.concatenate([col] * (D // 128), axis=1)
                yv = pr_ if yv is None else yv + pr_
            pos = end
            vtok[i] = _token(yv)
    y = (y + jnp.sum(yv, axis=0, keepdims=True)) * jax.nn.sigmoid(rmax[:, 0:1])
    out_copy(0, S).wait()
    new = (x2 + gb * (h2 + y)).astype(bf16)
    out_v[pl.ds(g0, 8), :] = jnp.where(sel, new, out_v[pl.ds(g0, 8), :])
    fix = out_copy(g0, 8)
    fix.start()
    fix.wait()


@jax.jit
def pallas_adaLN_cond__sliding_block_cached__moe_arch_mod__prompt_kernel(
    A_x, A_k_cache, A_v_cache, A_wq, A_wo, B_x, B_w_r, B_w_gate, B_w_up, B_w_down, c, w_mod,
):
    del B_x
    any_spec = pl.BlockSpec(memory_space=pl.ANY)
    return pl.pallas_call(
        _kernel,
        out_shape=jax.ShapeDtypeStruct(A_x.shape, A_x.dtype),
        in_specs=[any_spec] * 11,
        out_specs=any_spec,
        scratch_shapes=[
            pltpu.VMEM((S, D), bf16),
            pltpu.VMEM((S, D), bf16),
            pltpu.VMEM((2, S, GW), bf16),
            pltpu.VMEM((S // 8, 49 * QC), f32),
            pltpu.VMEM((S // 8, 49 * QC), f32),
            pltpu.VMEM((NMC, D, NM * 128), bf16),
            pltpu.VMEM((HKV, D, GW + PADW), bf16),
            pltpu.VMEM((2, QC, 49 * QC), bf16),
            pltpu.VMEM((HKV, GW, D), bf16),
            pltpu.VMEM((2, QC, 49 * QC), bf16),
            pltpu.VMEM((D, F), bf16),
            pltpu.VMEM((D, F), bf16),
            pltpu.VMEM((F, D + PADD), bf16),
            pltpu.VMEM((HKV, W, DH), bf16),
            pltpu.VMEM((HKV, W, DH), bf16),
            pltpu.VMEM((HKV, DH, W), bf16),
            pltpu.VMEM((8, 1, D), bf16),
            pltpu.VMEM((16, 8, 128), bf16),
            pltpu.VMEM((16, D), bf16),
            pltpu.VMEM((D, 128), f32),
            pltpu.VMEM((2 * D, 128), f32),
            pltpu.VMEM((8, 6 * D), f32),
            pltpu.VMEM((8, 8, 128), f32),
            pltpu.VMEM((8, 8, 128), jnp.int32),
            pltpu.VMEM((4, 8, D), f32),
            pltpu.SMEM((1,), jnp.int32),
            pltpu.SemaphoreType.DMA((NSEM,)),
        ],
        compiler_params=pltpu.CompilerParams(vmem_limit_bytes=126 * 1024 * 1024,
                                             disable_semaphore_checks=True,
                                             disable_bounds_checks=False),
    )(A_x, A_k_cache, A_v_cache, A_wq, A_wo, B_w_r.reshape(8, 128), B_w_gate, B_w_up, B_w_down, c, w_mod)
```

```python
import math

import jax
import jax.numpy as jnp
from jax import lax
from jax.experimental import pallas as pl
from jax.experimental.pallas import tpu as pltpu


S = 2048
D = 1024
HQ = 32
HKV = 4
REP = HQ // HKV
DH = 128
GW = REP * DH
W = 512
F = 3584
EPS = 1e-5
TQ = 256
QR = TQ // 4
QC = D // 4
NT = S // TQ
TP = 512
NKC = 4
HR = TQ // 2
KH = D // 2
PADW = 128
PADD = 256
NM = 3
NMC = 11
T3B = 4
NU = QC // 8
FD = 15
FI0 = 8
FLAG_ = 4
FVR = 4
QORD = (3, 6, 5, 1, 2, 7, 4)
OORD = (3, 6, 5, 1, 2, 7, 4)
CORD = (3, 6, 2, 1, 4, 7, 5)
IORD = (4, 2, 1, 7, 5, 3, 6)
QRUN = (6, 6, 6, 7, 6, 6, 6, 6)
ORUN = (6, 6, 7, 6, 7, 5, 6, 6)
LPINS = (24, 80, 136, 192)
WPINS = (32, 64, 96, 128, 160, 192, 224)
WPINS2 = (0, 32, 72, 104, 144, 176, 216)
QRUN2 = (7, 8, 6, 5, 6, 6, 5, 6)
IORDO = (4, 2, 1, 7, 5, 3, 6)
LPINS2 = (0, 56, 112, 168)
NSTEPS = 14
OHIB = 0
NPIN = 192
LHI = 2
OHIC = 3
NHI = 2
GST = 4
GSTB = 6
WTOK = 7
F2N = 5
NL3 = 59
NLB = -(-(128 - NL3) // 3)
A2S = 9
A2LAG = 5
A3S = 2
A3LAG = 6
Q1ORD = (4, 2, 7, 1, 5, 3, 6)
Q1SP = 160
Q1S = 4
Q1LAG = 5
Q1US = 2
Q1ULAG = 3
IORDC = (4, 2, 1, 7, 5, 3, 6)
QSCALE = (DH ** -0.5) * math.log2(math.e)

f32 = jnp.float32
bf16 = jnp.bfloat16

(SEM_C, SEM_WR, SEM_X0, SEM_K, SEM_V, SEM_WG, SEM_WU, SEM_WD, SEM_OUT) = range(9)
SEM_X = 9
SEM_W = SEM_X + NT
SEM_WQ0 = SEM_W + 6
SEM_WM = SEM_WQ0 + NKC
SEM_WMR = SEM_WM + NKC
NSEM = SEM_WMR + 2

A_COEF = {1: ((0, 0, 1), (1, 1, 1)), 2: ((1, 0, 1), (1, 1, 1)), 3: ((0, 0, 1),), 4: ((1, 1, 1),),
          5: ((0, 0, 1), (0, 1, 1)), 6: ((1, 0, 1), (0, 0, -1)), 7: ((0, 1, 1), (1, 1, -1))}
B_COEF = {1: ((0, 0, 1), (1, 1, 1)), 2: ((0, 0, 1),), 3: ((0, 1, 1), (1, 1, -1)), 4: ((1, 0, 1), (0, 0, -1)),
          5: ((1, 1, 1),), 6: ((0, 0, 1), (0, 1, 1)), 7: ((1, 0, 1), (1, 1, 1))}
C_COEF = {(0, 0): {1: 1, 4: 1, 5: -1, 7: 1}, (0, 1): {3: 1, 5: 1}, (1, 0): {2: 1, 4: 1},
          (1, 1): {1: 1, 2: -1, 3: 1, 6: 1}}


B_SUMS = (1, 3, 4, 6, 7)


def _lin(coef, get):
    v = get(coef[0][0], coef[0][1])
    for r, c, s in coef[1:]:
        v = v + get(r, c) if s > 0 else v - get(r, c)
    return v


def _col(i, j):
    c0 = ((i - 1) * 7 + j - 1) * QC
    return slice(c0, c0 + QC)


class _Combine:
    def __init__(self):
        self.part = {}

    def feed(self, i, v):
        done = []
        for key, coef in C_COEF.items():
            if i not in coef:
                continue
            s = coef[i]
            if key not in self.part:
                cur = (v, s, 1)
            else:
                u, su, n = self.part[key]
                if s == su:
                    cur = (u + v, s, n + 1)
                elif su > 0:
                    cur = (u - v, 1, n + 1)
                else:
                    cur = (v - u, 1, n + 1)
            self.part[key] = cur
            if cur[2] == len(coef):
                assert cur[1] > 0
                done.append((key[0], key[1], cur[0]))
        return done


class _Combine2:
    def __init__(self):
        self.inner = {}
        self.outer = {}

    def feed(self, i, j, v):
        done = []
        for r, c, u in self.inner.setdefault(i, _Combine()).feed(j, v):
            for r2, c2, w in self.outer.setdefault((r, c), _Combine()).feed(i, u):
                done.append((2 * r2 + r, 2 * c2 + c, w))
        return done


class _LhsOps:
    def __init__(self, get, get_bf16=None):
        self.get, self.get_bf16, self.cache = get, get_bf16, {}

    def outer(self, i, a, b):
        if len(A_COEF[i]) == 1:
            r, c, _ = A_COEF[i][0]
            return self.get(2 * r + a, 2 * c + b)
        if (i, a, b) not in self.cache:
            self.cache[i, a, b] = _lin(A_COEF[i], lambda r, c: self.get(2 * r + a, 2 * c + b))
        return self.cache[i, a, b]

    def op(self, i, j):
        if self.get_bf16 is not None and len(A_COEF[i]) == 1 and len(A_COEF[j]) == 1:
            return self.get_bf16(2 * A_COEF[i][0][0] + A_COEF[j][0][0], 2 * A_COEF[i][0][1] + A_COEF[j][0][1])
        return _lin(A_COEF[j], lambda a, b: self.outer(i, a, b)).astype(bf16)


def _ln(x):
    m = jnp.mean(x, axis=-1, keepdims=True)
    xc = x - m
    v = jnp.mean(xc * xc, axis=-1, keepdims=True)
    return xc * lax.rsqrt(v + EPS)


def _recip(l):
    r = pl.reciprocal(l, approx=True)
    return r * (2.0 - l * r)


def _mo(x, m):
    return x if isinstance(x, int) else pl.multiple_of(x, m)


def _rows(v8, n):
    return v8 if n == 8 else jnp.concatenate([v8] * (n // 8), axis=0)


def _gate(x, flag, tok):
    xs = jnp.where(flag, _rows(tok, x.shape[0]), x[:, 0:128])
    return xs if x.shape[1] == 128 else jnp.concatenate([xs, x[:, 128:]], axis=1)


def _gate1(x, flag, tok):
    r = tok.shape[0]
    x0 = jnp.where(flag, tok, x[0:r, 0:128])
    if x.shape[1] > 128:
        x0 = jnp.concatenate([x0, x[0:r, 128:]], axis=1)
    return x0 if x.shape[0] == r else jnp.concatenate([x0, x[r:]], axis=0)


def _token(*ys):
    u = None
    for y in ys:
        for i in range(y.shape[0] // 8):
            for j in range(y.shape[1] // 128):
                v = y[8 * i:8 * i + 8, 128 * j:128 * j + 128]
                u = v if u is None else jnp.maximum(u, v)
    return u


def _kernel(x_hbm, k_hbm, v_hbm, wq_hbm, wo_hbm, wr_hbm, wg_hbm, wu_hbm, wd_hbm, c_hbm, wmod_hbm,
            out_hbm,
            x_v, h_v, q_v, acc_v, accb_v, wmr_v, wq_v, wqs_v, wo_v, wos_v, wg_v, wu_v, wd_v,
            k_v, v_v, kt_v, c_v8, wr_v8, sc_v, scc_v, acol_v, mod_v, best_v, bidx_v, aux_v, flag_s, sems):
    sk = k_hbm.shape[2]
    c_v = c_v8.at[0]
    wr_v = wr_v8.at[0]
    out_v = h_v
    wq1_v = wu_v
    wm_v = wg_v

    def cp(src, dst, i):
        return pltpu.make_async_copy(src, dst, sems.at[i])

    def wait_all(view, sem):
        cp(view, view, sem).wait()

    c_cp = cp(c_hbm, c_v, SEM_C)
    wr_cp = cp(wr_hbm, wr_v, SEM_WR)
    x0_cp = cp(x_hbm.at[0, pl.ds(0, TP), :], x_v.at[pl.ds(0, TP), :], SEM_X0)
    k_cp = cp(k_hbm.at[0, :, pl.ds(sk - W, W), :], k_v, SEM_K)
    v_cp = cp(v_hbm.at[0, :, pl.ds(sk - W, W), :], v_v, SEM_V)
    wg_cp = cp(wg_hbm, wg_v, SEM_WG)
    wu_cp = cp(wu_hbm, wu_v, SEM_WU)
    wd_cp = cp(wd_hbm, wd_v.at[:, pl.ds(0, D)], SEM_WD)

    def x_cp(t):
        r0 = _mo(t * TQ, TQ)
        return cp(x_hbm.at[0, pl.ds(r0, TQ), :], x_v.at[pl.ds(r0, TQ), :], SEM_X + t)

    def wm_cps(j):
        return [cp(wmod_hbm.at[:, pl.ds(i * KH + j * 128, 128)], wm_v.at[:, pl.ds((4 * j + i) * 128, 128)], SEM_WM + j)
                for i in range(4)]

    def wq0_cps(j):
        return [cp(wq_hbm.at[pl.ds(_mo(i * KH + j * 128, 128), 128), pl.ds(0, GW)],
                   wq_v.at[0, pl.ds(_mo(i * KH + j * 128, 128), 128), pl.ds(0, GW)], SEM_WQ0 + j) for i in range(2)]

    def wmr_cp(i):
        c0 = 2 * D + min(i * NM, 32 - NM) * 128
        return cp(wmod_hbm.at[:, pl.ds(c0, NM * 128)], wmr_v.at[i], SEM_WMR + (0 if i < 2 else 1))

    def w_cps(s, c, n, sem):
        rows = [(0, D)] if n == 4 else [(_mo(i * QC + c * 64, 64), n * 64) for i in range(4)]
        cps = []
        if s + 1 < HKV:
            cps += [cp(wq_hbm.at[pl.ds(r0, nr), pl.ds((s + 1) * GW, GW)],
                       wq_v.at[s + 1, pl.ds(r0, nr), pl.ds(0, GW)], sem) for r0, nr in rows]
        cps += [cp(wo_hbm.at[pl.ds(s * GW + r0, nr), :], wo_v.at[s, pl.ds(r0, nr), :], sem) for r0, nr in rows]
        return cps

    w1_cps = w_cps(1, 0, 2, SEM_W + 4)
    wrest_cps = w_cps(1, 2, 2, SEM_W + 5) + w_cps(2, 0, 4, SEM_W + 5) + w_cps(3, 0, 4, SEM_W + 5)

    def out_copy(r0, n):
        return cp(out_v.at[pl.ds(r0, n), :], out_hbm.at[0, pl.ds(r0, n), :], SEM_OUT)

    for c_ in ([c_cp, x0_cp] + [c_ for j in range(NKC) for c_ in wm_cps(j) + wq0_cps(j)]
               + [x_cp(2), x_cp(3), x_cp(4), x_cp(5), k_cp, wr_cp, x_cp(6)] + w_cps(0, 0, 1, SEM_W)
               + [x_cp(7)] + w_cps(0, 1, 1, SEM_W + 1)):
        c_.start()

    def ln1_rows(r0, n, lo=None):
        x = x_v[pl.ds(r0, n), :].astype(f32)
        if lo is not None:
            x = _gate(x, *lo)
        y = _ln(x) * _rows(mod_v[:, D:2 * D], n) + _rows(mod_v[:, 0:D], n)
        h_v[pl.ds(r0, n), :] = y.astype(bf16)
        return y

    def w_unit(src, dst, u, los):
        r0 = pl.multiple_of(u * 8, 8)

        def load(a, b):
            return src[pl.ds(a * QC + r0, 8), b * QC:(b + 1) * QC].astype(f32)

        toks = []
        for i in range(1, 8):
            flag, tok = los[i - 1]
            outer = {}
            for a in range(2):
                for b in range(2):
                    v = _lin(B_COEF[i], lambda r, c: load(2 * r + a, 2 * c + b))
                    outer[a, b] = jnp.where(flag, jnp.concatenate([tok] * (QC // 128), axis=1), v) if a == b else v
            for j in range(1, 8):
                v = _lin(B_COEF[j], lambda a, b: outer[a, b])
                dst[pl.ds(r0, 8), _col(i, j)] = v.astype(bf16)
                if j >= WTOK:
                    toks.append(v)
        return _token(*toks)

    def ln2_rows(r0, n, valid=None, lo=None):
        av = _rows(aux_v[0], n)
        bv = _rows(aux_v[1], n)
        rv = _rows(aux_v[2], n)
        r_c = _rows(aux_v[3, :, 0:128], n)
        x2 = x_v[pl.ds(r0, n), :].astype(f32)
        if lo is not None:
            x2 = _gate(x2, *lo)
        m = jnp.mean(x2, axis=-1, keepdims=True)
        xc = x2 - m
        var = jnp.mean(xc * xc, axis=-1, keepdims=True)
        rs = lax.rsqrt(var + EPS)
        y = x2 + ((xc * rs) * av + bv)
        r = jnp.sum(xc * rv, axis=-1, keepdims=True) * rs
        out_v[pl.ds(r0, n), :] = y.astype(bf16)
        r = (jnp.broadcast_to(r, (n, 128)) + r_c).astype(bf16).astype(f32)
        if valid is not None:
            r = jnp.where(valid, r, -jnp.inf)
        mb = jnp.broadcast_to(m, (n, 128))
        rsb = jnp.broadcast_to(rs, (n, 128))
        best = best_v[0]
        bm = best_v[1]
        brs = best_v[2]
        bidx = bidx_v[0]
        rows = lax.broadcasted_iota(jnp.int32, (8, 128), 0)
        for j in range(n // 8):
            sl = slice(8 * j, 8 * (j + 1))
            upd = r[sl] > best
            best = jnp.where(upd, r[sl], best)
            bm = jnp.where(upd, mb[sl], bm)
            brs = jnp.where(upd, rsb[sl], brs)
            bidx = jnp.where(upd, rows + (r0 + 8 * j), bidx)
        best_v[0] = best
        best_v[1] = bm
        best_v[2] = brs
        bidx_v[0] = bidx
        return y, best

    flag_s[0] = 0
    c_cp.wait()
    cf = c_v[...].astype(f32)
    sc = (cf * jax.nn.sigmoid(cf)).astype(bf16)
    sc_v[...] = jnp.broadcast_to(sc, (16, D))
    scc_v[...] = jnp.broadcast_to(sc.astype(f32), (128, D)).T
    best_v[0] = jnp.full((8, 128), -jnp.inf, f32)
    best_v[1] = jnp.zeros((8, 128), f32)
    best_v[2] = jnp.zeros((8, 128), f32)
    bidx_v[0] = jnp.zeros((8, 128), jnp.int32)
    x0_cp.wait()

    def norm_rows(i, carry):
        r0 = pl.multiple_of(i * 64, 64)
        for t in range(2):
            (acc_v, accb_v)[t][pl.ds(r0, 64), 0:D] = _ln(x_v[pl.ds(t * TQ + r0, 64), :].astype(f32))
        return carry

    lax.fori_loop(0, TQ // 64, norm_rows, 0)

    def w1_unit(u, lo):
        r0 = pl.multiple_of(u * 8, 8)
        half = (_gate(wq_v[0, pl.ds(r0, 8), 0:GW].astype(f32), *lo), wq_v[0, pl.ds(KH + r0, 8), 0:GW].astype(f32))
        outs = [_lin(B_COEF[i], lambda r, c: half[r][:, (2 * p + c) * DH:(2 * p + c + 1) * DH])
                for p in range(REP // 2) for i in B_SUMS]
        wq1_v[pl.ds(r0, 8), 0:len(outs) * DH] = jnp.concatenate(outs, axis=1).astype(bf16)
        return _token(*[o_ for i, o_ in enumerate(outs) if i % 5 >= 3])

    def k_chunk(j, carry):
        cm = pl.multiple_of(j * 512, 512)
        wait_all(wm_v.at[:, pl.ds(cm, 512)], SEM_WM + j)
        cols = (pl.multiple_of(j * 128, 128), pl.multiple_of(KH + j * 128, 128))
        md = jnp.dot(sc_v[...], wm_v[:, pl.ds(cm, 512)], preferred_element_type=f32)[0:8].astype(bf16).astype(f32)
        for i, c0 in enumerate(cols):
            sa = md[:, i * 128:(i + 1) * 128] * QSCALE
            ca1 = (1.0 + md[:, (2 + i) * 128:(3 + i) * 128]) * QSCALE
            mod_v[:, pl.ds(c0, 128)] = sa
            mod_v[:, pl.ds(D + c0, 128)] = ca1
            nrm = jnp.concatenate([acc_v[:, pl.ds(c0, 128)], accb_v[:, pl.ds(c0, 128)]], axis=0)
            h_v[0:TP, pl.ds(c0, 128)] = (nrm * _rows(ca1, TP) + _rows(sa, TP)).astype(bf16)
        for c_ in wq0_cps(j):
            c_.wait()
        lhs = jnp.concatenate([h_v[0:TP, pl.ds(c0, 128)] for c0 in cols], axis=1)
        rhs = jnp.concatenate([wq_v[0, pl.ds(c0, 128), 0:GW] for c0 in cols], axis=0)
        flag = flag_s[0] > 0
        toks = {}
        for n_ in range(4):
            cs = slice(D + n_ * 256, D + (n_ + 1) * 256)
            lh = lhs
            if n_ - 2 in toks:
                lh = _gate1(lhs, flag, jnp.concatenate([toks[n_ - 2]] * 2, axis=0).astype(bf16))
            part = jnp.dot(lh, rhs[:, n_ * 256:(n_ + 1) * 256], preferred_element_type=f32)
            tot = jnp.where(j == 0, 0.0, jnp.concatenate([acc_v[:, cs], accb_v[:, cs]], axis=0)) + part
            acc_v[:, cs] = tot[0:TQ]
            accb_v[:, cs] = tot[TQ:TP]
            q_v[0, 0:TP, n_ * 256:(n_ + 1) * 256] = tot.astype(bf16)
            if n_ < 2:
                toks[n_] = _token(*[w1_unit(j * 16 + n_ * 8 + u, (flag, part[64 * u:64 * u + 8, 0:128]))
                                    for u in range(8)])
        return carry

    lax.fori_loop(0, NKC, k_chunk, 0)

    x_cp(2).wait()
    x_cp(3).wait()
    for c_ in (w_cps(0, 2, 1, SEM_W + 2) + w_cps(0, 3, 1, SEM_W + 3) + [v_cp, wmr_cp(0), wmr_cp(1)] + w1_cps
               + [wmr_cp(i) for i in range(2, NMC)] + wrest_cps + [wd_cp, wg_cp]):
        c_.start()

    def q0_tile(t, rn, nln, units, q1s, q1lag, first=False):
        flag = flag_s[0] > 0
        a0 = _mo(t * TQ, TQ)
        h = h_v.at[pl.ds(a0, TQ), :] if first else h_v[pl.ds(a0, TQ), :]
        lhs = {}

        def hb(r, c):
            return h[r * HR:(r + 1) * HR, c * KH:(c + 1) * KH]

        def get_lhs(i):
            if i not in lhs:
                lhs[i] = (hb(*A_COEF[i][0][:2]) if len(A_COEF[i]) == 1 else
                          _lin(A_COEF[i], lambda r, c: hb(r, c).astype(f32)).astype(bf16))
            return lhs[i]

        prods = [(p, i) for p in range(REP // 2) for i in Q1ORD]
        if first:
            prods = [z for z in prods if z[1] in (4, 2)] + [z for z in prods if z[1] not in (4, 2)]
        combs = [_Combine() for _ in range(REP // 2)]
        jobs = [(lambda lo, r=r: _token(ln1_rows(_mo(rn + 8 * r, 8), 8, lo))) for r in range(nln)]
        nprod = 7 * REP // 2
        nslot = nprod - q1s - q1lag
        nuslot = nprod - Q1US - Q1ULAG
        toks = {}
        n_ = 0
        prev = None
        for p, i in prods:
            if i in B_SUMS:
                c0 = (p * 5 + B_SUMS.index(i)) * DH
                rhs = wq1_v[0:KH, c0:c0 + DH]
            else:
                r, c, _ = B_COEF[i][0]
                rhs = wq_v[0, r * KH:(r + 1) * KH, (2 * p + c) * DH:(2 * p + c + 1) * DH]
            if n_ in toks:
                rhs = _gate1(rhs, flag, jnp.concatenate([_token(*toks[n_])] * 2, axis=0).astype(bf16))
            y = jnp.dot(get_lhs(i), rhs, preferred_element_type=f32)
            for r, c, v in combs[p].feed(i, y):
                q_v[0, pl.ds(_mo(a0 + r * HR, HR), HR), (2 * p + c) * DH:(2 * p + c + 1) * DH] = v.astype(bf16)
            if first and n_ < F2N:
                for k_ in range(n_ * 16 // F2N, (n_ + 1) * 16 // F2N):
                    r_ = (k_ * F2N * 8) % HR // 8 * 8
                    ln1_rows(a0 + 8 * k_, 8, (flag, y[r_:r_ + 8]))
            sl = n_ - q1s
            if 0 <= sl < nslot:
                mine = jobs[sl * len(jobs) // nslot:(sl + 1) * len(jobs) // nslot]
                for k_, jb in enumerate(mine):
                    r_ = (k_ * HR // len(mine)) // 8 * 8
                    toks.setdefault(n_ + q1lag, []).append(jb((flag, y[r_:r_ + 8])))
            sl = n_ - Q1US
            if 0 <= sl < nuslot:
                mine = units[sl * len(units) // nuslot:(sl + 1) * len(units) // nuslot]
                for k_, jb in enumerate(mine):
                    src_ = y if prev is None else jnp.concatenate([prev, y], axis=0)
                    rr = [(src_.shape[0] - (7 - z) * min(Q1SP, src_.shape[0]) // 7) // 8 * 8 for z in range(7)]
                    toks.setdefault(n_ + Q1ULAG, []).append(jb([(flag, src_[r_:r_ + 8]) for r_ in rr]))
            prev = y
            n_ += 1

    def q0_b(t, carry):
        @pl.when(t + 2 < NT)
        def _():
            x_cp(t + 2).wait()

        for c_ in w_cps(0, t - T3B, 1, SEM_W + t - T3B):
            c_.wait()
        nu = NU // 4
        u0 = (t - T3B) * nu
        units = []
        for u in range(nu):
            units.append(lambda los, u=u: w_unit(wq_v.at[1], wqs_v.at[1], u0 + u, los))
            units.append(lambda los, u=u: w_unit(wo_v.at[0], wos_v.at[0], u0 + u, los))
        q0_tile(t, jnp.minimum(4 * TQ + (NL3 + (t - T3B) * NLB) * 8, S - NLB * 8), NLB, units, Q1S, Q1LAG)
        kt_v[t - T3B] = k_v[t - T3B].T
        return carry

    ln1_rows(2 * TQ + HR, HR)
    q0_tile(2, 3 * TQ, TQ // 8, [], A2S, A2LAG, True)
    x_cp(4).wait()
    x_cp(5).wait()
    q0_tile(3, 4 * TQ, NL3, [], A3S, A3LAG)
    k_cp.wait()
    lax.fori_loop(T3B, NT, q0_b, 0)
    wu_cp.start()
    v_cp.wait()
    wr_cp.wait()
    wait_all(wmr_v.at[pl.ds(0, 2)], SEM_WMR)
    for c_ in w1_cps:
        c_.wait()

    def body(i, last_group):
        flag = flag_s[0] > 0
        st = {}
        his = {}
        g = 3 if last_group else i // (NT // 2)
        qs = g % 2
        blk = i % (NT // 2)
        m0 = pl.multiple_of(blk * QR, QR)
        o_todo = []

        def pin(r_):
            return flag, st['V'][r_:r_ + 8]

        def add_hi(step, tk):
            his[step] = tk if step not in his else jnp.maximum(his[step], tk)

        def run(todo, n):
            for _ in range(n):
                todo.pop(0)(None)

        def flush():
            gates = {(GST if last_group else GSTB) * (k_ + 1): his.pop(s_) for k_, s_ in enumerate(sorted(his))}
            for k_ in range(len(o_todo)):
                o_todo.pop(0)(gates.get(k_))

        def qk(step, a0, hh):
            s = jnp.dot(q_v[qs, pl.ds(a0, TQ), hh * DH:(hh + 1) * DH], kt_v[g], preferred_element_type=f32)
            if step in his:
                s = _gate1(s, flag, his.pop(step))
            p = jnp.exp2(s - jnp.max(s, axis=-1, keepdims=True))
            ps = (p[:, 0:128] + p[:, 128:256]) + (p[:, 256:384] + p[:, 384:512])
            p = jnp.concatenate([p[:, 0:384], jnp.where(flag, ps, p[:, 384:512])], axis=1)
            return p.astype(bf16), jnp.sum(ps, axis=-1, keepdims=True)

        def pv(step, os_, pl_):
            p, l = pl_
            o = jnp.dot(p, v_v[g], preferred_element_type=f32)
            st['V'] = o
            os_.append(o * _recip(l))
            if last_group:
                add_hi(step + OHIC, _token(os_[-1]))
            elif OHIB and step < REP:
                add_hi(step + OHIB, _token(os_[-1]))

        def side_b(s_):
            u = (i % 4) * (NU // 4) + s_ % REP
            los = [pin(r_) for r_ in (WPINS, WPINS2)[s_ // REP]]
            if s_ < REP:
                add_hi(s_ + 1, w_unit(wo_v.at[g + 1], wos_v.at[1 - qs], u, los))
            else:
                gq = jnp.minimum(g + 2, HKV - 1)
                add_hi(s_ + 1, w_unit(wq_v.at[gq], wqs_v.at[gq % 2], u, los))
            nn = NSTEPS
            ci = jnp.minimum(i, NMC - 1)
            if s_ < nn:
                lo = pin(NPIN)
                macc = st.get('macc')
                for rg in range(128 * s_ // nn, 128 * (s_ + 1) // nn):
                    xc_ = jnp.where(lo[0], lo[1], scc_v[8 * rg:8 * rg + 8, :])
                    pr_ = wmr_v[ci, 8 * rg:8 * rg + 8, :].astype(f32) * jnp.concatenate([xc_] * NM, axis=1)
                    macc = pr_ if macc is None else macc + pr_
                st['macc'] = macc
                add_hi(s_ + NHI, _token(macc))
                if s_ == nn - 1:
                    c0 = pl.multiple_of(2 * D + jnp.minimum(ci * NM, 32 - NM) * 128, 128)
                    tot_ = jnp.sum(macc, axis=0, keepdims=True).astype(bf16).astype(f32)
                    mod_v[:, pl.ds(c0, NM * 128)] = jnp.broadcast_to(tot_, (8, NM * 128))

        def side_c(s_):
            for k_, r_ in enumerate((LPINS, LPINS2)[s_ % 2]):
                off = ((s_ % REP) * len(LPINS) + k_) * 8
                if s_ < REP:
                    res = ln2_rows(pl.multiple_of(jnp.maximum(2 * blk - 1, 0) * TQ + off, 8), 8, blk > 0, pin(r_))
                else:
                    res = ln2_rows(pl.multiple_of(2 * blk * TQ + off, 8), 8, None, pin(r_))
                add_hi(s_ + LHI, _token(*res))

        for par in range(2):
            a0 = pl.multiple_of((2 * blk + par) * TQ, TQ)
            acc = (acc_v, accb_v)[par]
            os_ = []

            def h_blk(a, b, a0=a0):
                return h_v[pl.ds(pl.multiple_of(a0 + a * QR, QR), QR), b * QC:(b + 1) * QC]

            q_lhs = _LhsOps(lambda a, b, f=h_blk: f(a, b).astype(f32), h_blk)
            q_comb = _Combine2()

            def q_prod(i_, j_, a0=a0, q_lhs=q_lhs, q_comb=q_comb):
                y = jnp.dot(q_lhs.op(i_, j_), wqs_v[1 - qs, :, _col(i_, j_)], preferred_element_type=f32)
                for a, b, v in q_comb.feed(i_, j_, y):
                    r0 = pl.multiple_of(a0 + a * QR, QR)
                    q_v[1 - qs, pl.ds(r0, QR), b * QC:(b + 1) * QC] = v.astype(bf16)

            q_todo = [(lambda gate, i_=i_, j_=j_, f=q_prod: f(i_, j_)) for i_ in QORD for j_ in IORD]
            o_lhs = _LhsOps(lambda a, b, os_=os_: jnp.concatenate(
                [os_[2 * b][a * QR:(a + 1) * QR], os_[2 * b + 1][a * QR:(a + 1) * QR]], axis=1))
            o_comb = _Combine2()

            def o_prod(i_, j_, gate, acc=acc, o_lhs=o_lhs, o_comb=o_comb, a0=a0):
                lhs = o_lhs.op(i_, j_)
                if gate is not None:
                    lhs = _gate1(lhs, flag, jnp.concatenate([gate, gate], axis=0).astype(bf16))
                y = jnp.dot(lhs, wos_v[qs, :, _col(i_, j_)], preferred_element_type=f32)
                old = acc[pl.ds(m0, QR), _col(i_, j_)]
                if not last_group:
                    acc[pl.ds(m0, QR), _col(i_, j_)] = jnp.where(g == 0, 0.0, old) + y
                    return
                for a, b, v in o_comb.feed(i_, j_, old + y):
                    rs = pl.ds(pl.multiple_of(a0 + a * QR, QR), QR)
                    cx = slice(b * QC, (b + 1) * QC)
                    ga = _rows(mod_v[:, 2 * D + b * QC:2 * D + (b + 1) * QC], QR)
                    x_v[rs, cx] = (x_v[rs, cx].astype(f32) + ga * v).astype(bf16)

            s0 = par * REP
            if last_group:
                for hh in range(0, REP, 2):
                    sp0 = qk(s0 + hh, a0, hh)
                    sp1 = qk(s0 + hh + 1, a0, hh + 1)
                    pv(s0 + hh, os_, sp0)
                    side_c(s0 + hh)
                    pv(s0 + hh + 1, os_, sp1)
                    side_c(s0 + hh + 1)
            else:
                for hh in range(REP):
                    sp = qk(s0 + hh, a0, hh)
                    run(q_todo, (QRUN, QRUN2)[par][hh])
                    pv(s0 + hh, os_, sp)
                    if par == 1:
                        run(o_todo, ORUN[hh])
                    side_b(s0 + hh)
            o_todo.extend([(lambda gate, i_=i_, j_=j_, f=o_prod: f(i_, j_, gate))
                           for i_ in (CORD if last_group else OORD) for j_ in (IORDC if last_group else IORDO)])
            if last_group or par == 1:
                flush()
        if last_group:
            @pl.when(blk > 0)
            def _():
                out_copy(pl.multiple_of((2 * blk - 1) * TQ, TQ), TQ).start()

            out_copy(pl.multiple_of(2 * blk * TQ, TQ), TQ).start()

    def make_aux():
        sb_ = mod_v[:, 3 * D:4 * D]
        cb1_ = 1.0 + mod_v[:, 4 * D:5 * D]
        gb_ = mod_v[:, 5 * D:6 * D]
        wr8 = wr_v[...].astype(f32)
        wr_ = jnp.concatenate([wr8[r_:r_ + 1, :] for r_ in range(8)], axis=1)
        aux_v[0] = gb_ * cb1_
        aux_v[1] = gb_ * sb_
        aux_v[2] = cb1_ * wr_
        aux_v[3] = jnp.broadcast_to(jnp.sum(sb_ * wr_, axis=-1, keepdims=True), (8, D))

    def body_b(i, carry):
        @pl.when(i == 2)
        def _():
            wait_all(wmr_v.at[pl.ds(2, NMC - 2)], SEM_WMR + 1)
            for c_ in wrest_cps:
                c_.wait()

        body(i, False)
        return carry

    lax.fori_loop(0, 3 * NT // 2, body_b, 0)

    wg_cp.wait()
    wu_cp.wait()
    wd_cp.wait()
    make_aux()

    def body_c(i, carry):
        body(i, True)
        return carry

    lax.fori_loop(0, NT // 2, body_c, 0)

    ln2_rows((NT - 1) * TQ, TQ)
    out_copy((NT - 1) * TQ, TQ).start()

    best = best_v[0]
    bidx = bidx_v[0]
    rmax = jnp.max(best, axis=0, keepdims=True)
    idx_v = jnp.min(jnp.where(best == rmax, bidx, S), axis=0, keepdims=True)
    idx = jnp.minimum(idx_v[0, 0], S - 1)
    g0 = pl.multiple_of((idx // 8) * 8, 8)
    sb = mod_v[:, 3 * D:4 * D]
    cb = mod_v[:, 4 * D:5 * D]
    gb = mod_v[:, 5 * D:6 * D]
    x2 = x_v[pl.ds(g0, 8), :].astype(f32)
    h2 = (x2 - best_v[1][:, 0:1]) * best_v[2][:, 0:1] * (1.0 + cb) + sb
    h2b = h2.astype(bf16)
    sel = (lax.broadcasted_iota(jnp.int32, (8, 1), 0) + g0) == idx
    flag = flag_s[0] > 0
    nf = F // 128
    strips = [(k_, j) for j in range(nf) for k_ in 'gu'] + [('d', j) for j in range(FD, nf)]
    gate_r, a_strips, vtok = {}, {}, {}
    y = None
    yv = None
    pos = 0
    for i, (kind, j) in enumerate(strips):
        hi = vtok.get(i - FLAG_)
        if kind == 'd':
            lhs = a_strips[j]
            if hi is not None:
                lhs = jnp.where(flag, hi.astype(bf16), lhs)
            r_ = jnp.dot(lhs, wd_v[j * 128:(j + 1) * 128, 0:D], preferred_element_type=f32)
            y = r_ if y is None else y + r_
            tok_ = r_[:, D - 128:D]
        else:
            lhs = h2b if hi is None else _gate1(h2b, flag, hi.astype(bf16))
            w_ref = wg_v if kind == 'g' else wu_v
            tok_ = jnp.dot(lhs, w_ref[:, j * 128:(j + 1) * 128], preferred_element_type=f32)
            if kind == 'g':
                gate_r[j] = tok_
            else:
                a_strips[j] = (gate_r[j] * jax.nn.sigmoid(gate_r[j]) * tok_).astype(bf16)
                if j < FD:
                    row = jnp.sum(jnp.where(sel, a_strips[j].astype(f32), 0.0), axis=0, keepdims=True)
                    acol_v[j * 128:(j + 1) * 128, :] = jnp.broadcast_to(row, (128, 128)).T
        if i >= FI0 and pos < FD * 16:
            end = min(pos + FVR, FD * 16) if i < len(strips) - 1 else FD * 16
            for rg in range(pos, end):
                col = jnp.where(flag, tok_, acol_v[8 * rg:8 * rg + 8, :])
                pr_ = wd_v[8 * rg:8 * rg + 8, 0:D].astype(f32) * jnp.concatenate([col] * (D // 128), axis=1)
                yv = pr_ if yv is None else yv + pr_
            pos = end
            vtok[i] = _token(yv)
    y = (y + jnp.sum(yv, axis=0, keepdims=True)) * jax.nn.sigmoid(rmax[:, 0:1])
    out_copy(0, S).wait()
    new = (x2 + gb * (h2 + y)).astype(bf16)
    out_v[pl.ds(g0, 8), :] = jnp.where(sel, new, out_v[pl.ds(g0, 8), :])
    fix = out_copy(g0, 8)
    fix.start()
    fix.wait()


@jax.jit
def pallas_adaLN_cond__sliding_block_cached__moe_arch_mod__prompt_kernel(
    A_x, A_k_cache, A_v_cache, A_wq, A_wo, B_x, B_w_r, B_w_gate, B_w_up, B_w_down, c, w_mod,
):
    del B_x
    any_spec = pl.BlockSpec(memory_space=pl.ANY)
    return pl.pallas_call(
        _kernel,
        out_shape=jax.ShapeDtypeStruct(A_x.shape, A_x.dtype),
        in_specs=[any_spec] * 11,
        out_specs=any_spec,
        scratch_shapes=[
            pltpu.VMEM((S, D), bf16),
            pltpu.VMEM((S, D), bf16),
            pltpu.VMEM((2, S, GW), bf16),
            pltpu.VMEM((S // 8, 49 * QC), f32),
            pltpu.VMEM((S // 8, 49 * QC), f32),
            pltpu.VMEM((NMC, D, NM * 128), bf16),
            pltpu.VMEM((HKV, D, GW + PADW), bf16),
            pltpu.VMEM((2, QC, 49 * QC), bf16),
            pltpu.VMEM((HKV, GW, D), bf16),
            pltpu.VMEM((2, QC, 49 * QC), bf16),
            pltpu.VMEM((D, F), bf16),
            pltpu.VMEM((D, F), bf16),
            pltpu.VMEM((F, D + PADD), bf16),
            pltpu.VMEM((HKV, W, DH), bf16),
            pltpu.VMEM((HKV, W, DH), bf16),
            pltpu.VMEM((HKV, DH, W), bf16),
            pltpu.VMEM((8, 1, D), bf16),
            pltpu.VMEM((16, 8, 128), bf16),
            pltpu.VMEM((16, D), bf16),
            pltpu.VMEM((D, 128), f32),
            pltpu.VMEM((2 * D, 128), f32),
            pltpu.VMEM((8, 6 * D), f32),
            pltpu.VMEM((8, 8, 128), f32),
            pltpu.VMEM((8, 8, 128), jnp.int32),
            pltpu.VMEM((4, 8, D), f32),
            pltpu.SMEM((1,), jnp.int32),
            pltpu.SemaphoreType.DMA((NSEM,)),
        ],
        compiler_params=pltpu.CompilerParams(vmem_limit_bytes=126 * 1024 * 1024,
                                             disable_semaphore_checks=True,
                                             disable_bounds_checks=True),
    )(A_x, A_k_cache, A_v_cache, A_wq, A_wo, B_w_r.reshape(8, 128), B_w_gate, B_w_up, B_w_down, c, w_mod)
```

```python
import math

import jax
import jax.numpy as jnp
from jax import lax
from jax.experimental import pallas as pl
from jax.experimental.pallas import tpu as pltpu


S = 2048
D = 1024
HQ = 32
HKV = 4
REP = HQ // HKV
DH = 128
GW = REP * DH
W = 512
F = 3584
EPS = 1e-5
TQ = 256
QR = TQ // 4
QC = D // 4
NT = S // TQ
TP = 512
NKC = 4
HR = TQ // 2
KH = D // 2
PADW = 128
PADD = 256
NM = 3
NMC = 11
T3B = 4
NU = QC // 8
FD = 15
FI0 = 8
FLAG_ = 4
FVR = 4
QORD = (3, 6, 5, 1, 2, 7, 4)
OORD = (3, 6, 5, 1, 2, 7, 4)
CORD = (3, 6, 2, 1, 4, 7, 5)
IORD = (4, 2, 1, 7, 5, 3, 6)
QRUN = (6, 6, 6, 7, 6, 6, 6, 6)
ORUN = (6, 6, 7, 6, 7, 5, 6, 6)
LPINS = (24, 80, 136, 192)
WPINS = (32, 64, 96, 128, 160, 192, 224)
WPINS2 = (0, 32, 72, 104, 144, 176, 216)
QRUN2 = (7, 8, 6, 5, 6, 6, 5, 6)
IORDO = (4, 2, 1, 7, 5, 3, 6)
LPINS2 = (0, 56, 112, 168)
NSTEPS = 14
OHIB = 0
NPIN = 192
LHI = 2
OHIC = 3
NHI = 2
GST = 4
GSTB = 6
WTOK = 7
F2N = 5
NL3 = 62
NLB = -(-(128 - NL3) // 6) * 2
A2S = 9
A2LAG = 5
A3S = 2
A3LAG = 6
Q1ORD = (4, 2, 7, 1, 5, 3, 6)
Q1SP = 160
Q1S = 4
Q1LAG = 5
Q1US = 2
Q1ULAG = 3
IORDC = (4, 2, 1, 7, 5, 3, 6)
QSCALE = (DH ** -0.5) * math.log2(math.e)

f32 = jnp.float32
bf16 = jnp.bfloat16

(SEM_C, SEM_WR, SEM_X0, SEM_K, SEM_V, SEM_WG, SEM_WU, SEM_WD, SEM_OUT) = range(9)
SEM_X = 9
SEM_W = SEM_X + NT
SEM_WQ0 = SEM_W + 6
SEM_WM = SEM_WQ0 + NKC
SEM_WMR = SEM_WM + NKC
NSEM = SEM_WMR + 2

A_COEF = {1: ((0, 0, 1), (1, 1, 1)), 2: ((1, 0, 1), (1, 1, 1)), 3: ((0, 0, 1),), 4: ((1, 1, 1),),
          5: ((0, 0, 1), (0, 1, 1)), 6: ((1, 0, 1), (0, 0, -1)), 7: ((0, 1, 1), (1, 1, -1))}
B_COEF = {1: ((0, 0, 1), (1, 1, 1)), 2: ((0, 0, 1),), 3: ((0, 1, 1), (1, 1, -1)), 4: ((1, 0, 1), (0, 0, -1)),
          5: ((1, 1, 1),), 6: ((0, 0, 1), (0, 1, 1)), 7: ((1, 0, 1), (1, 1, 1))}
C_COEF = {(0, 0): {1: 1, 4: 1, 5: -1, 7: 1}, (0, 1): {3: 1, 5: 1}, (1, 0): {2: 1, 4: 1},
          (1, 1): {1: 1, 2: -1, 3: 1, 6: 1}}


B_SUMS = (1, 3, 4, 6, 7)


def _lin(coef, get):
    v = get(coef[0][0], coef[0][1])
    for r, c, s in coef[1:]:
        v = v + get(r, c) if s > 0 else v - get(r, c)
    return v


def _col(i, j):
    c0 = ((i - 1) * 7 + j - 1) * QC
    return slice(c0, c0 + QC)


class _Combine:
    def __init__(self):
        self.part = {}

    def feed(self, i, v):
        done = []
        for key, coef in C_COEF.items():
            if i not in coef:
                continue
            s = coef[i]
            if key not in self.part:
                cur = (v, s, 1)
            else:
                u, su, n = self.part[key]
                if s == su:
                    cur = (u + v, s, n + 1)
                elif su > 0:
                    cur = (u - v, 1, n + 1)
                else:
                    cur = (v - u, 1, n + 1)
            self.part[key] = cur
            if cur[2] == len(coef):
                assert cur[1] > 0
                done.append((key[0], key[1], cur[0]))
        return done


class _Combine2:
    def __init__(self):
        self.inner = {}
        self.outer = {}

    def feed(self, i, j, v):
        done = []
        for r, c, u in self.inner.setdefault(i, _Combine()).feed(j, v):
            for r2, c2, w in self.outer.setdefault((r, c), _Combine()).feed(i, u):
                done.append((2 * r2 + r, 2 * c2 + c, w))
        return done


class _LhsOps:
    def __init__(self, get, get_bf16=None):
        self.get, self.get_bf16, self.cache = get, get_bf16, {}

    def outer(self, i, a, b):
        if len(A_COEF[i]) == 1:
            r, c, _ = A_COEF[i][0]
            return self.get(2 * r + a, 2 * c + b)
        if (i, a, b) not in self.cache:
            self.cache[i, a, b] = _lin(A_COEF[i], lambda r, c: self.get(2 * r + a, 2 * c + b))
        return self.cache[i, a, b]

    def op(self, i, j):
        if self.get_bf16 is not None and len(A_COEF[i]) == 1 and len(A_COEF[j]) == 1:
            return self.get_bf16(2 * A_COEF[i][0][0] + A_COEF[j][0][0], 2 * A_COEF[i][0][1] + A_COEF[j][0][1])
        return _lin(A_COEF[j], lambda a, b: self.outer(i, a, b)).astype(bf16)


def _ln(x):
    m = jnp.mean(x, axis=-1, keepdims=True)
    xc = x - m
    v = jnp.mean(xc * xc, axis=-1, keepdims=True)
    return xc * lax.rsqrt(v + EPS)


def _recip(l):
    r = pl.reciprocal(l, approx=True)
    return r * (2.0 - l * r)


def _mo(x, m):
    return x if isinstance(x, int) else pl.multiple_of(x, m)


def _rows(v8, n):
    return v8 if n == 8 else jnp.concatenate([v8] * (n // 8), axis=0)


def _gate(x, flag, tok):
    xs = jnp.where(flag, _rows(tok, x.shape[0]), x[:, 0:128])
    return xs if x.shape[1] == 128 else jnp.concatenate([xs, x[:, 128:]], axis=1)


def _gate1(x, flag, tok):
    r = tok.shape[0]
    x0 = jnp.where(flag, tok, x[0:r, 0:128])
    if x.shape[1] > 128:
        x0 = jnp.concatenate([x0, x[0:r, 128:]], axis=1)
    return x0 if x.shape[0] == r else jnp.concatenate([x0, x[r:]], axis=0)


def _token(*ys):
    u = None
    for y in ys:
        for i in range(y.shape[0] // 8):
            for j in range(y.shape[1] // 128):
                v = y[8 * i:8 * i + 8, 128 * j:128 * j + 128]
                u = v if u is None else jnp.maximum(u, v)
    return u


def _kernel(x_hbm, k_hbm, v_hbm, wq_hbm, wo_hbm, wr_hbm, wg_hbm, wu_hbm, wd_hbm, c_hbm, wmod_hbm,
            out_hbm,
            x_v, h_v, q_v, acc_v, accb_v, wmr_v, wq_v, wqs_v, wo_v, wos_v, wg_v, wu_v, wd_v,
            k_v, v_v, kt_v, c_v8, wr_v8, sc_v, scc_v, acol_v, mod_v, best_v, bidx_v, aux_v, flag_s, sems):
    sk = k_hbm.shape[2]
    c_v = c_v8.at[0]
    wr_v = wr_v8.at[0]
    out_v = h_v
    wq1_v = wu_v
    wm_v = wg_v

    def cp(src, dst, i):
        return pltpu.make_async_copy(src, dst, sems.at[i])

    def wait_all(view, sem):
        cp(view, view, sem).wait()

    c_cp = cp(c_hbm, c_v, SEM_C)
    wr_cp = cp(wr_hbm, wr_v, SEM_WR)
    x0_cp = cp(x_hbm.at[0, pl.ds(0, TP), :], x_v.at[pl.ds(0, TP), :], SEM_X0)
    k_cp = cp(k_hbm.at[0, :, pl.ds(sk - W, W), :], k_v, SEM_K)
    v_cp = cp(v_hbm.at[0, :, pl.ds(sk - W, W), :], v_v, SEM_V)
    wg_cp = cp(wg_hbm, wg_v, SEM_WG)
    wu_cp = cp(wu_hbm, wu_v, SEM_WU)
    wd_cp = cp(wd_hbm, wd_v.at[:, pl.ds(0, D)], SEM_WD)

    def x_cp(t):
        r0 = _mo(t * TQ, TQ)
        return cp(x_hbm.at[0, pl.ds(r0, TQ), :], x_v.at[pl.ds(r0, TQ), :], SEM_X + t)

    def wm_cps(j):
        return [cp(wmod_hbm.at[:, pl.ds(i * KH + j * 128, 128)], wm_v.at[:, pl.ds((4 * j + i) * 128, 128)], SEM_WM + j)
                for i in range(4)]

    def wq0_cps(j):
        r0 = _mo((j % 2) * 128, 128)
        return [cp(wq_hbm.at[2 * i + j // 2, pl.ds(r0, 128), pl.ds(0, GW)],
                   wq_v.at[0, 2 * i + j // 2, pl.ds(r0, 128), pl.ds(0, GW)], SEM_WQ0 + j) for i in range(2)]

    def wmr_cp(i):
        c0 = 2 * D + min(i * NM, 32 - NM) * 128
        return cp(wmod_hbm.at[:, pl.ds(c0, NM * 128)], wmr_v.at[i], SEM_WMR + (0 if i < 2 else 1))

    def w_cps(s, c, n, sem):
        rows = pl.ds(_mo(c * 64, 64), n * 64)
        return [cp(wq_hbm.at[:, rows, pl.ds((s + 1) * GW, GW)], wq_v.at[s + 1, :, rows, pl.ds(0, GW)], sem),
                cp(wo_hbm.at[s, :, rows, :], wo_v.at[s, :, rows, :], sem)]

    w1_cps = w_cps(1, 0, 2, SEM_W + 4)
    wrest_cps = w_cps(1, 2, 2, SEM_W + 5) + w_cps(2, 0, 4, SEM_W + 5) + [cp(wo_hbm.at[3], wo_v.at[3], SEM_W + 5)]

    def out_copy(r0, n):
        return cp(out_v.at[pl.ds(r0, n), :], out_hbm.at[0, pl.ds(r0, n), :], SEM_OUT)

    for c_ in ([c_cp, x0_cp] + [c_ for j in range(NKC) for c_ in wm_cps(j) + wq0_cps(j)]
               + [x_cp(2), x_cp(3), x_cp(4), x_cp(5), k_cp, wr_cp, x_cp(6)] + w_cps(0, 0, 1, SEM_W)
               + [x_cp(7)] + w_cps(0, 1, 1, SEM_W + 1) + w_cps(0, 2, 1, SEM_W + 2) + w_cps(0, 3, 1, SEM_W + 3)
               + [v_cp, wmr_cp(0), wmr_cp(1)] + w1_cps + [wmr_cp(i) for i in range(2, NMC)] + wrest_cps + [wd_cp]):
        c_.start()

    def ln1_rows(base, off, n, lo=None):
        x = x_v.at[pl.ds(base, off + n)][off:off + n, :].astype(f32)
        if lo is not None:
            x = _gate(x, *lo)
        y = _ln(x) * _rows(mod_v[:, D:2 * D], n) + _rows(mod_v[:, 0:D], n)
        h_v.at[pl.ds(base, off + n)][off:off + n, :] = y.astype(bf16)
        return y

    def w_unit(src, dst, ch, u, los):
        rows = pl.ds(pl.multiple_of(ch * 64, 64), 64)
        src = src.at[:, rows]
        dst = dst.at[rows]

        def load(a, b):
            return src[a, 8 * u:8 * u + 8, b * QC:(b + 1) * QC].astype(f32)

        toks = []
        for i in range(1, 8):
            flag, tok = los[i - 1]
            outer = {}
            for a in range(2):
                for b in range(2):
                    v = _lin(B_COEF[i], lambda r, c: load(2 * r + a, 2 * c + b))
                    outer[a, b] = jnp.where(flag, jnp.concatenate([tok] * (QC // 128), axis=1), v) if a == b else v
            for j in range(1, 8):
                v = _lin(B_COEF[j], lambda a, b: outer[a, b])
                dst[8 * u:8 * u + 8, _col(i, j)] = v.astype(bf16)
                if j >= WTOK:
                    toks.append(v)
        return _token(*toks)

    def ln2_rows(base, off, n, valid=None, lo=None):
        av = _rows(aux_v[0], n)
        bv = _rows(aux_v[1], n)
        rv = _rows(aux_v[2], n)
        r_c = _rows(aux_v[3, :, 0:128], n)
        x2 = x_v.at[pl.ds(base, TQ)][off:off + n, :].astype(f32)
        if lo is not None:
            x2 = _gate(x2, *lo)
        m = jnp.mean(x2, axis=-1, keepdims=True)
        xc = x2 - m
        var = jnp.mean(xc * xc, axis=-1, keepdims=True)
        rs = lax.rsqrt(var + EPS)
        y = x2 + ((xc * rs) * av + bv)
        r = jnp.sum(xc * rv, axis=-1, keepdims=True) * rs
        out_v.at[pl.ds(base, TQ)][off:off + n, :] = y.astype(bf16)
        r = (jnp.broadcast_to(r, (n, 128)) + r_c).astype(bf16).astype(f32)
        if valid is not None:
            r = jnp.where(valid, r, -jnp.inf)
        mb = jnp.broadcast_to(m, (n, 128))
        rsb = jnp.broadcast_to(rs, (n, 128))
        best = best_v[0]
        bm = best_v[1]
        brs = best_v[2]
        bidx = bidx_v[0]
        rows = lax.broadcasted_iota(jnp.int32, (8, 128), 0)
        for j in range(n // 8):
            sl = slice(8 * j, 8 * (j + 1))
            upd = r[sl] > best
            best = jnp.where(upd, r[sl], best)
            bm = jnp.where(upd, mb[sl], bm)
            brs = jnp.where(upd, rsb[sl], brs)
            bidx = jnp.where(upd, rows + (base + (off + 8 * j)), bidx)
        best_v[0] = best
        best_v[1] = bm
        best_v[2] = brs
        bidx_v[0] = bidx
        return y, best

    flag_s[0] = 0
    c_cp.wait()
    cf = c_v[...].astype(f32)
    sc = (cf * jax.nn.sigmoid(cf)).astype(bf16)
    sc_v[...] = jnp.broadcast_to(sc, (16, D))
    scc_v[...] = jnp.broadcast_to(sc.astype(f32), (128, D)).T
    best_v[0] = jnp.full((8, 128), -jnp.inf, f32)
    best_v[1] = jnp.zeros((8, 128), f32)
    best_v[2] = jnp.zeros((8, 128), f32)
    bidx_v[0] = jnp.zeros((8, 128), jnp.int32)
    x0_cp.wait()

    def norm_rows(i, carry):
        r0 = pl.multiple_of(i * 64, 64)
        for t in range(2):
            (acc_v, accb_v)[t][pl.ds(r0, 64), 0:D] = _ln(x_v[pl.ds(t * TQ + r0, 64), :].astype(f32))
        return carry

    lax.fori_loop(0, TQ // 64, norm_rows, 0)

    def w1_unit(u, lo):
        r0 = pl.multiple_of(u * 8, 8)
        rq = pl.ds(pl.multiple_of((u % NU) * 8, 8), 8)
        half = (_gate(wq_v[0, u // NU, rq, 0:GW].astype(f32), *lo), wq_v[0, 2 + u // NU, rq, 0:GW].astype(f32))
        outs = [_lin(B_COEF[i], lambda r, c: half[r][:, (2 * p + c) * DH:(2 * p + c + 1) * DH])
                for p in range(REP // 2) for i in B_SUMS]
        wq1_v[pl.ds(r0, 8), 0:len(outs) * DH] = jnp.concatenate(outs, axis=1).astype(bf16)
        return _token(*[o_ for i, o_ in enumerate(outs) if i % 5 >= 3])

    def k_chunk(j, carry):
        cm = pl.multiple_of(j * 512, 512)
        wait_all(wm_v.at[:, pl.ds(cm, 512)], SEM_WM + j)
        cols = (pl.multiple_of(j * 128, 128), pl.multiple_of(KH + j * 128, 128))
        md = jnp.dot(sc_v[...], wm_v[:, pl.ds(cm, 512)], preferred_element_type=f32)[0:8].astype(bf16).astype(f32)
        for i, c0 in enumerate(cols):
            sa = md[:, i * 128:(i + 1) * 128] * QSCALE
            ca1 = (1.0 + md[:, (2 + i) * 128:(3 + i) * 128]) * QSCALE
            mod_v[:, pl.ds(c0, 128)] = sa
            mod_v[:, pl.ds(D + c0, 128)] = ca1
            nrm = jnp.concatenate([acc_v[:, pl.ds(c0, 128)], accb_v[:, pl.ds(c0, 128)]], axis=0)
            h_v[0:TP, pl.ds(c0, 128)] = (nrm * _rows(ca1, TP) + _rows(sa, TP)).astype(bf16)
        for c_ in wq0_cps(j):
            c_.wait()
        lhs = jnp.concatenate([h_v[0:TP, pl.ds(c0, 128)] for c0 in cols], axis=1)
        rhs = jnp.concatenate([wq_v[0, 2 * i + j // 2, pl.ds(pl.multiple_of((j % 2) * 128, 128), 128), 0:GW]
                               for i in range(2)], axis=0)
        flag = flag_s[0] > 0
        toks = {}
        for n_ in range(4):
            cs = slice(D + n_ * 256, D + (n_ + 1) * 256)
            lh = lhs
            if n_ - 2 in toks:
                lh = _gate1(lhs, flag, jnp.concatenate([toks[n_ - 2]] * 2, axis=0).astype(bf16))
            part = jnp.dot(lh, rhs[:, n_ * 256:(n_ + 1) * 256], preferred_element_type=f32)
            tot = jnp.where(j == 0, 0.0, jnp.concatenate([acc_v[:, cs], accb_v[:, cs]], axis=0)) + part
            acc_v[:, cs] = tot[0:TQ]
            accb_v[:, cs] = tot[TQ:TP]
            q_v[0, 0:TP, n_ * 256:(n_ + 1) * 256] = tot.astype(bf16)
            if n_ < 2:
                toks[n_] = _token(*[w1_unit(j * 16 + n_ * 8 + u, (flag, part[64 * u:64 * u + 8, 0:128]))
                                    for u in range(8)])
        return carry

    lax.fori_loop(0, NKC, k_chunk, 0)

    x_cp(2).wait()
    x_cp(3).wait()

    def q0_tile(t, rn, nln, units, q1s, q1lag, first=False):
        flag = flag_s[0] > 0
        a0 = _mo(t * TQ, TQ)
        h = h_v.at[pl.ds(a0, TQ), :] if first else h_v[pl.ds(a0, TQ), :]
        lhs = {}

        def hb(r, c):
            return h[r * HR:(r + 1) * HR, c * KH:(c + 1) * KH]

        def get_lhs(i):
            if i not in lhs:
                lhs[i] = (hb(*A_COEF[i][0][:2]) if len(A_COEF[i]) == 1 else
                          _lin(A_COEF[i], lambda r, c: hb(r, c).astype(f32)).astype(bf16))
            return lhs[i]

        prods = [(p, i) for p in range(REP // 2) for i in Q1ORD]
        if first:
            prods = [z for z in prods if z[1] in (4, 2)] + [z for z in prods if z[1] not in (4, 2)]
        combs = [_Combine() for _ in range(REP // 2)]
        jobs = [(lambda lo, r=r: _token(ln1_rows(_mo(rn, 16), 8 * r, 8, lo))) for r in range(nln)]
        nprod = 7 * REP // 2
        nslot = nprod - q1s - q1lag
        nuslot = nprod - Q1US - Q1ULAG
        toks = {}
        n_ = 0
        prev = None
        for p, i in prods:
            if i in B_SUMS:
                c0 = (p * 5 + B_SUMS.index(i)) * DH
                rhs = wq1_v[0:KH, c0:c0 + DH]
            else:
                r, c, _ = B_COEF[i][0]
                rhs = jnp.concatenate([wq_v[0, 2 * r + z, :, (2 * p + c) * DH:(2 * p + c + 1) * DH] for z in range(2)], axis=0)
            if n_ in toks:
                rhs = _gate1(rhs, flag, jnp.concatenate([_token(*toks[n_])] * 2, axis=0).astype(bf16))
            y = jnp.dot(get_lhs(i), rhs, preferred_element_type=f32)
            for r, c, v in combs[p].feed(i, y):
                q_v[0, pl.ds(_mo(a0 + r * HR, HR), HR), (2 * p + c) * DH:(2 * p + c + 1) * DH] = v.astype(bf16)
            if first and n_ < F2N:
                for k_ in range(n_ * 16 // F2N, (n_ + 1) * 16 // F2N):
                    r_ = (k_ * F2N * 8) % HR // 8 * 8
                    ln1_rows(a0, 8 * k_, 8, (flag, y[r_:r_ + 8]))
            sl = n_ - q1s
            if 0 <= sl < nslot:
                mine = jobs[sl * len(jobs) // nslot:(sl + 1) * len(jobs) // nslot]
                for k_, jb in enumerate(mine):
                    r_ = (k_ * HR // len(mine)) // 8 * 8
                    toks.setdefault(n_ + q1lag, []).append(jb((flag, y[r_:r_ + 8])))
            sl = n_ - Q1US
            if 0 <= sl < nuslot:
                mine = units[sl * len(units) // nuslot:(sl + 1) * len(units) // nuslot]
                for k_, jb in enumerate(mine):
                    src_ = y if prev is None else jnp.concatenate([prev, y], axis=0)
                    rr = [(src_.shape[0] - (7 - z) * min(Q1SP, src_.shape[0]) // 7) // 8 * 8 for z in range(7)]
                    toks.setdefault(n_ + Q1ULAG, []).append(jb([(flag, src_[r_:r_ + 8]) for r_ in rr]))
            prev = y
            n_ += 1

    def q0_b(t, carry):
        @pl.when(t + 2 < NT)
        def _():
            x_cp(t + 2).wait()

        for c_ in w_cps(0, t - T3B, 1, SEM_W + t - T3B):
            c_.wait()
        nu = NU // 4
        units = []
        for u in range(nu):
            units.append(lambda los, u=u: w_unit(wq_v.at[1], wqs_v.at[1], t - T3B, u, los))
            units.append(lambda los, u=u: w_unit(wo_v.at[0], wos_v.at[0], t - T3B, u, los))
        q0_tile(t, jnp.minimum(4 * TQ + (NL3 + (t - T3B) * NLB) * 8, S - NLB * 8), NLB, units, Q1S, Q1LAG)
        kt_v[t - T3B] = k_v[t - T3B].T
        return carry

    ln1_rows(2 * TQ, HR, HR)
    q0_tile(2, 3 * TQ, TQ // 8, [], A2S, A2LAG, True)
    x_cp(4).wait()
    x_cp(5).wait()
    q0_tile(3, 4 * TQ, NL3, [], A3S, A3LAG)
    k_cp.wait()
    lax.fori_loop(T3B, NT, q0_b, 0)
    wg_cp.start()
    wu_cp.start()
    v_cp.wait()
    wr_cp.wait()
    wait_all(wmr_v.at[pl.ds(0, 2)], SEM_WMR)
    for c_ in w1_cps:
        c_.wait()

    def body(i, last_group):
        flag = flag_s[0] > 0
        st = {}
        his = {}
        g = 3 if last_group else i // (NT // 2)
        qs = g % 2
        blk = i % (NT // 2)
        m0 = pl.multiple_of(blk * QR, QR)
        o_todo = []

        def pin(r_):
            return flag, st['V'][r_:r_ + 8]

        def add_hi(step, tk):
            his[step] = tk if step not in his else jnp.maximum(his[step], tk)

        def run(todo, n):
            for _ in range(n):
                todo.pop(0)(None)

        def flush():
            gates = {(GST if last_group else GSTB) * (k_ + 1): his.pop(s_) for k_, s_ in enumerate(sorted(his))}
            for k_ in range(len(o_todo)):
                o_todo.pop(0)(gates.get(k_))

        def qk(step, a0, hh):
            s = jnp.dot(q_v[qs, pl.ds(a0, TQ), hh * DH:(hh + 1) * DH], kt_v[g], preferred_element_type=f32)
            if step in his:
                s = _gate1(s, flag, his.pop(step))
            p = jnp.exp2(s - jnp.max(s, axis=-1, keepdims=True))
            ps = (p[:, 0:128] + p[:, 128:256]) + (p[:, 256:384] + p[:, 384:512])
            p = jnp.concatenate([p[:, 0:384], jnp.where(flag, ps, p[:, 384:512])], axis=1)
            return p.astype(bf16), jnp.sum(ps, axis=-1, keepdims=True)

        def pv(step, os_, pl_):
            p, l = pl_
            o = jnp.dot(p, v_v[g], preferred_element_type=f32)
            st['V'] = o
            os_.append(o * _recip(l))
            if last_group:
                add_hi(step + OHIC, _token(os_[-1]))
            elif OHIB and step < REP:
                add_hi(step + OHIB, _token(os_[-1]))

        def side_b(s_):
            los = [pin(r_) for r_ in (WPINS, WPINS2)[s_ // REP]]
            if s_ < REP:
                add_hi(s_ + 1, w_unit(wo_v.at[g + 1], wos_v.at[1 - qs], blk, s_ % REP, los))
            else:
                gq = jnp.minimum(g + 2, HKV - 1)
                add_hi(s_ + 1, w_unit(wq_v.at[gq], wqs_v.at[gq % 2], blk, s_ % REP, los))
            nn = NSTEPS
            ci = jnp.minimum(i, NMC - 1)
            if s_ < nn:
                lo = pin(NPIN)
                macc = st.get('macc')
                for rg in range(128 * s_ // nn, 128 * (s_ + 1) // nn):
                    xc_ = jnp.where(lo[0], lo[1], scc_v[8 * rg:8 * rg + 8, :])
                    pr_ = wmr_v[ci, 8 * rg:8 * rg + 8, :].astype(f32) * jnp.concatenate([xc_] * NM, axis=1)
                    macc = pr_ if macc is None else macc + pr_
                st['macc'] = macc
                add_hi(s_ + NHI, _token(macc))
                if s_ == nn - 1:
                    c0 = pl.multiple_of(2 * D + jnp.minimum(ci * NM, 32 - NM) * 128, 128)
                    tot_ = jnp.sum(macc, axis=0, keepdims=True).astype(bf16).astype(f32)
                    mod_v[:, pl.ds(c0, NM * 128)] = jnp.broadcast_to(tot_, (8, NM * 128))

        def side_c(s_):
            for k_, r_ in enumerate((LPINS, LPINS2)[s_ % 2]):
                off = ((s_ % REP) * len(LPINS) + k_) * 8
                if s_ < REP:
                    res = ln2_rows(pl.multiple_of(jnp.maximum(2 * blk - 1, 0) * TQ, TQ), off, 8, blk > 0, pin(r_))
                else:
                    res = ln2_rows(pl.multiple_of(2 * blk * TQ, TQ), off, 8, None, pin(r_))
                add_hi(s_ + LHI, _token(*res))

        for par in range(2):
            a0 = pl.multiple_of((2 * blk + par) * TQ, TQ)
            acc = (acc_v, accb_v)[par]
            os_ = []

            def h_blk(a, b, a0=a0):
                return h_v[pl.ds(pl.multiple_of(a0 + a * QR, QR), QR), b * QC:(b + 1) * QC]

            q_lhs = _LhsOps(lambda a, b, f=h_blk: f(a, b).astype(f32), h_blk)
            q_comb = _Combine2()

            def q_prod(i_, j_, a0=a0, q_lhs=q_lhs, q_comb=q_comb):
                y = jnp.dot(q_lhs.op(i_, j_), wqs_v[1 - qs, :, _col(i_, j_)], preferred_element_type=f32)
                for a, b, v in q_comb.feed(i_, j_, y):
                    r0 = pl.multiple_of(a0 + a * QR, QR)
                    q_v[1 - qs, pl.ds(r0, QR), b * QC:(b + 1) * QC] = v.astype(bf16)

            q_todo = [(lambda gate, i_=i_, j_=j_, f=q_prod: f(i_, j_)) for i_ in QORD for j_ in IORD]
            o_lhs = _LhsOps(lambda a, b, os_=os_: jnp.concatenate(
                [os_[2 * b][a * QR:(a + 1) * QR], os_[2 * b + 1][a * QR:(a + 1) * QR]], axis=1))
            o_comb = _Combine2()

            def o_prod(i_, j_, gate, acc=acc, o_lhs=o_lhs, o_comb=o_comb, a0=a0):
                lhs = o_lhs.op(i_, j_)
                if gate is not None:
                    lhs = _gate1(lhs, flag, jnp.concatenate([gate, gate], axis=0).astype(bf16))
                y = jnp.dot(lhs, wos_v[qs, :, _col(i_, j_)], preferred_element_type=f32)
                old = acc[pl.ds(m0, QR), _col(i_, j_)]
                if not last_group:
                    acc[pl.ds(m0, QR), _col(i_, j_)] = jnp.where(g == 0, 0.0, old) + y
                    return
                for a, b, v in o_comb.feed(i_, j_, old + y):
                    rs = pl.ds(pl.multiple_of(a0 + a * QR, QR), QR)
                    cx = slice(b * QC, (b + 1) * QC)
                    ga = _rows(mod_v[:, 2 * D + b * QC:2 * D + (b + 1) * QC], QR)
                    x_v[rs, cx] = (x_v[rs, cx].astype(f32) + ga * v).astype(bf16)

            s0 = par * REP
            if last_group:
                for hh in range(0, REP, 2):
                    sp0 = qk(s0 + hh, a0, hh)
                    sp1 = qk(s0 + hh + 1, a0, hh + 1)
                    pv(s0 + hh, os_, sp0)
                    side_c(s0 + hh)
                    pv(s0 + hh + 1, os_, sp1)
                    side_c(s0 + hh + 1)
            else:
                for hh in range(REP):
                    sp = qk(s0 + hh, a0, hh)
                    run(q_todo, (QRUN, QRUN2)[par][hh])
                    pv(s0 + hh, os_, sp)
                    if par == 1:
                        run(o_todo, ORUN[hh])
                    side_b(s0 + hh)
            o_todo.extend([(lambda gate, i_=i_, j_=j_, f=o_prod: f(i_, j_, gate))
                           for i_ in (CORD if last_group else OORD) for j_ in (IORDC if last_group else IORDO)])
            if last_group or par == 1:
                flush()
        if last_group:
            @pl.when(blk > 0)
            def _():
                out_copy(pl.multiple_of((2 * blk - 1) * TQ, TQ), TQ).start()

            out_copy(pl.multiple_of(2 * blk * TQ, TQ), TQ).start()

    def make_aux():
        sb_ = mod_v[:, 3 * D:4 * D]
        cb1_ = 1.0 + mod_v[:, 4 * D:5 * D]
        gb_ = mod_v[:, 5 * D:6 * D]
        wr8 = wr_v[...].astype(f32)
        wr_ = jnp.concatenate([wr8[r_:r_ + 1, :] for r_ in range(8)], axis=1)
        aux_v[0] = gb_ * cb1_
        aux_v[1] = gb_ * sb_
        aux_v[2] = cb1_ * wr_
        aux_v[3] = jnp.broadcast_to(jnp.sum(sb_ * wr_, axis=-1, keepdims=True), (8, D))

    def body_b(i, carry):
        @pl.when(i == 2)
        def _():
            wait_all(wmr_v.at[pl.ds(2, NMC - 2)], SEM_WMR + 1)
            for c_ in wrest_cps:
                c_.wait()

        body(i, False)
        return carry

    lax.fori_loop(0, 3 * NT // 2, body_b, 0)

    wg_cp.wait()
    wu_cp.wait()
    wd_cp.wait()
    make_aux()

    def body_c(i, carry):
        body(i, True)
        return carry

    lax.fori_loop(0, NT // 2, body_c, 0)

    ln2_rows((NT - 1) * TQ, 0, TQ)
    out_copy((NT - 1) * TQ, TQ).start()

    best = best_v[0]
    bidx = bidx_v[0]
    rmax = jnp.max(best, axis=0, keepdims=True)
    idx_v = jnp.min(jnp.where(best == rmax, bidx, S), axis=0, keepdims=True)
    idx = jnp.minimum(idx_v[0, 0], S - 1)
    g0 = pl.multiple_of((idx // 8) * 8, 8)
    sb = mod_v[:, 3 * D:4 * D]
    cb = mod_v[:, 4 * D:5 * D]
    gb = mod_v[:, 5 * D:6 * D]
    x2 = x_v[pl.ds(g0, 8), :].astype(f32)
    h2 = (x2 - best_v[1][:, 0:1]) * best_v[2][:, 0:1] * (1.0 + cb) + sb
    h2b = h2.astype(bf16)
    sel = (lax.broadcasted_iota(jnp.int32, (8, 1), 0) + g0) == idx
    flag = flag_s[0] > 0
    nf = F // 128
    strips = [(k_, j) for j in range(nf) for k_ in 'gu'] + [('d', j) for j in range(FD, nf)]
    gate_r, a_strips, vtok = {}, {}, {}
    y = None
    yv = None
    pos = 0
    for i, (kind, j) in enumerate(strips):
        hi = vtok.get(i - FLAG_)
        if kind == 'd':
            lhs = a_strips[j]
            if hi is not None:
                lhs = jnp.where(flag, hi.astype(bf16), lhs)
            r_ = jnp.dot(lhs, wd_v[j * 128:(j + 1) * 128, 0:D], preferred_element_type=f32)
            y = r_ if y is None else y + r_
            tok_ = r_[:, D - 128:D]
        else:
            lhs = h2b if hi is None else _gate1(h2b, flag, hi.astype(bf16))
            w_ref = wg_v if kind == 'g' else wu_v
            tok_ = jnp.dot(lhs, w_ref[:, j * 128:(j + 1) * 128], preferred_element_type=f32)
            if kind == 'g':
                gate_r[j] = tok_
            else:
                a_strips[j] = (gate_r[j] * jax.nn.sigmoid(gate_r[j]) * tok_).astype(bf16)
                if j < FD:
                    row = jnp.sum(jnp.where(sel, a_strips[j].astype(f32), 0.0), axis=0, keepdims=True)
                    acol_v[j * 128:(j + 1) * 128, :] = jnp.broadcast_to(row, (128, 128)).T
        if i >= FI0 and pos < FD * 16:
            end = min(pos + FVR, FD * 16) if i < len(strips) - 1 else FD * 16
            for rg in range(pos, end):
                col = jnp.where(flag, tok_, acol_v[8 * rg:8 * rg + 8, :])
                pr_ = wd_v[8 * rg:8 * rg + 8, 0:D].astype(f32) * jnp.concatenate([col] * (D // 128), axis=1)
                yv = pr_ if yv is None else yv + pr_
            pos = end
            vtok[i] = _token(yv)
    y = (y + jnp.sum(yv, axis=0, keepdims=True)) * jax.nn.sigmoid(rmax[:, 0:1])
    out_copy(0, S).wait()
    new = (x2 + gb * (h2 + y)).astype(bf16)
    out_v[pl.ds(g0, 8), :] = jnp.where(sel, new, out_v[pl.ds(g0, 8), :])
    fix = out_copy(g0, 8)
    fix.start()
    fix.wait()


@jax.jit
def pallas_adaLN_cond__sliding_block_cached__moe_arch_mod__prompt_kernel(
    A_x, A_k_cache, A_v_cache, A_wq, A_wo, B_x, B_w_r, B_w_gate, B_w_up, B_w_down, c, w_mod,
):
    del B_x
    any_spec = pl.BlockSpec(memory_space=pl.ANY)
    return pl.pallas_call(
        _kernel,
        out_shape=jax.ShapeDtypeStruct(A_x.shape, A_x.dtype),
        in_specs=[any_spec] * 11,
        out_specs=any_spec,
        scratch_shapes=[
            pltpu.VMEM((S, D), bf16),
            pltpu.VMEM((S, D), bf16),
            pltpu.VMEM((2, S, GW), bf16),
            pltpu.VMEM((S // 8, 49 * QC), f32),
            pltpu.VMEM((S // 8, 49 * QC), f32),
            pltpu.VMEM((NMC, D, NM * 128), bf16),
            pltpu.VMEM((HKV, 4, QC, GW + PADW), bf16),
            pltpu.VMEM((2, QC, 49 * QC), bf16),
            pltpu.VMEM((HKV, 4, QC, D), bf16),
            pltpu.VMEM((2, QC, 49 * QC), bf16),
            pltpu.VMEM((D, F), bf16),
            pltpu.VMEM((D, F), bf16),
            pltpu.VMEM((F, D + PADD), bf16),
            pltpu.VMEM((HKV, W, DH), bf16),
            pltpu.VMEM((HKV, W, DH), bf16),
            pltpu.VMEM((HKV, DH, W), bf16),
            pltpu.VMEM((8, 1, D), bf16),
            pltpu.VMEM((16, 8, 128), bf16),
            pltpu.VMEM((16, D), bf16),
            pltpu.VMEM((D, 128), f32),
            pltpu.VMEM((2 * D, 128), f32),
            pltpu.VMEM((8, 6 * D), f32),
            pltpu.VMEM((8, 8, 128), f32),
            pltpu.VMEM((8, 8, 128), jnp.int32),
            pltpu.VMEM((4, 8, D), f32),
            pltpu.SMEM((1,), jnp.int32),
            pltpu.SemaphoreType.DMA((NSEM,)),
        ],
        compiler_params=pltpu.CompilerParams(vmem_limit_bytes=126 * 1024 * 1024,
                                             disable_semaphore_checks=True,
                                             disable_bounds_checks=True),
    )(A_x, A_k_cache, A_v_cache, A_wq.reshape(4, QC, HQ * DH), A_wo.reshape(HKV, 4, QC, D), B_w_r.reshape(8, 128), B_w_gate, B_w_up, B_w_down, c, w_mod)
```

```python
import math

import jax
import jax.numpy as jnp
from jax import lax
from jax.experimental import pallas as pl
from jax.experimental.pallas import tpu as pltpu


S = 2048
D = 1024
HQ = 32
HKV = 4
REP = HQ // HKV
DH = 128
GW = REP * DH
W = 512
F = 3584
EPS = 1e-5
TQ = 256
QR = TQ // 4
QC = D // 4
NT = S // TQ
TP = 512
NKC = 4
HR = TQ // 2
KH = D // 2
PADW = 128
PADD = 256
NM = 3
NMC = 11
T3B = 4
NU = QC // 8
FD = 15
FI0 = 8
FLAG_ = 4
FVR = 4
QORD = (3, 6, 5, 1, 2, 7, 4)
OORD = (3, 6, 5, 1, 2, 7, 4)
CORD = (3, 6, 1, 2, 4, 7, 5)
IORD = (4, 2, 1, 7, 5, 3, 6)
QRUN = (6, 6, 6, 7, 6, 6, 6, 6)
ORUN = (6, 6, 7, 6, 7, 5, 6, 6)
LPINS = (24, 80, 136, 192)
WPINS = (32, 64, 96, 128, 160, 192, 224)
WPINS2 = (0, 32, 72, 104, 144, 176, 216)
QRUN2 = (7, 8, 6, 5, 6, 6, 5, 6)
IORDO = (4, 2, 1, 7, 5, 3, 6)
LPINS2 = (0, 56, 112, 168)
NSTEPS = 14
OHIB = 0
NPIN = 192
LHI = 2
OHIC = 3
NHI = 2
GST = 4
GSTB = 6
WTOK = 7
F2N = 2
NL3 = 62
NLB = -(-(128 - NL3) // 6) * 2
A2S = 8
A2LAG = 5
A3S = 0
A3LAG = 7
Q1ORD = (4, 2, 7, 1, 5, 3, 6)
Q1SP = 160
Q1S = 3
Q1LAG = 5
Q1US = 2
Q1ULAG = 3
IORDC = (4, 2, 7, 1, 5, 3, 6)
QSCALE = (DH ** -0.5) * math.log2(math.e)

f32 = jnp.float32
bf16 = jnp.bfloat16

(SEM_C, SEM_WR, SEM_X0, SEM_K, SEM_V, SEM_WG, SEM_WU, SEM_WD, SEM_OUT) = range(9)
SEM_X = 9
SEM_W = SEM_X + NT
SEM_WQ0 = SEM_W + 6
SEM_WM = SEM_WQ0 + NKC
SEM_WMR = SEM_WM + NKC
NSEM = SEM_WMR + 2

A_COEF = {1: ((0, 0, 1), (1, 1, 1)), 2: ((1, 0, 1), (1, 1, 1)), 3: ((0, 0, 1),), 4: ((1, 1, 1),),
          5: ((0, 0, 1), (0, 1, 1)), 6: ((1, 0, 1), (0, 0, -1)), 7: ((0, 1, 1), (1, 1, -1))}
B_COEF = {1: ((0, 0, 1), (1, 1, 1)), 2: ((0, 0, 1),), 3: ((0, 1, 1), (1, 1, -1)), 4: ((1, 0, 1), (0, 0, -1)),
          5: ((1, 1, 1),), 6: ((0, 0, 1), (0, 1, 1)), 7: ((1, 0, 1), (1, 1, 1))}
C_COEF = {(0, 0): {1: 1, 4: 1, 5: -1, 7: 1}, (0, 1): {3: 1, 5: 1}, (1, 0): {2: 1, 4: 1},
          (1, 1): {1: 1, 2: -1, 3: 1, 6: 1}}


B_SUMS = (1, 3, 4, 6, 7)


def _lin(coef, get):
    v = get(coef[0][0], coef[0][1])
    for r, c, s in coef[1:]:
        v = v + get(r, c) if s > 0 else v - get(r, c)
    return v


def _col(i, j):
    c0 = ((i - 1) * 7 + j - 1) * QC
    return slice(c0, c0 + QC)


class _Combine:
    def __init__(self):
        self.part = {}

    def feed(self, i, v):
        done = []
        for key, coef in C_COEF.items():
            if i not in coef:
                continue
            s = coef[i]
            if key not in self.part:
                cur = (v, s, 1)
            else:
                u, su, n = self.part[key]
                if s == su:
                    cur = (u + v, s, n + 1)
                elif su > 0:
                    cur = (u - v, 1, n + 1)
                else:
                    cur = (v - u, 1, n + 1)
            self.part[key] = cur
            if cur[2] == len(coef):
                assert cur[1] > 0
                done.append((key[0], key[1], cur[0]))
        return done


class _Combine2:
    def __init__(self):
        self.inner = {}
        self.outer = {}

    def feed(self, i, j, v):
        done = []
        for r, c, u in self.inner.setdefault(i, _Combine()).feed(j, v):
            for r2, c2, w in self.outer.setdefault((r, c), _Combine()).feed(i, u):
                done.append((2 * r2 + r, 2 * c2 + c, w))
        return done


class _LhsOps:
    def __init__(self, get, get_bf16=None):
        self.get, self.get_bf16, self.cache = get, get_bf16, {}

    def outer(self, i, a, b):
        if len(A_COEF[i]) == 1:
            r, c, _ = A_COEF[i][0]
            return self.get(2 * r + a, 2 * c + b)
        if (i, a, b) not in self.cache:
            self.cache[i, a, b] = _lin(A_COEF[i], lambda r, c: self.get(2 * r + a, 2 * c + b))
        return self.cache[i, a, b]

    def op(self, i, j):
        if self.get_bf16 is not None and len(A_COEF[i]) == 1 and len(A_COEF[j]) == 1:
            return self.get_bf16(2 * A_COEF[i][0][0] + A_COEF[j][0][0], 2 * A_COEF[i][0][1] + A_COEF[j][0][1])
        return _lin(A_COEF[j], lambda a, b: self.outer(i, a, b)).astype(bf16)


def _ln(x):
    m = jnp.mean(x, axis=-1, keepdims=True)
    xc = x - m
    v = jnp.mean(xc * xc, axis=-1, keepdims=True)
    return xc * lax.rsqrt(v + EPS)


def _recip(l):
    r = pl.reciprocal(l, approx=True)
    return r * (2.0 - l * r)


def _mo(x, m):
    return x if isinstance(x, int) else pl.multiple_of(x, m)


def _rows(v8, n):
    return v8 if n == 8 else jnp.concatenate([v8] * (n // 8), axis=0)


def _gate(x, flag, tok):
    xs = jnp.where(flag, _rows(tok, x.shape[0]), x[:, 0:128])
    return xs if x.shape[1] == 128 else jnp.concatenate([xs, x[:, 128:]], axis=1)


def _gate1(x, flag, tok):
    r = tok.shape[0]
    x0 = jnp.where(flag, tok, x[0:r, 0:128])
    if x.shape[1] > 128:
        x0 = jnp.concatenate([x0, x[0:r, 128:]], axis=1)
    return x0 if x.shape[0] == r else jnp.concatenate([x0, x[r:]], axis=0)


def _token(*ys):
    u = None
    for y in ys:
        for i in range(y.shape[0] // 8):
            for j in range(y.shape[1] // 128):
                v = y[8 * i:8 * i + 8, 128 * j:128 * j + 128]
                u = v if u is None else jnp.maximum(u, v)
    return u


def _kernel(x_hbm, k_hbm, v_hbm, wq_hbm, wo_hbm, wr_hbm, wg_hbm, wu_hbm, wd_hbm, c_hbm, wmod_hbm,
            out_hbm,
            x_v, h_v, q_v, acc_v, accb_v, wmr_v, wq_v, wqs_v, wo_v, wos_v, wg_v, wu_v, wd_v,
            k_v, v_v, kt_v, c_v8, wr_v8, sc_v, scc_v, acol_v, mod_v, best_v, bidx_v, aux_v, flag_s, sems):
    sk = k_hbm.shape[2]
    c_v = c_v8.at[0]
    wr_v = wr_v8.at[0]
    out_v = h_v
    wq1_v = wu_v
    wm_v = wg_v

    def cp(src, dst, i):
        return pltpu.make_async_copy(src, dst, sems.at[i])

    def wait_all(view, sem):
        cp(view, view, sem).wait()

    c_cp = cp(c_hbm, c_v, SEM_C)
    wr_cp = cp(wr_hbm, wr_v, SEM_WR)
    x0_cp = cp(x_hbm.at[0, pl.ds(0, TP), :], x_v.at[pl.ds(0, TP), :], SEM_X0)
    k_cp = cp(k_hbm.at[0, :, pl.ds(sk - W, W), :], k_v, SEM_K)
    v_cp = cp(v_hbm.at[0, :, pl.ds(sk - W, W), :], v_v, SEM_V)
    wg_cp = cp(wg_hbm, wg_v, SEM_WG)
    wu_cp = cp(wu_hbm, wu_v, SEM_WU)
    wd_cp = cp(wd_hbm, wd_v.at[:, pl.ds(0, D)], SEM_WD)

    def x_cp(t):
        r0 = _mo(t * TQ, TQ)
        return cp(x_hbm.at[0, pl.ds(r0, TQ), :], x_v.at[pl.ds(r0, TQ), :], SEM_X + t)

    def wm_cps(j):
        return [cp(wmod_hbm.at[:, pl.ds(i * KH + j * 128, 128)], wm_v.at[:, pl.ds((4 * j + i) * 128, 128)], SEM_WM + j)
                for i in range(4)]

    def wq0_cps(j):
        r0 = _mo((j % 2) * 128, 128)
        return [cp(wq_hbm.at[2 * i + j // 2, pl.ds(r0, 128), pl.ds(0, GW)],
                   wq_v.at[0, 2 * i + j // 2, pl.ds(r0, 128), pl.ds(0, GW)], SEM_WQ0 + j) for i in range(2)]

    def wmr_cp(i):
        c0 = 2 * D + min(i * NM, 32 - NM) * 128
        return cp(wmod_hbm.at[:, pl.ds(c0, NM * 128)], wmr_v.at[i], SEM_WMR + (0 if i < 2 else 1))

    def w_cps(s, c, n, sem):
        rows = pl.ds(_mo(c * 64, 64), n * 64)
        return [cp(wq_hbm.at[:, rows, pl.ds((s + 1) * GW, GW)], wq_v.at[s + 1, :, rows, pl.ds(0, GW)], sem),
                cp(wo_hbm.at[s, :, rows, :], wo_v.at[s, :, rows, :], sem)]

    w1_cps = w_cps(1, 0, 2, SEM_W + 4)
    wrest_cps = w_cps(1, 2, 2, SEM_W + 5) + w_cps(2, 0, 4, SEM_W + 5) + [cp(wo_hbm.at[3], wo_v.at[3], SEM_W + 5)]

    def out_copy(r0, n):
        return cp(out_v.at[pl.ds(r0, n), :], out_hbm.at[0, pl.ds(r0, n), :], SEM_OUT)

    for c_ in ([c_cp, x0_cp] + [c_ for j in range(NKC) for c_ in wm_cps(j) + wq0_cps(j)]
               + [x_cp(2), x_cp(3), x_cp(4), x_cp(5), k_cp, wr_cp, x_cp(6)] + w_cps(0, 0, 1, SEM_W)
               + [x_cp(7)] + w_cps(0, 1, 1, SEM_W + 1) + w_cps(0, 2, 1, SEM_W + 2) + w_cps(0, 3, 1, SEM_W + 3)
               + [v_cp, wmr_cp(0), wmr_cp(1)] + w1_cps + [wmr_cp(i) for i in range(2, NMC)] + wrest_cps + [wd_cp]):
        c_.start()

    def ln1_rows(base, off, n, lo=None):
        x = x_v.at[pl.ds(base, off + n)][off:off + n, :].astype(f32)
        if lo is not None:
            x = _gate(x, *lo)
        y = _ln(x) * _rows(mod_v[:, D:2 * D], n) + _rows(mod_v[:, 0:D], n)
        h_v.at[pl.ds(base, off + n)][off:off + n, :] = y.astype(bf16)
        return y

    def w_unit(src, dst, ch, u, los):
        rows = pl.ds(pl.multiple_of(ch * 64, 64), 64)
        src = src.at[:, rows]
        dst = dst.at[rows]

        def load(a, b):
            return src[a, 8 * u:8 * u + 8, b * QC:(b + 1) * QC].astype(f32)

        toks = []
        for i in range(1, 8):
            flag, tok = los[i - 1]
            outer = {}
            for a in range(2):
                for b in range(2):
                    v = _lin(B_COEF[i], lambda r, c: load(2 * r + a, 2 * c + b))
                    outer[a, b] = jnp.where(flag, jnp.concatenate([tok] * (QC // 128), axis=1), v) if a == b else v
            for j in range(1, 8):
                v = _lin(B_COEF[j], lambda a, b: outer[a, b])
                dst[8 * u:8 * u + 8, _col(i, j)] = v.astype(bf16)
                if j >= WTOK:
                    toks.append(v)
        return _token(*toks)

    def ln2_rows(base, off, n, valid=None, lo=None):
        av = _rows(aux_v[0], n)
        bv = _rows(aux_v[1], n)
        rv = _rows(aux_v[2], n)
        r_c = _rows(aux_v[3, :, 0:128], n)
        x2 = x_v.at[pl.ds(base, TQ)][off:off + n, :].astype(f32)
        if lo is not None:
            x2 = _gate(x2, *lo)
        m = jnp.mean(x2, axis=-1, keepdims=True)
        xc = x2 - m
        var = jnp.mean(xc * xc, axis=-1, keepdims=True)
        rs = lax.rsqrt(var + EPS)
        y = x2 + ((xc * rs) * av + bv)
        r = jnp.sum(xc * rv, axis=-1, keepdims=True) * rs
        out_v.at[pl.ds(base, TQ)][off:off + n, :] = y.astype(bf16)
        r = (jnp.broadcast_to(r, (n, 128)) + r_c).astype(bf16).astype(f32)
        if valid is not None:
            r = jnp.where(valid, r, -jnp.inf)
        mb = jnp.broadcast_to(m, (n, 128))
        rsb = jnp.broadcast_to(rs, (n, 128))
        best = best_v[0]
        bm = best_v[1]
        brs = best_v[2]
        bidx = bidx_v[0]
        rows = lax.broadcasted_iota(jnp.int32, (8, 128), 0)
        for j in range(n // 8):
            sl = slice(8 * j, 8 * (j + 1))
            upd = r[sl] > best
            best = jnp.where(upd, r[sl], best)
            bm = jnp.where(upd, mb[sl], bm)
            brs = jnp.where(upd, rsb[sl], brs)
            bidx = jnp.where(upd, rows + (base + (off + 8 * j)), bidx)
        best_v[0] = best
        best_v[1] = bm
        best_v[2] = brs
        bidx_v[0] = bidx
        return y, best

    flag_s[0] = 0
    c_cp.wait()
    cf = c_v[...].astype(f32)
    sc = (cf * jax.nn.sigmoid(cf)).astype(bf16)
    sc_v[...] = jnp.broadcast_to(sc, (16, D))
    scc_v[...] = jnp.broadcast_to(sc.astype(f32), (128, D)).T
    best_v[0] = jnp.full((8, 128), -jnp.inf, f32)
    best_v[1] = jnp.zeros((8, 128), f32)
    best_v[2] = jnp.zeros((8, 128), f32)
    bidx_v[0] = jnp.zeros((8, 128), jnp.int32)
    x0_cp.wait()

    def norm_rows(i, carry):
        r0 = pl.multiple_of(i * 64, 64)
        for t in range(2):
            (acc_v, accb_v)[t][pl.ds(r0, 64), 0:D] = _ln(x_v[pl.ds(t * TQ + r0, 64), :].astype(f32))
        return carry

    lax.fori_loop(0, TQ // 64, norm_rows, 0)

    def w1_unit(u, lo):
        r0 = pl.multiple_of(u * 8, 8)
        rq = pl.ds(pl.multiple_of((u % NU) * 8, 8), 8)
        half = (_gate(wq_v[0, u // NU, rq, 0:GW].astype(f32), *lo), wq_v[0, 2 + u // NU, rq, 0:GW].astype(f32))
        outs = [_lin(B_COEF[i], lambda r, c: half[r][:, (2 * p + c) * DH:(2 * p + c + 1) * DH])
                for p in range(REP // 2) for i in B_SUMS]
        wq1_v[pl.ds(r0, 8), 0:len(outs) * DH] = jnp.concatenate(outs, axis=1).astype(bf16)
        return _token(*[o_ for i, o_ in enumerate(outs) if i % 5 >= 3])

    def k_chunk(j, carry):
        cm = pl.multiple_of(j * 512, 512)
        wait_all(wm_v.at[:, pl.ds(cm, 512)], SEM_WM + j)
        cols = (pl.multiple_of(j * 128, 128), pl.multiple_of(KH + j * 128, 128))
        md = jnp.dot(sc_v[...], wm_v[:, pl.ds(cm, 512)], preferred_element_type=f32)[0:8].astype(bf16).astype(f32)
        for i, c0 in enumerate(cols):
            sa = md[:, i * 128:(i + 1) * 128] * QSCALE
            ca1 = (1.0 + md[:, (2 + i) * 128:(3 + i) * 128]) * QSCALE
            mod_v[:, pl.ds(c0, 128)] = sa
            mod_v[:, pl.ds(D + c0, 128)] = ca1
            nrm = jnp.concatenate([acc_v[:, pl.ds(c0, 128)], accb_v[:, pl.ds(c0, 128)]], axis=0)
            h_v[0:TP, pl.ds(c0, 128)] = (nrm * _rows(ca1, TP) + _rows(sa, TP)).astype(bf16)
        for c_ in wq0_cps(j):
            c_.wait()
        lhs = jnp.concatenate([h_v[0:TP, pl.ds(c0, 128)] for c0 in cols], axis=1)
        rhs = jnp.concatenate([wq_v[0, 2 * i + j // 2, pl.ds(pl.multiple_of((j % 2) * 128, 128), 128), 0:GW]
                               for i in range(2)], axis=0)
        flag = flag_s[0] > 0
        toks = {}
        for n_ in range(4):
            cs = slice(D + n_ * 256, D + (n_ + 1) * 256)
            lh = lhs
            if n_ - 2 in toks:
                lh = _gate1(lhs, flag, jnp.concatenate([toks[n_ - 2]] * 2, axis=0).astype(bf16))
            part = jnp.dot(lh, rhs[:, n_ * 256:(n_ + 1) * 256], preferred_element_type=f32)
            tot = jnp.where(j == 0, 0.0, jnp.concatenate([acc_v[:, cs], accb_v[:, cs]], axis=0)) + part
            acc_v[:, cs] = tot[0:TQ]
            accb_v[:, cs] = tot[TQ:TP]
            q_v[0, 0:TP, n_ * 256:(n_ + 1) * 256] = tot.astype(bf16)
            if n_ < 2:
                toks[n_] = _token(*[w1_unit(j * 16 + n_ * 8 + u, (flag, part[64 * u:64 * u + 8, 0:128]))
                                    for u in range(8)])
        return carry

    lax.fori_loop(0, NKC, k_chunk, 0)

    x_cp(2).wait()
    x_cp(3).wait()

    def q0_tile(t, rn, nln, units, q1s, q1lag, first=False):
        flag = flag_s[0] > 0
        a0 = _mo(t * TQ, TQ)
        h = h_v.at[pl.ds(a0, TQ), :] if first else h_v[pl.ds(a0, TQ), :]
        lhs = {}

        def hb(r, c):
            return h[r * HR:(r + 1) * HR, c * KH:(c + 1) * KH]

        def get_lhs(i):
            if i not in lhs:
                lhs[i] = (hb(*A_COEF[i][0][:2]) if len(A_COEF[i]) == 1 else
                          _lin(A_COEF[i], lambda r, c: hb(r, c).astype(f32)).astype(bf16))
            return lhs[i]

        prods = [(p, i) for p in range(REP // 2) for i in Q1ORD]
        if first:
            prods = [z for z in prods if z[1] in (4, 2)] + [z for z in prods if z[1] not in (4, 2)]
        combs = [_Combine() for _ in range(REP // 2)]
        jobs = [(lambda lo, r=r: _token(ln1_rows(_mo(rn, 16), 8 * r, 8, lo))) for r in range(nln)]
        nprod = 7 * REP // 2
        nslot = nprod - q1s - q1lag
        nuslot = nprod - Q1US - Q1ULAG
        toks = {}
        n_ = 0
        prev = None
        for p, i in prods:
            if i in B_SUMS:
                c0 = (p * 5 + B_SUMS.index(i)) * DH
                rhs = wq1_v[0:KH, c0:c0 + DH]
            else:
                r, c, _ = B_COEF[i][0]
                rhs = jnp.concatenate([wq_v[0, 2 * r + z, :, (2 * p + c) * DH:(2 * p + c + 1) * DH] for z in range(2)], axis=0)
            if n_ in toks:
                rhs = _gate1(rhs, flag, jnp.concatenate([_token(*toks[n_])] * 2, axis=0).astype(bf16))
            y = jnp.dot(get_lhs(i), rhs, preferred_element_type=f32)
            for r, c, v in combs[p].feed(i, y):
                q_v[0, pl.ds(_mo(a0 + r * HR, HR), HR), (2 * p + c) * DH:(2 * p + c + 1) * DH] = v.astype(bf16)
            if first and n_ < F2N:
                for k_ in range(n_ * 16 // F2N, (n_ + 1) * 16 // F2N):
                    r_ = (k_ * F2N * 8) % HR // 8 * 8
                    ln1_rows(a0, 8 * k_, 8, (flag, y[r_:r_ + 8]))
            sl = n_ - q1s
            if 0 <= sl < nslot:
                mine = jobs[sl * len(jobs) // nslot:(sl + 1) * len(jobs) // nslot]
                for k_, jb in enumerate(mine):
                    r_ = (k_ * HR // len(mine)) // 8 * 8
                    toks.setdefault(n_ + q1lag, []).append(jb((flag, y[r_:r_ + 8])))
            sl = n_ - Q1US
            if 0 <= sl < nuslot:
                mine = units[sl * len(units) // nuslot:(sl + 1) * len(units) // nuslot]
                for k_, jb in enumerate(mine):
                    src_ = y if prev is None else jnp.concatenate([prev, y], axis=0)
                    rr = [(src_.shape[0] - (7 - z) * min(Q1SP, src_.shape[0]) // 7) // 8 * 8 for z in range(7)]
                    toks.setdefault(n_ + Q1ULAG, []).append(jb([(flag, src_[r_:r_ + 8]) for r_ in rr]))
            prev = y
            n_ += 1

    def q0_b(t, carry):
        @pl.when(t + 2 < NT)
        def _():
            x_cp(t + 2).wait()

        for c_ in w_cps(0, t - T3B, 1, SEM_W + t - T3B):
            c_.wait()
        nu = NU // 4
        units = []
        for u in range(nu):
            units.append(lambda los, u=u: w_unit(wq_v.at[1], wqs_v.at[1], t - T3B, u, los))
            units.append(lambda los, u=u: w_unit(wo_v.at[0], wos_v.at[0], t - T3B, u, los))
        q0_tile(t, jnp.minimum(4 * TQ + (NL3 + (t - T3B) * NLB) * 8, S - NLB * 8), NLB, units, Q1S, Q1LAG)
        kt_v[t - T3B] = k_v[t - T3B].T
        return carry

    ln1_rows(2 * TQ, HR, HR)
    q0_tile(2, 3 * TQ, TQ // 8, [], A2S, A2LAG, True)
    x_cp(4).wait()
    x_cp(5).wait()
    q0_tile(3, 4 * TQ, NL3, [], A3S, A3LAG)
    k_cp.wait()
    lax.fori_loop(T3B, NT, q0_b, 0)
    wg_cp.start()
    wu_cp.start()
    v_cp.wait()
    wr_cp.wait()
    wait_all(wmr_v.at[pl.ds(0, 2)], SEM_WMR)
    for c_ in w1_cps:
        c_.wait()

    def body(i, last_group):
        flag = flag_s[0] > 0
        st = {}
        his = {}
        g = 3 if last_group else i // (NT // 2)
        qs = g % 2
        blk = i % (NT // 2)
        m0 = pl.multiple_of(blk * QR, QR)
        o_todo = []

        def pin(r_):
            return flag, st['V'][r_:r_ + 8]

        def add_hi(step, tk):
            his[step] = tk if step not in his else jnp.maximum(his[step], tk)

        def run(todo, n):
            for _ in range(n):
                todo.pop(0)(None)

        def flush():
            gates = {(GST if last_group else GSTB) * (k_ + 1): his.pop(s_) for k_, s_ in enumerate(sorted(his))}
            for k_ in range(len(o_todo)):
                o_todo.pop(0)(gates.get(k_))

        def qk(step, a0, hh):
            s = jnp.dot(q_v[qs, pl.ds(a0, TQ), hh * DH:(hh + 1) * DH], kt_v[g], preferred_element_type=f32)
            if step in his:
                s = _gate1(s, flag, his.pop(step))
            p = jnp.exp2(s - jnp.max(s, axis=-1, keepdims=True))
            ps = (p[:, 0:128] + p[:, 128:256]) + (p[:, 256:384] + p[:, 384:512])
            p = jnp.concatenate([p[:, 0:384], jnp.where(flag, ps, p[:, 384:512])], axis=1)
            return p.astype(bf16), jnp.sum(ps, axis=-1, keepdims=True)

        def pv(step, os_, pl_):
            p, l = pl_
            o = jnp.dot(p, v_v[g], preferred_element_type=f32)
            st['V'] = o
            os_.append(o * _recip(l))
            if last_group:
                add_hi(step + OHIC, _token(os_[-1]))
            elif OHIB and step < REP:
                add_hi(step + OHIB, _token(os_[-1]))

        def side_b(s_):
            los = [pin(r_) for r_ in (WPINS, WPINS2)[s_ // REP]]
            if s_ < REP:
                add_hi(s_ + 1, w_unit(wo_v.at[g + 1], wos_v.at[1 - qs], blk, s_ % REP, los))
            else:
                gq = jnp.minimum(g + 2, HKV - 1)
                add_hi(s_ + 1, w_unit(wq_v.at[gq], wqs_v.at[gq % 2], blk, s_ % REP, los))
            nn = NSTEPS
            ci = jnp.minimum(i, NMC - 1)
            if s_ < nn:
                lo = pin(NPIN)
                macc = st.get('macc')
                for rg in range(128 * s_ // nn, 128 * (s_ + 1) // nn):
                    xc_ = jnp.where(lo[0], lo[1], scc_v[8 * rg:8 * rg + 8, :])
                    pr_ = wmr_v[ci, 8 * rg:8 * rg + 8, :].astype(f32) * jnp.concatenate([xc_] * NM, axis=1)
                    macc = pr_ if macc is None else macc + pr_
                st['macc'] = macc
                add_hi(s_ + NHI, _token(macc))
                if s_ == nn - 1:
                    c0 = pl.multiple_of(2 * D + jnp.minimum(ci * NM, 32 - NM) * 128, 128)
                    tot_ = jnp.sum(macc, axis=0, keepdims=True).astype(bf16).astype(f32)
                    mod_v[:, pl.ds(c0, NM * 128)] = jnp.broadcast_to(tot_, (8, NM * 128))

        def side_c(s_):
            for k_, r_ in enumerate((LPINS, LPINS2)[s_ % 2]):
                off = ((s_ % REP) * len(LPINS) + k_) * 8
                if s_ < REP:
                    res = ln2_rows(pl.multiple_of(jnp.maximum(2 * blk - 1, 0) * TQ, TQ), off, 8, blk > 0, pin(r_))
                else:
                    res = ln2_rows(pl.multiple_of(2 * blk * TQ, TQ), off, 8, None, pin(r_))
                add_hi(s_ + LHI, _token(*res))

        for par in range(2):
            a0 = pl.multiple_of((2 * blk + par) * TQ, TQ)
            acc = (acc_v, accb_v)[par]
            os_ = []

            def h_blk(a, b, a0=a0):
                return h_v[pl.ds(pl.multiple_of(a0 + a * QR, QR), QR), b * QC:(b + 1) * QC]

            q_lhs = _LhsOps(lambda a, b, f=h_blk: f(a, b).astype(f32), h_blk)
            q_comb = _Combine2()

            def q_prod(i_, j_, a0=a0, q_lhs=q_lhs, q_comb=q_comb):
                y = jnp.dot(q_lhs.op(i_, j_), wqs_v[1 - qs, :, _col(i_, j_)], preferred_element_type=f32)
                for a, b, v in q_comb.feed(i_, j_, y):
                    r0 = pl.multiple_of(a0 + a * QR, QR)
                    q_v[1 - qs, pl.ds(r0, QR), b * QC:(b + 1) * QC] = v.astype(bf16)

            q_todo = [(lambda gate, i_=i_, j_=j_, f=q_prod: f(i_, j_)) for i_ in QORD for j_ in IORD]
            o_lhs = _LhsOps(lambda a, b, os_=os_: jnp.concatenate(
                [os_[2 * b][a * QR:(a + 1) * QR], os_[2 * b + 1][a * QR:(a + 1) * QR]], axis=1))
            o_comb = _Combine2()

            def o_prod(i_, j_, gate, acc=acc, o_lhs=o_lhs, o_comb=o_comb, a0=a0):
                lhs = o_lhs.op(i_, j_)
                if gate is not None:
                    lhs = _gate1(lhs, flag, jnp.concatenate([gate, gate], axis=0).astype(bf16))
                y = jnp.dot(lhs, wos_v[qs, :, _col(i_, j_)], preferred_element_type=f32)
                old = acc[pl.ds(m0, QR), _col(i_, j_)]
                if not last_group:
                    acc[pl.ds(m0, QR), _col(i_, j_)] = jnp.where(g == 0, 0.0, old) + y
                    return
                for a, b, v in o_comb.feed(i_, j_, old + y):
                    rs = pl.ds(pl.multiple_of(a0 + a * QR, QR), QR)
                    cx = slice(b * QC, (b + 1) * QC)
                    ga = _rows(mod_v[:, 2 * D + b * QC:2 * D + (b + 1) * QC], QR)
                    x_v[rs, cx] = (x_v[rs, cx].astype(f32) + ga * v).astype(bf16)

            s0 = par * REP
            if last_group:
                for hh in range(0, REP, 2):
                    sp0 = qk(s0 + hh, a0, hh)
                    sp1 = qk(s0 + hh + 1, a0, hh + 1)
                    pv(s0 + hh, os_, sp0)
                    side_c(s0 + hh)
                    pv(s0 + hh + 1, os_, sp1)
                    side_c(s0 + hh + 1)
            else:
                for hh in range(REP):
                    sp = qk(s0 + hh, a0, hh)
                    run(q_todo, (QRUN, QRUN2)[par][hh])
                    pv(s0 + hh, os_, sp)
                    if par == 1:
                        run(o_todo, ORUN[hh])
                    side_b(s0 + hh)
            o_todo.extend([(lambda gate, i_=i_, j_=j_, f=o_prod: f(i_, j_, gate))
                           for i_ in (CORD if last_group else OORD) for j_ in (IORDC if last_group else IORDO)])
            if last_group or par == 1:
                flush()
        if last_group:
            @pl.when(blk > 0)
            def _():
                out_copy(pl.multiple_of((2 * blk - 1) * TQ, TQ), TQ).start()

            out_copy(pl.multiple_of(2 * blk * TQ, TQ), TQ).start()

    def make_aux():
        sb_ = mod_v[:, 3 * D:4 * D]
        cb1_ = 1.0 + mod_v[:, 4 * D:5 * D]
        gb_ = mod_v[:, 5 * D:6 * D]
        wr8 = wr_v[...].astype(f32)
        wr_ = jnp.concatenate([wr8[r_:r_ + 1, :] for r_ in range(8)], axis=1)
        aux_v[0] = gb_ * cb1_
        aux_v[1] = gb_ * sb_
        aux_v[2] = cb1_ * wr_
        aux_v[3] = jnp.broadcast_to(jnp.sum(sb_ * wr_, axis=-1, keepdims=True), (8, D))

    def body_b(i, carry):
        @pl.when(i == 2)
        def _():
            wait_all(wmr_v.at[pl.ds(2, NMC - 2)], SEM_WMR + 1)
            for c_ in wrest_cps:
                c_.wait()

        body(i, False)
        return carry

    lax.fori_loop(0, 3 * NT // 2, body_b, 0)

    wg_cp.wait()
    wu_cp.wait()
    wd_cp.wait()
    make_aux()

    def body_c(i, carry):
        body(i, True)
        return carry

    lax.fori_loop(0, NT // 2, body_c, 0)

    ln2_rows((NT - 1) * TQ, 0, TQ)
    out_copy((NT - 1) * TQ, TQ).start()

    best = best_v[0]
    bidx = bidx_v[0]
    rmax = jnp.max(best, axis=0, keepdims=True)
    idx_v = jnp.min(jnp.where(best == rmax, bidx, S), axis=0, keepdims=True)
    idx = jnp.minimum(idx_v[0, 0], S - 1)
    g0 = pl.multiple_of((idx // 8) * 8, 8)
    sb = mod_v[:, 3 * D:4 * D]
    cb = mod_v[:, 4 * D:5 * D]
    gb = mod_v[:, 5 * D:6 * D]
    x2 = x_v[pl.ds(g0, 8), :].astype(f32)
    h2 = (x2 - best_v[1][:, 0:1]) * best_v[2][:, 0:1] * (1.0 + cb) + sb
    h2b = h2.astype(bf16)
    sel = (lax.broadcasted_iota(jnp.int32, (8, 1), 0) + g0) == idx
    flag = flag_s[0] > 0
    nf = F // 128
    strips = [(k_, j) for j in range(nf) for k_ in 'gu'] + [('d', j) for j in range(FD, nf)]
    gate_r, a_strips, vtok = {}, {}, {}
    y = None
    yv = None
    pos = 0
    for i, (kind, j) in enumerate(strips):
        hi = vtok.get(i - FLAG_)
        if kind == 'd':
            lhs = a_strips[j]
            if hi is not None:
                lhs = jnp.where(flag, hi.astype(bf16), lhs)
            r_ = jnp.dot(lhs, wd_v[j * 128:(j + 1) * 128, 0:D], preferred_element_type=f32)
            y = r_ if y is None else y + r_
            tok_ = r_[:, D - 128:D]
        else:
            lhs = h2b if hi is None else _gate1(h2b, flag, hi.astype(bf16))
            w_ref = wg_v if kind == 'g' else wu_v
            tok_ = jnp.dot(lhs, w_ref[:, j * 128:(j + 1) * 128], preferred_element_type=f32)
            if kind == 'g':
                gate_r[j] = tok_
            else:
                a_strips[j] = (gate_r[j] * jax.nn.sigmoid(gate_r[j]) * tok_).astype(bf16)
                if j < FD:
                    row = jnp.sum(jnp.where(sel, a_strips[j].astype(f32), 0.0), axis=0, keepdims=True)
                    acol_v[j * 128:(j + 1) * 128, :] = jnp.broadcast_to(row, (128, 128)).T
        if i >= FI0 and pos < FD * 16:
            end = min(pos + FVR, FD * 16) if i < len(strips) - 1 else FD * 16
            for rg in range(pos, end):
                col = jnp.where(flag, tok_, acol_v[8 * rg:8 * rg + 8, :])
                pr_ = wd_v[8 * rg:8 * rg + 8, 0:D].astype(f32) * jnp.concatenate([col] * (D // 128), axis=1)
                yv = pr_ if yv is None else yv + pr_
            pos = end
            vtok[i] = _token(yv)
    y = (y + jnp.sum(yv, axis=0, keepdims=True)) * jax.nn.sigmoid(rmax[:, 0:1])
    out_copy(0, S).wait()
    new = (x2 + gb * (h2 + y)).astype(bf16)
    out_v[pl.ds(g0, 8), :] = jnp.where(sel, new, out_v[pl.ds(g0, 8), :])
    fix = out_copy(g0, 8)
    fix.start()
    fix.wait()


@jax.jit
def pallas_adaLN_cond__sliding_block_cached__moe_arch_mod__prompt_kernel(
    A_x, A_k_cache, A_v_cache, A_wq, A_wo, B_x, B_w_r, B_w_gate, B_w_up, B_w_down, c, w_mod,
):
    del B_x
    any_spec = pl.BlockSpec(memory_space=pl.ANY)
    return pl.pallas_call(
        _kernel,
        out_shape=jax.ShapeDtypeStruct(A_x.shape, A_x.dtype),
        in_specs=[any_spec] * 11,
        out_specs=any_spec,
        scratch_shapes=[
            pltpu.VMEM((S, D), bf16),
            pltpu.VMEM((S, D), bf16),
            pltpu.VMEM((2, S, GW), bf16),
            pltpu.VMEM((S // 8, 49 * QC), f32),
            pltpu.VMEM((S // 8, 49 * QC), f32),
            pltpu.VMEM((NMC, D, NM * 128), bf16),
            pltpu.VMEM((HKV, 4, QC, GW + PADW), bf16),
            pltpu.VMEM((2, QC, 49 * QC), bf16),
            pltpu.VMEM((HKV, 4, QC, D), bf16),
            pltpu.VMEM((2, QC, 49 * QC), bf16),
            pltpu.VMEM((D, F), bf16),
            pltpu.VMEM((D, F), bf16),
            pltpu.VMEM((F, D + PADD), bf16),
            pltpu.VMEM((HKV, W, DH), bf16),
            pltpu.VMEM((HKV, W, DH), bf16),
            pltpu.VMEM((HKV, DH, W), bf16),
            pltpu.VMEM((8, 1, D), bf16),
            pltpu.VMEM((16, 8, 128), bf16),
            pltpu.VMEM((16, D), bf16),
            pltpu.VMEM((D, 128), f32),
            pltpu.VMEM((2 * D, 128), f32),
            pltpu.VMEM((8, 6 * D), f32),
            pltpu.VMEM((8, 8, 128), f32),
            pltpu.VMEM((8, 8, 128), jnp.int32),
            pltpu.VMEM((4, 8, D), f32),
            pltpu.SMEM((1,), jnp.int32),
            pltpu.SemaphoreType.DMA((NSEM,)),
        ],
        compiler_params=pltpu.CompilerParams(vmem_limit_bytes=126 * 1024 * 1024,
                                             disable_semaphore_checks=True,
                                             disable_bounds_checks=True),
    )(A_x, A_k_cache, A_v_cache, A_wq.reshape(4, QC, HQ * DH), A_wo.reshape(HKV, 4, QC, D), B_w_r.reshape(8, 128), B_w_gate, B_w_up, B_w_down, c, w_mod)
```
